```python
import jax
import jax.numpy as jnp

def _softmax(x, axis=-1):
    return jax.nn.softmax(x, axis=axis)

def _gelu(x):
    return jax.nn.gelu(x, approximate=True)

def _silu(x):
    return jax.nn.silu(x)

def _sigmoid(x):
    return jax.nn.sigmoid(x)

def _layernorm(x, axis=-1, eps=1e-05):
    m = jnp.mean(x, axis=axis, keepdims=True)
    v = jnp.var(x, axis=axis, keepdims=True)
    return (x - m) / jnp.sqrt(v + eps)

def _scatter_add(tgt, idx, src, axis=0):
    return tgt.at[idx].add(src)

def _segment_sum(src, seg, n):
    return jax.ops.segment_sum(src, seg, n)

class _Rng:

    def __init__(self, key):
        self._k = key

    def _next(self):
        self._k, sub = jax.random.split(self._k)
        return sub

    def normal(self, shape):
        return jax.random.normal(self._next(), shape, dtype=jnp.bfloat16)

    def randint(self, lo, hi, shape):
        return jax.random.randint(self._next(), shape, lo, hi, dtype=jnp.int32)

    def uniform(self, shape, lo=0.0, hi=1.0):
        return jax.random.uniform(self._next(), shape, jnp.bfloat16, lo, hi)

    def permutation(self, n):
        return jax.random.permutation(self._next(), n)
kernel_name = 'interleave_layers__memory_aug_recurrent_mem_tr__glu_gated_glu__prompt'

def setup_inputs():
    _rng = _Rng(jax.random.key(int.from_bytes(__import__("os").urandom(4), "little")))
    _w = lambda a: (lambda t: t.astype(jnp.bfloat16) if jnp.issubdtype(t.dtype, jnp.floating) else t)(jnp.asarray(a))

    def _A_setup():
        B, S, Dm = (1, 2048, 1024)
        H, Dh = (32, 128)
        M, seg = (8, 32)
        seg = min(seg, S)
        S = S // seg * seg
        return {'x': _w((lambda *s: _rng.normal(s) * 0.05)(B, S, Dm)), 'mem0': _w((lambda *s: _rng.normal(s) * 0.05)(B, M, Dm)), 'Wq': _w((lambda *s: _rng.normal(s) * 0.05)(Dm, H, Dh) * Dm ** (-0.5)), 'Wk': _w((lambda *s: _rng.normal(s) * 0.05)(Dm, H, Dh) * Dm ** (-0.5)), 'Wv': _w((lambda *s: _rng.normal(s) * 0.05)(Dm, H, Dh) * Dm ** (-0.5)), 'Wo': _w((lambda *s: _rng.normal(s) * 0.05)(H, Dh, Dm) * (H * Dh) ** (-0.5)), 'seg_len': seg}
    _A_in = _A_setup()

    def _B_setup():
        B, S, D, F = (1, 2048, 1024, 3584)
        return {'x': _w((lambda *s: _rng.normal(s) * 0.05)(B, S, D)), 'w_gate': _w((lambda *s: _rng.normal(s) * 0.05)(D, F)), 'w_up': _w((lambda *s: _rng.normal(s) * 0.05)(D, F)), 'w_down': _w((lambda *s: _rng.normal(s) * 0.05)(F, D))}
    _B_in = _B_setup()
    return {'A_x': _A_in['x'], 'A_mem0': _A_in['mem0'], 'A_Wq': _A_in['Wq'], 'A_Wk': _A_in['Wk'], 'A_Wv': _A_in['Wv'], 'A_Wo': _A_in['Wo'], 'A_seg_len': _A_in['seg_len'], 'B_x': _B_in['x'], 'B_w_gate': _B_in['w_gate'], 'B_w_up': _B_in['w_up'], 'B_w_down': _B_in['w_down']}

def reference(A_x, A_mem0, A_Wq, A_Wk, A_Wv, A_Wo, A_seg_len, B_x, B_w_gate, B_w_up, B_w_down):

    def _A_ref(x, mem0, Wq, Wk, Wv, Wo, seg_len):
        B, S, Dm = x.shape
        H, Dh = (Wq.shape[1], Wq.shape[2])
        M = mem0.shape[1]
        scale = Dh ** (-0.5)
        n_seg = S // seg_len
        L = M + seg_len
        idx = jnp.arange(L)
        mask = (idx[:, None] < M) | (idx[:, None] >= idx[None, :])
        mem = mem0
        outs = []
        for s in range(n_seg):
            xs = x[:, s * seg_len:(s + 1) * seg_len, :].copy()
            h = jnp.concatenate([mem, xs], axis=1)
            q = jnp.einsum('btd,dhe->bhte', h, Wq)
            k = jnp.einsum('btd,dhe->bhte', h, Wk)
            v = jnp.einsum('btd,dhe->bhte', h, Wv)
            scores = jnp.einsum('bhqe,bhke->bhqk', q, k) * scale
            scores = jnp.where(mask[None, None], scores, -1000000000.0)
            p = _softmax(scores, axis=-1)
            o = jnp.einsum('bhqk,bhke->bhqe', p, v)
            o = jnp.einsum('bhte,hed->btd', o, Wo)
            mem = o[:, :M, :].copy()
            outs.append(o[:, M:, :])
        return jnp.concatenate(outs, axis=1)

    def _B_ref(x, w_gate, w_up, w_down):
        g = jnp.einsum('bsd,df->bsf', x, w_gate)
        u = jnp.einsum('bsd,df->bsf', x, w_up)
        h = _sigmoid(g) * u
        return jnp.einsum('bsf,fd->bsd', h, w_down)
    x = A_x
    x = x + _A_ref(_layernorm(x, axis=-1), A_mem0, A_Wq, A_Wk, A_Wv, A_Wo, A_seg_len)
    x = x + _B_ref(_layernorm(x, axis=-1), B_w_gate, B_w_up, B_w_down)
    x = x + _A_ref(_layernorm(x, axis=-1), A_mem0, A_Wq, A_Wk, A_Wv, A_Wo, A_seg_len)
    x = x + _B_ref(_layernorm(x, axis=-1), B_w_gate, B_w_up, B_w_down)
    return x
```

```python
import functools
import math

import jax
import jax.numpy as jnp
import numpy as np
from jax import lax
import jax.experimental.pallas as pl
import jax.experimental.pallas.tpu as pltpu

F32 = jnp.float32
BF16 = jnp.bfloat16
U32 = jnp.uint32
EPS = 1e-05


def _layernorm(x):
    m = jnp.mean(x, axis=-1, keepdims=True)
    c = x - m
    v = jnp.mean(c * c, axis=-1, keepdims=True)
    return c * lax.rsqrt(v + EPS)


def _dot(a, b):
    return jnp.dot(a, b, preferred_element_type=F32)


def _dot_nt(a, b):
    return lax.dot_general(a, b, (((1,), (1,)), ((), ())), preferred_element_type=F32)


def _make_kernel(S, D, H, DH, M, SEG, FF, cfg):
    G = cfg.get("G", 4)
    FC = cfg.get("FC", 512)
    NC = cfg.get("NC", 512)
    DC = cfg.get("DC", 128)
    NSTAGE = cfg.get("NSTAGE", 4)
    NSEG = S // SEG
    R = 2 * (M + SEG)
    RB = 2 * SEG
    NG = H // G
    scale = DH ** (-0.5)
    c_exp = scale * math.log2(math.e)

    def kernel(x_hbm, mem0_ref, wq_hbm, wk_hbm, wv_hbm, wo_hbm, wg_hbm, wu_hbm, wd_hbm,
               out_hbm,
               x_v, out_v, wqkv_v, wo_v, wg_v, wu_v, wd_v, stage_v,
               h_v, xa_v, ya_v, hb_v, o_v, act_v, fill_v, keep_v,
               sem_in, sem_stage, sem_out):
        x_cp = pltpu.make_async_copy(x_hbm, x_v, sem_in.at[0])
        wo_cp = pltpu.make_async_copy(wo_hbm, wo_v, sem_in.at[1])
        wg_cp = pltpu.make_async_copy(wg_hbm, wg_v, sem_in.at[2])
        wu_cp = pltpu.make_async_copy(wu_hbm, wu_v, sem_in.at[3])
        wd_cp = pltpu.make_async_copy(wd_hbm, wd_v, sem_in.at[4])
        NDC = D // DC
        chunks = [(w, c) for w in range(3) for c in range(NDC)]
        srcs = (wq_hbm, wk_hbm, wv_hbm)

        def stage_cp(i):
            w, c = chunks[i]
            return pltpu.make_async_copy(
                srcs[w].at[pl.ds(c * DC * H, DC * H), :], stage_v.at[i % NSTAGE],
                sem_stage.at[i % NSTAGE])

        for i in range(NSTAGE):
            stage_cp(i).start()
        x_cp.start()

        ri = lax.broadcasted_iota(jnp.int32, (R, R), 0)
        ci = lax.broadcasted_iota(jnp.int32, (R, R), 1)

        def layer_of(i):
            return jnp.where(i < 2 * M, (i >= M).astype(jnp.int32),
                             (i >= 2 * M + SEG).astype(jnp.int32))

        same = layer_of(ri) == layer_of(ci)
        visible = (ri < 2 * M) | (ri >= ci)
        keep_v[...] = (same & visible).astype(jnp.int32)
        fill_v[...] = jnp.where(same, -1e9 / scale, -jnp.inf).astype(F32)
        ya_v[...] = jnp.zeros(ya_v.shape, F32)

        for i, (w, c) in enumerate(chunks):
            stage_cp(i).wait()
            st = stage_v.at[i % NSTAGE].bitcast(U32)

            for j in range(H // 2):
                ev = st[pl.ds(j, DC // 2, stride=H), :]
                od = st[pl.ds(H // 2 + j, DC // 2, stride=H), :]
                lo = (ev & 0xFFFF) | (od << 16)
                hi = (ev >> 16) | (od & np.uint32(0xFFFF0000))
                for r, val in ((0, lo), (1, hi)):
                    hd = 2 * j + r
                    g, k = hd // G, hd % G
                    col = (w * G + k) * DH
                    wqkv_v[g, c * DC:(c + 1) * DC, col:col + DH] = pltpu.bitcast(val, BF16)
            if i + NSTAGE < len(chunks):
                stage_cp(i + NSTAGE).start()
            if i + NSTAGE == len(chunks) - 1:
                wg_cp.start()
                wu_cp.start()
                wd_cp.start()
                wo_cp.start()

        x_cp.wait()
        mem0 = mem0_ref[...].astype(F32)
        h_v[0:2 * M, :] = jnp.concatenate([mem0, mem0], axis=0).astype(BF16)
        x0 = x_v[0:SEG, :].astype(F32)
        xa_v[0:SEG, :] = x0
        xa_v[SEG:, :] = jnp.zeros((SEG, D), F32)
        h_v[2 * M:2 * M + SEG, :] = _layernorm(x0).astype(BF16)
        h_v[2 * M + SEG:, :] = jnp.zeros((SEG, D), BF16)
        wg_cp.wait()
        wu_cp.wait()
        wd_cp.wait()
        wo_cp.wait()

        def attend(g, qkv):
            keep = keep_v[...] != 0
            fill = fill_v[...]
            for k in range(G):
                q = qkv[:, k * DH:(k + 1) * DH]
                kk = qkv[:, (G + k) * DH:(G + k + 1) * DH]
                v = qkv[:, (2 * G + k) * DH:(2 * G + k + 1) * DH]
                s = jnp.where(keep, _dot_nt(q, kk), fill)
                mx = jnp.max(s, axis=-1, keepdims=True)
                e = jnp.exp2((s - mx) * c_exp)
                den = jnp.sum(e, axis=-1, keepdims=True)
                p = e * pl.reciprocal(den)
                o = _dot(p.astype(BF16), v)
                hd = g * G + k
                o_v[:, hd * DH:(hd + 1) * DH] = o.astype(BF16)

        def step(t, carry):
            hb_v[...] = _layernorm(ya_v[...]).astype(BF16)
            h = h_v[...]
            prev = None
            for g in range(NG):
                qkv = _dot(h, wqkv_v[g]).astype(BF16)
                if cfg.get("swp", True):
                    if prev is not None:
                        attend(g - 1, prev)
                    prev = qkv
                else:
                    attend(g, qkv)
            hb = hb_v[...]
            for j in range(FF // FC):
                gate = _dot(hb, wg_v[:, j * FC:(j + 1) * FC])
                up = _dot(hb, wu_v[:, j * FC:(j + 1) * FC])
                if j == 0 and prev is not None:
                    attend(NG - 1, prev)
                act_v[:, j * FC:(j + 1) * FC] = (jax.nn.sigmoid(gate) * up).astype(BF16)
            act = act_v[...]
            z = jnp.concatenate(
                [ya_v[:, n * NC:(n + 1) * NC] + _dot(act, wd_v[:, n * NC:(n + 1) * NC])
                 for n in range(D // NC)], axis=1)
            so = jnp.clip(t - 3, 0, NSEG - 1)
            out_v[pl.ds(pl.multiple_of(so * SEG, SEG), SEG), :] = z[SEG:].astype(BF16)
            o = o_v[...]
            xa = xa_v[...]
            for n in range(D // NC):
                r = _dot(o, wo_v[:, n * NC:(n + 1) * NC])
                ya_v[:, n * NC:(n + 1) * NC] = xa[:, n * NC:(n + 1) * NC] + r[2 * M:]
                m2 = jnp.where(t < 2, mem0_ref[:, n * NC:(n + 1) * NC].astype(F32), r[M:2 * M])
                h_v[0:2 * M, n * NC:(n + 1) * NC] = jnp.concatenate(
                    [r[0:M], m2], axis=0).astype(BF16)
            sn = jnp.minimum(t + 1, NSEG - 1)
            xn = jnp.concatenate(
                [x_v[pl.ds(pl.multiple_of(sn * SEG, SEG), SEG), :].astype(F32), z[:SEG]], axis=0)
            xa_v[...] = xn
            h_v[2 * M:, :] = _layernorm(xn).astype(BF16)

            @pl.when(t >= 3)
            def _():
                r0 = pl.multiple_of(so * SEG, SEG)
                pltpu.make_async_copy(out_v.at[pl.ds(r0, SEG), :],
                                      out_hbm.at[pl.ds(r0, SEG), :], sem_out).start()
            return carry

        lax.fori_loop(0, cfg.get("nsteps", NSEG + 3), step, 0)
        pltpu.make_async_copy(out_v, out_hbm, sem_out).wait()

    scratch = [
        pltpu.VMEM((S, D), BF16),
        pltpu.VMEM((S, D), BF16),
        pltpu.VMEM((NG, D, 3 * G * DH), BF16),
        pltpu.VMEM((H * DH, D), BF16),
        pltpu.VMEM((D, FF), BF16),
        pltpu.VMEM((D, FF), BF16),
        pltpu.VMEM((FF, D), BF16),
        pltpu.VMEM((NSTAGE, DC * H, DH), BF16),
        pltpu.VMEM((R, D), BF16),
        pltpu.VMEM((RB, D), F32),
        pltpu.VMEM((RB, D), F32),
        pltpu.VMEM((RB, D), BF16),
        pltpu.VMEM((R, H * DH), BF16),
        pltpu.VMEM((RB, FF), BF16),
        pltpu.VMEM((R, R), F32),
        pltpu.VMEM((R, R), jnp.int32),
        pltpu.SemaphoreType.DMA((5,)),
        pltpu.SemaphoreType.DMA((NSTAGE,)),
        pltpu.SemaphoreType.DMA(()),
    ]
    return kernel, scratch


def _build(cfg):
    @functools.partial(jax.jit, static_argnames=("A_seg_len",))
    def fn(A_x, A_mem0, A_Wq, A_Wk, A_Wv, A_Wo, A_seg_len, B_x, B_w_gate, B_w_up, B_w_down):
        B, S, D = A_x.shape
        _, H, DH = A_Wq.shape
        M = A_mem0.shape[1]
        FF = B_w_gate.shape[1]
        kernel, scratch = _make_kernel(S, D, H, DH, M, A_seg_len, FF, cfg)
        any_spec = pl.BlockSpec(memory_space=pl.ANY)
        out = pl.pallas_call(
            kernel,
            out_shape=jax.ShapeDtypeStruct((S, D), A_x.dtype),
            in_specs=[any_spec, pl.BlockSpec(memory_space=pltpu.VMEM)] + [any_spec] * 7,
            out_specs=any_spec,
            scratch_shapes=scratch,
            compiler_params=pltpu.CompilerParams(vmem_limit_bytes=110 * 1024 * 1024,
                                                 flags=cfg.get("flags")),
        )(A_x.reshape(S, D), A_mem0.reshape(M, D),
          A_Wq.reshape(D * H, DH), A_Wk.reshape(D * H, DH), A_Wv.reshape(D * H, DH),
          A_Wo.reshape(H * DH, D), B_w_gate, B_w_up, B_w_down)
        return out.reshape(B, S, D)
    return fn


pallas_interleave_layers__memory_aug_recurrent_mem_tr__glu_gated_glu__prompt_kernel = _build({})
```

```python
import functools
import math

import jax
import jax.numpy as jnp
import numpy as np
from jax import lax
import jax.experimental.pallas as pl
import jax.experimental.pallas.tpu as pltpu

F32 = jnp.float32
BF16 = jnp.bfloat16
U32 = jnp.uint32
EPS = 1e-05
LANES = 128

STRASSEN = (2, (
    ({(1, 0): 1, (1, 1): 1}, {(0, 0): 1}, {(1, 0): 1, (1, 1): -1}, {0: 1, 1: 1}, {0: 1}),
    ({(1, 1): 1}, {(1, 0): 1, (0, 0): -1}, {(0, 0): 1, (1, 0): 1}, {1: 1}, {0: 1}),
    ({(0, 0): 1}, {(0, 1): 1, (1, 1): -1}, {(0, 1): 1, (1, 1): 1}, {0: 1}, {1: 1}),
    ({(0, 0): 1, (0, 1): 1}, {(1, 1): 1}, {(0, 0): -1, (0, 1): 1}, {0: 1, 1: 1}, {1: 1}),
    ({(0, 0): 1, (1, 1): 1}, {(0, 0): 1, (1, 1): 1}, {(0, 0): 1, (1, 1): 1}, None, None),
    ({(1, 0): 1, (0, 0): -1}, {(0, 0): 1, (0, 1): 1}, {(1, 1): 1}, None, None),
    ({(0, 1): 1, (1, 1): -1}, {(1, 0): 1, (1, 1): 1}, {(0, 0): 1}, None, None),
))
SCHEMES = {"strassen": STRASSEN}


def _combine(coefs, vals):
    acc = None
    for key, c in sorted(coefs.items(), key=lambda kv: -kv[1]):
        v = vals[key]
        if abs(c) != 1:
            v = v * abs(c)
        if acc is None:
            acc = v if c > 0 else -v
        else:
            acc = acc + v if c > 0 else acc - v
    return acc


def _accumulate(accs, coefs, v):
    for key, c in coefs.items():
        t = v if abs(c) == 1 else v * abs(c)
        if key not in accs:
            accs[key] = t if c > 0 else -t
        else:
            accs[key] = accs[key] + t if c > 0 else accs[key] - t


def _layernorm(x):
    m = jnp.mean(x, axis=-1, keepdims=True)
    c = x - m
    v = jnp.mean(c * c, axis=-1, keepdims=True)
    return c * lax.rsqrt(v + EPS)


def _dot(a, b):
    return jnp.dot(a, b, preferred_element_type=F32)


def _dot_nt(a, b):
    return lax.dot_general(a, b, (((1,), (1,)), ((), ())), preferred_element_type=F32)


def _pack(x):
    return pltpu.bitcast(x.astype(BF16), U32)


def _unpack(x):
    return pltpu.bitcast(x, BF16)


def _make_kernel(S, D, H, DH, M, SEG, FF, cfg):
    NB, prods = SCHEMES[cfg.get("scheme", "strassen")]
    NP = len(prods)
    NSEG = S // SEG
    MM = 2 * M
    R = MM + 2 * SEG
    RL = MM + SEG
    DB, HB, FB = D // NB, H // NB, FF // NB
    EB = HB * DH
    OC = cfg.get("OC", 256)
    QR = cfg.get("QR", 128) // NB
    WR = cfg.get("WR", 512) // NB
    GR = cfg.get("GR", 128) // NB
    NST = cfg.get("NST", 3)
    scale = DH ** (-0.5)
    c_exp = scale * math.log2(math.e)

    def store_lhs(ref, cols, tok, mem):
        for r, (u, _, _, um, _) in enumerate(prods):
            if tok is not None:
                ref[r, ref.shape[1] - SEG // 2:, cols] = _pack(_combine(u, tok))
            if mem is not None and um is not None:
                ref[r, 0:MM // 2, cols] = _pack(_combine(um, mem))

    def fast_dot(lhs_ref, w_of, with_mem, hooks=None):
        tok, mem = {}, {}
        for r, (_, _, w, um, wm) in enumerate(prods):
            if hooks and r in hooks:
                hooks[r]()
            if with_mem and um is not None:
                p = _dot(_unpack(lhs_ref[r]), _unpack(w_of(r)))
                _accumulate(mem, wm, p[:MM])
                _accumulate(tok, w, p[MM:])
            else:
                p = _dot(_unpack(lhs_ref[r, lhs_ref.shape[1] - SEG // 2:, :]), _unpack(w_of(r)))
                _accumulate(tok, w, p)
        return tok, mem

    def split_tokens(x):
        return {(hf, i): x[hf * SEG:(hf + 1) * SEG, i * DB:(i + 1) * DB]
                for hf in range(2) for i in range(NB)}

    def kernel(x_hbm, mem0_ref, wq_hbm, wk_hbm, wv_hbm, wo_hbm, wg_hbm, wu_hbm, wd_hbm,
               out_hbm,
               x_v, out_v, wqkv_v, wo_v, wgu_v, wd_v,
               la_v, lo_v, lb_v, ld_v, xa_v, ya_v, z_v, fill_v, keep_v,
               sem_x, sem_st, sem_out):

        def staged(srcs, rows, row_mul, nchunk, width, process, before_drain):
            def run(stage):
                def copies(w, c, slot):
                    blk = srcs[w].shape[0] // NB
                    return [pltpu.make_async_copy(
                        srcs[w].at[pl.ds(pl.multiple_of(i * blk + c * rows * row_mul, 16),
                                         rows * row_mul), :],
                        stage.at[slot, i], sem_st.at[slot, i]) for i in range(NB)]

                total = len(srcs) * nchunk
                for n in range(NST):
                    for cp in copies(n // nchunk, n % nchunk, n):
                        cp.start()
                for w in range(len(srcs)):
                    def body(c, carry, w=w):
                        n = w * nchunk + c
                        slot = n % NST
                        for cp in copies(w, c, slot):
                            cp.wait()
                        process(w, c, stage, slot)

                        @pl.when(c + NST < nchunk)
                        def _():
                            for cp in copies(w, c + NST, slot):
                                cp.start()

                        if w + 1 < len(srcs):
                            @pl.when(c + NST >= nchunk)
                            def _():
                                for cp in copies(w + 1, c + NST - nchunk, slot):
                                    cp.start()
                        return carry
                    lax.fori_loop(0, nchunk, body, 0)
            pl.run_scoped(run, pltpu.VMEM((NST, NB, rows * row_mul, width), BF16))

        def prep_qkv(w, c, stage, slot):
            r0 = pl.multiple_of(c * (QR // 2), 8)

            for jp in range(HB // 2):
                lo, hi = {}, {}
                for i in range(NB):
                    st = stage.at[slot, i].bitcast(U32)
                    for j in range(NB):
                        x = st[pl.ds(j * (HB // 2) + jp, QR, stride=H // 2), :]
                        lo[i, j] = pltpu.bitcast(x << 16, F32)
                        hi[i, j] = pltpu.bitcast(x & np.uint32(0xFFFF0000), F32)
                for r, (_, v, _, _, _) in enumerate(prods):
                    for k, vals in enumerate((lo, hi)):
                        wqkv_v[2 * jp + k, r, pl.ds(r0, QR // 2), w * DH:(w + 1) * DH] = _pack(
                            _combine(v, vals))

        def prep_plain(dst_of, rows, nb):
            def process(w, c, stage, slot):
                def sub(s, carry):
                    rs = pl.multiple_of(s * 16, 16)
                    vals = {(i, j): stage[slot, i, pl.ds(rs, 16), j * nb:(j + 1) * nb].astype(F32)
                            for i in range(NB) for j in range(NB)}
                    r0 = pl.multiple_of(c * (rows // 2) + s * 8, 8)
                    for r, (_, v, _, _, _) in enumerate(prods):
                        dst_of(w, r, r0, _pack(_combine(v, vals)))
                    return carry
                lax.fori_loop(0, rows // 16, sub, 0)
            return process

        def put_o(w, r, r0, val):
            wo_v[r, pl.ds(r0, 8), :] = val

        def put_d(w, r, r0, val):
            wd_v[r, pl.ds(r0, 8), :] = val

        def put_gu(w, r, r0, val):
            for c in range(FB // LANES):
                wgu_v[c, r, pl.ds(r0, 8), w * LANES:(w + 1) * LANES] = (
                    val[:, c * LANES:(c + 1) * LANES])

        x_cp = pltpu.make_async_copy(x_hbm, x_v, sem_x)
        x_cp.start()

        ri = lax.broadcasted_iota(jnp.int32, (R, R), 0)
        ci = lax.broadcasted_iota(jnp.int32, (R, R), 1)

        def layer_of(i):
            return jnp.where(i < MM, (i >= M).astype(jnp.int32), (i >= MM + SEG).astype(jnp.int32))

        same = layer_of(ri) == layer_of(ci)
        visible = (ri < MM) | (ri >= ci)
        keep_v[...] = (same & visible).astype(jnp.int32)
        fill_v[...] = jnp.where(same, -1e9 / scale, -jnp.inf).astype(F32)
        ya_v[...] = jnp.zeros(ya_v.shape, F32)

        staged((wq_hbm, wk_hbm, wv_hbm), QR, H, DB // QR, DH, prep_qkv, None)
        staged((wo_hbm,), WR, 1, EB // WR, D, prep_plain(put_o, WR, DB), None)
        staged((wg_hbm, wu_hbm), GR, 1, DB // GR, FF, prep_plain(put_gu, GR, FB), None)
        staged((wd_hbm,), WR // 2, 1, FB // (WR // 2), D, prep_plain(put_d, WR // 2, DB), None)

        x_cp.wait()
        mem0 = mem0_ref[...].astype(F32)
        mem0 = jnp.concatenate([mem0, mem0], axis=0)
        x0 = jnp.concatenate([x_v[0:SEG, :].astype(F32), jnp.zeros((SEG, D), F32)], axis=0)
        xa_v[...] = x0
        store_lhs(la_v, slice(None), split_tokens(_layernorm(x0)),
                  {i: mem0[:, i * DB:(i + 1) * DB] for i in range(NB)})

        def attention_hooks(c, tok, mem):
            pv = {}

            def scores():
                keep = keep_v[...] != 0
                fill = fill_v[...]
                for j in range(NB):
                    qkv = jnp.concatenate([mem[j], tok[0, j], tok[1, j]], axis=0).astype(BF16)
                    q, k, v = (qkv[:, w * DH:(w + 1) * DH] for w in range(3))
                    s = jnp.where(keep, _dot_nt(q, k), fill)
                    mx = jnp.max(s, axis=-1, keepdims=True)
                    e = jnp.exp2((s - mx) * c_exp)
                    den = jnp.sum(e, axis=-1, keepdims=True)
                    pv[j] = ((e * pl.reciprocal(den)).astype(BF16), v)

            def values():
                o_tok, o_mem = {}, {}
                for j in range(NB):
                    o = _dot(*pv[j])
                    o_mem[j] = o[:MM]
                    o_tok[0, j] = o[MM:MM + SEG]
                    o_tok[1, j] = o[MM + SEG:]
                store_lhs(lo_v, slice(c * DH, (c + 1) * DH), o_tok, o_mem)

            return scores, values

        def step(t, carry):
            store_lhs(lb_v, slice(None), split_tokens(_layernorm(ya_v[...])), None)
            h0, h1 = cfg.get("h0", 1), cfg.get("h1", NP - 1)
            hooks = None
            for c in range(HB):
                cur = fast_dot(la_v, lambda r: wqkv_v[c, r], True, hooks)
                scores, values = attention_hooks(c, *cur)
                hooks = {h0: scores, h1: values}
            for c in range(FB // LANES):
                hooks = {0: {2: scores}, 1: {2: values}}.get(c)
                gu, _ = fast_dot(lb_v, lambda r: wgu_v[c, r], False, hooks)
                act = {k: jax.nn.sigmoid(v[:, :LANES]) * v[:, LANES:] for k, v in gu.items()}
                store_lhs(ld_v, slice(c * LANES, (c + 1) * LANES), act, None)
            for c in range(DB // OC):
                dn, _ = fast_dot(ld_v, lambda r: wd_v[r, :, c * OC:(c + 1) * OC], False)
                for (hf, j), v in dn.items():
                    rows = slice(hf * SEG, (hf + 1) * SEG)
                    cols = slice(j * DB + c * OC, j * DB + (c + 1) * OC)
                    z_v[rows, cols] = ya_v[rows, cols] + v
            so = jnp.clip(t - 3, 0, NSEG - 1)
            out_v[pl.ds(pl.multiple_of(so * SEG, SEG), SEG), :] = z_v[SEG:, :].astype(BF16)
            for c in range(DB // OC):
                tok, mem = fast_dot(lo_v, lambda r: wo_v[r, :, c * OC:(c + 1) * OC], True)
                for (hf, j), v in tok.items():
                    rows = slice(hf * SEG, (hf + 1) * SEG)
                    cols = slice(j * DB + c * OC, j * DB + (c + 1) * OC)
                    ya_v[rows, cols] = xa_v[rows, cols] + v
                for j in range(NB):
                    m0 = mem0_ref[:, j * DB + c * OC:j * DB + (c + 1) * OC].astype(F32)
                    mem[j] = jnp.concatenate(
                        [mem[j][:M], jnp.where(t < 2, m0, mem[j][M:])], axis=0)
                store_lhs(la_v, slice(c * OC, (c + 1) * OC), None, mem)
            sn = jnp.minimum(t + 1, NSEG - 1)
            xn = jnp.concatenate(
                [x_v[pl.ds(pl.multiple_of(sn * SEG, SEG), SEG), :].astype(F32), z_v[:SEG, :]],
                axis=0)
            xa_v[...] = xn
            store_lhs(la_v, slice(None), split_tokens(_layernorm(xn)), None)

            @pl.when(t >= 3)
            def _():
                r0 = pl.multiple_of(so * SEG, SEG)
                pltpu.make_async_copy(out_v.at[pl.ds(r0, SEG), :],
                                      out_hbm.at[pl.ds(r0, SEG), :], sem_out).start()
            return carry

        lax.fori_loop(0, cfg.get("nsteps", NSEG + 3), step, 0)
        nd = (cfg.get("nsteps", NSEG + 3) - 3) * SEG
        pltpu.make_async_copy(out_v.at[pl.ds(0, nd), :], out_hbm.at[pl.ds(0, nd), :], sem_out).wait()

    scratch = [
        pltpu.VMEM((S, D), BF16),
        pltpu.VMEM((S, D), BF16),
        pltpu.VMEM((HB, NP, DB // 2, 3 * DH), U32),
        pltpu.VMEM((NP, EB // 2, DB), U32),
        pltpu.VMEM((FB // LANES, NP, DB // 2, 2 * LANES), U32),
        pltpu.VMEM((NP, FB // 2, DB), U32),
        pltpu.VMEM((NP, RL // 2, DB), U32),
        pltpu.VMEM((NP, RL // 2, EB), U32),
        pltpu.VMEM((NP, SEG // 2, DB), U32),
        pltpu.VMEM((NP, SEG // 2, FB), U32),
        pltpu.VMEM((2 * SEG, D), F32),
        pltpu.VMEM((2 * SEG, D), F32),
        pltpu.VMEM((2 * SEG, D), F32),
        pltpu.VMEM((R, R), F32),
        pltpu.VMEM((R, R), jnp.int32),
        pltpu.SemaphoreType.DMA(()),
        pltpu.SemaphoreType.DMA((NST, NB)),
        pltpu.SemaphoreType.DMA(()),
    ]
    return kernel, scratch


def _build(cfg):
    @functools.partial(jax.jit, static_argnames=("A_seg_len",))
    def fn(A_x, A_mem0, A_Wq, A_Wk, A_Wv, A_Wo, A_seg_len, B_x, B_w_gate, B_w_up, B_w_down):
        B, S, D = A_x.shape
        _, H, DH = A_Wq.shape
        M = A_mem0.shape[1]
        FF = B_w_gate.shape[1]
        kernel, scratch = _make_kernel(S, D, H, DH, M, A_seg_len, FF, cfg)
        any_spec = pl.BlockSpec(memory_space=pl.ANY)
        out = pl.pallas_call(
            kernel,
            out_shape=jax.ShapeDtypeStruct((S, D), A_x.dtype),
            in_specs=[any_spec, pl.BlockSpec(memory_space=pltpu.VMEM)] + [any_spec] * 7,
            out_specs=any_spec,
            scratch_shapes=scratch,
            compiler_params=pltpu.CompilerParams(vmem_limit_bytes=cfg.get("vmem", 120) * 1024 * 1024,
                                                 flags=cfg.get("flags")),
        )(A_x.reshape(S, D), A_mem0.reshape(M, D),
          A_Wq.reshape(D * H, DH), A_Wk.reshape(D * H, DH), A_Wv.reshape(D * H, DH),
          A_Wo.reshape(H * DH, D), B_w_gate, B_w_up, B_w_down)
        return out.reshape(B, S, D)
    return fn


pallas_interleave_layers__memory_aug_recurrent_mem_tr__glu_gated_glu__prompt_kernel = _build({})
```

```python
import functools
import math

import jax
import jax.numpy as jnp
import numpy as np
from jax import lax
import jax.experimental.pallas as pl
import jax.experimental.pallas.tpu as pltpu

F32 = jnp.float32
BF16 = jnp.bfloat16
U32 = jnp.uint32
EPS = 1e-05
LANES = 128

STRASSEN = (2, (
    ({(1, 0): 1, (1, 1): 1}, {(0, 0): 1}, {(1, 0): 1, (1, 1): -1}, {0: 1, 1: 1}, {0: 1}),
    ({(1, 1): 1}, {(1, 0): 1, (0, 0): -1}, {(0, 0): 1, (1, 0): 1}, {1: 1}, {0: 1}),
    ({(0, 0): 1}, {(0, 1): 1, (1, 1): -1}, {(0, 1): 1, (1, 1): 1}, {0: 1}, {1: 1}),
    ({(0, 0): 1, (0, 1): 1}, {(1, 1): 1}, {(0, 0): -1, (0, 1): 1}, {0: 1, 1: 1}, {1: 1}),
    ({(0, 0): 1, (1, 1): 1}, {(0, 0): 1, (1, 1): 1}, {(0, 0): 1, (1, 1): 1}, None, None),
    ({(1, 0): 1, (0, 0): -1}, {(0, 0): 1, (0, 1): 1}, {(1, 1): 1}, None, None),
    ({(0, 1): 1, (1, 1): -1}, {(1, 0): 1, (1, 1): 1}, {(0, 0): 1}, None, None),
))
HK26 = (4, (
    ({(0, 0): 1}, {(0, 0): 1, (0, 2): 1, (1, 0): -1, (3, 0): 1}, {(0, 0): 1, (1, 0): -1}, None, None),
    ({(0, 0): 1, (1, 0): 1}, {(0, 0): 1, (0, 1): -1, (2, 0): 1, (3, 0): -1}, {(1, 0): 1}, {0: 1}, {0: 1}),
    ({(1, 1): 1}, {(0, 1): 1, (1, 1): -1, (1, 2): -1, (3, 1): 1}, {(0, 1): 1, (1, 1): -1}, {1: 1}, {1: -1}),
    ({(0, 1): 1, (1, 1): 1}, {(0, 3): -1, (1, 0): -1, (1, 1): 1, (1, 3): 1, (2, 1): -1, (3, 0): 1}, {(0, 1): 1}, None, None),
    ({(0, 2): 1}, {(1, 2): -1, (2, 0): 1, (2, 2): 1, (2, 3): 1}, {(0, 2): 1}, None, None),
    ({(1, 2): 1}, {(0, 2): 1, (2, 1): 1, (2, 2): 1, (3, 2): -1}, {(1, 2): 1}, {2: 1}, {2: 1}),
    ({(0, 3): 1}, {(0, 3): 1, (1, 3): -1, (3, 2): 1, (3, 3): 1}, {(0, 3): 1, (1, 3): -1}, None, None),
    ({(0, 3): 1, (1, 3): 1}, {(0, 3): -1, (2, 3): -1, (3, 1): 1, (3, 3): 1}, {(1, 3): 1}, {3: 1}, {3: 1}),
    ({(0, 0): 1, (1, 1): -1}, {(0, 1): 1, (1, 0): -1, (3, 0): 1}, {(0, 1): 1, (1, 0): 1}, {1: 1}, {0: -1}),
    ({(1, 0): 1, (1, 1): 1}, {(0, 1): 1}, {(1, 0): 1, (1, 1): 1}, {0: 1, 1: 1}, {0: 1, 1: 1}),
    ({(0, 0): 1, (0, 1): 1}, {(0, 3): 1, (1, 0): 1, (3, 0): -1}, {(0, 0): 1, (0, 1): 1}, None, None),
    ({(0, 0): 1, (1, 0): 1, (1, 2): -1}, {(0, 2): 1, (2, 0): -1}, {(0, 0): -1, (0, 2): 1, (1, 0): 1}, None, None),
    ({(1, 0): 1, (1, 2): -1}, {(0, 2): -1}, {(0, 0): -1, (0, 2): 1, (1, 0): 1, (1, 2): -1}, {0: 1, 2: -1}, {2: -1}),
    ({(0, 0): 1, (0, 2): -1, (1, 0): 1, (1, 2): -1}, {(2, 0): 1}, {(0, 0): -1, (0, 2): 1}, {0: 1, 2: -1}, {0: -1}),
    ({(0, 1): 1, (0, 2): 1, (1, 1): 1}, {(1, 2): 1, (2, 1): 1}, {(0, 1): 1, (1, 1): -1, (1, 2): 1}, None, None),
    ({(0, 1): 1, (0, 2): 1}, {(1, 2): 1}, {(0, 1): -1, (0, 2): 1, (1, 1): 1, (1, 2): -1}, {1: 1}, {1: -1, 2: 1}),
    ({(0, 1): 1, (0, 2): 1, (1, 1): 1, (1, 2): 1}, {(2, 1): -1}, {(1, 1): -1, (1, 2): 1}, {2: 1}, {1: -1, 2: 1}),
    ({(0, 3): -1, (1, 1): 1}, {(0, 3): -1, (1, 3): 1, (3, 1): 1}, {(0, 1): -1, (1, 3): 1}, {1: 1}, {3: 1}),
    ({(0, 1): 1, (0, 3): 1}, {(0, 3): -1, (1, 3): 1, (3, 0): 1}, {(0, 1): -1, (0, 3): 1}, None, None),
    ({(1, 1): 1, (1, 3): 1}, {(3, 1): -1}, {(1, 1): -1, (1, 3): 1}, {1: 1, 3: 1}, {1: -1, 3: 1}),
    ({(0, 3): 1, (1, 2): 1, (1, 3): 1}, {(2, 3): -1, (3, 2): -1}, {(0, 2): -1, (0, 3): 1, (1, 3): -1}, None, None),
    ({(0, 2): 1, (0, 3): 1, (1, 2): 1, (1, 3): 1}, {(2, 3): 1}, {(0, 2): -1, (0, 3): 1}, {2: 1, 3: 1}, {3: 1}),
    ({(1, 2): 1, (1, 3): 1}, {(3, 2): 1}, {(0, 2): -1, (0, 3): 1, (1, 2): 1, (1, 3): -1}, {2: 1, 3: 1}, {2: 1}),
    ({(0, 0): 1, (1, 0): 1, (1, 1): 1, (1, 3): 1}, {(3, 0): -1}, {(0, 0): 1, (0, 1): 1, (0, 3): -1, (1, 0): -1}, {0: 1, 1: 1, 3: 1}, {0: -1}),
    ({(0, 0): 1, (0, 1): 1, (0, 3): 1, (1, 0): 1, (1, 1): 1, (1, 3): 1}, {(0, 3): -1, (3, 0): 1}, {(0, 0): 1, (0, 1): 1, (0, 3): -1}, None, None),
    ({(0, 3): 1, (1, 0): 1, (1, 1): 1, (1, 3): 1}, {(0, 3): 1}, {(0, 0): 1, (0, 1): 1, (0, 3): -1, (1, 3): 1}, {0: 1, 1: 1, 3: 1}, {3: 1}),
))
SCHEMES = {"strassen": STRASSEN, "hk26": HK26}


def _combine(coefs, vals):
    acc = None
    for key, c in sorted(coefs.items(), key=lambda kv: -kv[1]):
        v = vals[key]
        if abs(c) != 1:
            v = v * abs(c)
        if acc is None:
            acc = v if c > 0 else -v
        else:
            acc = acc + v if c > 0 else acc - v
    return acc


def _accumulate(accs, coefs, v):
    for key, c in coefs.items():
        t = v if abs(c) == 1 else v * abs(c)
        if key not in accs:
            accs[key] = t if c > 0 else -t
        else:
            accs[key] = accs[key] + t if c > 0 else accs[key] - t


def _layernorm(x):
    m = jnp.mean(x, axis=-1, keepdims=True)
    c = x - m
    v = jnp.mean(c * c, axis=-1, keepdims=True)
    return c * lax.rsqrt(v + EPS)


def _dot(a, b):
    return jnp.dot(a, b, preferred_element_type=F32)


def _dot_nt(a, b):
    return lax.dot_general(a, b, (((1,), (1,)), ((), ())), preferred_element_type=F32)


def _halves(x):
    return [pltpu.unpack_elementwise(x, index=k, packed_dtype=BF16, unpacked_dtype=F32)
            for k in range(2)]


def _pair(lo, hi):
    return pltpu.pack_elementwise([lo, hi], packed_dtype=BF16)


def _make_kernel(S, D, H, DH, M, SEG, FF, cfg):
    NB, prods = SCHEMES[cfg.get("scheme", "hk26")]
    if "order" in cfg:
        prods = tuple(prods[i] for i in cfg["order"])
    NP = len(prods)
    NSEG = S // SEG
    MM = 2 * M
    R = MM + 2 * SEG
    RL = MM + SEG
    DB, HB, FB = D // NB, H // NB, FF // NB
    EB = HB * DH
    OC = DB // 2
    QR = cfg.get("QR", 128) // NB
    QST = cfg.get("QST", 4)
    WR = 512 // NB
    OST = FF // (WR * NB)
    GST = 4
    GR, DR = DB // GST, FB // GST
    XH = 2 * SEG
    scale = DH ** (-0.5)
    c_exp = scale * math.log2(math.e)

    def put_lhs(ref, r, tile0, rows, val):
        for k in range(val.shape[1] // LANES):
            ref[r, tile0 + k, rows, :] = val[:, k * LANES:(k + 1) * LANES].astype(BF16)

    def store_lhs(ref, tile0, tok, mem):
        for r, (u, _, _, um, _) in enumerate(prods):
            if tok is not None:
                put_lhs(ref, r, tile0, slice(ref.shape[2] - SEG, None), _combine(u, tok))
            if mem is not None and um is not None:
                put_lhs(ref, r, tile0, slice(0, mem[0].shape[0]), _combine(um, mem))

    def fast_dot(lhs_ref, w_of, with_tok, with_mem, hooks=None):
        def lhs(r, rows):
            return jnp.concatenate(
                [lhs_ref[r, k, rows, :] for k in range(lhs_ref.shape[1])], axis=1)

        tok, mem = {}, {}
        for r, (_, _, w, um, wm) in enumerate(prods):
            if hooks and r in hooks:
                hooks[r]()
            if with_mem and um is not None:
                p = _dot(lhs(r, slice(None)), pltpu.bitcast(w_of(r), BF16))
                if with_tok:
                    _accumulate(mem, wm, p[:MM])
                    _accumulate(tok, w, p[MM:])
                else:
                    _accumulate(mem, wm, p)
            elif with_tok:
                p = _dot(lhs(r, slice(lhs_ref.shape[2] - SEG, None)), pltpu.bitcast(w_of(r), BF16))
                _accumulate(tok, w, p)
        return tok, mem

    def split_tokens(x):
        return {(hf, i): x[hf * SEG:(hf + 1) * SEG, i * DB:(i + 1) * DB]
                for hf in range(2) for i in range(NB)}

    def split_cols(x):
        return {i: x[:, i * DB:(i + 1) * DB] for i in range(NB)}

    def out_cols(j, c):
        return slice(j * DB + c * OC, j * DB + (c + 1) * OC)

    def kernel(x_hbm, mem0_ref, wq_hbm, wk_hbm, wv_hbm, wo_hbm, wg_hbm, wu_hbm, wd_hbm,
               out_hbm,
               x_v, big_v, gst_v, qst_v, qtr_v, wqkv_v, wo_v, wgu_v, wd_v,
               la_v, lo_v, lb_v, ld_v, mem_v, xa_v, ya_v, z_v, fill_v, keep_v,
               sem_x, sem_q, sem_o, sem_g, sem_d, sem_out):

        def rows_at(start, size):
            return pl.ds(start if isinstance(start, int) else pl.multiple_of(start, 16), size)

        def q_copies(w, c, slot):
            src = (wq_hbm, wk_hbm, wv_hbm)[w]
            return [pltpu.make_async_copy(src.at[rows_at((i * DB + c * QR) * H, QR * H), :],
                                          qst_v.at[slot, i], sem_q.at[slot, i]) for i in range(NB)]

        def o_copies(c):
            slot = c % OST
            return [pltpu.make_async_copy(wo_hbm.at[rows_at(i * EB + c * WR, WR), :],
                                          big_v.at[rows_at((slot * NB + i) * WR, WR), :],
                                          sem_o.at[slot, i]) for i in range(NB)]

        def g_copies(src, c):
            return [pltpu.make_async_copy(src.at[rows_at(i * DB + c * GR, GR), :],
                                          gst_v.at[c, i], sem_g.at[c, i]) for i in range(NB)]

        def d_copies(c):
            return [pltpu.make_async_copy(wd_hbm.at[rows_at(i * FB + c * DR, DR), :],
                                          big_v.at[rows_at(i * FB + c * DR, DR), :],
                                          sem_d.at[c, i]) for i in range(NB)]

        def start(copies):
            for cp in copies:
                cp.start()

        def wait(copies):
            for cp in copies:
                cp.wait()

        def prep_tiles(load, put, nrows, ncols, mul=None):
            def tile(n, carry):
                s, k = lax.div(n, ncols), lax.rem(n, ncols)
                lo, hi = {}, {}
                for i in range(NB):
                    for j in range(NB):
                        x = load(i, j, pl.multiple_of(s * 16, 16), k)
                        lo[i, j], hi[i, j] = _halves(pltpu.bitcast(x, U32))
                        if mul is not None:
                            lo[i, j], hi[i, j] = lo[i, j] * mul, hi[i, j] * mul
                for r, (_, v, _, _, _) in enumerate(prods):
                    put(r, s * 8, k, _pair(_combine(v, lo), _combine(v, hi)))
                return carry
            lax.fori_loop(0, nrows // 16 * ncols, tile, 0)

        def lanes_at(k):
            return pl.ds(pl.multiple_of(k * LANES, LANES), LANES)

        def words_at(row):
            return pl.ds(pl.multiple_of(row, 8), 8)

        def prep_qkv(w, c, slot):
            def heads(i, carry):
                st = qst_v.at[slot, i].bitcast(U32)
                for jp in range(H // 2):
                    for k, x in enumerate(_halves(st[pl.ds(jp, QR, stride=H // 2), :])):
                        qtr_v[i, 2 * jp + k] = x.astype(BF16)
                return carry
            lax.fori_loop(0, NB, heads, 0)

            def put(r, row, k, val):
                wqkv_v[k, r, words_at(c * (QR // 2) + row), lanes_at(w)] = val
            prep_tiles(lambda i, j, row, k: qtr_v[i, j * HB + k, pl.ds(row, 16), :], put, QR, HB)

        def prep_from_big(dst, base, blk, c, nrows):
            def load(i, j, row, k):
                return big_v[rows_at(base + i * blk + row, 16), lanes_at(j * (DB // LANES) + k)]

            def put(r, row, k, val):
                dst[r, words_at(c * (nrows // 2) + row), lanes_at(k)] = val
            prep_tiles(load, put, nrows, DB // LANES)

        def prep_gu(w, c):
            def load(i, j, row, k):
                return gst_v[c, i, pl.ds(row, 16), lanes_at(j * (FB // LANES) + k)]

            def put(r, row, k, val):
                wgu_v[k, r, words_at(c * (GR // 2) + row), w * LANES:(w + 1) * LANES] = val
            prep_tiles(load, put, GR, FB // LANES, 0.5)

        x_head = pltpu.make_async_copy(x_hbm.at[0:XH, :], x_v.at[0:XH, :], sem_x.at[0])
        x_tail = pltpu.make_async_copy(x_hbm.at[XH:, :], x_v.at[XH:, :], sem_x.at[1])
        NQ, NO = DB // QR, EB // WR
        ONEXT = min(QST * QR * H * DH // (WR * D), OST)
        for n in range(QST):
            start(q_copies(0, n, n))
        x_head.start()

        ri = lax.broadcasted_iota(jnp.int32, (R, LANES), 0)
        ci = lax.broadcasted_iota(jnp.int32, (R, LANES), 1)

        def layer_of(i):
            return jnp.where(i < MM, (i >= M).astype(jnp.int32), (i >= MM + SEG).astype(jnp.int32))

        same = (layer_of(ri) == layer_of(ci)) & (ci < R)
        visible = (ri < MM) | (ri >= ci)
        keep_v[...] = (same & visible).astype(jnp.int32)
        fill_v[...] = jnp.where(same, -1e9 / scale, -jnp.inf).astype(F32)
        mem_v[0:M, :] = mem0_ref[...].astype(F32)
        mem_v[M:, :] = mem0_ref[...].astype(F32)

        for w in range(3):
            def q_body(c, carry, w=w):
                slot = (w * NQ + c) % QST
                wait(q_copies(w, c, slot))
                prep_qkv(w, c, slot)
                pl.when(c + QST < NQ)(lambda: start(q_copies(w, c + QST, slot)))
                if w < 2:
                    pl.when(c + QST >= NQ)(lambda: start(q_copies(w + 1, c + QST - NQ, slot)))
                else:
                    pl.when((c + QST >= NQ) & (c + QST - NQ < ONEXT))(
                        lambda: start(o_copies(c + QST - NQ)))
                return carry
            lax.fori_loop(0, NQ, q_body, 0)

        def o_body(c, carry):
            wait(o_copies(c))
            prep_from_big(wo_v, (c % OST) * NB * WR, WR, c, WR)
            pl.when(c + ONEXT < NO)(lambda: start(o_copies(c + ONEXT)))
            pl.when(c >= NO - GST)(lambda: start(g_copies(wg_hbm, c - (NO - GST))))
            return carry
        lax.fori_loop(0, NO, o_body, 0)
        for c in range(GST):
            start(d_copies(c))
        x_head.wait()
        xa_v[...] = x_v[0:XH, :].astype(F32)

        def load_glu_weights():
            def gate(c, carry):
                wait(g_copies(wg_hbm, c))
                prep_gu(0, c)
                start(g_copies(wu_hbm, c))
                return carry

            def down(c, carry):
                wait(d_copies(c))
                prep_from_big(wd_v, c * DR, FB, c, DR)
                return carry

            def up(c, carry):
                wait(g_copies(wu_hbm, c))
                prep_gu(1, c)
                return carry
            lax.fori_loop(0, GST, gate, 0)
            lax.fori_loop(0, GST, down, 0)
            lax.fori_loop(0, GST, up, 0)
            x_tail.start()

        def attention(rows_of, emit):
            pv = {}

            def scores():
                for j in range(NB):
                    qkv = rows_of(j).astype(BF16)
                    n = qkv.shape[0]
                    q, k, v = (qkv[:, w * DH:(w + 1) * DH] for w in range(3))
                    pad = jnp.zeros((LANES - n, DH), BF16)
                    k, v = jnp.concatenate([k, pad], axis=0), jnp.concatenate([v, pad], axis=0)
                    s = jnp.where(keep_v[0:n, :] != 0, _dot_nt(q, k), fill_v[0:n, :])
                    mx = jnp.max(s, axis=-1, keepdims=True)
                    e = jnp.exp2((s - mx) * c_exp)
                    den = jnp.sum(e, axis=-1, keepdims=True)
                    inv = pl.reciprocal(den, approx=True)
                    inv = inv * (2.0 - den * inv)
                    pv[j] = ((e * inv).astype(BF16), v)

            def values():
                emit({j: _dot(*pv[j]) for j in range(NB)})

            return scores, values

        h0, h1 = cfg.get("h0", 4), cfg.get("h1", 16)

        def gate_up(hooks):
            for c in range(FB // LANES):
                gu, _ = fast_dot(lb_v, lambda r: wgu_v[c, r], True, False, hooks if c == 0 else None)
                act = {k: jnp.tanh(v[:, :LANES]) * v[:, LANES:] + v[:, LANES:] for k, v in gu.items()}
                store_lhs(ld_v, c, act, None)

        def down():
            for c in range(DB // OC):
                dn, _ = fast_dot(ld_v, lambda r: wd_v[r, :, c * OC:(c + 1) * OC], True, False)
                for (hf, j), v in dn.items():
                    z_v[hf * SEG:(hf + 1) * SEG, out_cols(j, c)] += v

        def glu_input():
            ya = ya_v[0:2 * SEG, :]
            z_v[...] = ya
            store_lhs(lb_v, 0, split_tokens(_layernorm(ya)), None)

        def out_copy(row, n):
            return pltpu.make_async_copy(big_v.at[pl.ds(row, n), :],
                                         out_hbm.at[pl.ds(row, n), :], sem_out)

        def attention_single(mrow, xrow, yrow):
            m = mem_v[pl.ds(mrow, M), :]
            x = xa_v[pl.ds(xrow, SEG), :]
            store_lhs(la_v, 0, None, split_cols(jnp.concatenate([m, m, _layernorm(x)], axis=0)))
            hooks = None
            for c in range(HB):
                _, cur = fast_dot(la_v, lambda r: wqkv_v[c, r], False, True, hooks)
                scores, values = attention(
                    lambda j, cur=cur: cur[j], lambda o, c=c: store_lhs(lo_v, c, None, o))
                hooks = {h0: scores, NP - 1: values}
            scores()
            values()
            for c in range(DB // OC):
                _, o = fast_dot(lo_v, lambda r: wo_v[r, :, c * OC:(c + 1) * OC], False, True)
                for j in range(NB):
                    mem_v[pl.ds(mrow, M), out_cols(j, c)] = o[j][:M]
                    ya_v[pl.ds(yrow, SEG), out_cols(j, c)] = (
                        xa_v[pl.ds(xrow, SEG), out_cols(j, c)] + o[j][MM:])

        def step(t, carry):
            glu_input()
            hooks = None
            for c in range(HB):
                tok, mem = fast_dot(la_v, lambda r: wqkv_v[c, r], True, True, hooks)
                scores, values = attention(
                    lambda j, tok=tok, mem=mem: jnp.concatenate(
                        [mem[j], tok[0, j], tok[1, j]], axis=0),
                    lambda o, c=c: store_lhs(
                        lo_v, c,
                        {(hf, j): o[j][MM + hf * SEG:MM + (hf + 1) * SEG]
                         for hf in range(2) for j in range(NB)},
                        {j: o[j][:MM] for j in range(NB)}))
                hooks = {h0: scores, h1: values}
            gate_up({h0: scores, NP - 1: values})

            def project(c, hooks=None):
                tok, mem = fast_dot(lo_v, lambda r: wo_v[r, :, c * OC:(c + 1) * OC], True, True, hooks)
                for (hf, j), v in tok.items():
                    rows = slice(hf * SEG, (hf + 1) * SEG)
                    ya_v[rows, out_cols(j, c)] = xa_v[rows, out_cols(j, c)] + v
                for j in range(NB):
                    mem_v[:, out_cols(j, c)] = mem[j]
                store_lhs(la_v, c * OC // LANES, None, mem)

            project(0)
            down()
            row = pl.multiple_of(jnp.maximum(t - 3, 0) * SEG, SEG)
            big_v[pl.ds(row, SEG), :] = z_v[SEG:, :].astype(BF16)
            nxt = pl.multiple_of(jnp.minimum(t + 1, NSEG - 1) * SEG, SEG)
            xn = jnp.concatenate([x_v[pl.ds(nxt, SEG), :].astype(F32), z_v[:SEG, :]], axis=0)
            store_lhs(la_v, 0, split_tokens(_layernorm(xn)), None)
            project(1)
            xa_v[:SEG, :] = x_v[pl.ds(nxt, SEG), :].astype(F32)
            xa_v[SEG:, :] = z_v[:SEG, :]
            pl.when(t >= 3)(lambda: out_copy(row, SEG).start())
            return carry

        def phase(ph, carry):
            attention_single(pl.multiple_of(jnp.where(ph < 2, 0, M), M),
                             pl.multiple_of(jnp.where(ph == 0, 0, SEG), SEG),
                             pl.multiple_of(jnp.where(ph == 3, 1, ph) * SEG, SEG))
            pl.when(ph == 1)(load_glu_weights)

            @pl.when(ph >= 1)
            def _():
                glu_input()
                gate_up(None)
                down()

            @pl.when(ph == 1)
            def _():
                x_tail.wait()
                ya_v[0:SEG, :] = ya_v[SEG:2 * SEG, :]
                xn = jnp.concatenate(
                    [x_v[2 * SEG:3 * SEG, :].astype(F32), z_v[:SEG, :]], axis=0)
                xa_v[...] = xn
                store_lhs(la_v, 0, split_tokens(_layernorm(xn)), split_cols(mem_v[...]))
                lax.fori_loop(2, cfg.get("nsteps", NSEG), step, 0)

            @pl.when(ph == 2)
            def _():
                xa_v[SEG:, :] = z_v[:SEG, :]
                ya_v[0:SEG, :] = ya_v[2 * SEG:, :]
                big_v[S - 3 * SEG:S - 2 * SEG, :] = z_v[SEG:, :].astype(BF16)
                out_copy(S - 3 * SEG, SEG).start()

            @pl.when(ph == 3)
            def _():
                big_v[S - 2 * SEG:S, :] = z_v[...].astype(BF16)
                out_copy(S - 2 * SEG, 2 * SEG).start()
            return carry

        lax.fori_loop(0, cfg.get('nph', 4), phase, 0)
        out_copy(0, cfg.get("nsteps", NSEG) * SEG).wait()

    scratch = [
        pltpu.VMEM((S, D), BF16),
        pltpu.VMEM((FF, D), BF16),
        pltpu.VMEM((GST, NB, GR, FF), BF16),
        pltpu.VMEM((QST, NB, QR * H, DH), BF16),
        pltpu.VMEM((NB, H, QR, DH), BF16),
        pltpu.VMEM((HB, NP, DB // 2, 3 * DH), U32),
        pltpu.VMEM((NP, EB // 2, DB), U32),
        pltpu.VMEM((FB // LANES, NP, DB // 2, 2 * LANES), U32),
        pltpu.VMEM((NP, FB // 2, DB), U32),
        pltpu.VMEM((NP, DB // LANES, RL, LANES), BF16),
        pltpu.VMEM((NP, EB // LANES, RL, LANES), BF16),
        pltpu.VMEM((NP, DB // LANES, SEG, LANES), BF16),
        pltpu.VMEM((NP, FB // LANES, SEG, LANES), BF16),
        pltpu.VMEM((MM, D), F32),
        pltpu.VMEM((2 * SEG, D), F32),
        pltpu.VMEM((3 * SEG, D), F32),
        pltpu.VMEM((2 * SEG, D), F32),
        pltpu.VMEM((R, LANES), F32),
        pltpu.VMEM((R, LANES), jnp.int32),
        pltpu.SemaphoreType.DMA((2,)),
        pltpu.SemaphoreType.DMA((QST, NB)),
        pltpu.SemaphoreType.DMA((OST, NB)),
        pltpu.SemaphoreType.DMA((GST, NB)),
        pltpu.SemaphoreType.DMA((GST, NB)),
        pltpu.SemaphoreType.DMA(()),
    ]
    return kernel, scratch


def _build(cfg):
    @functools.partial(jax.jit, static_argnames=("A_seg_len",))
    def fn(A_x, A_mem0, A_Wq, A_Wk, A_Wv, A_Wo, A_seg_len, B_x, B_w_gate, B_w_up, B_w_down):
        B, S, D = A_x.shape
        _, H, DH = A_Wq.shape
        M = A_mem0.shape[1]
        FF = B_w_gate.shape[1]
        kernel, scratch = _make_kernel(S, D, H, DH, M, A_seg_len, FF, cfg)
        any_spec = pl.BlockSpec(memory_space=pl.ANY)
        out = pl.pallas_call(
            kernel,
            out_shape=jax.ShapeDtypeStruct((S, D), A_x.dtype),
            in_specs=[any_spec, pl.BlockSpec(memory_space=pltpu.VMEM)] + [any_spec] * 7,
            out_specs=any_spec,
            scratch_shapes=scratch,
            compiler_params=pltpu.CompilerParams(vmem_limit_bytes=cfg.get("vmem", 124) * 1024 * 1024,
                                                 flags=cfg.get("flags")),
        )(A_x.reshape(S, D), A_mem0.reshape(M, D),
          A_Wq.reshape(D * H, DH), A_Wk.reshape(D * H, DH), A_Wv.reshape(D * H, DH),
          A_Wo.reshape(H * DH, D), B_w_gate, B_w_up, B_w_down)
        return out.reshape(B, S, D)
    return fn


pallas_interleave_layers__memory_aug_recurrent_mem_tr__glu_gated_glu__prompt_kernel = _build({})
```

```python
import functools
import itertools
import math

import jax
import jax.numpy as jnp
import numpy as np
from jax import lax
import jax.experimental.pallas as pl
import jax.experimental.pallas.tpu as pltpu

F32 = jnp.float32
BF16 = jnp.bfloat16
U32 = jnp.uint32
EPS = 1e-05
LANES = 128

STRASSEN = (2, (
    ({(1, 0): 1, (1, 1): 1}, {(0, 0): 1}, {(1, 0): 1, (1, 1): -1}, {0: 1, 1: 1}, {0: 1}),
    ({(1, 1): 1}, {(1, 0): 1, (0, 0): -1}, {(0, 0): 1, (1, 0): 1}, {1: 1}, {0: 1}),
    ({(0, 0): 1}, {(0, 1): 1, (1, 1): -1}, {(0, 1): 1, (1, 1): 1}, {0: 1}, {1: 1}),
    ({(0, 0): 1, (0, 1): 1}, {(1, 1): 1}, {(0, 0): -1, (0, 1): 1}, {0: 1, 1: 1}, {1: 1}),
    ({(0, 0): 1, (1, 1): 1}, {(0, 0): 1, (1, 1): 1}, {(0, 0): 1, (1, 1): 1}, None, None),
    ({(1, 0): 1, (0, 0): -1}, {(0, 0): 1, (0, 1): 1}, {(1, 1): 1}, None, None),
    ({(0, 1): 1, (1, 1): -1}, {(1, 0): 1, (1, 1): 1}, {(0, 0): 1}, None, None),
))
HK26 = (4, (
    ({(0, 0): 1}, {(0, 0): 1, (0, 2): 1, (1, 0): -1, (3, 0): 1}, {(0, 0): 1, (1, 0): -1}, None, None),
    ({(0, 0): 1, (1, 0): 1}, {(0, 0): 1, (0, 1): -1, (2, 0): 1, (3, 0): -1}, {(1, 0): 1}, {0: 1}, {0: 1}),
    ({(1, 1): 1}, {(0, 1): 1, (1, 1): -1, (1, 2): -1, (3, 1): 1}, {(0, 1): 1, (1, 1): -1}, {1: 1}, {1: -1}),
    ({(0, 1): 1, (1, 1): 1}, {(0, 3): -1, (1, 0): -1, (1, 1): 1, (1, 3): 1, (2, 1): -1, (3, 0): 1}, {(0, 1): 1}, None, None),
    ({(0, 2): 1}, {(1, 2): -1, (2, 0): 1, (2, 2): 1, (2, 3): 1}, {(0, 2): 1}, None, None),
    ({(1, 2): 1}, {(0, 2): 1, (2, 1): 1, (2, 2): 1, (3, 2): -1}, {(1, 2): 1}, {2: 1}, {2: 1}),
    ({(0, 3): 1}, {(0, 3): 1, (1, 3): -1, (3, 2): 1, (3, 3): 1}, {(0, 3): 1, (1, 3): -1}, None, None),
    ({(0, 3): 1, (1, 3): 1}, {(0, 3): -1, (2, 3): -1, (3, 1): 1, (3, 3): 1}, {(1, 3): 1}, {3: 1}, {3: 1}),
    ({(0, 0): 1, (1, 1): -1}, {(0, 1): 1, (1, 0): -1, (3, 0): 1}, {(0, 1): 1, (1, 0): 1}, {1: 1}, {0: -1}),
    ({(1, 0): 1, (1, 1): 1}, {(0, 1): 1}, {(1, 0): 1, (1, 1): 1}, {0: 1, 1: 1}, {0: 1, 1: 1}),
    ({(0, 0): 1, (0, 1): 1}, {(0, 3): 1, (1, 0): 1, (3, 0): -1}, {(0, 0): 1, (0, 1): 1}, None, None),
    ({(0, 0): 1, (1, 0): 1, (1, 2): -1}, {(0, 2): 1, (2, 0): -1}, {(0, 0): -1, (0, 2): 1, (1, 0): 1}, None, None),
    ({(1, 0): 1, (1, 2): -1}, {(0, 2): -1}, {(0, 0): -1, (0, 2): 1, (1, 0): 1, (1, 2): -1}, {0: 1, 2: -1}, {2: -1}),
    ({(0, 0): 1, (0, 2): -1, (1, 0): 1, (1, 2): -1}, {(2, 0): 1}, {(0, 0): -1, (0, 2): 1}, {0: 1, 2: -1}, {0: -1}),
    ({(0, 1): 1, (0, 2): 1, (1, 1): 1}, {(1, 2): 1, (2, 1): 1}, {(0, 1): 1, (1, 1): -1, (1, 2): 1}, None, None),
    ({(0, 1): 1, (0, 2): 1}, {(1, 2): 1}, {(0, 1): -1, (0, 2): 1, (1, 1): 1, (1, 2): -1}, {1: 1}, {1: -1, 2: 1}),
    ({(0, 1): 1, (0, 2): 1, (1, 1): 1, (1, 2): 1}, {(2, 1): -1}, {(1, 1): -1, (1, 2): 1}, {2: 1}, {1: -1, 2: 1}),
    ({(0, 3): -1, (1, 1): 1}, {(0, 3): -1, (1, 3): 1, (3, 1): 1}, {(0, 1): -1, (1, 3): 1}, {1: 1}, {3: 1}),
    ({(0, 1): 1, (0, 3): 1}, {(0, 3): -1, (1, 3): 1, (3, 0): 1}, {(0, 1): -1, (0, 3): 1}, None, None),
    ({(1, 1): 1, (1, 3): 1}, {(3, 1): -1}, {(1, 1): -1, (1, 3): 1}, {1: 1, 3: 1}, {1: -1, 3: 1}),
    ({(0, 3): 1, (1, 2): 1, (1, 3): 1}, {(2, 3): -1, (3, 2): -1}, {(0, 2): -1, (0, 3): 1, (1, 3): -1}, None, None),
    ({(0, 2): 1, (0, 3): 1, (1, 2): 1, (1, 3): 1}, {(2, 3): 1}, {(0, 2): -1, (0, 3): 1}, {2: 1, 3: 1}, {3: 1}),
    ({(1, 2): 1, (1, 3): 1}, {(3, 2): 1}, {(0, 2): -1, (0, 3): 1, (1, 2): 1, (1, 3): -1}, {2: 1, 3: 1}, {2: 1}),
    ({(0, 0): 1, (1, 0): 1, (1, 1): 1, (1, 3): 1}, {(3, 0): -1}, {(0, 0): 1, (0, 1): 1, (0, 3): -1, (1, 0): -1}, {0: 1, 1: 1, 3: 1}, {0: -1}),
    ({(0, 0): 1, (0, 1): 1, (0, 3): 1, (1, 0): 1, (1, 1): 1, (1, 3): 1}, {(0, 3): -1, (3, 0): 1}, {(0, 0): 1, (0, 1): 1, (0, 3): -1}, None, None),
    ({(0, 3): 1, (1, 0): 1, (1, 1): 1, (1, 3): 1}, {(0, 3): 1}, {(0, 0): 1, (0, 1): 1, (0, 3): -1, (1, 3): 1}, {0: 1, 1: 1, 3: 1}, {3: 1}),
))
SCHEMES = {"strassen": STRASSEN, "hk26": HK26}


def _combine(coefs, vals):
    acc = None
    for key, c in sorted(coefs.items(), key=lambda kv: -kv[1]):
        v = vals[key]
        if abs(c) != 1:
            v = v * abs(c)
        if acc is None:
            acc = v if c > 0 else -v
        else:
            acc = acc + v if c > 0 else acc - v
    return acc


def _accumulate(accs, coefs, v):
    for key, c in coefs.items():
        t = v if abs(c) == 1 else v * abs(c)
        if key not in accs:
            accs[key] = t if c > 0 else -t
        else:
            accs[key] = accs[key] + t if c > 0 else accs[key] - t


def _layernorm(x):
    m = jnp.mean(x, axis=-1, keepdims=True)
    c = x - m
    v = jnp.mean(c * c, axis=-1, keepdims=True)
    return c * lax.rsqrt(v + EPS)


def _dot(a, b):
    return jnp.dot(a, b, preferred_element_type=F32)


def _dot_nt(a, b):
    return lax.dot_general(a, b, (((1,), (1,)), ((), ())), preferred_element_type=F32)


def _halves(x):
    return [pltpu.unpack_elementwise(x, index=k, packed_dtype=BF16, unpacked_dtype=F32)
            for k in range(2)]


def _pair(lo, hi):
    return pltpu.pack_elementwise([lo, hi], packed_dtype=BF16)


def _make_kernel(S, D, H, DH, M, SEG, FF, cfg):
    NB, prods = SCHEMES[cfg.get("scheme", "hk26")]
    if "order" in cfg:
        prods = tuple(prods[i] for i in cfg["order"])
    NP = len(prods)
    NSEG = S // SEG
    MM = 2 * M
    R = MM + 2 * SEG
    RL = MM + SEG
    DB, HB, FB = D // NB, H // NB, FF // NB
    EB = HB * DH
    OC = DB // 2
    QR = cfg.get("QR", 128) // NB
    QST = cfg.get("QST", 4)
    WR = 512 // NB
    OST = FF // (WR * NB)
    GST = 4
    GR, DR = DB // GST, FB // GST
    XH = 2 * SEG
    scale = DH ** (-0.5)
    c_exp = scale * math.log2(math.e)

    def put_lhs(ref, r, tile0, rows, val):
        for k in range(val.shape[1] // LANES):
            ref[r, tile0 + k, rows, :] = val[:, k * LANES:(k + 1) * LANES].astype(BF16)

    def store_lhs(ref, tile0, tok, mem):
        for r, (u, _, _, um, _) in enumerate(prods):
            if tok is not None:
                put_lhs(ref, r, tile0, slice(ref.shape[2] - SEG, None), _combine(u, tok))
            if mem is not None and um is not None:
                put_lhs(ref, r, tile0, slice(0, mem[0].shape[0]), _combine(um, mem))

    def fast_dot(*args):
        res = []
        for _ in fast_dot_steps(res, *args):
            pass
        return res

    def fast_dot_steps(res, lhs_ref, w_of, with_tok, with_mem, hooks=None, source=None):
        def lhs(r, rows):
            if source is None:
                return jnp.concatenate(
                    [lhs_ref[r, k, rows, :] for k in range(lhs_ref.shape[1])], axis=1)
            u, um = prods[r][0], prods[r][3]
            tok_ref, mem_ref = source
            val = _combine(u, {(hf, i): tok_ref[hf * SEG:(hf + 1) * SEG, i * DB:(i + 1) * DB]
                               for hf, i in u})
            if with_mem and um is not None:
                val = jnp.concatenate(
                    [_combine(um, {i: mem_ref[:, i * DB:(i + 1) * DB] for i in um}), val], axis=0)
            val = val.astype(BF16)
            put_lhs(lhs_ref, r, 0, rows, val)
            return val

        tok, mem = {}, {}
        for r, (_, _, w, um, wm) in enumerate(prods):
            if hooks and r in hooks:
                hooks[r]()
            if with_mem and um is not None:
                p = _dot(lhs(r, slice(None)), pltpu.bitcast(w_of(r), BF16))
                if with_tok:
                    _accumulate(mem, wm, p[:MM])
                    _accumulate(tok, w, p[MM:])
                else:
                    _accumulate(mem, wm, p)
            elif with_tok:
                p = _dot(lhs(r, slice(lhs_ref.shape[2] - SEG, None)), pltpu.bitcast(w_of(r), BF16))
                _accumulate(tok, w, p)
            yield
        res += [tok, mem]

    def split_tokens(x):
        return {(hf, i): x[hf * SEG:(hf + 1) * SEG, i * DB:(i + 1) * DB]
                for hf in range(2) for i in range(NB)}

    def split_cols(x):
        return {i: x[:, i * DB:(i + 1) * DB] for i in range(NB)}

    def out_cols(j, c):
        return slice(j * DB + c * OC, j * DB + (c + 1) * OC)

    def kernel(x_hbm, mem0_ref, wq_hbm, wk_hbm, wv_hbm, wo_hbm, wg_hbm, wu_hbm, wd_hbm,
               out_hbm,
               x_v, big_v, gst_v, qst_v, qtr_v, wqkv_v, wo_v, wgu_v, wd_v,
               la_v, lo_v, lb_v, ld_v, mem_v, xa_v, na_v, nb_v, ya_v, z_v, qkv_v, fill_v, keep_v,
               sem_x, sem_q, sem_o, sem_g, sem_d, sem_out):

        def rows_at(start, size):
            return pl.ds(start if isinstance(start, int) else pl.multiple_of(start, 16), size)

        def q_copies(w, c, slot):
            src = (wq_hbm, wk_hbm, wv_hbm)[w]
            return [pltpu.make_async_copy(src.at[rows_at((i * DB + c * QR) * H, QR * H), :],
                                          qst_v.at[slot, i], sem_q.at[slot, i]) for i in range(NB)]

        def o_copies(c):
            slot = c % OST
            return [pltpu.make_async_copy(wo_hbm.at[rows_at(i * EB + c * WR, WR), :],
                                          big_v.at[rows_at((slot * NB + i) * WR, WR), :],
                                          sem_o.at[slot, i]) for i in range(NB)]

        def g_copies(src, c):
            return [pltpu.make_async_copy(src.at[rows_at(i * DB + c * GR, GR), :],
                                          gst_v.at[c, i], sem_g.at[c, i]) for i in range(NB)]

        def d_copies(c):
            return [pltpu.make_async_copy(wd_hbm.at[rows_at(i * FB + c * DR, DR), :],
                                          big_v.at[rows_at(i * FB + c * DR, DR), :],
                                          sem_d.at[c, i]) for i in range(NB)]

        def start(copies):
            for cp in copies:
                cp.start()

        def wait(copies):
            for cp in copies:
                cp.wait()

        def prep_tiles(load, put, nrows, ncols, mul=None):
            def tile(n, carry):
                s, k = lax.div(n, ncols), lax.rem(n, ncols)
                lo, hi = {}, {}
                for i in range(NB):
                    for j in range(NB):
                        x = load(i, j, pl.multiple_of(s * 16, 16), k)
                        lo[i, j], hi[i, j] = _halves(pltpu.bitcast(x, U32))
                        if mul is not None:
                            lo[i, j], hi[i, j] = lo[i, j] * mul, hi[i, j] * mul
                for r, (_, v, _, _, _) in enumerate(prods):
                    put(r, s * 8, k, _pair(_combine(v, lo), _combine(v, hi)))
                return carry
            lax.fori_loop(0, nrows // 16 * ncols, tile, 0)

        def lanes_at(k):
            return pl.ds(pl.multiple_of(k * LANES, LANES), LANES)

        def words_at(row):
            return pl.ds(pl.multiple_of(row, 8), 8)

        def prep_qkv(w, c, slot):
            def heads(i, carry):
                st = qst_v.at[slot, i].bitcast(U32)
                for jp in range(H // 2):
                    for k, x in enumerate(_halves(st[pl.ds(jp, QR, stride=H // 2), :])):
                        qtr_v[i, 2 * jp + k] = x.astype(BF16)
                return carry
            lax.fori_loop(0, NB, heads, 0)

            def put(r, row, k, val):
                wqkv_v[k, r, words_at(c * (QR // 2) + row), lanes_at(w)] = val
            prep_tiles(lambda i, j, row, k: qtr_v[i, j * HB + k, pl.ds(row, 16), :], put, QR, HB)

        def prep_from_big(dst, base, blk, c, nrows):
            def load(i, j, row, k):
                return big_v[rows_at(base + i * blk + row, 16), lanes_at(j * (DB // LANES) + k)]

            def put(r, row, k, val):
                dst[r, words_at(c * (nrows // 2) + row), lanes_at(k)] = val
            prep_tiles(load, put, nrows, DB // LANES)

        def prep_gu(w, c):
            def load(i, j, row, k):
                return gst_v[c, i, pl.ds(row, 16), lanes_at(j * (FB // LANES) + k)]

            def put(r, row, k, val):
                wgu_v[k, r, words_at(c * (GR // 2) + row), w * LANES:(w + 1) * LANES] = val
            prep_tiles(load, put, GR, FB // LANES, 0.5)

        x_head = pltpu.make_async_copy(x_hbm.at[0:XH, :], x_v.at[0:XH, :], sem_x.at[0])
        x_tail = pltpu.make_async_copy(x_hbm.at[XH:, :], x_v.at[XH:, :], sem_x.at[1])
        NQ, NO = DB // QR, EB // WR
        ONEXT = min(QST * QR * H * DH // (WR * D), OST)
        for n in range(QST):
            start(q_copies(0, n, n))
        x_head.start()

        ri = lax.broadcasted_iota(jnp.int32, (R, LANES), 0)
        ci = lax.broadcasted_iota(jnp.int32, (R, LANES), 1)

        def layer_of(i):
            return jnp.where(i < MM, (i >= M).astype(jnp.int32), (i >= MM + SEG).astype(jnp.int32))

        same = (layer_of(ri) == layer_of(ci)) & (ci < R)
        visible = (ri < MM) | (ri >= ci)
        keep_v[...] = (same & visible).astype(jnp.int32)
        fill_v[...] = jnp.where(same, -1e9 / scale, -jnp.inf).astype(F32)
        qkv_v[...] = jnp.zeros(qkv_v.shape, BF16)
        mem_v[0:M, :] = mem0_ref[...].astype(F32)
        mem_v[M:, :] = mem0_ref[...].astype(F32)

        for w in range(3):
            def q_body(c, carry, w=w):
                slot = (w * NQ + c) % QST
                wait(q_copies(w, c, slot))
                prep_qkv(w, c, slot)
                pl.when(c + QST < NQ)(lambda: start(q_copies(w, c + QST, slot)))
                if w < 2:
                    pl.when(c + QST >= NQ)(lambda: start(q_copies(w + 1, c + QST - NQ, slot)))
                else:
                    pl.when((c + QST >= NQ) & (c + QST - NQ < ONEXT))(
                        lambda: start(o_copies(c + QST - NQ)))
                return carry
            lax.fori_loop(0, NQ, q_body, 0)

        def o_body(c, carry):
            wait(o_copies(c))
            prep_from_big(wo_v, (c % OST) * NB * WR, WR, c, WR)
            pl.when(c + ONEXT < NO)(lambda: start(o_copies(c + ONEXT)))
            pl.when(c >= NO - GST)(lambda: start(g_copies(wg_hbm, c - (NO - GST))))
            return carry
        lax.fori_loop(0, NO, o_body, 0)
        for c in range(GST):
            start(d_copies(c))
        x_head.wait()
        xa_v[...] = x_v[0:XH, :].astype(F32)

        def load_glu_weights():
            def gate(c, carry):
                wait(g_copies(wg_hbm, c))
                prep_gu(0, c)
                start(g_copies(wu_hbm, c))
                return carry

            def down(c, carry):
                wait(d_copies(c))
                prep_from_big(wd_v, c * DR, FB, c, DR)
                return carry

            def up(c, carry):
                wait(g_copies(wu_hbm, c))
                prep_gu(1, c)
                return carry
            lax.fori_loop(0, GST, gate, 0)
            lax.fori_loop(0, GST, down, 0)
            lax.fori_loop(0, GST, up, 0)
            x_tail.start()

        def attention(rows_of, emit):
            pv = {}

            def scores():
                for j in range(NB):
                    qkv = rows_of(j)
                    n = qkv.shape[0]
                    for w in range(3):
                        qkv_v[j, w, 0:n, :] = qkv[:, w * DH:(w + 1) * DH].astype(BF16)
                    s = _dot_nt(qkv_v[j, 0, 0:n, :], qkv_v[j, 1])
                    s = jnp.where(keep_v[0:n, :] != 0, s, fill_v[0:n, :])
                    mx = jnp.max(s, axis=-1, keepdims=True)
                    e = jnp.exp2((s - mx) * c_exp)
                    den = jnp.sum(e, axis=-1, keepdims=True)
                    inv = pl.reciprocal(den, approx=True)
                    inv = inv * (2.0 - den * inv)
                    pv[j] = (e * inv).astype(BF16)

            def values():
                emit({j: _dot(pv[j], qkv_v[j, 2]) for j in range(NB)})

            return scores, values

        h0, h1 = cfg.get("h0", 4), cfg.get("h1", 16)

        def gate_up(c, hooks=None):
            for _ in gate_up_steps(c, hooks):
                pass

        def gate_up_steps(c, hooks=None):
            res = []
            yield from fast_dot_steps(res, lb_v, lambda r: wgu_v[c, r], True, False, hooks,
                                      (nb_v, None) if c == 0 else None)
            gu = res[0]
            act = {k: jnp.tanh(v[:, :LANES]) * v[:, LANES:] + v[:, LANES:] for k, v in gu.items()}
            store_lhs(ld_v, c, act, None)

        def down(c, hooks=None):
            dn, _ = fast_dot(ld_v, lambda r: wd_v[r, :, c * OC:(c + 1) * OC], True, False, hooks)
            for (hf, j), v in dn.items():
                rows = slice(hf * SEG, (hf + 1) * SEG)
                z_v[rows, out_cols(j, c)] = ya_v[rows, out_cols(j, c)] + v

        def glu_input():
            nb_v[...] = _layernorm(ya_v[0:2 * SEG, :])

        def out_copy(row, n):
            return pltpu.make_async_copy(big_v.at[pl.ds(row, n), :],
                                         out_hbm.at[pl.ds(row, n), :], sem_out)

        def attention_single(mrow, xrow, yrow):
            m = mem_v[pl.ds(mrow, M), :]
            x = xa_v[pl.ds(xrow, SEG), :]
            store_lhs(la_v, 0, None, split_cols(jnp.concatenate([m, m, _layernorm(x)], axis=0)))
            hooks = None
            for c in range(HB):
                _, cur = fast_dot(la_v, lambda r: wqkv_v[c, r], False, True, hooks)
                scores, values = attention(
                    lambda j, cur=cur: cur[j], lambda o, c=c: store_lhs(lo_v, c, None, o))
                hooks = {h0: scores, NP - 1: values}
            scores()
            values()
            for c in range(DB // OC):
                _, o = fast_dot(lo_v, lambda r: wo_v[r, :, c * OC:(c + 1) * OC], False, True)
                for j in range(NB):
                    mem_v[pl.ds(mrow, M), out_cols(j, c)] = o[j][:M]
                    ya_v[pl.ds(yrow, SEG), out_cols(j, c)] = (
                        xa_v[pl.ds(xrow, SEG), out_cols(j, c)] + o[j][MM:])

        def step(t, carry):
            hooks = {cfg.get("g0", 2): glu_input}
            for c in range(HB):
                res = []
                mode = cfg.get("mode", 2)
                gens = [fast_dot_steps(res, la_v, lambda r: wqkv_v[c, r], True, True, hooks,
                                       (na_v, mem_v) if c == 0 else None)]
                if mode == 4 and c < 2:
                    if c == 0:
                        first = gate_up_steps(0)
                        gens.append(itertools.chain([None] * cfg.get("lag", 13),
                                                    itertools.islice(first, NP - cfg.get("lag", 13))))
                    else:
                        gens.append(first)
                if c > 0 and (mode == 2 or (mode == 3 and c == 1)):
                    gens.append(gate_up_steps(c - 1))
                for _ in itertools.zip_longest(*gens):
                    pass
                tok, mem = res
                scores, values = attention(
                    lambda j, tok=tok, mem=mem: jnp.concatenate(
                        [mem[j], tok[0, j], tok[1, j]], axis=0),
                    lambda o, c=c: store_lhs(
                        lo_v, c,
                        {(hf, j): o[j][MM + hf * SEG:MM + (hf + 1) * SEG]
                         for hf in range(2) for j in range(NB)},
                        {j: o[j][:MM] for j in range(NB)}))
                if c < FB // LANES:
                    if mode == 2 or (mode >= 3 and c == 0):
                        hooks = {h0: scores, cfg.get("h4", 14): values}
                    elif mode == 0:
                        gate_up(c)
                        hooks = {h0: scores, h1: values}
                    else:
                        gate_up(c, {h0: scores})
                        hooks = {h1: values}
            down(0, {cfg.get('d0', 3): scores, cfg.get('d1', 16): values})
            down(1)

            def project(c, hooks=None):
                tok, mem = fast_dot(lo_v, lambda r: wo_v[r, :, c * OC:(c + 1) * OC], True, True, hooks)
                for (hf, j), v in tok.items():
                    res = (x_v[pl.ds(cur, SEG), out_cols(j, c)].astype(F32) if hf == 0
                           else xa_v[SEG:, out_cols(j, c)])
                    ya_v[hf * SEG:(hf + 1) * SEG, out_cols(j, c)] = res + v
                for j in range(NB):
                    mem_v[:, out_cols(j, c)] = mem[j]

            row = pl.multiple_of(jnp.maximum(t - 3, 0) * SEG, SEG)
            nxt = pl.multiple_of(jnp.minimum(t + 1, NSEG - 1) * SEG, SEG)

            big_v[pl.ds(row, SEG), :] = z_v[SEG:, :].astype(BF16)
            cur = pl.multiple_of(t * SEG, SEG)

            def next_input():
                na_v[:SEG, :] = _layernorm(x_v[pl.ds(nxt, SEG), :].astype(F32))
                na_v[SEG:, :] = _layernorm(z_v[:SEG, :])

            project(0, {cfg.get("h2", 2): next_input})
            project(1)
            xa_v[SEG:, :] = z_v[:SEG, :]
            pl.when(t >= 3)(lambda: out_copy(row, SEG).start())
            return carry

        def phase(ph, carry):
            attention_single(pl.multiple_of(jnp.where(ph < 2, 0, M), M),
                             pl.multiple_of(jnp.where(ph == 0, 0, SEG), SEG),
                             pl.multiple_of(jnp.where(ph == 3, 1, ph) * SEG, SEG))
            pl.when(ph == 1)(load_glu_weights)

            @pl.when(ph >= 1)
            def _():
                glu_input()
                for c in range(FB // LANES):
                    gate_up(c)
                for c in range(DB // OC):
                    down(c)

            @pl.when(ph == 1)
            def _():
                x_tail.wait()
                ya_v[0:SEG, :] = ya_v[SEG:2 * SEG, :]
                xn = jnp.concatenate(
                    [x_v[2 * SEG:3 * SEG, :].astype(F32), z_v[:SEG, :]], axis=0)
                xa_v[...] = xn
                na_v[...] = _layernorm(xn)
                lax.fori_loop(2, cfg.get("nsteps", NSEG), step, 0)

            @pl.when(ph == 2)
            def _():
                xa_v[SEG:, :] = z_v[:SEG, :]
                ya_v[0:SEG, :] = ya_v[2 * SEG:, :]
                big_v[S - 3 * SEG:S - 2 * SEG, :] = z_v[SEG:, :].astype(BF16)
                out_copy(S - 3 * SEG, SEG).start()

            @pl.when(ph == 3)
            def _():
                big_v[S - 2 * SEG:S, :] = z_v[...].astype(BF16)
                out_copy(S - 2 * SEG, 2 * SEG).start()
            return carry

        lax.fori_loop(0, cfg.get('nph', 4), phase, 0)
        out_copy(0, cfg.get("nsteps", NSEG) * SEG).wait()

    scratch = [
        pltpu.VMEM((S, D), BF16),
        pltpu.VMEM((FF, D), BF16),
        pltpu.VMEM((GST, NB, GR, FF), BF16),
        pltpu.VMEM((QST, NB, QR * H, DH), BF16),
        pltpu.VMEM((NB, H, QR, DH), BF16),
        pltpu.VMEM((HB, NP, DB // 2, 3 * DH), U32),
        pltpu.VMEM((NP, EB // 2, DB), U32),
        pltpu.VMEM((FB // LANES, NP, DB // 2, 2 * LANES), U32),
        pltpu.VMEM((NP, FB // 2, DB), U32),
        pltpu.VMEM((NP, DB // LANES, RL, LANES), BF16),
        pltpu.VMEM((NP, EB // LANES, RL, LANES), BF16),
        pltpu.VMEM((NP, DB // LANES, SEG, LANES), BF16),
        pltpu.VMEM((NP, FB // LANES, SEG, LANES), BF16),
        pltpu.VMEM((MM, D), F32),
        pltpu.VMEM((2 * SEG, D), F32),
        pltpu.VMEM((2 * SEG, D), F32),
        pltpu.VMEM((2 * SEG, D), F32),
        pltpu.VMEM((3 * SEG, D), F32),
        pltpu.VMEM((2 * SEG, D), F32),
        pltpu.VMEM((NB, 3, LANES, DH), BF16),
        pltpu.VMEM((R, LANES), F32),
        pltpu.VMEM((R, LANES), jnp.int32),
        pltpu.SemaphoreType.DMA((2,)),
        pltpu.SemaphoreType.DMA((QST, NB)),
        pltpu.SemaphoreType.DMA((OST, NB)),
        pltpu.SemaphoreType.DMA((GST, NB)),
        pltpu.SemaphoreType.DMA((GST, NB)),
        pltpu.SemaphoreType.DMA(()),
    ]
    return kernel, scratch


def _build(cfg):
    @functools.partial(jax.jit, static_argnames=("A_seg_len",))
    def fn(A_x, A_mem0, A_Wq, A_Wk, A_Wv, A_Wo, A_seg_len, B_x, B_w_gate, B_w_up, B_w_down):
        B, S, D = A_x.shape
        _, H, DH = A_Wq.shape
        M = A_mem0.shape[1]
        FF = B_w_gate.shape[1]
        kernel, scratch = _make_kernel(S, D, H, DH, M, A_seg_len, FF, cfg)
        any_spec = pl.BlockSpec(memory_space=pl.ANY)
        out = pl.pallas_call(
            kernel,
            out_shape=jax.ShapeDtypeStruct((S, D), A_x.dtype),
            in_specs=[any_spec, pl.BlockSpec(memory_space=pltpu.VMEM)] + [any_spec] * 7,
            out_specs=any_spec,
            scratch_shapes=scratch,
            compiler_params=pltpu.CompilerParams(vmem_limit_bytes=cfg.get("vmem", 124) * 1024 * 1024,
                                                 flags=cfg.get("flags")),
        )(A_x.reshape(S, D), A_mem0.reshape(M, D),
          A_Wq.reshape(D * H, DH), A_Wk.reshape(D * H, DH), A_Wv.reshape(D * H, DH),
          A_Wo.reshape(H * DH, D), B_w_gate, B_w_up, B_w_down)
        return out.reshape(B, S, D)
    return fn


pallas_interleave_layers__memory_aug_recurrent_mem_tr__glu_gated_glu__prompt_kernel = _build({"mode":1,"h0":8,"h1":4})
```

```python
import functools
import math

import jax
import jax.numpy as jnp
import numpy as np
from jax import lax
import jax.experimental.pallas as pl
import jax.experimental.pallas.tpu as pltpu

F32 = jnp.float32
BF16 = jnp.bfloat16
U32 = jnp.uint32
EPS = 1e-05
LANES = 128

STRASSEN = (2, (
    ({(1, 0): 1, (1, 1): 1}, {(0, 0): 1}, {(1, 0): 1, (1, 1): -1}, {0: 1, 1: 1}, {0: 1}),
    ({(1, 1): 1}, {(1, 0): 1, (0, 0): -1}, {(0, 0): 1, (1, 0): 1}, {1: 1}, {0: 1}),
    ({(0, 0): 1}, {(0, 1): 1, (1, 1): -1}, {(0, 1): 1, (1, 1): 1}, {0: 1}, {1: 1}),
    ({(0, 0): 1, (0, 1): 1}, {(1, 1): 1}, {(0, 0): -1, (0, 1): 1}, {0: 1, 1: 1}, {1: 1}),
    ({(0, 0): 1, (1, 1): 1}, {(0, 0): 1, (1, 1): 1}, {(0, 0): 1, (1, 1): 1}, None, None),
    ({(1, 0): 1, (0, 0): -1}, {(0, 0): 1, (0, 1): 1}, {(1, 1): 1}, None, None),
    ({(0, 1): 1, (1, 1): -1}, {(1, 0): 1, (1, 1): 1}, {(0, 0): 1}, None, None),
))
HK26 = (4, (
    ({(0, 0): 1}, {(0, 0): 1, (0, 2): 1, (1, 0): -1, (3, 0): 1}, {(0, 0): 1, (1, 0): -1}, None, None),
    ({(0, 0): 1, (1, 0): 1}, {(0, 0): 1, (0, 1): -1, (2, 0): 1, (3, 0): -1}, {(1, 0): 1}, {0: 1}, {0: 1}),
    ({(1, 1): 1}, {(0, 1): 1, (1, 1): -1, (1, 2): -1, (3, 1): 1}, {(0, 1): 1, (1, 1): -1}, {1: 1}, {1: -1}),
    ({(0, 1): 1, (1, 1): 1}, {(0, 3): -1, (1, 0): -1, (1, 1): 1, (1, 3): 1, (2, 1): -1, (3, 0): 1}, {(0, 1): 1}, None, None),
    ({(0, 2): 1}, {(1, 2): -1, (2, 0): 1, (2, 2): 1, (2, 3): 1}, {(0, 2): 1}, None, None),
    ({(1, 2): 1}, {(0, 2): 1, (2, 1): 1, (2, 2): 1, (3, 2): -1}, {(1, 2): 1}, {2: 1}, {2: 1}),
    ({(0, 3): 1}, {(0, 3): 1, (1, 3): -1, (3, 2): 1, (3, 3): 1}, {(0, 3): 1, (1, 3): -1}, None, None),
    ({(0, 3): 1, (1, 3): 1}, {(0, 3): -1, (2, 3): -1, (3, 1): 1, (3, 3): 1}, {(1, 3): 1}, {3: 1}, {3: 1}),
    ({(0, 0): 1, (1, 1): -1}, {(0, 1): 1, (1, 0): -1, (3, 0): 1}, {(0, 1): 1, (1, 0): 1}, {1: 1}, {0: -1}),
    ({(1, 0): 1, (1, 1): 1}, {(0, 1): 1}, {(1, 0): 1, (1, 1): 1}, {0: 1, 1: 1}, {0: 1, 1: 1}),
    ({(0, 0): 1, (0, 1): 1}, {(0, 3): 1, (1, 0): 1, (3, 0): -1}, {(0, 0): 1, (0, 1): 1}, None, None),
    ({(0, 0): 1, (1, 0): 1, (1, 2): -1}, {(0, 2): 1, (2, 0): -1}, {(0, 0): -1, (0, 2): 1, (1, 0): 1}, None, None),
    ({(1, 0): 1, (1, 2): -1}, {(0, 2): -1}, {(0, 0): -1, (0, 2): 1, (1, 0): 1, (1, 2): -1}, {0: 1, 2: -1}, {2: -1}),
    ({(0, 0): 1, (0, 2): -1, (1, 0): 1, (1, 2): -1}, {(2, 0): 1}, {(0, 0): -1, (0, 2): 1}, {0: 1, 2: -1}, {0: -1}),
    ({(0, 1): 1, (0, 2): 1, (1, 1): 1}, {(1, 2): 1, (2, 1): 1}, {(0, 1): 1, (1, 1): -1, (1, 2): 1}, None, None),
    ({(0, 1): 1, (0, 2): 1}, {(1, 2): 1}, {(0, 1): -1, (0, 2): 1, (1, 1): 1, (1, 2): -1}, {1: 1}, {1: -1, 2: 1}),
    ({(0, 1): 1, (0, 2): 1, (1, 1): 1, (1, 2): 1}, {(2, 1): -1}, {(1, 1): -1, (1, 2): 1}, {2: 1}, {1: -1, 2: 1}),
    ({(0, 3): -1, (1, 1): 1}, {(0, 3): -1, (1, 3): 1, (3, 1): 1}, {(0, 1): -1, (1, 3): 1}, {1: 1}, {3: 1}),
    ({(0, 1): 1, (0, 3): 1}, {(0, 3): -1, (1, 3): 1, (3, 0): 1}, {(0, 1): -1, (0, 3): 1}, None, None),
    ({(1, 1): 1, (1, 3): 1}, {(3, 1): -1}, {(1, 1): -1, (1, 3): 1}, {1: 1, 3: 1}, {1: -1, 3: 1}),
    ({(0, 3): 1, (1, 2): 1, (1, 3): 1}, {(2, 3): -1, (3, 2): -1}, {(0, 2): -1, (0, 3): 1, (1, 3): -1}, None, None),
    ({(0, 2): 1, (0, 3): 1, (1, 2): 1, (1, 3): 1}, {(2, 3): 1}, {(0, 2): -1, (0, 3): 1}, {2: 1, 3: 1}, {3: 1}),
    ({(1, 2): 1, (1, 3): 1}, {(3, 2): 1}, {(0, 2): -1, (0, 3): 1, (1, 2): 1, (1, 3): -1}, {2: 1, 3: 1}, {2: 1}),
    ({(0, 0): 1, (1, 0): 1, (1, 1): 1, (1, 3): 1}, {(3, 0): -1}, {(0, 0): 1, (0, 1): 1, (0, 3): -1, (1, 0): -1}, {0: 1, 1: 1, 3: 1}, {0: -1}),
    ({(0, 0): 1, (0, 1): 1, (0, 3): 1, (1, 0): 1, (1, 1): 1, (1, 3): 1}, {(0, 3): -1, (3, 0): 1}, {(0, 0): 1, (0, 1): 1, (0, 3): -1}, None, None),
    ({(0, 3): 1, (1, 0): 1, (1, 1): 1, (1, 3): 1}, {(0, 3): 1}, {(0, 0): 1, (0, 1): 1, (0, 3): -1, (1, 3): 1}, {0: 1, 1: 1, 3: 1}, {3: 1}),
))
SCHEMES = {"strassen": STRASSEN, "hk26": HK26}


def _combine(coefs, vals):
    acc = None
    for key, c in sorted(coefs.items(), key=lambda kv: -kv[1]):
        v = vals[key]
        if abs(c) != 1:
            v = v * abs(c)
        if acc is None:
            acc = v if c > 0 else -v
        else:
            acc = acc + v if c > 0 else acc - v
    return acc


def _accumulate(accs, coefs, v):
    for key, c in coefs.items():
        t = v if abs(c) == 1 else v * abs(c)
        if key not in accs:
            accs[key] = t if c > 0 else -t
        else:
            accs[key] = accs[key] + t if c > 0 else accs[key] - t


def _layernorm(x):
    m = jnp.mean(x, axis=-1, keepdims=True)
    c = x - m
    v = jnp.mean(c * c, axis=-1, keepdims=True)
    return c * lax.rsqrt(v + EPS)


def _dot(a, b):
    return lax.dot_general(a, b, (((1,), (0,)), ((), ())), preferred_element_type=F32)


def _dot_nt(a, b):
    return lax.dot_general(a, b, (((1,), (1,)), ((), ())), preferred_element_type=F32)


def _halves(x):
    return [pltpu.unpack_elementwise(x, index=k, packed_dtype=BF16, unpacked_dtype=F32)
            for k in range(2)]


def _pair(lo, hi):
    return pltpu.pack_elementwise([lo, hi], packed_dtype=BF16)


def _make_kernel(S, D, H, DH, M, SEG, FF, cfg):
    NB, prods = SCHEMES[cfg.get("scheme", "hk26")]
    if "order" in cfg:
        prods = tuple(prods[i] for i in cfg["order"])
    NP = len(prods)
    NSEG = S // SEG
    L = M + SEG
    DB, HB, FB = D // NB, H // NB, FF // NB
    EB = HB * DH
    OC = DB // 2
    QR = cfg.get("QR", 128) // NB
    QST = cfg.get("QST", 4)
    WR = 512 // NB
    OST = FF // (WR * NB)
    GST = 4
    GR, DR = DB // GST, FB // GST
    XH = 2 * SEG
    scale = DH ** (-0.5)
    c_exp = scale * math.log2(math.e)

    def store_lhs(ref, cols, blocks, paired):
        for r, (u, _, _, u1, _) in enumerate(prods):
            if paired or u1 is not None:
                ref[r, :, cols] = _combine(u if paired else u1, blocks)

    def fast_dot(lhs_ref, w_of, paired, hooks=None, src_ref=None):
        n = lhs_ref.shape[1]
        acc = {}
        for r, (u, _, w, u1, w1) in enumerate(prods):
            if hooks and r in hooks:
                hooks[r]()
            if not paired and u1 is None:
                continue
            if src_ref is None:
                lhs = lhs_ref[r]
            else:
                if paired:
                    lhs = _combine(u, {(hf, i): src_ref[hf * n:(hf + 1) * n, i * DB:(i + 1) * DB]
                                       for hf, i in u})
                else:
                    lhs = _combine(u1, {i: src_ref[0:n, i * DB:(i + 1) * DB] for i in u1})
                lhs_ref[r] = lhs
            _accumulate(acc, w if paired else w1, _dot(lhs, pltpu.bitcast(w_of(r), BF16)))
        return acc

    def out_cols(j, c):
        return slice(j * DB + c * OC, j * DB + (c + 1) * OC)

    def kernel(x_hbm, mem0_ref, wq_hbm, wk_hbm, wv_hbm, wo_hbm, wg_hbm, wu_hbm, wd_hbm,
               out_hbm,
               x_v, big_v, gst_v, qst_v, qtr_v, wqkv_v, wo_v, wgu_v, wd_v,
               la_v, lo_v, lb_v, ld_v, mem_v, xa_v, na_v, nb_v, ya_v, z_v, kv_v, fill_v, keep_v,
               sem_x, sem_q, sem_o, sem_g, sem_d, sem_out):

        def rows_at(start, size):
            return pl.ds(start if isinstance(start, int) else pl.multiple_of(start, 16), size)

        def q_copies(w, c, slot):
            src = (wq_hbm, wk_hbm, wv_hbm)[w]
            return [pltpu.make_async_copy(src.at[rows_at((i * DB + c * QR) * H, QR * H), :],
                                          qst_v.at[slot, i], sem_q.at[slot, i]) for i in range(NB)]

        def o_copies(c):
            slot = c % OST
            return [pltpu.make_async_copy(wo_hbm.at[rows_at(i * EB + c * WR, WR), :],
                                          big_v.at[rows_at((slot * NB + i) * WR, WR), :],
                                          sem_o.at[slot, i]) for i in range(NB)]

        def g_copies(src, c):
            return [pltpu.make_async_copy(src.at[rows_at(i * DB + c * GR, GR), :],
                                          gst_v.at[c, i], sem_g.at[c, i]) for i in range(NB)]

        def d_copies(c):
            return [pltpu.make_async_copy(wd_hbm.at[rows_at(i * FB + c * DR, DR), :],
                                          big_v.at[rows_at(i * FB + c * DR, DR), :],
                                          sem_d.at[c, i]) for i in range(NB)]

        def start(copies):
            for cp in copies:
                cp.start()

        def wait(copies):
            for cp in copies:
                cp.wait()

        def prep_tiles(load, put, nrows, ncols, mul=None):
            def tile(n, carry):
                s, k = lax.div(n, ncols), lax.rem(n, ncols)
                lo, hi = {}, {}
                for i in range(NB):
                    for j in range(NB):
                        x = load(i, j, pl.multiple_of(s * 16, 16), k)
                        lo[i, j], hi[i, j] = _halves(pltpu.bitcast(x, U32))
                        if mul is not None:
                            lo[i, j], hi[i, j] = lo[i, j] * mul, hi[i, j] * mul
                for r, (_, v, _, _, _) in enumerate(prods):
                    put(r, s * 8, k, _pair(_combine(v, lo), _combine(v, hi)))
                return carry
            lax.fori_loop(0, nrows // 16 * ncols, tile, 0)

        def lanes_at(k):
            return pl.ds(pl.multiple_of(k * LANES, LANES), LANES)

        def words_at(row):
            return pl.ds(pl.multiple_of(row, 8), 8)

        def prep_qkv(w, c, slot):
            def heads(i, carry):
                st = qst_v.at[slot, i].bitcast(U32)
                for jp in range(H // 2):
                    for k, x in enumerate(_halves(st[pl.ds(jp, QR, stride=H // 2), :])):
                        qtr_v[i, 2 * jp + k] = x.astype(BF16)
                return carry
            lax.fori_loop(0, NB, heads, 0)

            def put(r, row, k, val):
                wqkv_v[k, r, words_at(c * (QR // 2) + row), lanes_at(w)] = val
            prep_tiles(lambda i, j, row, k: qtr_v[i, j * HB + k, pl.ds(row, 16), :], put, QR, HB)

        def prep_from_big(dst, base, blk, c, nrows):
            def load(i, j, row, k):
                return big_v[rows_at(base + i * blk + row, 16), lanes_at(j * (DB // LANES) + k)]

            def put(r, row, k, val):
                dst[r, words_at(c * (nrows // 2) + row), lanes_at(k)] = val
            prep_tiles(load, put, nrows, DB // LANES)

        def prep_gu(w, c):
            def load(i, j, row, k):
                return gst_v[c, i, pl.ds(row, 16), lanes_at(j * (FB // LANES) + k)]

            def put(r, row, k, val):
                wgu_v[k, r, words_at(c * (GR // 2) + row), w * LANES:(w + 1) * LANES] = val
            prep_tiles(load, put, GR, FB // LANES, 0.5)

        x_head = pltpu.make_async_copy(x_hbm.at[0:XH, :], x_v.at[0:XH, :], sem_x.at[0])
        x_tail = pltpu.make_async_copy(x_hbm.at[XH:, :], x_v.at[XH:, :], sem_x.at[1])
        NQ, NO = DB // QR, EB // WR
        ONEXT = min(QST * QR * H * DH // (WR * D), OST)
        for n in range(QST):
            start(q_copies(0, n, n))
        x_head.start()

        ri = lax.broadcasted_iota(jnp.int32, (2 * L, LANES), 0)
        ci = lax.broadcasted_iota(jnp.int32, (2 * L, LANES), 1)
        first = jnp.where(ri < L, 0, L)
        same = (ci >= first) & (ci < first + L)
        visible = (ri < first + M) | (ri >= ci)
        keep_v[...] = (same & visible).astype(jnp.int32)
        fill_v[...] = jnp.where(same, -1e9 / scale, -jnp.inf).astype(F32)
        kv_v[...] = jnp.zeros(kv_v.shape, BF16)
        mem_v[0:M, :] = mem0_ref[...].astype(F32)
        mem_v[M:, :] = mem0_ref[...].astype(F32)

        for w in range(3):
            def q_body(c, carry, w=w):
                slot = (w * NQ + c) % QST
                wait(q_copies(w, c, slot))
                prep_qkv(w, c, slot)
                pl.when(c + QST < NQ)(lambda: start(q_copies(w, c + QST, slot)))
                if w < 2:
                    pl.when(c + QST >= NQ)(lambda: start(q_copies(w + 1, c + QST - NQ, slot)))
                else:
                    pl.when((c + QST >= NQ) & (c + QST - NQ < ONEXT))(
                        lambda: start(o_copies(c + QST - NQ)))
                return carry
            lax.fori_loop(0, NQ, q_body, 0)

        def o_body(c, carry):
            wait(o_copies(c))
            prep_from_big(wo_v, (c % OST) * NB * WR, WR, c, WR)
            pl.when(c + ONEXT < NO)(lambda: start(o_copies(c + ONEXT)))
            pl.when(c >= NO - GST)(lambda: start(g_copies(wg_hbm, c - (NO - GST))))
            return carry
        lax.fori_loop(0, NO, o_body, 0)
        for c in range(GST):
            start(d_copies(c))
        x_head.wait()
        xa_v[...] = x_v[0:XH, :].astype(F32)

        def load_glu_weights():
            def gate(c, carry):
                wait(g_copies(wg_hbm, c))
                prep_gu(0, c)
                start(g_copies(wu_hbm, c))
                return carry

            def down(c, carry):
                wait(d_copies(c))
                prep_from_big(wd_v, c * DR, FB, c, DR)
                return carry

            def up(c, carry):
                wait(g_copies(wu_hbm, c))
                prep_gu(1, c)
                return carry
            lax.fori_loop(0, GST, gate, 0)
            lax.fori_loop(0, GST, down, 0)
            lax.fori_loop(0, GST, up, 0)
            x_tail.start()

        def attention(c, qkv, paired):
            probs = {}

            def scores():
                for j in range(NB):
                    x = jnp.concatenate([qkv[0, j], qkv[1, j]], axis=0) if paired else qkv[j]
                    n = x.shape[0]
                    for w in range(2):
                        kv_v[j, w, 0:n, :] = x[:, (w + 1) * DH:(w + 2) * DH].astype(BF16)
                    s = _dot_nt(x[:, :DH], kv_v[j, 0])
                    s = jnp.where(keep_v[0:n, :] != 0, s, fill_v[0:n, :])
                    mx = jnp.max(s, axis=-1, keepdims=True)
                    e = jnp.exp2((s - mx) * c_exp)
                    den = jnp.sum(e, axis=-1, keepdims=True)
                    inv = pl.reciprocal(den, approx=True)
                    inv = inv * (2.0 - den * inv)
                    probs[j] = e * inv

            def values():
                o = {j: _dot(probs[j], kv_v[j, 1]) for j in range(NB)}
                if paired:
                    o = {(hf, j): o[j][hf * L:(hf + 1) * L] for hf in range(2) for j in range(NB)}
                store_lhs(lo_v, slice(c * DH, (c + 1) * DH), o, paired)

            return scores, values

        def gate_up(c, hooks=None):
            gu = fast_dot(lb_v, lambda r: wgu_v[c, r], True, hooks, nb_v if c == 0 else None)
            act = {k: jnp.tanh(v[:, :LANES]) * v[:, LANES:] + v[:, LANES:] for k, v in gu.items()}
            store_lhs(ld_v, slice(c * LANES, (c + 1) * LANES), act, True)

        def down(c, hooks=None):
            dn = fast_dot(ld_v, lambda r: wd_v[r, :, c * OC:(c + 1) * OC], True, hooks)
            for (hf, j), v in dn.items():
                rows = slice(hf * SEG, (hf + 1) * SEG)
                z_v[rows, out_cols(j, c)] = ya_v[rows, out_cols(j, c)] + v

        def glu_input():
            nb_v[...] = _layernorm(ya_v[0:2 * SEG, :])

        def out_copy(row, n):
            return pltpu.make_async_copy(big_v.at[pl.ds(row, n), :],
                                         out_hbm.at[pl.ds(row, n), :], sem_out)

        def attention_single(mrow, xrow, yrow):
            na_v[0:M, :] = mem_v[pl.ds(mrow, M), :]
            na_v[M:L, :] = _layernorm(xa_v[pl.ds(xrow, SEG), :])
            hooks = None
            for c in range(HB):
                qkv = fast_dot(la_v, lambda r: wqkv_v[c, r], False, hooks, na_v if c == 0 else None)
                scores, values = attention(c, qkv, False)
                hooks = {5: scores, NP - 1: values}
            scores()
            values()
            for c in range(DB // OC):
                o = fast_dot(lo_v, lambda r: wo_v[r, :, c * OC:(c + 1) * OC], False)
                for j in range(NB):
                    mem_v[pl.ds(mrow, M), out_cols(j, c)] = o[j][:M]
                    ya_v[pl.ds(yrow, SEG), out_cols(j, c)] = (
                        xa_v[pl.ds(xrow, SEG), out_cols(j, c)] + o[j][M:])

        def step(t, carry):
            cur = pl.multiple_of(t * SEG, SEG)
            nxt = pl.multiple_of(jnp.minimum(t + 1, NSEG - 1) * SEG, SEG)
            row = pl.multiple_of(jnp.maximum(t - 3, 0) * SEG, SEG)
            hooks = {cfg.get("g0", 2): glu_input}
            for c in range(HB):
                qkv = fast_dot(la_v, lambda r: wqkv_v[c, r], True, hooks, na_v if c == 0 else None)
                scores, values = attention(c, qkv, True)
                if c < FB // LANES:
                    gate_up(c, {cfg.get("h0", 8): scores})
                    hooks = {cfg.get("h1", 4): values}
            down(0, {cfg.get("d0", 3): scores, cfg.get("d1", 16): values})
            down(1)
            big_v[pl.ds(row, SEG), :] = z_v[SEG:, :].astype(BF16)

            def next_input():
                na_v[M:L, :] = _layernorm(x_v[pl.ds(nxt, SEG), :].astype(F32))
                na_v[L + M:, :] = _layernorm(z_v[:SEG, :])

            for c in range(DB // OC):
                o = fast_dot(lo_v, lambda r: wo_v[r, :, c * OC:(c + 1) * OC], True,
                             {cfg.get("h2", 2): next_input} if c == 0 else None)
                for (hf, j), v in o.items():
                    res = (x_v[pl.ds(cur, SEG), out_cols(j, c)].astype(F32) if hf == 0
                           else xa_v[SEG:, out_cols(j, c)])
                    na_v[hf * L:hf * L + M, out_cols(j, c)] = v[:M]
                    ya_v[hf * SEG:(hf + 1) * SEG, out_cols(j, c)] = res + v[M:]
            xa_v[SEG:, :] = z_v[:SEG, :]
            pl.when(t >= 3)(lambda: out_copy(row, SEG).start())
            return carry

        def phase(ph, carry):
            attention_single(pl.multiple_of(jnp.where(ph < 2, 0, M), M),
                             pl.multiple_of(jnp.where(ph == 0, 0, SEG), SEG),
                             pl.multiple_of(jnp.where(ph == 3, 1, ph) * SEG, SEG))
            pl.when(ph == 1)(load_glu_weights)

            @pl.when(ph >= 1)
            def _():
                glu_input()
                for c in range(FB // LANES):
                    gate_up(c)
                for c in range(DB // OC):
                    down(c)

            @pl.when(ph == 1)
            def _():
                x_tail.wait()
                ya_v[0:SEG, :] = ya_v[SEG:2 * SEG, :]
                xa_v[SEG:, :] = z_v[:SEG, :]
                na_v[0:M, :] = mem_v[0:M, :]
                na_v[M:L, :] = _layernorm(x_v[2 * SEG:3 * SEG, :].astype(F32))
                na_v[L:L + M, :] = mem_v[M:, :]
                na_v[L + M:, :] = _layernorm(z_v[:SEG, :])
                lax.fori_loop(2, cfg.get("nsteps", NSEG), step, 0)
                mem_v[M:, :] = na_v[L:L + M, :]

            @pl.when(ph == 2)
            def _():
                xa_v[SEG:, :] = z_v[:SEG, :]
                ya_v[0:SEG, :] = ya_v[2 * SEG:, :]
                big_v[S - 3 * SEG:S - 2 * SEG, :] = z_v[SEG:, :].astype(BF16)
                out_copy(S - 3 * SEG, SEG).start()

            @pl.when(ph == 3)
            def _():
                big_v[S - 2 * SEG:S, :] = z_v[...].astype(BF16)
                out_copy(S - 2 * SEG, 2 * SEG).start()
            return carry

        lax.fori_loop(0, cfg.get('nph', 4), phase, 0)
        out_copy(0, cfg.get("nsteps", NSEG) * SEG).wait()

    scratch = [
        pltpu.VMEM((S, D), BF16),
        pltpu.VMEM((FF, D), BF16),
        pltpu.VMEM((GST, NB, GR, FF), BF16),
        pltpu.VMEM((QST, NB, QR * H, DH), BF16),
        pltpu.VMEM((NB, H, QR, DH), BF16),
        pltpu.VMEM((HB, NP, DB // 2, 3 * DH), U32),
        pltpu.VMEM((NP, EB // 2, DB), U32),
        pltpu.VMEM((FB // LANES, NP, DB // 2, 2 * LANES), U32),
        pltpu.VMEM((NP, FB // 2, DB), U32),
        pltpu.VMEM((NP, L, DB), F32),
        pltpu.VMEM((NP, L, EB), F32),
        pltpu.VMEM((NP, SEG, DB), F32),
        pltpu.VMEM((NP, SEG, FB), F32),
        pltpu.VMEM((2 * M, D), F32),
        pltpu.VMEM((2 * SEG, D), F32),
        pltpu.VMEM((2 * L, D), F32),
        pltpu.VMEM((2 * SEG, D), F32),
        pltpu.VMEM((3 * SEG, D), F32),
        pltpu.VMEM((2 * SEG, D), F32),
        pltpu.VMEM((NB, 2, LANES, DH), BF16),
        pltpu.VMEM((2 * L, LANES), F32),
        pltpu.VMEM((2 * L, LANES), jnp.int32),
        pltpu.SemaphoreType.DMA((2,)),
        pltpu.SemaphoreType.DMA((QST, NB)),
        pltpu.SemaphoreType.DMA((OST, NB)),
        pltpu.SemaphoreType.DMA((GST, NB)),
        pltpu.SemaphoreType.DMA((GST, NB)),
        pltpu.SemaphoreType.DMA(()),
    ]
    return kernel, scratch


def _build(cfg):
    @functools.partial(jax.jit, static_argnames=("A_seg_len",))
    def fn(A_x, A_mem0, A_Wq, A_Wk, A_Wv, A_Wo, A_seg_len, B_x, B_w_gate, B_w_up, B_w_down):
        B, S, D = A_x.shape
        _, H, DH = A_Wq.shape
        M = A_mem0.shape[1]
        FF = B_w_gate.shape[1]
        kernel, scratch = _make_kernel(S, D, H, DH, M, A_seg_len, FF, cfg)
        any_spec = pl.BlockSpec(memory_space=pl.ANY)
        out = pl.pallas_call(
            kernel,
            out_shape=jax.ShapeDtypeStruct((S, D), A_x.dtype),
            in_specs=[any_spec, pl.BlockSpec(memory_space=pltpu.VMEM)] + [any_spec] * 7,
            out_specs=any_spec,
            scratch_shapes=scratch,
            compiler_params=pltpu.CompilerParams(vmem_limit_bytes=cfg.get("vmem", 124) * 1024 * 1024,
                                                 flags=cfg.get("flags")),
        )(A_x.reshape(S, D), A_mem0.reshape(M, D),
          A_Wq.reshape(D * H, DH), A_Wk.reshape(D * H, DH), A_Wv.reshape(D * H, DH),
          A_Wo.reshape(H * DH, D), B_w_gate, B_w_up, B_w_down)
        return out.reshape(B, S, D)
    return fn


pallas_interleave_layers__memory_aug_recurrent_mem_tr__glu_gated_glu__prompt_kernel = _build({})
```

```python
import functools
import itertools
import math

import jax
import jax.numpy as jnp
import numpy as np
from jax import lax
import jax.experimental.pallas as pl
import jax.experimental.pallas.tpu as pltpu

F32 = jnp.float32
BF16 = jnp.bfloat16
U32 = jnp.uint32
EPS = 1e-05
LANES = 128

STRASSEN = (2, (
    ({(1, 0): 1, (1, 1): 1}, {(0, 0): 1}, {(1, 0): 1, (1, 1): -1}, {0: 1, 1: 1}, {0: 1}),
    ({(1, 1): 1}, {(1, 0): 1, (0, 0): -1}, {(0, 0): 1, (1, 0): 1}, {1: 1}, {0: 1}),
    ({(0, 0): 1}, {(0, 1): 1, (1, 1): -1}, {(0, 1): 1, (1, 1): 1}, {0: 1}, {1: 1}),
    ({(0, 0): 1, (0, 1): 1}, {(1, 1): 1}, {(0, 0): -1, (0, 1): 1}, {0: 1, 1: 1}, {1: 1}),
    ({(0, 0): 1, (1, 1): 1}, {(0, 0): 1, (1, 1): 1}, {(0, 0): 1, (1, 1): 1}, None, None),
    ({(1, 0): 1, (0, 0): -1}, {(0, 0): 1, (0, 1): 1}, {(1, 1): 1}, None, None),
    ({(0, 1): 1, (1, 1): -1}, {(1, 0): 1, (1, 1): 1}, {(0, 0): 1}, None, None),
))
HK26 = (4, (
    ({(0, 0): 1}, {(0, 0): 1, (0, 2): 1, (1, 0): -1, (3, 0): 1}, {(0, 0): 1, (1, 0): -1}, None, None),
    ({(0, 0): 1, (1, 0): 1}, {(0, 0): 1, (0, 1): -1, (2, 0): 1, (3, 0): -1}, {(1, 0): 1}, {0: 1}, {0: 1}),
    ({(0, 0): 1, (1, 1): -1}, {(0, 1): 1, (1, 0): -1, (3, 0): 1}, {(0, 1): 1, (1, 0): 1}, {1: 1}, {0: -1}),
    ({(1, 0): 1, (1, 1): 1}, {(0, 1): 1}, {(1, 0): 1, (1, 1): 1}, {0: 1, 1: 1}, {0: 1, 1: 1}),
    ({(0, 0): 1, (0, 1): 1}, {(0, 3): 1, (1, 0): 1, (3, 0): -1}, {(0, 0): 1, (0, 1): 1}, None, None),
    ({(0, 0): 1, (1, 0): 1, (1, 1): 1, (1, 3): 1}, {(3, 0): -1}, {(0, 0): 1, (0, 1): 1, (0, 3): -1, (1, 0): -1}, {0: 1, 1: 1, 3: 1}, {0: -1}),
    ({(0, 0): 1, (0, 1): 1, (0, 3): 1, (1, 0): 1, (1, 1): 1, (1, 3): 1}, {(0, 3): -1, (3, 0): 1}, {(0, 0): 1, (0, 1): 1, (0, 3): -1}, None, None),
    ({(0, 3): 1, (1, 0): 1, (1, 1): 1, (1, 3): 1}, {(0, 3): 1}, {(0, 0): 1, (0, 1): 1, (0, 3): -1, (1, 3): 1}, {0: 1, 1: 1, 3: 1}, {3: 1}),
    ({(0, 0): 1, (1, 0): 1, (1, 2): -1}, {(0, 2): 1, (2, 0): -1}, {(0, 0): -1, (0, 2): 1, (1, 0): 1}, None, None),
    ({(1, 0): 1, (1, 2): -1}, {(0, 2): -1}, {(0, 0): -1, (0, 2): 1, (1, 0): 1, (1, 2): -1}, {0: 1, 2: -1}, {2: -1}),
    ({(0, 0): 1, (0, 2): -1, (1, 0): 1, (1, 2): -1}, {(2, 0): 1}, {(0, 0): -1, (0, 2): 1}, {0: 1, 2: -1}, {0: -1}),
    ({(1, 1): 1}, {(0, 1): 1, (1, 1): -1, (1, 2): -1, (3, 1): 1}, {(0, 1): 1, (1, 1): -1}, {1: 1}, {1: -1}),
    ({(0, 1): 1, (1, 1): 1}, {(0, 3): -1, (1, 0): -1, (1, 1): 1, (1, 3): 1, (2, 1): -1, (3, 0): 1}, {(0, 1): 1}, None, None),
    ({(0, 3): -1, (1, 1): 1}, {(0, 3): -1, (1, 3): 1, (3, 1): 1}, {(0, 1): -1, (1, 3): 1}, {1: 1}, {3: 1}),
    ({(0, 1): 1, (0, 3): 1}, {(0, 3): -1, (1, 3): 1, (3, 0): 1}, {(0, 1): -1, (0, 3): 1}, None, None),
    ({(1, 1): 1, (1, 3): 1}, {(3, 1): -1}, {(1, 1): -1, (1, 3): 1}, {1: 1, 3: 1}, {1: -1, 3: 1}),
    ({(0, 1): 1, (0, 2): 1, (1, 1): 1}, {(1, 2): 1, (2, 1): 1}, {(0, 1): 1, (1, 1): -1, (1, 2): 1}, None, None),
    ({(0, 1): 1, (0, 2): 1}, {(1, 2): 1}, {(0, 1): -1, (0, 2): 1, (1, 1): 1, (1, 2): -1}, {1: 1}, {1: -1, 2: 1}),
    ({(0, 1): 1, (0, 2): 1, (1, 1): 1, (1, 2): 1}, {(2, 1): -1}, {(1, 1): -1, (1, 2): 1}, {2: 1}, {1: -1, 2: 1}),
    ({(0, 3): 1, (1, 2): 1, (1, 3): 1}, {(2, 3): -1, (3, 2): -1}, {(0, 2): -1, (0, 3): 1, (1, 3): -1}, None, None),
    ({(0, 2): 1, (0, 3): 1, (1, 2): 1, (1, 3): 1}, {(2, 3): 1}, {(0, 2): -1, (0, 3): 1}, {2: 1, 3: 1}, {3: 1}),
    ({(1, 2): 1, (1, 3): 1}, {(3, 2): 1}, {(0, 2): -1, (0, 3): 1, (1, 2): 1, (1, 3): -1}, {2: 1, 3: 1}, {2: 1}),
    ({(0, 2): 1}, {(1, 2): -1, (2, 0): 1, (2, 2): 1, (2, 3): 1}, {(0, 2): 1}, None, None),
    ({(1, 2): 1}, {(0, 2): 1, (2, 1): 1, (2, 2): 1, (3, 2): -1}, {(1, 2): 1}, {2: 1}, {2: 1}),
    ({(0, 3): 1}, {(0, 3): 1, (1, 3): -1, (3, 2): 1, (3, 3): 1}, {(0, 3): 1, (1, 3): -1}, None, None),
    ({(0, 3): 1, (1, 3): 1}, {(0, 3): -1, (2, 3): -1, (3, 1): 1, (3, 3): 1}, {(1, 3): 1}, {3: 1}, {3: 1}),
))
SCHEMES = {"strassen": STRASSEN, "hk26": HK26}


def _combine(coefs, vals):
    acc = None
    for key, c in sorted(coefs.items(), key=lambda kv: -kv[1]):
        v = vals[key]
        if abs(c) != 1:
            v = v * abs(c)
        if acc is None:
            acc = v if c > 0 else -v
        else:
            acc = acc + v if c > 0 else acc - v
    return acc


def _accumulate(accs, group):
    terms = {}
    for n, (coefs, _) in enumerate(group):
        for key, c in coefs.items():
            terms.setdefault(key, []).append((n, c))
    sums = {((n, 1),): v for n, (_, v) in enumerate(group)}
    for key, tm in sorted(terms.items(), key=lambda kv: len(kv[1])):
        sign = tm[0][1]
        tm = tuple((n, c * sign) for n, c in tm)
        if tm not in sums:
            base = max((s for s in sums if all(t in tm for t in s)), key=len)
            val = sums[base]
            for n, c in tm:
                if (n, c) not in base:
                    val = val + group[n][1] if c > 0 else val - group[n][1]
            sums[tm] = val
        if key not in accs:
            accs[key] = sums[tm] if sign > 0 else -sums[tm]
        else:
            accs[key] = accs[key] + sums[tm] if sign > 0 else accs[key] - sums[tm]


def _layernorm(x):
    m = jnp.mean(x, axis=-1, keepdims=True)
    c = x - m
    v = jnp.mean(c * c, axis=-1, keepdims=True)
    return c * lax.rsqrt(v + EPS)


def _dot(a, b):
    return lax.dot_general(a, b, (((1,), (0,)), ((), ())), preferred_element_type=F32)


def _dot_nt(a, b):
    return lax.dot_general(a, b, (((1,), (1,)), ((), ())), preferred_element_type=F32)


def _halves(x):
    return [pltpu.unpack_elementwise(x, index=k, packed_dtype=BF16, unpacked_dtype=F32)
            for k in range(2)]


def _pair(lo, hi):
    return pltpu.pack_elementwise([lo, hi], packed_dtype=BF16)


def _make_kernel(S, D, H, DH, M, SEG, FF, cfg):
    NB, prods = SCHEMES[cfg.get("scheme", "hk26")]
    if "order" in cfg:
        prods = tuple(prods[i] for i in cfg["order"])
    NP = len(prods)
    NSEG = S // SEG
    L = M + SEG
    DB, HB, FB = D // NB, H // NB, FF // NB
    EB = HB * DH
    OC = DB // 2
    QR = cfg.get("QR", 128) // NB
    QST = cfg.get("QST", 4)
    WR = 512 // NB
    OST = FF // (WR * NB)
    GST = 4
    GR, DR = DB // GST, FB // GST
    XH = 2 * SEG
    scale = DH ** (-0.5)
    c_exp = scale * math.log2(math.e)

    def put_lhs(ref, r, tile0, val):
        for k in range(val.shape[1] // LANES):
            ref[r, tile0 + k] = val[:, k * LANES:(k + 1) * LANES].astype(ref.dtype)

    def store_lhs(ref, cols, blocks, paired):
        for r, (u, _, _, u1, _) in enumerate(prods):
            if paired or u1 is not None:
                put_lhs(ref, r, cols.start // LANES, _combine(u if paired else u1, blocks))

    ends = cfg.get("ends", (1, 4, 7, 10, 12, 15, 18, 21, 23, 25))

    def fast_dot(*args):
        acc = {}
        for _ in fast_dot_steps(acc, *args):
            pass
        return acc

    def fast_dot_steps(acc, lhs_ref, w_of, paired, hooks=None, src_ref=None):
        n = lhs_ref.shape[2]
        group = []
        for r, (u, _, w, u1, w1) in enumerate(prods):
            if hooks and r in hooks:
                hooks[r]()
            if not paired and u1 is None:
                continue
            if src_ref is None:
                lhs = jnp.concatenate([lhs_ref[r, k] for k in range(lhs_ref.shape[1])], axis=1)
            else:
                if paired:
                    lhs = _combine(u, {(hf, i): src_ref[hf * n:(hf + 1) * n, i * DB:(i + 1) * DB]
                                       for hf, i in u})
                else:
                    lhs = _combine(u1, {i: src_ref[0:n, i * DB:(i + 1) * DB] for i in u1})
                lhs = lhs.astype(lhs_ref.dtype)
                put_lhs(lhs_ref, r, 0, lhs)
            group.append((w if paired else w1, _dot(lhs, pltpu.bitcast(w_of(r), BF16))))
            if r in ends or not paired:
                _accumulate(acc, group)
                group = []
                yield

    def out_cols(j, c):
        return slice(j * DB + c * OC, j * DB + (c + 1) * OC)

    def kernel(x_hbm, mem0_ref, wq_hbm, wk_hbm, wv_hbm, wo_hbm, wg_hbm, wu_hbm, wd_hbm,
               out_hbm,
               x_v, big_v, gst_v, qst_v, qtr_v, wqkv_v, wo_v, wgu_v, wd_v,
               la_v, lo_v, lb_v, ld_v, mem_v, xa_v, na_v, nb_v, ya_v, z_v, kv_v, fill_v, keep_v,
               sem_x, sem_q, sem_o, sem_g, sem_d, sem_out):

        def rows_at(start, size):
            return pl.ds(start if isinstance(start, int) else pl.multiple_of(start, 16), size)

        def q_copies(w, c, slot):
            src = (wq_hbm, wk_hbm, wv_hbm)[w]
            return [pltpu.make_async_copy(src.at[rows_at((i * DB + c * QR) * H, QR * H), :],
                                          qst_v.at[slot, i, 0:QR * H, :], sem_q.at[slot, i]) for i in range(NB)]

        def o_copies(c):
            slot = c % OST
            return [pltpu.make_async_copy(wo_hbm.at[rows_at(i * EB + c * WR, WR), :],
                                          big_v.at[rows_at((slot * NB + i) * WR, WR), :],
                                          sem_o.at[slot, i]) for i in range(NB)]

        def g_copies(src, c):
            return [pltpu.make_async_copy(src.at[rows_at(i * DB + c * GR, GR), :],
                                          gst_v.at[c, i], sem_g.at[c, i]) for i in range(NB)]

        def d_copies(c):
            return [pltpu.make_async_copy(wd_hbm.at[rows_at(i * FB + c * DR, DR), :],
                                          big_v.at[rows_at(i * FB + c * DR, DR), :],
                                          sem_d.at[c, i]) for i in range(NB)]

        def start(copies):
            for cp in copies:
                cp.start()

        def wait(copies):
            for cp in copies:
                cp.wait()

        def prep_tiles(load, put, nrows, ncols, mul=None):
            def tile(s, k):
                lo, hi = {}, {}
                for i in range(NB):
                    for j in range(NB):
                        x = load(i, j, pl.multiple_of(s * 16, 16), k)
                        lo[i, j], hi[i, j] = _halves(pltpu.bitcast(x, U32))
                        if mul is not None:
                            lo[i, j], hi[i, j] = lo[i, j] * mul, hi[i, j] * mul
                for r, (_, v, _, _, _) in enumerate(prods):
                    put(r, s * 8, k, _pair(_combine(v, lo), _combine(v, hi)))

            pu = cfg.get("pu", 1)

            def tiles(n, pos):
                s, k = pos
                for d in range(pu):
                    tile(s * pu + d, k)
                wrap = k + 1 == ncols
                return jnp.where(wrap, s + 1, s), jnp.where(wrap, 0, k + 1)
            lax.fori_loop(0, nrows // (16 * pu) * ncols, tiles, (0, 0))

        def lanes_at(k):
            return pl.ds(pl.multiple_of(k * LANES, LANES), LANES)

        def words_at(row):
            return pl.ds(pl.multiple_of(row, 8), 8)

        def prep_qkv(w, c, slot):
            def heads(i, carry):
                st = qst_v.at[slot, i].bitcast(U32)
                for jp in range(H // 2):
                    for k, x in enumerate(_halves(st[pl.ds(jp, QR, stride=H // 2), :])):
                        qtr_v[i, 2 * jp + k] = x.astype(BF16)
                return carry
            lax.fori_loop(0, NB, heads, 0)

            def put(r, row, k, val):
                wqkv_v[k, r, words_at(c * (QR // 2) + row), lanes_at(w)] = val
            prep_tiles(lambda i, j, row, k: qtr_v[i, j * HB + k, pl.ds(row, 16), :], put, QR, HB)

        def prep_from_big(dst, base, blk, c, nrows):
            def load(i, j, row, k):
                return big_v[rows_at(base + i * blk + row, 16), lanes_at(j * (DB // LANES) + k)]

            def put(r, row, k, val):
                dst[r, words_at(c * (nrows // 2) + row), lanes_at(k)] = val
            prep_tiles(load, put, nrows, DB // LANES)

        def prep_gu(w, c):
            def load(i, j, row, k):
                return gst_v[c, i, pl.ds(row, 16), lanes_at(j * (FB // LANES) + k)]

            def put(r, row, k, val):
                wgu_v[k, r, words_at(c * (GR // 2) + row), w * LANES:(w + 1) * LANES] = val
            prep_tiles(load, put, GR, FB // LANES, 0.5)

        x_head = pltpu.make_async_copy(x_hbm.at[0:XH, :], x_v.at[0:XH, :], sem_x.at[0])
        x_tail = pltpu.make_async_copy(x_hbm.at[XH:, :], x_v.at[XH:, :], sem_x.at[1])
        NQ, NO = DB // QR, EB // WR
        ONEXT = min(QST, OST)
        for n in range(QST):
            start(q_copies(0, n, n))
        x_head.start()

        ri = lax.broadcasted_iota(jnp.int32, (2 * L, LANES), 0)
        ci = lax.broadcasted_iota(jnp.int32, (2 * L, LANES), 1)
        first = jnp.where(ri < L, 0, L)
        same = (ci >= first) & (ci < first + L)
        visible = (ri < first + M) | (ri >= ci)
        keep_v[...] = (same & visible).astype(jnp.int32)
        fill_v[...] = jnp.where(same, -1e9 / scale, -jnp.inf).astype(F32)
        kv_v[...] = jnp.zeros(kv_v.shape, BF16)
        mem_v[0:M, :] = mem0_ref[...].astype(F32)
        mem_v[M:, :] = mem0_ref[...].astype(F32)

        for w in range(3):
            def q_body(c, carry, w=w):
                slot = (w * NQ + c) % QST
                wait(q_copies(w, c, slot))
                prep_qkv(w, c, slot)
                pl.when(c + QST < NQ)(lambda: start(q_copies(w, c + QST, slot)))
                if w < 2:
                    pl.when(c + QST >= NQ)(lambda: start(q_copies(w + 1, c + QST - NQ, slot)))
                else:
                    pl.when((c + QST >= NQ) & (c + QST - NQ < ONEXT))(
                        lambda: start(o_copies(c + QST - NQ)))
                return carry
            lax.fori_loop(0, NQ, q_body, 0)

        def o_body(c, carry):
            wait(o_copies(c))
            prep_from_big(wo_v, (c % OST) * NB * WR, WR, c, WR)
            pl.when(c + ONEXT < NO)(lambda: start(o_copies(c + ONEXT)))
            pl.when(c >= NO - GST)(lambda: start(g_copies(wg_hbm, c - (NO - GST))))
            return carry
        lax.fori_loop(0, NO, o_body, 0)
        for c in range(GST):
            start(d_copies(c))
        x_head.wait()
        xa_v[...] = x_v[0:XH, :].astype(F32)

        def load_glu_weights():
            def gate(c, carry):
                wait(g_copies(wg_hbm, c))
                prep_gu(0, c)
                start(g_copies(wu_hbm, c))
                return carry

            def down(c, carry):
                wait(d_copies(c))
                prep_from_big(wd_v, c * DR, FB, c, DR)
                return carry

            def up(c, carry):
                wait(g_copies(wu_hbm, c))
                prep_gu(1, c)
                return carry
            lax.fori_loop(0, GST, gate, 0)
            lax.fori_loop(0, GST, down, 0)
            lax.fori_loop(0, GST, up, 0)
            x_tail.start()

        def attention(c, qkv, paired):
            probs = {}

            def scores():
                for j in range(NB):
                    x = jnp.concatenate([qkv[0, j], qkv[1, j]], axis=0) if paired else qkv[j]
                    n = x.shape[0]
                    for w in range(2):
                        kv_v[j, w, 0:n, :] = x[:, (w + 1) * DH:(w + 2) * DH].astype(BF16)
                    s = _dot_nt(x[:, :DH], kv_v[j, 0])
                    s = jnp.where(keep_v[0:n, :] != 0, s, fill_v[0:n, :])
                    mx = jnp.max(s, axis=-1, keepdims=True)
                    e = jnp.exp2((s - mx) * c_exp)
                    den = jnp.sum(e, axis=-1, keepdims=True)
                    inv = pl.reciprocal(den, approx=True)
                    inv = inv * (2.0 - den * inv)
                    probs[j] = e * inv

            def values():
                o = {j: _dot(probs[j], kv_v[j, 1]) for j in range(NB)}
                if paired:
                    o = {(hf, j): o[j][hf * L:(hf + 1) * L] for hf in range(2) for j in range(NB)}
                store_lhs(lo_v, slice(c * DH, (c + 1) * DH), o, paired)

            return scores, values

        def gate_up(c, hooks=None):
            if cfg.get("sg", 0):
                parts = [fast_dot(lb_v, lambda r: wgu_v[c, r, :, w * LANES:(w + 1) * LANES], True,
                                  hooks if w == 0 else None, nb_v if c + w == 0 else None)
                         for w in range(2)]
                gu = {k: jnp.concatenate([p[k] for p in parts], axis=1) for k in parts[0]}
            else:
                gu = fast_dot(lb_v, lambda r: wgu_v[c, r], True, hooks, nb_v if c == 0 else None)
            act = {k: jnp.tanh(v[:, :LANES]) * v[:, LANES:] + v[:, LANES:] for k, v in gu.items()}
            store_lhs(ld_v, slice(c * LANES, (c + 1) * LANES), act, True)

        def down(c, hooks=None):
            dn = fast_dot(ld_v, lambda r: wd_v[r, :, c * OC:(c + 1) * OC], True, hooks)
            for (hf, j), v in dn.items():
                rows = slice(hf * SEG, (hf + 1) * SEG)
                z_v[rows, out_cols(j, c)] = ya_v[rows, out_cols(j, c)] + v

        def glu_input():
            nb_v[...] = _layernorm(ya_v[0:2 * SEG, :])

        def out_copy(row, n):
            return pltpu.make_async_copy(big_v.at[pl.ds(row, n), :],
                                         out_hbm.at[pl.ds(row, n), :], sem_out)

        def attention_single(mrow, xrow, yrow):
            na_v[0:M, :] = mem_v[pl.ds(mrow, M), :]
            na_v[M:L, :] = _layernorm(xa_v[pl.ds(xrow, SEG), :])
            hooks = None
            for c in range(HB):
                qkv = fast_dot(la_v, lambda r: wqkv_v[c, r], False, hooks, na_v if c == 0 else None)
                scores, values = attention(c, qkv, False)
                hooks = {5: scores, NP - 1: values}
            scores()
            values()
            for c in range(DB // OC):
                o = fast_dot(lo_v, lambda r: wo_v[r, :, c * OC:(c + 1) * OC], False)
                for j in range(NB):
                    mem_v[pl.ds(mrow, M), out_cols(j, c)] = o[j][:M]
                    ya_v[pl.ds(yrow, SEG), out_cols(j, c)] = (
                        xa_v[pl.ds(xrow, SEG), out_cols(j, c)] + o[j][M:])

        def step(t, carry):
            cur = pl.multiple_of(t * SEG, SEG)
            nxt = pl.multiple_of(jnp.minimum(t + 1, NSEG - 1) * SEG, SEG)
            row = pl.multiple_of(jnp.maximum(t - 3, 0) * SEG, SEG)
            hooks = {0: {cfg.get("g0", 2): glu_input}}
            for c in range(HB):
                parts = [{}, {}, {}]
                gens = [fast_dot_steps(parts[w], la_v, functools.partial(
                    lambda w, r: wqkv_v[c, r, :, w * DH:(w + 1) * DH], w), True,
                    (hooks or {}).get(w), na_v if c + w == 0 else None) for w in range(3)]
                mode = cfg.get("mode", 0)
                if mode == 1 and c > 0:
                    gu = [{}, {}]
                    gg = [fast_dot_steps(gu[w], lb_v, functools.partial(
                        lambda w, r: wgu_v[c - 1, r, :, w * LANES:(w + 1) * LANES], w), True,
                        None, nb_v if c + w == 1 else None) for w in range(2)]
                    for w in range(2):
                        for _ in itertools.zip_longest(gens[w], gg[w]):
                            pass
                    act = {k: jnp.tanh(gu[0][k]) * gu[1][k] + gu[1][k] for k in gu[0]}
                    store_lhs(ld_v, slice((c - 1) * LANES, c * LANES), act, True)
                for g in gens:
                    for _ in g:
                        pass
                qkv = {k: jnp.concatenate([p[k] for p in parts], axis=1) for k in parts[0]}
                scores, values = attention(c, qkv, True)
                if mode == 1:
                    hooks = {0: {cfg.get("h0", 8): scores}, cfg.get("hw", 1): {cfg.get("h1", 10): values}}
                elif mode == 2:
                    if c < FB // LANES:
                        gate_up(c)
                    hooks = {1: {cfg.get("h0", 8): scores}, 2: {cfg.get("h1", 14): values}}
                elif c < FB // LANES:
                    gate_up(c, {cfg.get("h0", 8): scores})
                    hooks = {cfg.get("hw", 0): {cfg.get("h1", 10): values}}
            down(0, {cfg.get("d0", 3): scores, cfg.get("d1", 16): values})
            down(1)
            big_v[pl.ds(row, SEG), :] = z_v[SEG:, :].astype(BF16)

            def next_input():
                na_v[M:L, :] = _layernorm(x_v[pl.ds(nxt, SEG), :].astype(F32))
                na_v[L + M:, :] = _layernorm(z_v[:SEG, :])

            for c in range(DB // OC):
                o = fast_dot(lo_v, lambda r: wo_v[r, :, c * OC:(c + 1) * OC], True,
                             {cfg.get("h2", 2): next_input} if c == 0 else None)
                for (hf, j), v in o.items():
                    res = (x_v[pl.ds(cur, SEG), out_cols(j, c)].astype(F32) if hf == 0
                           else xa_v[SEG:, out_cols(j, c)])
                    na_v[hf * L:hf * L + M, out_cols(j, c)] = v[:M]
                    ya_v[hf * SEG:(hf + 1) * SEG, out_cols(j, c)] = res + v[M:]
            xa_v[SEG:, :] = z_v[:SEG, :]
            pl.when(t >= 3)(lambda: out_copy(row, SEG).start())
            return carry

        def phase(ph, carry):
            attention_single(pl.multiple_of(jnp.where(ph < 2, 0, M), M),
                             pl.multiple_of(jnp.where(ph == 0, 0, SEG), SEG),
                             pl.multiple_of(jnp.where(ph == 3, 1, ph) * SEG, SEG))
            pl.when(ph == 1)(load_glu_weights)

            @pl.when(ph >= 1)
            def _():
                glu_input()
                for c in range(FB // LANES):
                    gate_up(c)
                for c in range(DB // OC):
                    down(c)

            @pl.when(ph == 1)
            def _():
                x_tail.wait()
                ya_v[0:SEG, :] = ya_v[SEG:2 * SEG, :]
                xa_v[SEG:, :] = z_v[:SEG, :]
                na_v[0:M, :] = mem_v[0:M, :]
                na_v[M:L, :] = _layernorm(x_v[2 * SEG:3 * SEG, :].astype(F32))
                na_v[L:L + M, :] = mem_v[M:, :]
                na_v[L + M:, :] = _layernorm(z_v[:SEG, :])
                lax.fori_loop(2, cfg.get("nsteps", NSEG), step, 0, unroll=cfg.get("un", 1))
                mem_v[M:, :] = na_v[L:L + M, :]

            @pl.when(ph == 2)
            def _():
                xa_v[SEG:, :] = z_v[:SEG, :]
                ya_v[0:SEG, :] = ya_v[2 * SEG:, :]
                big_v[S - 3 * SEG:S - 2 * SEG, :] = z_v[SEG:, :].astype(BF16)
                out_copy(S - 3 * SEG, SEG).start()

            @pl.when(ph == 3)
            def _():
                big_v[S - 2 * SEG:S, :] = z_v[...].astype(BF16)
                out_copy(S - 2 * SEG, 2 * SEG).start()
            return carry

        lax.fori_loop(0, cfg.get('nph', 4), phase, 0)
        out_copy(0, cfg.get("nsteps", NSEG) * SEG).wait()

    scratch = [
        pltpu.VMEM((S, D), BF16),
        pltpu.VMEM((FF, D), BF16),
        pltpu.VMEM((GST, NB, GR, FF), BF16),
        pltpu.VMEM((QST, NB, (QR + 1) * H, DH), BF16),
        pltpu.VMEM((NB, H, QR, DH), BF16),
        pltpu.VMEM((HB, NP, DB // 2, 3 * DH), U32),
        pltpu.VMEM((NP, EB // 2, DB), U32),
        pltpu.VMEM((FB // LANES, NP, DB // 2, 2 * LANES), U32),
        pltpu.VMEM((NP, FB // 2, DB), U32),
        pltpu.VMEM((NP, DB // LANES, L, LANES), F32),
        pltpu.VMEM((NP, EB // LANES, L, LANES), F32),
        pltpu.VMEM((NP, DB // LANES, SEG, LANES), BF16 if cfg.get('bb', 1) else F32),
        pltpu.VMEM((NP, FB // LANES, SEG, LANES), BF16 if cfg.get('bd', 0) else F32),
        pltpu.VMEM((2 * M, D), F32),
        pltpu.VMEM((2 * SEG, D), F32),
        pltpu.VMEM((2 * L, D), F32),
        pltpu.VMEM((2 * SEG, D), F32),
        pltpu.VMEM((3 * SEG, D), F32),
        pltpu.VMEM((2 * SEG, D), F32),
        pltpu.VMEM((NB, 2, LANES, DH), BF16),
        pltpu.VMEM((2 * L, LANES), F32),
        pltpu.VMEM((2 * L, LANES), jnp.int32),
        pltpu.SemaphoreType.DMA((2,)),
        pltpu.SemaphoreType.DMA((QST, NB)),
        pltpu.SemaphoreType.DMA((OST, NB)),
        pltpu.SemaphoreType.DMA((GST, NB)),
        pltpu.SemaphoreType.DMA((GST, NB)),
        pltpu.SemaphoreType.DMA(()),
    ]
    return kernel, scratch


def _build(cfg):
    @functools.partial(jax.jit, static_argnames=("A_seg_len",))
    def fn(A_x, A_mem0, A_Wq, A_Wk, A_Wv, A_Wo, A_seg_len, B_x, B_w_gate, B_w_up, B_w_down):
        B, S, D = A_x.shape
        _, H, DH = A_Wq.shape
        M = A_mem0.shape[1]
        FF = B_w_gate.shape[1]
        kernel, scratch = _make_kernel(S, D, H, DH, M, A_seg_len, FF, cfg)
        any_spec = pl.BlockSpec(memory_space=pl.ANY)
        out = pl.pallas_call(
            kernel,
            out_shape=jax.ShapeDtypeStruct((S, D), A_x.dtype),
            in_specs=[any_spec, pl.BlockSpec(memory_space=pltpu.VMEM)] + [any_spec] * 7,
            out_specs=any_spec,
            scratch_shapes=scratch,
            compiler_params=pltpu.CompilerParams(vmem_limit_bytes=cfg.get("vmem", 124) * 1024 * 1024,
                                                 flags=cfg.get("flags")),
        )(A_x.reshape(S, D), A_mem0.reshape(M, D),
          A_Wq.reshape(D * H, DH), A_Wk.reshape(D * H, DH), A_Wv.reshape(D * H, DH),
          A_Wo.reshape(H * DH, D), B_w_gate, B_w_up, B_w_down)
        return out.reshape(B, S, D)
    return fn


pallas_interleave_layers__memory_aug_recurrent_mem_tr__glu_gated_glu__prompt_kernel = _build({})
```

```python
import functools
import math

import jax
import jax.numpy as jnp
import numpy as np
from jax import lax
import jax.experimental.pallas as pl
import jax.experimental.pallas.tpu as pltpu

F32 = jnp.float32
BF16 = jnp.bfloat16
U32 = jnp.uint32
EPS = 1e-05
LANES = 128

_SCHEME_4 = """
+00 | +00 +02 -10 +30 | +00 -10
+00 +10 | +00 -01 +20 -30 | +10

+00 -11 | +01 -10 +30 | +01 +10
+10 +11 | +01 | +10 +11
+00 +01 | +03 +10 -30 | +00 +01

+00 +10 +11 +13 | +30 | -00 -01 +03 +10
+00 +01 +03 +10 +11 +13 | -03 +30 | +00 +01 -03
+03 +10 +11 +13 | +03 | +00 +01 -03 +13

+00 +10 -12 | +02 -20 | -00 +02 +10
+10 -12 | +02 | +00 -02 -10 +12
+00 -02 +10 -12 | +20 | -00 +02

+11 | +01 -11 -12 +31 | +01 -11
+01 +11 | -03 -10 +11 +13 -21 +30 | +01

-03 +11 | -03 +13 +31 | -01 +13
+01 +03 | -03 +13 +30 | -01 +03
+11 +13 | +31 | +11 -13

+01 +02 +11 | +12 +21 | +01 -11 +12
+01 +02 | +12 | -01 +02 +11 -12
+01 +02 +11 +12 | +21 | +11 -12

+03 +12 +13 | -23 -32 | -02 +03 -13
+02 +03 +12 +13 | +23 | -02 +03
+12 +13 | +32 | -02 +03 +12 -13

+02 | -12 +20 +22 +23 | +02
+12 | +02 +21 +22 -32 | +12

+03 | +03 -13 +32 +33 | +03 -13
+03 +13 | -03 -23 +31 +33 | +13
"""
_SCHEME_8 = """
+01 +10 | +01 +10 | +00 +11
+00 -01 | +01 | +00 +01
+10 -11 | +10 | -10 -11

+00 +02 +10 | +02 +20 | +00 -10 +12
+00 +02 | +02 | -00 +02 +10 -12
+00 +02 +10 +12 | +20 | +10 -12

+00 +03 -04 +10 | +30 | +00 -10 -13 -14
+00 +03 -04 +10 +13 -14 | +03 +30 | +10 +13 +14
+00 +03 -04 +13 | +03 | +03 -10 -13 -14

+04 +10 | +04 +30 +40 -74 | +00 +14
+00 -04 | +04 -47 -74 | +00 +04
+10 -14 | -03 -30 -40 | +10 +14

+00 -05 +10 | +05 +50 | -00 +10 +15
+00 -05 | +05 | +00 +05 -10 -15
+00 -05 +10 -15 | +50 | -10 -15

+00 +06 +07 +10 | +60 | +00 -10 -16 +17
+00 +06 +07 +10 +16 +17 | +06 +60 | +10 +16 -17
+00 +06 +07 +16 | +06 | +06 -10 -16 +17

-07 +10 | +07 +47 -60 +70 | -00 +17
+00 +07 | +07 +47 +74 | -00 +07
+10 +17 | +06 +60 -70 | -10 +17

+10 | -00 -02 +05 -10 -30 -40 -60 +70 | +00 -10
+00 +10 | +00 -01 -04 +07 -20 -30 +47 +50 -60 +74 | +00

+01 +11 -12 | +12 +21 | +01 +02 -11
+11 -12 | +12 | -01 -02 +11 +12
+01 -02 +11 -12 | +21 | -01 -02

+01 +13 | +13 +31 +63 -71 | +03 +11
+11 -13 | +13 -36 +63 | +11 +13
+01 -03 | -17 -31 +71 | +01 +03

+01 +11 +14 -16 | +41 | -01 +04 +06 +11
+01 +04 -06 +11 +14 -16 | -14 +41 | +01 -04 -06
+04 +11 +14 -16 | +14 | +01 -04 -06 +14

+01 +11 +15 | +15 -51 | +01 +05 -11
+11 +15 | +15 | -01 -05 +11 +15
+01 +05 +11 +15 | +51 | +01 +05

+01 +16 | +16 +36 -41 -61 | +06 -11
+11 -16 | +16 +36 -63 | -11 +16
+01 -06 | -14 +41 +61 | -01 +06

+01 +11 -13 -17 | +71 | +01 +03 +07 -11
+01 -03 -07 +11 -13 -17 | +17 -71 | +01 +03 +07
-07 +11 -13 -17 | +17 | -01 -03 -07 +17

+01 | +01 +11 -12 -15 +31 +41 +61 -71 | +01 -11
+01 +11 | -10 +11 -13 +16 +21 +36 -41 -51 -63 +71 | +11

+02 +03 +13 | +23 -32 -52 | +03 -12 -13
+02 +03 +12 +13 | +23 | +12 +13
+02 +03 | +25 +32 +52 | +02 +03 -12 -13

-04 +12 -14 | -24 -42 | +02 +04 -14
+02 -04 +12 -14 | +24 | +02 +04
+12 -14 | +42 | +02 +04 -12 -14

+03 -05 +12 +13 -15 | +52 | -02 -03 +05 +13 -15
+12 +13 -15 | +25 +52 | +02 +03 -05 -12 -13 +15
+02 +03 +12 +13 -15 | +25 | -02 -03 +05 +12 +13

+02 +06 +16 | +26 -62 | +06 -12 -16
+02 +06 +12 +16 | +26 | +12 +16
+02 +06 | +62 | +02 +06 -12 -16

+07 +12 +17 | -27 -72 | -02 +07 -17
+02 +07 +12 +17 | +27 | -02 +07
+12 +17 | +72 | -02 +07 +12 -17

+02 | -02 -21 +22 -24 +27 -32 -52 -62 | +02
+12 | +12 +20 +22 -23 -26 +42 +52 -72 | +12

+04 +13 | +03 +34 +43 | +03 +14
+03 -04 | +34 | +03 +04
+13 -14 | -03 -30 -43 | +13 +14

+03 -05 +13 | -25 +35 -53 | +03 -13 +15
+03 -05 | -25 +35 -52 | -03 +05 +13 -15
+03 -05 +13 -15 | +53 | -13 +15

-01 +03 +06 +13 | +63 | +03 -11 -13 +16
-01 +03 +06 -11 +13 +16 | -36 +63 | +11 +13 -16
-01 +03 +06 +16 | +36 | +06 +11 +13 -16

-07 +13 | +17 +37 -73 | +03 +17
+03 +07 | +17 +37 -71 | +03 +07
+13 +17 | +73 | +13 +17

+13 | -03 -13 +25 +32 -33 -35 -43 +52 -63 +73 | +03 -13
+03 +13 | -03 -17 -23 -31 +33 -34 -37 +53 -63 +71 | +03

+04 +14 +15 | +45 -54 | +04 +05 -14
+14 +15 | +45 | -04 -05 +14 +15
+04 +05 +14 +15 | +54 | +04 +05

+04 +16 | +14 +46 +64 | +06 +14
+14 -16 | +46 | +14 +16
+04 -06 | -14 +41 -64 | +04 +06

+04 -10 +14 -17 | +74 | +00 +04 -07 -14
-00 +04 -07 -10 +14 -17 | -47 -74 | +00 +04 -07
-07 -10 +14 -17 | +47 | +00 +04 -07 +17

+04 | +04 +14 +34 -42 +44 -45 +64 -74 | +04 -14
+04 +14 | -03 -14 +24 -30 -40 -43 +44 -46 -54 +74 | +14

+05 +06 +16 | +56 -65 | +06 -15 -16
+05 +06 +15 +16 | +56 | +15 +16
+05 +06 | +65 | +05 +06 -15 -16

+07 +15 +17 | -57 -75 | -05 +07 -17
+05 +07 +15 +17 | +57 | -05 +07
+15 +17 | +75 | -05 +07 +15 -17

+05 | +05 -25 +35 -51 -54 +55 +57 -65 | +05
+15 | -15 +25 -45 -50 +53 +55 -56 -75 | +15

-07 +16 | -06 +67 +76 | -06 +17
+06 +07 | +67 | -06 +07
+16 +17 | +06 +60 -76 | -16 +17

+16 | -06 -16 -36 -46 +62 +65 -66 +76 | +06 -16
+06 +16 | -06 -14 -26 -36 +41 -56 +61 -64 +66 +67 | +06

+07 | -07 -17 -37 -47 -67 +72 +75 +77 | +07 -17
+07 +17 | -06 +17 -27 +47 -57 -60 +70 -73 +76 +77 | +17
"""


class _Scheme:
    def __init__(self, n, text):
        def terms(field):
            return {(int(t[1]), int(t[2])): 1 if t[0] == "+" else -1 for t in field.split()}

        def fold(coefs, weights):
            out = {}
            for (h, i), c in coefs.items():
                out[i] = out.get(i, 0) + weights[h] * c
            return {i: c for i, c in out.items() if c}

        self.n = n
        self.prods, self.ends = [], []
        for group in text.strip().split("\n\n"):
            self.prods += [tuple(terms(f) for f in line.split("|")) for line in group.split("\n")]
            self.ends.append(len(self.prods) - 1)
        folded = [(fold(u, (-1, 1)), fold(w, (0, 1))) for u, _, w in self.prods]
        self.single = [(u, w) if u and w else None for u, w in folded]


def _combine(coefs, vals):
    acc = None
    for key, c in sorted(coefs.items(), key=lambda kv: -kv[1]):
        v = vals[key]
        if abs(c) != 1:
            v = v * abs(c)
        if acc is None:
            acc = v if c > 0 else -v
        else:
            acc = acc + v if c > 0 else acc - v
    return acc


def _accumulate(accs, group):
    terms = {}
    for n, (coefs, _) in enumerate(group):
        for key, c in coefs.items():
            terms.setdefault(key, []).append((n, c))
    sums = {((n, 1),): v for n, (_, v) in enumerate(group)}
    for key, tm in sorted(terms.items(), key=lambda kv: len(kv[1])):
        sign = tm[0][1]
        tm = tuple((n, c * sign) for n, c in tm)
        if tm not in sums:
            base = max((s for s in sums if all(t in tm for t in s)), key=len)
            val = sums[base]
            for n, c in tm:
                if (n, c) not in base:
                    val = val + group[n][1] if c > 0 else val - group[n][1]
            sums[tm] = val
        if key not in accs:
            accs[key] = sums[tm] if sign > 0 else -sums[tm]
        else:
            accs[key] = accs[key] + sums[tm] if sign > 0 else accs[key] - sums[tm]


def _layernorm(x, gain=1.0):
    m = jnp.mean(x, axis=-1, keepdims=True)
    c = x - m
    v = jnp.mean(c * c, axis=-1, keepdims=True)
    inv = lax.rsqrt(v + EPS)
    return c * (inv if gain == 1.0 else inv * gain)


def _dot(a, b):
    return lax.dot_general(a, b, (((1,), (0,)), ((), ())), preferred_element_type=F32)


def _dot_nt(a, b):
    return lax.dot_general(a, b, (((1,), (1,)), ((), ())), preferred_element_type=F32)


def _halves(x):
    return [pltpu.unpack_elementwise(x, index=k, packed_dtype=BF16, unpacked_dtype=F32)
            for k in range(2)]


def _pair(lo, hi):
    return pltpu.pack_elementwise([lo, hi], packed_dtype=BF16)


def _make_kernel(S, D, H, DH, M, SEG, FF, cfg):
    SA = _Scheme(8, _SCHEME_8) if cfg.get("na", 8) == 8 else _Scheme(4, _SCHEME_4)
    SB = _Scheme(4, _SCHEME_4)
    NA, NB = SA.n, SB.n
    PA, PB = len(SA.prods), len(SB.prods)
    NSEG = S // SEG
    L = M + SEG
    DA, HB = D // NA, H // NA
    EB = HB * DH
    DB, FB = D // NB, FF // NB
    QR = cfg.get("QR", 128) // NA
    QST = cfg.get("QST", 4)
    WR = 512 // NA
    OST = FF // (WR * NA)
    GST = 4
    GR, DR = DB // GST, FB // GST
    XH = 2 * SEG
    scale = DH ** (-0.5)
    c_exp = scale * math.log2(math.e)

    def put_lhs(ref, r, tile0, val):
        for k in range(val.shape[1] // LANES):
            ref[r, tile0 + k] = val[:, k * LANES:(k + 1) * LANES].astype(ref.dtype)

    def store_lhs(sch, ref, tile, blocks, paired):
        for r, (u, _, _) in enumerate(sch.prods):
            if paired or sch.single[r]:
                put_lhs(ref, r, tile, _combine(u if paired else sch.single[r][0], blocks))

    def fast_dot(sch, lhs_ref, w_of, paired, hooks=None, src_ref=None):
        n, kb = lhs_ref.shape[2], lhs_ref.shape[1] * LANES
        acc, group = {}, []
        for r, (u, _, w) in enumerate(sch.prods):
            if hooks and r in hooks:
                hooks[r]()
            if paired or sch.single[r]:
                if not paired:
                    u, w = sch.single[r]
                if src_ref is None:
                    lhs = jnp.concatenate([lhs_ref[r, k] for k in range(kb // LANES)], axis=1)
                else:
                    keys = u if paired else {i: (0, i) for i in u}
                    lhs = _combine(u, {
                        key: src_ref[hf * n:(hf + 1) * n, i * kb:(i + 1) * kb]
                        for key, (hf, i) in zip(u, keys if paired else keys.values())})
                    put_lhs(lhs_ref, r, 0, lhs)
                group.append((w, _dot(lhs, pltpu.bitcast(w_of(r), BF16))))
            if r in sch.ends:
                _accumulate(acc, group)
                group = []
        return acc

    def tile_of(j, blk, c):
        return slice(j * blk + c * LANES, j * blk + (c + 1) * LANES)

    def kernel(x_hbm, mem0_ref, wq_hbm, wk_hbm, wv_hbm, wo_hbm, wg_hbm, wu_hbm, wd_hbm,
               out_hbm,
               x_v, big_v, gst_v, qst_v, qtr_v, wqkv_v, wo_v, wgu_v, wd_v,
               la_v, lo_v, lb_v, ld_v, mem_v, xa_v, na_v, nb_v, ya_v, z_v, kv_v, fill_v, keep_v,
               sem_x, sem_q, sem_o, sem_g, sem_d, sem_out):

        def rows_at(start, size):
            return pl.ds(start if isinstance(start, int) else pl.multiple_of(start, 16), size)

        def q_copies(w, c, slot):
            src = (wq_hbm, wk_hbm, wv_hbm)[w]
            return [pltpu.make_async_copy(src.at[rows_at((i * DA + c * QR) * H, QR * H), :],
                                          qst_v.at[slot, i, 0:QR * H, :], sem_q.at[slot, i])
                    for i in range(NA)]

        def o_copies(c):
            slot = c % OST
            return [pltpu.make_async_copy(wo_hbm.at[rows_at(i * EB + c * WR, WR), :],
                                          big_v.at[rows_at((slot * NA + i) * WR, WR), :],
                                          sem_o.at[slot, i]) for i in range(NA)]

        def g_copies(src, c):
            return [pltpu.make_async_copy(src.at[rows_at(i * DB + c * GR, GR), :],
                                          gst_v.at[c, i], sem_g.at[c, i]) for i in range(NB)]

        def d_copies(c):
            return [pltpu.make_async_copy(wd_hbm.at[rows_at(i * FB + c * DR, DR), :],
                                          big_v.at[rows_at(i * FB + c * DR, DR), :],
                                          sem_d.at[c, i]) for i in range(NB)]

        def start(copies):
            for cp in copies:
                cp.start()

        def wait(copies):
            for cp in copies:
                cp.wait()

        def prep_tiles(sch, load, put, nrows, ncols):
            def tile(_, pos):
                s, k = pos
                words = {}
                for r, (_, v, _) in enumerate(sch.prods):
                    for key in v:
                        if key not in words or sch.n > 4:
                            words[key] = pltpu.bitcast(
                                load(*key, pl.multiple_of(s * 16, 16), k), U32)
                    if len(v) == 1:
                        put(r, s * 8, k, words[next(iter(v))])
                    else:
                        halves = {key: _halves(words[key]) for key in v}
                        put(r, s * 8, k, _pair(*(
                            _combine(v, {key: hv[p] for key, hv in halves.items()})
                            for p in range(2))))
                wrap = k + 1 == ncols
                return jnp.where(wrap, s + 1, s), jnp.where(wrap, 0, k + 1)
            lax.fori_loop(0, nrows // 16 * ncols, tile, (0, 0))

        def lanes_at(k):
            return pl.ds(pl.multiple_of(k * LANES, LANES), LANES)

        def words_at(row):
            return pl.ds(pl.multiple_of(row, 8), 8)

        def prep_qkv(w, c, slot):
            def heads(i, carry):
                st = qst_v.at[slot, i].bitcast(U32)
                for jp in range(H // 2):
                    for k, x in enumerate(_halves(st[pl.ds(jp, QR, stride=H // 2), :])):
                        qtr_v[i, 2 * jp + k] = x.astype(BF16)
                return carry
            lax.fori_loop(0, NA, heads, 0)

            def put(r, row, k, val):
                wqkv_v[w, k, r, words_at(c * (QR // 2) + row), :] = val
            prep_tiles(SA, lambda i, j, row, k: qtr_v[i, j * HB + k, pl.ds(row, 16), :], put, QR, HB)

        def prep_from_big(sch, dst, base, blk, c, nrows):
            ncols = D // sch.n // LANES

            def load(i, j, row, k):
                return big_v[rows_at(base + i * blk + row, 16), lanes_at(j * ncols + k)]

            def put(r, row, k, val):
                dst[k, r, words_at(c * (nrows // 2) + row), :] = val
            prep_tiles(sch, load, put, nrows, ncols)

        def prep_gu(w, c):
            def load(i, j, row, k):
                return gst_v[c, i, pl.ds(row, 16), lanes_at(j * (FB // LANES) + k)]

            def put(r, row, k, val):
                wgu_v[k, r, words_at(c * (GR // 2) + row), w * LANES:(w + 1) * LANES] = val
            prep_tiles(SB, load, put, GR, FB // LANES)

        x_head = pltpu.make_async_copy(x_hbm.at[0:XH, :], x_v.at[0:XH, :], sem_x.at[0])
        x_tail = pltpu.make_async_copy(x_hbm.at[XH:, :], x_v.at[XH:, :], sem_x.at[1])
        NQ, NO = DA // QR, EB // WR
        ONEXT = min(QST, OST)
        for n in range(QST):
            start(q_copies(0, n, n))
        x_head.start()

        ri = lax.broadcasted_iota(jnp.int32, (2 * L, LANES), 0)
        ci = lax.broadcasted_iota(jnp.int32, (2 * L, LANES), 1)
        first = jnp.where(ri < L, 0, L)
        same = (ci >= first) & (ci < first + L)
        visible = (ri < first + M) | (ri >= ci)
        keep_v[...] = (same & visible).astype(jnp.int32)
        fill_v[...] = jnp.where(same, -1e9 / scale, -jnp.inf).astype(F32)
        kv_v[...] = jnp.zeros(kv_v.shape, BF16)
        mem_v[0:M, :] = mem0_ref[...].astype(F32)
        mem_v[M:, :] = mem0_ref[...].astype(F32)

        for w in range(3):
            def q_body(c, carry, w=w):
                slot = (w * NQ + c) % QST
                wait(q_copies(w, c, slot))
                prep_qkv(w, c, slot)
                pl.when(c + QST < NQ)(lambda: start(q_copies(w, c + QST, slot)))
                if w < 2:
                    pl.when(c + QST >= NQ)(lambda: start(q_copies(w + 1, c + QST - NQ, slot)))
                else:
                    pl.when((c + QST >= NQ) & (c + QST - NQ < ONEXT))(
                        lambda: start(o_copies(c + QST - NQ)))
                return carry
            lax.fori_loop(0, NQ, q_body, 0)

        def o_body(c, carry):
            wait(o_copies(c))
            prep_from_big(SA, wo_v, (c % OST) * NA * WR, WR, c, WR)
            pl.when(c + ONEXT < NO)(lambda: start(o_copies(c + ONEXT)))
            pl.when(c >= NO - GST)(lambda: start(g_copies(wg_hbm, c - (NO - GST))))
            return carry
        lax.fori_loop(0, NO, o_body, 0)
        for c in range(GST):
            start(d_copies(c))
        x_head.wait()
        xa_v[...] = x_v[0:XH, :].astype(F32)

        def load_glu_weights():
            def gate(c, carry):
                wait(g_copies(wg_hbm, c))
                prep_gu(0, c)
                start(g_copies(wu_hbm, c))
                return carry

            def down(c, carry):
                wait(d_copies(c))
                prep_from_big(SB, wd_v, c * DR, FB, c, DR)
                return carry

            def up(c, carry):
                wait(g_copies(wu_hbm, c))
                prep_gu(1, c)
                return carry
            lax.fori_loop(0, GST, gate, 0)
            lax.fori_loop(0, GST, down, 0)
            lax.fori_loop(0, GST, up, 0)
            x_tail.start()

        def attention(c, qkv, paired):
            probs = {}

            def scores():
                for j in range(NA):
                    x = [jnp.concatenate([p[0, j], p[1, j]], axis=0) if paired else p[j]
                         for p in qkv]
                    n = x[0].shape[0]
                    for w in range(2):
                        kv_v[j, w, 0:n, :] = x[w + 1].astype(BF16)
                    s = _dot_nt(x[0], kv_v[j, 0])
                    s = jnp.where(keep_v[0:n, :] != 0, s, fill_v[0:n, :])
                    mx = jnp.max(s, axis=-1, keepdims=True)
                    e = jnp.exp2((s - mx) * c_exp)
                    den = jnp.sum(e, axis=-1, keepdims=True)
                    inv = pl.reciprocal(den, approx=True)
                    inv = inv * (2.0 - den * inv)
                    probs[j] = e * inv

            def values():
                o = {j: _dot(probs[j], kv_v[j, 1]) for j in range(NA)}
                if paired:
                    o = {(hf, j): o[j][hf * L:(hf + 1) * L] for hf in range(2) for j in range(NA)}
                store_lhs(SA, lo_v, c, o, paired)

            return scores, values

        def project_qkv(w, c, paired, hooks):
            return fast_dot(SA, la_v, lambda r: wqkv_v[w, c, r], paired, hooks,
                            na_v if w + c == 0 else None)

        def glu_input():
            nb_v[...] = _layernorm(ya_v[0:2 * SEG, :], 0.5)

        def gate_up(c):
            gu = fast_dot(SB, lb_v, lambda r: wgu_v[c, r], True, None, nb_v if c == 0 else None)
            act = {k: jnp.tanh(v[:, :LANES]) * v[:, LANES:] + v[:, LANES:] for k, v in gu.items()}
            store_lhs(SB, ld_v, c, act, True)

        def down(c, hooks=None):
            for (hf, j), v in fast_dot(SB, ld_v, lambda r: wd_v[c, r], True, hooks).items():
                rows = slice(hf * SEG, (hf + 1) * SEG)
                z_v[rows, tile_of(j, DB, c)] = ya_v[rows, tile_of(j, DB, c)] + v

        def out_copy(row, n):
            return pltpu.make_async_copy(big_v.at[pl.ds(row, n), :],
                                         out_hbm.at[pl.ds(row, n), :], sem_out)

        def attention_single(mrow, xrow, yrow):
            na_v[0:M, :] = mem_v[pl.ds(mrow, M), :]
            na_v[M:L, :] = _layernorm(xa_v[pl.ds(xrow, SEG), :])
            hooks = {}
            for c in range(HB):
                qkv = [project_qkv(w, c, False, hooks.get(w)) for w in range(3)]
                scores, values = attention(c, qkv, False)
                hooks = {0: {PA // 3: scores}, 2: {0: values}}
            scores()
            values()
            for c in range(DA // LANES):
                for j, v in fast_dot(SA, lo_v, lambda r: wo_v[c, r], False).items():
                    mem_v[pl.ds(mrow, M), tile_of(j, DA, c)] = v[:M]
                    ya_v[pl.ds(yrow, SEG), tile_of(j, DA, c)] = (
                        xa_v[pl.ds(xrow, SEG), tile_of(j, DA, c)] + v[M:])

        def step(t, carry):
            cur = pl.multiple_of(t * SEG, SEG)
            nxt = pl.multiple_of(jnp.minimum(t + 1, NSEG - 1) * SEG, SEG)
            row = pl.multiple_of(jnp.maximum(t - 3, 0) * SEG, SEG)
            hooks = {0: {cfg.get("g0", 2): glu_input}}
            gpos = cfg.get("gpos", [1, 2, 4, 5, 7, 8, 10] if NA == 8 else [2, 5, 8, 11, 14, 17, 20])
            for c in range(HB):
                qkv = []
                for w in range(3):
                    qkv.append(project_qkv(w, c, True, hooks.get(w)))
                    if 3 * c + w in gpos:
                        gate_up(gpos.index(3 * c + w))
                scores, values = attention(c, qkv, True)
                hooks = {cfg.get("sw", 0): {cfg.get("h0", 15): scores},
                         cfg.get("vw", 1): {cfg.get("h1", 15): values}}
            down(0, {cfg.get("d0", 0): scores})
            down(1, {cfg.get("d1", 4): values})
            big_v[pl.ds(row, SEG), :] = z_v[SEG:, :].astype(BF16)

            def next_input():
                na_v[M:L, :] = _layernorm(x_v[pl.ds(nxt, SEG), :].astype(F32))
                na_v[L + M:, :] = _layernorm(z_v[:SEG, :])

            for c in range(DA // LANES):
                o = fast_dot(SA, lo_v, lambda r: wo_v[c, r], True,
                             {cfg.get("h2", 2): next_input} if c == 0 else None)
                for (hf, j), v in o.items():
                    cols = tile_of(j, DA, c)
                    res = x_v[pl.ds(cur, SEG), cols].astype(F32) if hf == 0 else xa_v[SEG:, cols]
                    na_v[hf * L:hf * L + M, cols] = v[:M]
                    ya_v[hf * SEG:(hf + 1) * SEG, cols] = res + v[M:]
            xa_v[SEG:, :] = z_v[:SEG, :]
            pl.when(t >= 3)(lambda: out_copy(row, SEG).start())
            return carry

        def phase(ph, carry):
            attention_single(pl.multiple_of(jnp.where(ph < 2, 0, M), M),
                             pl.multiple_of(jnp.where(ph == 0, 0, SEG), SEG),
                             pl.multiple_of(jnp.where(ph == 3, 1, ph) * SEG, SEG))
            pl.when(ph == 1)(load_glu_weights)

            @pl.when(ph >= 1)
            def _():
                glu_input()
                for c in range(FB // LANES):
                    gate_up(c)
                for c in range(DB // LANES):
                    down(c)

            @pl.when(ph == 1)
            def _():
                x_tail.wait()
                ya_v[0:SEG, :] = ya_v[SEG:2 * SEG, :]
                xa_v[SEG:, :] = z_v[:SEG, :]
                na_v[0:M, :] = mem_v[0:M, :]
                na_v[M:L, :] = _layernorm(x_v[2 * SEG:3 * SEG, :].astype(F32))
                na_v[L:L + M, :] = mem_v[M:, :]
                na_v[L + M:, :] = _layernorm(z_v[:SEG, :])
                lax.fori_loop(2, cfg.get("nsteps", NSEG), step, 0, unroll=cfg.get("un", 1))
                mem_v[M:, :] = na_v[L:L + M, :]

            @pl.when(ph == 2)
            def _():
                xa_v[SEG:, :] = z_v[:SEG, :]
                ya_v[0:SEG, :] = ya_v[2 * SEG:, :]
                big_v[S - 3 * SEG:S - 2 * SEG, :] = z_v[SEG:, :].astype(BF16)
                out_copy(S - 3 * SEG, SEG).start()

            @pl.when(ph == 3)
            def _():
                big_v[S - 2 * SEG:S, :] = z_v[...].astype(BF16)
                out_copy(S - 2 * SEG, 2 * SEG).start()
            return carry

        lax.fori_loop(0, cfg.get('nph', 4), phase, 0)
        out_copy(0, cfg.get("nsteps", NSEG) * SEG).wait()

    scratch = [
        pltpu.VMEM((S, D), BF16),
        pltpu.VMEM((FF, D), BF16),
        pltpu.VMEM((GST, NB, GR, FF), BF16),
        pltpu.VMEM((QST, NA, (QR + 1) * H, DH), BF16),
        pltpu.VMEM((NA, H, QR, DH), BF16),
        pltpu.VMEM((3, HB, PA, DA // 2, DH), U32),
        pltpu.VMEM((DA // LANES, PA, EB // 2, LANES), U32),
        pltpu.VMEM((FB // LANES, PB, DB // 2, 2 * LANES), U32),
        pltpu.VMEM((DB // LANES, PB, FB // 2, LANES), U32),
        pltpu.VMEM((PA, DA // LANES, L, LANES), F32),
        pltpu.VMEM((PA, EB // LANES, L, LANES), F32),
        pltpu.VMEM((PB, DB // LANES, SEG, LANES), F32),
        pltpu.VMEM((PB, FB // LANES, SEG, LANES), F32),
        pltpu.VMEM((2 * M, D), F32),
        pltpu.VMEM((2 * SEG, D), F32),
        pltpu.VMEM((2 * L, D), F32),
        pltpu.VMEM((2 * SEG, D), F32),
        pltpu.VMEM((3 * SEG, D), F32),
        pltpu.VMEM((2 * SEG, D), F32),
        pltpu.VMEM((NA, 2, LANES, DH), BF16),
        pltpu.VMEM((2 * L, LANES), F32),
        pltpu.VMEM((2 * L, LANES), jnp.int32),
        pltpu.SemaphoreType.DMA((2,)),
        pltpu.SemaphoreType.DMA((QST, NA)),
        pltpu.SemaphoreType.DMA((OST, NA)),
        pltpu.SemaphoreType.DMA((GST, NB)),
        pltpu.SemaphoreType.DMA((GST, NB)),
        pltpu.SemaphoreType.DMA(()),
    ]
    return kernel, scratch


def _build(cfg):
    @functools.partial(jax.jit, static_argnames=("A_seg_len",))
    def fn(A_x, A_mem0, A_Wq, A_Wk, A_Wv, A_Wo, A_seg_len, B_x, B_w_gate, B_w_up, B_w_down):
        B, S, D = A_x.shape
        _, H, DH = A_Wq.shape
        M = A_mem0.shape[1]
        FF = B_w_gate.shape[1]
        kernel, scratch = _make_kernel(S, D, H, DH, M, A_seg_len, FF, cfg)
        any_spec = pl.BlockSpec(memory_space=pl.ANY)
        out = pl.pallas_call(
            kernel,
            out_shape=jax.ShapeDtypeStruct((S, D), A_x.dtype),
            in_specs=[any_spec, pl.BlockSpec(memory_space=pltpu.VMEM)] + [any_spec] * 7,
            out_specs=any_spec,
            scratch_shapes=scratch,
            compiler_params=pltpu.CompilerParams(vmem_limit_bytes=cfg.get("vmem", 126) * 1024 * 1024,
                                                 flags=cfg.get("flags")),
        )(A_x.reshape(S, D), A_mem0.reshape(M, D),
          A_Wq.reshape(D * H, DH), A_Wk.reshape(D * H, DH), A_Wv.reshape(D * H, DH),
          A_Wo.reshape(H * DH, D), B_w_gate, B_w_up, B_w_down)
        return out.reshape(B, S, D)
    return fn


pallas_interleave_layers__memory_aug_recurrent_mem_tr__glu_gated_glu__prompt_kernel = _build({})
```

```python
import functools
import math

import jax
import jax.numpy as jnp
import numpy as np
from jax import lax
import jax.experimental.pallas as pl
import jax.experimental.pallas.tpu as pltpu

F32 = jnp.float32
BF16 = jnp.bfloat16
U32 = jnp.uint32
EPS = 1e-05
LANES = 128

_SCHEME_4 = """
+00 | +00 +02 -10 +30 | +00 -10
+00 +10 | +00 -01 +20 -30 | +10

+00 -11 | +01 -10 +30 | +01 +10
+10 +11 | +01 | +10 +11
+00 +01 | +03 +10 -30 | +00 +01

+00 +10 +11 +13 | +30 | -00 -01 +03 +10
+00 +01 +03 +10 +11 +13 | -03 +30 | +00 +01 -03
+03 +10 +11 +13 | +03 | +00 +01 -03 +13

+00 +10 -12 | +02 -20 | -00 +02 +10
+10 -12 | +02 | +00 -02 -10 +12
+00 -02 +10 -12 | +20 | -00 +02

+11 | +01 -11 -12 +31 | +01 -11
+01 +11 | -03 -10 +11 +13 -21 +30 | +01

-03 +11 | -03 +13 +31 | -01 +13
+01 +03 | -03 +13 +30 | -01 +03
+11 +13 | +31 | +11 -13

+01 +02 +11 | +12 +21 | +01 -11 +12
+01 +02 | +12 | -01 +02 +11 -12
+01 +02 +11 +12 | +21 | +11 -12

+03 +12 +13 | -23 -32 | -02 +03 -13
+02 +03 +12 +13 | +23 | -02 +03
+12 +13 | +32 | -02 +03 +12 -13

+02 | -12 +20 +22 +23 | +02
+12 | +02 +21 +22 -32 | +12

+03 | +03 -13 +32 +33 | +03 -13
+03 +13 | -03 -23 +31 +33 | +13
"""
_SCHEME_8 = """
+01 +10 | +01 +10 | +00 +11
+00 -01 | +01 | +00 +01
+10 -11 | +10 | -10 -11

+00 +02 +10 | +02 +20 | +00 -10 +12
+00 +02 | +02 | -00 +02 +10 -12
+00 +02 +10 +12 | +20 | +10 -12

+00 +03 -04 +10 | +30 | +00 -10 -13 -14
+00 +03 -04 +10 +13 -14 | +03 +30 | +10 +13 +14
+00 +03 -04 +13 | +03 | +03 -10 -13 -14

+04 +10 | +04 +30 +40 -74 | +00 +14
+00 -04 | +04 -47 -74 | +00 +04
+10 -14 | -03 -30 -40 | +10 +14

+00 -05 +10 | +05 +50 | -00 +10 +15
+00 -05 | +05 | +00 +05 -10 -15
+00 -05 +10 -15 | +50 | -10 -15

+00 +06 +07 +10 | +60 | +00 -10 -16 +17
+00 +06 +07 +10 +16 +17 | +06 +60 | +10 +16 -17
+00 +06 +07 +16 | +06 | +06 -10 -16 +17

-07 +10 | +07 +47 -60 +70 | -00 +17
+00 +07 | +07 +47 +74 | -00 +07
+10 +17 | +06 +60 -70 | -10 +17

+10 | -00 -02 +05 -10 -30 -40 -60 +70 | +00 -10
+00 +10 | +00 -01 -04 +07 -20 -30 +47 +50 -60 +74 | +00

+01 +11 -12 | +12 +21 | +01 +02 -11
+11 -12 | +12 | -01 -02 +11 +12
+01 -02 +11 -12 | +21 | -01 -02

+01 +13 | +13 +31 +63 -71 | +03 +11
+11 -13 | +13 -36 +63 | +11 +13
+01 -03 | -17 -31 +71 | +01 +03

+01 +11 +14 -16 | +41 | -01 +04 +06 +11
+01 +04 -06 +11 +14 -16 | -14 +41 | +01 -04 -06
+04 +11 +14 -16 | +14 | +01 -04 -06 +14

+01 +11 +15 | +15 -51 | +01 +05 -11
+11 +15 | +15 | -01 -05 +11 +15
+01 +05 +11 +15 | +51 | +01 +05

+01 +16 | +16 +36 -41 -61 | +06 -11
+11 -16 | +16 +36 -63 | -11 +16
+01 -06 | -14 +41 +61 | -01 +06

+01 +11 -13 -17 | +71 | +01 +03 +07 -11
+01 -03 -07 +11 -13 -17 | +17 -71 | +01 +03 +07
-07 +11 -13 -17 | +17 | -01 -03 -07 +17

+01 | +01 +11 -12 -15 +31 +41 +61 -71 | +01 -11
+01 +11 | -10 +11 -13 +16 +21 +36 -41 -51 -63 +71 | +11

+02 +03 +13 | +23 -32 -52 | +03 -12 -13
+02 +03 +12 +13 | +23 | +12 +13
+02 +03 | +25 +32 +52 | +02 +03 -12 -13

-04 +12 -14 | -24 -42 | +02 +04 -14
+02 -04 +12 -14 | +24 | +02 +04
+12 -14 | +42 | +02 +04 -12 -14

+03 -05 +12 +13 -15 | +52 | -02 -03 +05 +13 -15
+12 +13 -15 | +25 +52 | +02 +03 -05 -12 -13 +15
+02 +03 +12 +13 -15 | +25 | -02 -03 +05 +12 +13

+02 +06 +16 | +26 -62 | +06 -12 -16
+02 +06 +12 +16 | +26 | +12 +16
+02 +06 | +62 | +02 +06 -12 -16

+07 +12 +17 | -27 -72 | -02 +07 -17
+02 +07 +12 +17 | +27 | -02 +07
+12 +17 | +72 | -02 +07 +12 -17

+02 | -02 -21 +22 -24 +27 -32 -52 -62 | +02
+12 | +12 +20 +22 -23 -26 +42 +52 -72 | +12

+04 +13 | +03 +34 +43 | +03 +14
+03 -04 | +34 | +03 +04
+13 -14 | -03 -30 -43 | +13 +14

+03 -05 +13 | -25 +35 -53 | +03 -13 +15
+03 -05 | -25 +35 -52 | -03 +05 +13 -15
+03 -05 +13 -15 | +53 | -13 +15

-01 +03 +06 +13 | +63 | +03 -11 -13 +16
-01 +03 +06 -11 +13 +16 | -36 +63 | +11 +13 -16
-01 +03 +06 +16 | +36 | +06 +11 +13 -16

-07 +13 | +17 +37 -73 | +03 +17
+03 +07 | +17 +37 -71 | +03 +07
+13 +17 | +73 | +13 +17

+13 | -03 -13 +25 +32 -33 -35 -43 +52 -63 +73 | +03 -13
+03 +13 | -03 -17 -23 -31 +33 -34 -37 +53 -63 +71 | +03

+04 +14 +15 | +45 -54 | +04 +05 -14
+14 +15 | +45 | -04 -05 +14 +15
+04 +05 +14 +15 | +54 | +04 +05

+04 +16 | +14 +46 +64 | +06 +14
+14 -16 | +46 | +14 +16
+04 -06 | -14 +41 -64 | +04 +06

+04 -10 +14 -17 | +74 | +00 +04 -07 -14
-00 +04 -07 -10 +14 -17 | -47 -74 | +00 +04 -07
-07 -10 +14 -17 | +47 | +00 +04 -07 +17

+04 | +04 +14 +34 -42 +44 -45 +64 -74 | +04 -14
+04 +14 | -03 -14 +24 -30 -40 -43 +44 -46 -54 +74 | +14

+05 +06 +16 | +56 -65 | +06 -15 -16
+05 +06 +15 +16 | +56 | +15 +16
+05 +06 | +65 | +05 +06 -15 -16

+07 +15 +17 | -57 -75 | -05 +07 -17
+05 +07 +15 +17 | +57 | -05 +07
+15 +17 | +75 | -05 +07 +15 -17

+05 | +05 -25 +35 -51 -54 +55 +57 -65 | +05
+15 | -15 +25 -45 -50 +53 +55 -56 -75 | +15

-07 +16 | -06 +67 +76 | -06 +17
+06 +07 | +67 | -06 +07
+16 +17 | +06 +60 -76 | -16 +17

+16 | -06 -16 -36 -46 +62 +65 -66 +76 | +06 -16
+06 +16 | -06 -14 -26 -36 +41 -56 +61 -64 +66 +67 | +06

+07 | -07 -17 -37 -47 -67 +72 +75 +77 | +07 -17
+07 +17 | -06 +17 -27 +47 -57 -60 +70 -73 +76 +77 | +17
"""


class _Scheme:
    def __init__(self, n, text):
        def terms(field):
            return {(int(t[1]), int(t[2])): 1 if t[0] == "+" else -1 for t in field.split()}

        def fold(coefs, weights):
            out = {}
            for (h, i), c in coefs.items():
                out[i] = out.get(i, 0) + weights[h] * c
            return {i: c for i, c in out.items() if c}

        self.n = n
        self.prods, self.ends = [], []
        for group in text.strip().split("\n\n"):
            self.prods += [tuple(terms(f) for f in line.split("|")) for line in group.split("\n")]
            self.ends.append(len(self.prods) - 1)
        folded = [(fold(u, (-1, 1)), fold(w, (0, 1))) for u, _, w in self.prods]
        self.single = [(u, w) if u and w else None for u, w in folded]


def _combine(coefs, vals):
    acc = None
    for key, c in sorted(coefs.items(), key=lambda kv: -kv[1]):
        v = vals[key]
        if abs(c) != 1:
            v = v * abs(c)
        if acc is None:
            acc = v if c > 0 else -v
        else:
            acc = acc + v if c > 0 else acc - v
    return acc


def _accumulate(accs, group):
    terms = {}
    for n, (coefs, _) in enumerate(group):
        for key, c in coefs.items():
            terms.setdefault(key, []).append((n, c))
    sums = {((n, 1),): v for n, (_, v) in enumerate(group)}
    for key, tm in sorted(terms.items(), key=lambda kv: len(kv[1])):
        sign = tm[0][1]
        tm = tuple((n, c * sign) for n, c in tm)
        if tm not in sums:
            base = max((s for s in sums if all(t in tm for t in s)), key=len)
            val = sums[base]
            for n, c in tm:
                if (n, c) not in base:
                    val = val + group[n][1] if c > 0 else val - group[n][1]
            sums[tm] = val
        if key not in accs:
            accs[key] = sums[tm] if sign > 0 else -sums[tm]
        else:
            accs[key] = accs[key] + sums[tm] if sign > 0 else accs[key] - sums[tm]


def _layernorm(x, gain=1.0):
    m = jnp.mean(x, axis=-1, keepdims=True)
    c = x - m
    v = jnp.mean(c * c, axis=-1, keepdims=True)
    inv = lax.rsqrt(v + EPS)
    return c * (inv if gain == 1.0 else inv * gain)


def _dot(a, b):
    return lax.dot_general(a, b, (((1,), (0,)), ((), ())), preferred_element_type=F32)


def _dot_nt(a, b):
    return lax.dot_general(a, b, (((1,), (1,)), ((), ())), preferred_element_type=F32)


def _halves(x):
    return [pltpu.unpack_elementwise(x, index=k, packed_dtype=BF16, unpacked_dtype=F32)
            for k in range(2)]


def _pair(lo, hi):
    return pltpu.pack_elementwise([lo, hi], packed_dtype=BF16)


def _make_kernel(S, D, H, DH, M, SEG, FF, cfg):
    SA = _Scheme(8, _SCHEME_8) if cfg.get("na", 8) == 8 else _Scheme(4, _SCHEME_4)
    SB = _Scheme(4, _SCHEME_4)
    NA, NB = SA.n, SB.n
    PA, PB = len(SA.prods), len(SB.prods)
    NSEG = S // SEG
    L = M + SEG
    DA, HB = D // NA, H // NA
    EB = HB * DH
    DB, FB = D // NB, FF // NB
    QR = cfg.get("QR", 128) // NA
    QST = cfg.get("QST", 4)
    WR = 512 // NA
    OST = FF // (WR * NA)
    GST = 4
    GR, DR = DB // GST, FB // GST
    XH = 2 * SEG
    scale = DH ** (-0.5)
    c_exp = scale * math.log2(math.e)

    def fast_dot(sch, paired, w_of, block, kept_ref=None, fresh=True, hooks=None, sums=False):
        acc, group = {}, []
        for r, (u, _, w) in enumerate(sch.prods):
            if hooks and r in hooks:
                hooks[r]()
            if paired or sch.single[r]:
                if not paired:
                    u, w = sch.single[r]
                if fresh:
                    if not paired:
                        u = {(0, i): c for i, c in u.items()}
                    elif sums:
                        u = {(2 if u.get((1 - hf, i)) == c else hf, i): c
                             for (hf, i), c in u.items()}
                    lhs = _combine(u, {key: block(*key) for key in u})
                    if kept_ref is not None:
                        kept_ref[r] = lhs
                else:
                    lhs = kept_ref[r]
                group.append((w, _dot(lhs, pltpu.bitcast(w_of(r), BF16))))
            if r in sch.ends:
                _accumulate(acc, group)
                group = []
        return acc

    def blocks_of(ref, rows, cols):
        return lambda hf, i: ref[hf * rows:(hf + 1) * rows, i * cols:(i + 1) * cols]

    def spread(pieces, first, stride):
        return {first + n * stride: piece for n, piece in enumerate(pieces)}

    def tile_of(j, blk, c):
        return slice(j * blk + c * LANES, j * blk + (c + 1) * LANES)

    def kernel(x_hbm, mem0_ref, wq_hbm, wk_hbm, wv_hbm, wo_hbm, wg_hbm, wu_hbm, wd_hbm,
               out_hbm,
               x_v, big_v, gst_v, qst_v, qtr_v, wqkv_v, wo_v, wgu_v, wd_v,
               la_v, lb_v, o_v, act_v, mem_v, ma_v, xa_v, na_v, nb_v, ya_v, z_v, q_v, kv_v, fill_v, keep_v,
               sem_x, sem_q, sem_o, sem_g, sem_d, sem_out):

        def rows_at(start, size):
            return pl.ds(start if isinstance(start, int) else pl.multiple_of(start, 16), size)

        def q_copies(w, c, slot):
            src = (wq_hbm, wk_hbm, wv_hbm)[w]
            return [pltpu.make_async_copy(src.at[rows_at((i * DA + c * QR) * H, QR * H), :],
                                          qst_v.at[slot, i, 0:QR * H, :], sem_q.at[slot, i])
                    for i in range(NA)]

        def o_copies(c):
            slot = c % OST
            return [pltpu.make_async_copy(wo_hbm.at[rows_at(i * EB + c * WR, WR), :],
                                          big_v.at[rows_at((slot * NA + i) * WR, WR), :],
                                          sem_o.at[slot, i]) for i in range(NA)]

        def g_copies(src, c):
            return [pltpu.make_async_copy(src.at[rows_at(i * DB + c * GR, GR), :],
                                          gst_v.at[c, i], sem_g.at[c, i]) for i in range(NB)]

        def d_copies(c):
            return [pltpu.make_async_copy(wd_hbm.at[rows_at(i * FB + c * DR, DR), :],
                                          big_v.at[rows_at(i * FB + c * DR, DR), :],
                                          sem_d.at[c, i]) for i in range(NB)]

        def start(copies):
            for cp in copies:
                cp.start()

        def wait(copies):
            for cp in copies:
                cp.wait()

        def prep_tiles(sch, load, put, nrows, ncols):
            def tile(_, pos):
                s, k = pos
                words = {}
                for r, (_, v, _) in enumerate(sch.prods):
                    for key in v:
                        if key not in words or sch.n > 4:
                            words[key] = pltpu.bitcast(
                                load(*key, pl.multiple_of(s * 16, 16), k), U32)
                    if len(v) == 1:
                        put(r, s * 8, k, words[next(iter(v))])
                    else:
                        halves = {key: _halves(words[key]) for key in v}
                        put(r, s * 8, k, _pair(*(
                            _combine(v, {key: hv[p] for key, hv in halves.items()})
                            for p in range(2))))
                wrap = k + 1 == ncols
                return jnp.where(wrap, s + 1, s), jnp.where(wrap, 0, k + 1)
            lax.fori_loop(0, nrows // 16 * ncols, tile, (0, 0))

        def lanes_at(k):
            return pl.ds(pl.multiple_of(k * LANES, LANES), LANES)

        def words_at(row):
            return pl.ds(pl.multiple_of(row, 8), 8)

        def prep_qkv(w, c, slot):
            def heads(i, carry):
                st = qst_v.at[slot, i].bitcast(U32)
                for jp in range(H // 2):
                    for k, x in enumerate(_halves(st[pl.ds(jp, QR, stride=H // 2), :])):
                        qtr_v[i, 2 * jp + k] = x.astype(BF16)
                return carry
            lax.fori_loop(0, NA, heads, 0)

            def put(r, row, k, val):
                wqkv_v[w, k, r, words_at(c * (QR // 2) + row), :] = val
            prep_tiles(SA, lambda i, j, row, k: qtr_v[i, j * HB + k, pl.ds(row, 16), :], put, QR, HB)

        def prep_from_big(sch, dst, base, blk, c, nrows):
            ncols = D // sch.n // LANES

            def load(i, j, row, k):
                return big_v[rows_at(base + i * blk + row, 16), lanes_at(j * ncols + k)]

            def put(r, row, k, val):
                dst[k, r, words_at(c * (nrows // 2) + row), :] = val
            prep_tiles(sch, load, put, nrows, ncols)

        def prep_gu(w, c):
            def load(i, j, row, k):
                return gst_v[c, i, pl.ds(row, 16), lanes_at(j * (FB // LANES) + k)]

            def put(r, row, k, val):
                wgu_v[k, r, words_at(c * (GR // 2) + row), w * LANES:(w + 1) * LANES] = val
            prep_tiles(SB, load, put, GR, FB // LANES)

        x_head = pltpu.make_async_copy(x_hbm.at[0:XH, :], x_v.at[0:XH, :], sem_x.at[0])
        x_tail = pltpu.make_async_copy(x_hbm.at[XH:, :], x_v.at[XH:, :], sem_x.at[1])
        NQ, NO = DA // QR, EB // WR
        ONEXT = min(QST, OST)
        for n in range(QST):
            start(q_copies(0, n, n))
        x_head.start()

        ri = lax.broadcasted_iota(jnp.int32, (2 * L, LANES), 0)
        ci = lax.broadcasted_iota(jnp.int32, (2 * L, LANES), 1)
        first = jnp.where(ri < L, 0, L)
        same = (ci >= first) & (ci < first + L)
        visible = (ri < first + M) | (ri >= ci)
        keep_v[...] = (same & visible).astype(jnp.int32)
        fill_v[...] = jnp.where(same, -1e9 / scale, -jnp.inf).astype(F32)
        kv_v[...] = jnp.zeros(kv_v.shape, BF16)
        mem_v[0:M, :] = mem0_ref[...].astype(F32)
        mem_v[M:, :] = mem0_ref[...].astype(F32)

        for w in range(3):
            def q_body(c, carry, w=w):
                slot = (w * NQ + c) % QST
                wait(q_copies(w, c, slot))
                prep_qkv(w, c, slot)
                pl.when(c + QST < NQ)(lambda: start(q_copies(w, c + QST, slot)))
                if w < 2:
                    pl.when(c + QST >= NQ)(lambda: start(q_copies(w + 1, c + QST - NQ, slot)))
                else:
                    pl.when((c + QST >= NQ) & (c + QST - NQ < ONEXT))(
                        lambda: start(o_copies(c + QST - NQ)))
                return carry
            lax.fori_loop(0, NQ, q_body, 0)

        def o_body(c, carry):
            wait(o_copies(c))
            prep_from_big(SA, wo_v, (c % OST) * NA * WR, WR, c, WR)
            pl.when(c + ONEXT < NO)(lambda: start(o_copies(c + ONEXT)))
            pl.when(c >= NO - GST)(lambda: start(g_copies(wg_hbm, c - (NO - GST))))
            return carry
        lax.fori_loop(0, NO, o_body, 0)
        for c in range(GST):
            start(d_copies(c))
        x_head.wait()
        xa_v[...] = x_v[0:XH, :].astype(F32)

        def load_glu_weights():
            def gate(c, carry):
                wait(g_copies(wg_hbm, c))
                prep_gu(0, c)
                start(g_copies(wu_hbm, c))
                return carry

            def down(c, carry):
                wait(d_copies(c))
                prep_from_big(SB, wd_v, c * DR, FB, c, DR)
                return carry

            def up(c, carry):
                wait(g_copies(wu_hbm, c))
                prep_gu(1, c)
                return carry
            lax.fori_loop(0, GST, gate, 0)
            lax.fori_loop(0, GST, down, 0)
            lax.fori_loop(0, GST, up, 0)
            x_tail.start()

        def attention(c, paired):
            n = 2 * L if paired else L
            probs = {}

            def scores(j):
                s = _dot_nt(q_v[j, 0:n, :], kv_v[0, j])
                s = jnp.where(keep_v[0:n, :] != 0, s, fill_v[0:n, :])
                mx = jnp.max(s, axis=-1, keepdims=True)
                e = jnp.exp2((s - mx) * c_exp)
                den = jnp.sum(e, axis=-1, keepdims=True)
                inv = pl.reciprocal(den, approx=True)
                inv = inv * (2.0 - den * inv)
                probs[j] = e * inv

            def values(j):
                o = _dot(probs[j], kv_v[1, j])
                o_v[0:n, tile_of(j, EB, c)] = o
                if paired:
                    o_v[n:, tile_of(j, EB, c)] = o[:L] + o[L:]

            return ([functools.partial(scores, j) for j in range(NA)],
                    [functools.partial(values, j) for j in range(NA)])

        def project_qkv(w, c, paired, hooks):
            def block(hf, i):
                cols = slice(i * DA, (i + 1) * DA)
                return jnp.concatenate([ma_v[hf * M:(hf + 1) * M, cols],
                                        na_v[hf * SEG:(hf + 1) * SEG, cols]], axis=0)

            p = fast_dot(SA, paired, lambda r: wqkv_v[w, c, r], block, la_v, w + c == 0, hooks)
            for j in range(NA):
                x = jnp.concatenate([p[0, j], p[1, j]], axis=0) if paired else p[j]
                if w == 0:
                    q_v[j, 0:x.shape[0], :] = x
                else:
                    kv_v[w - 1, j, 0:x.shape[0], :] = x.astype(BF16)

        def project_out(c, paired, hooks=None):
            return fast_dot(SA, paired, lambda r: wo_v[c, r], blocks_of(o_v, L, EB),
                            hooks=hooks, sums=True)

        def glu_input():
            nb_v[...] = _layernorm(ya_v[0:2 * SEG, :], 0.5)

        def gate_up(c, hooks=None):
            gu = fast_dot(SB, True, lambda r: wgu_v[c, r], blocks_of(nb_v, SEG, DB), lb_v, c == 0,
                          hooks)
            for j in range(NB):
                act = [jnp.tanh(v[:, :LANES]) * v[:, LANES:] + v[:, LANES:]
                       for v in (gu[0, j], gu[1, j])]
                act_v[:, tile_of(j, FB, c)] = jnp.concatenate(act + [act[0] + act[1]], axis=0)

        def down(c, hooks=None):
            dn = fast_dot(SB, True, lambda r: wd_v[c, r], blocks_of(act_v, SEG, FB),
                          hooks=hooks, sums=True)
            for (hf, j), v in dn.items():
                rows = slice(hf * SEG, (hf + 1) * SEG)
                z_v[rows, tile_of(j, DB, c)] = ya_v[rows, tile_of(j, DB, c)] + v

        def out_copy(row, n):
            return pltpu.make_async_copy(big_v.at[pl.ds(row, n), :],
                                         out_hbm.at[pl.ds(row, n), :], sem_out)

        def attention_single(mrow, xrow, yrow):
            ma_v[0:M, :] = mem_v[pl.ds(mrow, M), :]
            na_v[0:SEG, :] = _layernorm(xa_v[pl.ds(xrow, SEG), :])
            hooks = None
            for c in range(HB):
                scores, values = attention(c, False)
                project_qkv(0, c, False, hooks)
                project_qkv(1, c, False, None)
                project_qkv(2, c, False, spread(scores, cfg.get("a0", 20), cfg.get("a1", 7)))
                hooks = spread(values, cfg.get("a2", 24), cfg.get("a3", 9))
            for piece in values:
                piece()
            for c in range(DA // LANES):
                for j, v in project_out(c, False).items():
                    mem_v[pl.ds(mrow, M), tile_of(j, DA, c)] = v[:M]
                    ya_v[pl.ds(yrow, SEG), tile_of(j, DA, c)] = (
                        xa_v[pl.ds(xrow, SEG), tile_of(j, DA, c)] + v[M:])

        def step(t, carry):
            cur = pl.multiple_of(t * SEG, SEG)
            nxt = pl.multiple_of(jnp.minimum(t + 1, NSEG - 1) * SEG, SEG)
            row = pl.multiple_of(jnp.maximum(t - 3, 0) * SEG, SEG)
            hooks = {cfg.get("g0", 2): glu_input}
            gpos = cfg.get("gpos", [1, 3, 4, 6, 7, 9, 10])
            for c in range(HB):
                scores, values = attention(c, True)
                for w in range(3):
                    project_qkv(w, c, True, (hooks, None, spread(
                        scores, cfg.get("h0", 20), cfg.get("s0", 10)))[w])
                    if 3 * c + w in gpos:
                        gate_up(gpos.index(3 * c + w))
                hooks = spread(values, cfg.get("h1", 20), cfg.get("s1", 10))
            down(0, spread(values, cfg.get("d0", 6), cfg.get("s2", 1)))
            down(1)
            big_v[pl.ds(row, SEG), :] = z_v[SEG:, :].astype(BF16)

            def next_input():
                na_v[SEG:, :] = _layernorm(z_v[:SEG, :])

            def next_tokens():
                na_v[:SEG, :] = _layernorm(x_v[pl.ds(nxt, SEG), :].astype(F32))

            next_tokens()
            for c in range(DA // LANES):
                o = project_out(c, True, {cfg.get("h2", 2): next_input} if c == 0 else None)
                for (hf, j), v in o.items():
                    cols = tile_of(j, DA, c)
                    res = x_v[pl.ds(cur, SEG), cols].astype(F32) if hf == 0 else xa_v[SEG:, cols]
                    ma_v[hf * M:(hf + 1) * M, cols] = v[:M]
                    ya_v[hf * SEG:(hf + 1) * SEG, cols] = res + v[M:]
            xa_v[SEG:, :] = z_v[:SEG, :]
            pl.when(t >= 3)(lambda: out_copy(row, SEG).start())
            return carry

        def phase(ph, carry):
            attention_single(pl.multiple_of(jnp.where(ph < 2, 0, M), M),
                             pl.multiple_of(jnp.where(ph == 0, 0, SEG), SEG),
                             pl.multiple_of(jnp.where(ph == 3, 1, ph) * SEG, SEG))
            pl.when(ph == 1)(load_glu_weights)

            @pl.when(ph >= 1)
            def _():
                glu_input()
                for c in range(FB // LANES):
                    gate_up(c)
                for c in range(DB // LANES):
                    down(c)

            @pl.when(ph == 1)
            def _():
                x_tail.wait()
                ya_v[0:SEG, :] = ya_v[SEG:2 * SEG, :]
                xa_v[SEG:, :] = z_v[:SEG, :]
                ma_v[...] = mem_v[...]
                na_v[:SEG, :] = _layernorm(x_v[2 * SEG:3 * SEG, :].astype(F32))
                na_v[SEG:, :] = _layernorm(z_v[:SEG, :])
                lax.fori_loop(2, cfg.get("nsteps", NSEG), step, 0)
                mem_v[...] = ma_v[...]

            @pl.when(ph == 2)
            def _():
                xa_v[SEG:, :] = z_v[:SEG, :]
                ya_v[0:SEG, :] = ya_v[2 * SEG:, :]
                big_v[S - 3 * SEG:S - 2 * SEG, :] = z_v[SEG:, :].astype(BF16)
                out_copy(S - 3 * SEG, SEG).start()

            @pl.when(ph == 3)
            def _():
                big_v[S - 2 * SEG:S, :] = z_v[...].astype(BF16)
                out_copy(S - 2 * SEG, 2 * SEG).start()
            return carry

        lax.fori_loop(0, cfg.get('nph', 4), phase, 0)
        out_copy(0, cfg.get("nsteps", NSEG) * SEG).wait()

    scratch = [
        pltpu.VMEM((S, D), BF16),
        pltpu.VMEM((FF, D), BF16),
        pltpu.VMEM((GST, NB, GR, FF), BF16),
        pltpu.VMEM((QST, NA, (QR + 1) * H, DH), BF16),
        pltpu.VMEM((NA, H, QR, DH), BF16),
        pltpu.VMEM((3, HB, PA, DA // 2, DH), U32),
        pltpu.VMEM((DA // LANES, PA, EB // 2, LANES), U32),
        pltpu.VMEM((FB // LANES, PB, DB // 2, 2 * LANES), U32),
        pltpu.VMEM((DB // LANES, PB, FB // 2, LANES), U32),
        pltpu.VMEM((PA, L, DA), F32),
        pltpu.VMEM((PB, SEG, DB), F32),
        pltpu.VMEM((3 * L, H * DH), F32),
        pltpu.VMEM((3 * SEG, FF), F32),
        pltpu.VMEM((2 * M, D), F32),
        pltpu.VMEM((2 * M, D), F32),
        pltpu.VMEM((2 * SEG, D), F32),
        pltpu.VMEM((2 * SEG, D), F32),
        pltpu.VMEM((2 * SEG, D), F32),
        pltpu.VMEM((3 * SEG, D), F32),
        pltpu.VMEM((2 * SEG, D), F32),
        pltpu.VMEM((NA, 2 * L, DH), F32),
        pltpu.VMEM((2, NA, LANES, DH), BF16),
        pltpu.VMEM((2 * L, LANES), F32),
        pltpu.VMEM((2 * L, LANES), jnp.int32),
        pltpu.SemaphoreType.DMA((2,)),
        pltpu.SemaphoreType.DMA((QST, NA)),
        pltpu.SemaphoreType.DMA((OST, NA)),
        pltpu.SemaphoreType.DMA((GST, NB)),
        pltpu.SemaphoreType.DMA((GST, NB)),
        pltpu.SemaphoreType.DMA(()),
    ]
    return kernel, scratch


def _build(cfg):
    @functools.partial(jax.jit, static_argnames=("A_seg_len",))
    def fn(A_x, A_mem0, A_Wq, A_Wk, A_Wv, A_Wo, A_seg_len, B_x, B_w_gate, B_w_up, B_w_down):
        B, S, D = A_x.shape
        _, H, DH = A_Wq.shape
        M = A_mem0.shape[1]
        FF = B_w_gate.shape[1]
        kernel, scratch = _make_kernel(S, D, H, DH, M, A_seg_len, FF, cfg)
        any_spec = pl.BlockSpec(memory_space=pl.ANY)
        out = pl.pallas_call(
            kernel,
            out_shape=jax.ShapeDtypeStruct((S, D), A_x.dtype),
            in_specs=[any_spec, pl.BlockSpec(memory_space=pltpu.VMEM)] + [any_spec] * 7,
            out_specs=any_spec,
            scratch_shapes=scratch,
            compiler_params=pltpu.CompilerParams(vmem_limit_bytes=cfg.get("vmem", 126) * 1024 * 1024,
                                                 flags=cfg.get("flags")),
        )(A_x.reshape(S, D), A_mem0.reshape(M, D),
          A_Wq.reshape(D * H, DH), A_Wk.reshape(D * H, DH), A_Wv.reshape(D * H, DH),
          A_Wo.reshape(H * DH, D), B_w_gate, B_w_up, B_w_down)
        return out.reshape(B, S, D)
    return fn


pallas_interleave_layers__memory_aug_recurrent_mem_tr__glu_gated_glu__prompt_kernel = _build({})
```

```python
import functools
import math

import jax
import jax.numpy as jnp
import numpy as np
from jax import lax
import jax.experimental.pallas as pl
import jax.experimental.pallas.tpu as pltpu

F32 = jnp.float32
BF16 = jnp.bfloat16
U32 = jnp.uint32
EPS = 1e-05
LANES = 128

_SCHEME_4 = """
+00 | +00 +02 -10 +30 | +00 -10
+00 +10 | +00 -01 +20 -30 | +10

+00 -11 | +01 -10 +30 | +01 +10
+10 +11 | +01 | +10 +11
+00 +01 | +03 +10 -30 | +00 +01

+00 +10 +11 +13 | +30 | -00 -01 +03 +10
+00 +01 +03 +10 +11 +13 | -03 +30 | +00 +01 -03
+03 +10 +11 +13 | +03 | +00 +01 -03 +13

+00 +10 -12 | +02 -20 | -00 +02 +10
+10 -12 | +02 | +00 -02 -10 +12
+00 -02 +10 -12 | +20 | -00 +02

+11 | +01 -11 -12 +31 | +01 -11
+01 +11 | -03 -10 +11 +13 -21 +30 | +01

-03 +11 | -03 +13 +31 | -01 +13
+01 +03 | -03 +13 +30 | -01 +03
+11 +13 | +31 | +11 -13

+01 +02 +11 | +12 +21 | +01 -11 +12
+01 +02 | +12 | -01 +02 +11 -12
+01 +02 +11 +12 | +21 | +11 -12

+03 +12 +13 | -23 -32 | -02 +03 -13
+02 +03 +12 +13 | +23 | -02 +03
+12 +13 | +32 | -02 +03 +12 -13

+02 | -12 +20 +22 +23 | +02
+12 | +02 +21 +22 -32 | +12

+03 | +03 -13 +32 +33 | +03 -13
+03 +13 | -03 -23 +31 +33 | +13
"""
_SCHEME_8 = """
+01 +10 | +01 +10 | +00 +11
+00 -01 | +01 | +00 +01
+10 -11 | +10 | -10 -11

+00 +02 +10 | +02 +20 | +00 -10 +12
+00 +02 | +02 | -00 +02 +10 -12
+00 +02 +10 +12 | +20 | +10 -12

+00 +03 -04 +10 | +30 | +00 -10 -13 -14
+00 +03 -04 +10 +13 -14 | +03 +30 | +10 +13 +14
+00 +03 -04 +13 | +03 | +03 -10 -13 -14

+04 +10 | +04 +30 +40 -74 | +00 +14
+00 -04 | +04 -47 -74 | +00 +04
+10 -14 | -03 -30 -40 | +10 +14

+00 -05 +10 | +05 +50 | -00 +10 +15
+00 -05 | +05 | +00 +05 -10 -15
+00 -05 +10 -15 | +50 | -10 -15

+00 +06 +07 +10 | +60 | +00 -10 -16 +17
+00 +06 +07 +10 +16 +17 | +06 +60 | +10 +16 -17
+00 +06 +07 +16 | +06 | +06 -10 -16 +17

-07 +10 | +07 +47 -60 +70 | -00 +17
+00 +07 | +07 +47 +74 | -00 +07
+10 +17 | +06 +60 -70 | -10 +17

+10 | -00 -02 +05 -10 -30 -40 -60 +70 | +00 -10
+00 +10 | +00 -01 -04 +07 -20 -30 +47 +50 -60 +74 | +00

+01 +11 -12 | +12 +21 | +01 +02 -11
+11 -12 | +12 | -01 -02 +11 +12
+01 -02 +11 -12 | +21 | -01 -02

+01 +13 | +13 +31 +63 -71 | +03 +11
+11 -13 | +13 -36 +63 | +11 +13
+01 -03 | -17 -31 +71 | +01 +03

+01 +11 +14 -16 | +41 | -01 +04 +06 +11
+01 +04 -06 +11 +14 -16 | -14 +41 | +01 -04 -06
+04 +11 +14 -16 | +14 | +01 -04 -06 +14

+01 +11 +15 | +15 -51 | +01 +05 -11
+11 +15 | +15 | -01 -05 +11 +15
+01 +05 +11 +15 | +51 | +01 +05

+01 +16 | +16 +36 -41 -61 | +06 -11
+11 -16 | +16 +36 -63 | -11 +16
+01 -06 | -14 +41 +61 | -01 +06

+01 +11 -13 -17 | +71 | +01 +03 +07 -11
+01 -03 -07 +11 -13 -17 | +17 -71 | +01 +03 +07
-07 +11 -13 -17 | +17 | -01 -03 -07 +17

+01 | +01 +11 -12 -15 +31 +41 +61 -71 | +01 -11
+01 +11 | -10 +11 -13 +16 +21 +36 -41 -51 -63 +71 | +11

+02 +03 +13 | +23 -32 -52 | +03 -12 -13
+02 +03 +12 +13 | +23 | +12 +13
+02 +03 | +25 +32 +52 | +02 +03 -12 -13

-04 +12 -14 | -24 -42 | +02 +04 -14
+02 -04 +12 -14 | +24 | +02 +04
+12 -14 | +42 | +02 +04 -12 -14

+03 -05 +12 +13 -15 | +52 | -02 -03 +05 +13 -15
+12 +13 -15 | +25 +52 | +02 +03 -05 -12 -13 +15
+02 +03 +12 +13 -15 | +25 | -02 -03 +05 +12 +13

+02 +06 +16 | +26 -62 | +06 -12 -16
+02 +06 +12 +16 | +26 | +12 +16
+02 +06 | +62 | +02 +06 -12 -16

+07 +12 +17 | -27 -72 | -02 +07 -17
+02 +07 +12 +17 | +27 | -02 +07
+12 +17 | +72 | -02 +07 +12 -17

+02 | -02 -21 +22 -24 +27 -32 -52 -62 | +02
+12 | +12 +20 +22 -23 -26 +42 +52 -72 | +12

+04 +13 | +03 +34 +43 | +03 +14
+03 -04 | +34 | +03 +04
+13 -14 | -03 -30 -43 | +13 +14

+03 -05 +13 | -25 +35 -53 | +03 -13 +15
+03 -05 | -25 +35 -52 | -03 +05 +13 -15
+03 -05 +13 -15 | +53 | -13 +15

-01 +03 +06 +13 | +63 | +03 -11 -13 +16
-01 +03 +06 -11 +13 +16 | -36 +63 | +11 +13 -16
-01 +03 +06 +16 | +36 | +06 +11 +13 -16

-07 +13 | +17 +37 -73 | +03 +17
+03 +07 | +17 +37 -71 | +03 +07
+13 +17 | +73 | +13 +17

+13 | -03 -13 +25 +32 -33 -35 -43 +52 -63 +73 | +03 -13
+03 +13 | -03 -17 -23 -31 +33 -34 -37 +53 -63 +71 | +03

+04 +14 +15 | +45 -54 | +04 +05 -14
+14 +15 | +45 | -04 -05 +14 +15
+04 +05 +14 +15 | +54 | +04 +05

+04 +16 | +14 +46 +64 | +06 +14
+14 -16 | +46 | +14 +16
+04 -06 | -14 +41 -64 | +04 +06

+04 -10 +14 -17 | +74 | +00 +04 -07 -14
-00 +04 -07 -10 +14 -17 | -47 -74 | +00 +04 -07
-07 -10 +14 -17 | +47 | +00 +04 -07 +17

+04 | +04 +14 +34 -42 +44 -45 +64 -74 | +04 -14
+04 +14 | -03 -14 +24 -30 -40 -43 +44 -46 -54 +74 | +14

+05 +06 +16 | +56 -65 | +06 -15 -16
+05 +06 +15 +16 | +56 | +15 +16
+05 +06 | +65 | +05 +06 -15 -16

+07 +15 +17 | -57 -75 | -05 +07 -17
+05 +07 +15 +17 | +57 | -05 +07
+15 +17 | +75 | -05 +07 +15 -17

+05 | +05 -25 +35 -51 -54 +55 +57 -65 | +05
+15 | -15 +25 -45 -50 +53 +55 -56 -75 | +15

-07 +16 | -06 +67 +76 | -06 +17
+06 +07 | +67 | -06 +07
+16 +17 | +06 +60 -76 | -16 +17

+16 | -06 -16 -36 -46 +62 +65 -66 +76 | +06 -16
+06 +16 | -06 -14 -26 -36 +41 -56 +61 -64 +66 +67 | +06

+07 | -07 -17 -37 -47 -67 +72 +75 +77 | +07 -17
+07 +17 | -06 +17 -27 +47 -57 -60 +70 -73 +76 +77 | +17
"""


class _Scheme:
    def __init__(self, n, text):
        def terms(field):
            return {(int(t[1]), int(t[2])): 1 if t[0] == "+" else -1 for t in field.split()}

        def fold(coefs, weights):
            out = {}
            for (h, i), c in coefs.items():
                out[i] = out.get(i, 0) + weights[h] * c
            return {i: c for i, c in out.items() if c}

        self.n = n
        self.prods, self.ends = [], []
        for group in text.strip().split("\n\n"):
            self.prods += [tuple(terms(f) for f in line.split("|")) for line in group.split("\n")]
            self.ends.append(len(self.prods) - 1)
        folded = [(fold(u, (-1, 1)), fold(w, (0, 1))) for u, _, w in self.prods]
        self.single = [(u, w) if u and w else None for u, w in folded]


def _combine(coefs, vals):
    acc = None
    for key, c in sorted(coefs.items(), key=lambda kv: -kv[1]):
        v = vals[key]
        if abs(c) != 1:
            v = v * abs(c)
        if acc is None:
            acc = v if c > 0 else -v
        else:
            acc = acc + v if c > 0 else acc - v
    return acc


def _accumulate(accs, group):
    terms = {}
    for n, (coefs, _) in enumerate(group):
        for key, c in coefs.items():
            terms.setdefault(key, []).append((n, c))
    sums = {((n, 1),): v for n, (_, v) in enumerate(group)}
    for key, tm in sorted(terms.items(), key=lambda kv: len(kv[1])):
        sign = tm[0][1]
        tm = tuple((n, c * sign) for n, c in tm)
        if tm not in sums:
            base = max((s for s in sums if all(t in tm for t in s)), key=len)
            val = sums[base]
            for n, c in tm:
                if (n, c) not in base:
                    val = val + group[n][1] if c > 0 else val - group[n][1]
            sums[tm] = val
        if key not in accs:
            accs[key] = sums[tm] if sign > 0 else -sums[tm]
        else:
            accs[key] = accs[key] + sums[tm] if sign > 0 else accs[key] - sums[tm]


def _layernorm(x, gain=1.0):
    m = jnp.mean(x, axis=-1, keepdims=True)
    c = x - m
    v = jnp.mean(c * c, axis=-1, keepdims=True)
    inv = lax.rsqrt(v + EPS)
    return c * (inv if gain == 1.0 else inv * gain)


def _dot(a, b):
    return lax.dot_general(a, b, (((1,), (0,)), ((), ())), preferred_element_type=F32)


def _dot_nt(a, b):
    return lax.dot_general(a, b, (((1,), (1,)), ((), ())), preferred_element_type=F32)


def _halves(x):
    return [pltpu.unpack_elementwise(x, index=k, packed_dtype=BF16, unpacked_dtype=F32)
            for k in range(2)]


def _pair(lo, hi):
    return pltpu.pack_elementwise([lo, hi], packed_dtype=BF16)


def _make_kernel(S, D, H, DH, M, SEG, FF, cfg):
    SA = _Scheme(8, _SCHEME_8)
    SB = _Scheme(4, _SCHEME_4)
    NA, NB = SA.n, SB.n
    PA, PB = len(SA.prods), len(SB.prods)
    NSEG = S // SEG
    L = M + SEG
    DA, HB = D // NA, H // NA
    EB = HB * DH
    NG = FF // (NA * LANES)
    FA = NG * LANES
    F8 = NA * FA
    DB = D // NB
    assert DA == LANES and DH == LANES and FF - F8 == NB * LANES
    QR = cfg.get("QR", 128) // NA
    QST = cfg.get("QST", 4)
    WR = 512 // NA
    OST = FF // (WR * NA)
    GST = 4
    GR, DR, ER = DA // GST, FA // GST, LANES // GST
    XH = 2 * SEG
    scale = DH ** (-0.5)
    c_exp = scale * math.log2(math.e)

    def fast_dot(sch, paired, w_of, block, kept_ref=None, fresh=True, hooks=None, sums=False,
                 acc=None):
        acc, group = dict(acc or {}), []
        for r, (u, _, w) in enumerate(sch.prods):
            if hooks and r in hooks:
                hooks[r]()
            if paired or sch.single[r]:
                if not paired:
                    u, w = sch.single[r]
                if fresh:
                    if not paired:
                        u = {(0, i): c for i, c in u.items()}
                    elif sums:
                        u = {(2 if u.get((1 - hf, i)) == c else hf, i): c
                             for (hf, i), c in u.items()}
                    lhs = _combine(u, {key: block(*key) for key in u})
                    if kept_ref is not None:
                        kept_ref[r] = lhs
                else:
                    lhs = kept_ref[r]
                group.append((w, _dot(lhs, pltpu.bitcast(w_of(r), BF16))))
            if r in sch.ends:
                _accumulate(acc, group)
                group = []
        return acc

    def blocks_of(ref, rows, cols, c0=0):
        return lambda hf, i: ref[hf * rows:(hf + 1) * rows, c0 + i * cols:c0 + (i + 1) * cols]

    def spread(pieces, first, stride):
        return {first + n * stride: piece for n, piece in enumerate(pieces)}

    def tile_of(j, blk, c):
        return slice(j * blk + c * LANES, j * blk + (c + 1) * LANES)

    def kernel(x_hbm, mem0_ref, wq_hbm, wk_hbm, wv_hbm, wo_hbm, wg_hbm, wu_hbm, wd_hbm,
               out_hbm,
               x_v, big_v, gst_v, qst_v, qtr_v, wqkv_v, wo_v, wgu8_v, wgu4_v, wd8_v, wd4_v,
               la_v, lb_v, o_v, act_v, mem_v, ma_v, xa_v, na_v, nb_v, ya_v, z_v, q_v, kv_v, fill_v, keep_v,
               sem_x, sem_q, sem_o, sem_g, sem_d, sem_out):

        def rows_at(start, size):
            return pl.ds(start if isinstance(start, int) else pl.multiple_of(start, 16), size)

        def q_copies(w, c, slot):
            src = (wq_hbm, wk_hbm, wv_hbm)[w]
            return [pltpu.make_async_copy(src.at[rows_at((i * DA + c * QR) * H, QR * H), :],
                                          qst_v.at[slot, i, 0:QR * H, :], sem_q.at[slot, i])
                    for i in range(NA)]

        def o_copies(c):
            slot = c % OST
            return [pltpu.make_async_copy(wo_hbm.at[rows_at(i * EB + c * WR, WR), :],
                                          big_v.at[rows_at((slot * NA + i) * WR, WR), :],
                                          sem_o.at[slot, i]) for i in range(NA)]

        def g_copies(src, c):
            return [pltpu.make_async_copy(src.at[rows_at(i * DA + c * GR, GR), :],
                                          gst_v.at[c, i], sem_g.at[c, i]) for i in range(NA)]

        def d_copies(c):
            rows = ([rows_at(i * FA + c * DR, DR) for i in range(NA)]
                    + [rows_at(F8 + i * LANES + c * ER, ER) for i in range(NB)])
            return [pltpu.make_async_copy(wd_hbm.at[r, :], big_v.at[r, :], sem_d.at[c, n])
                    for n, r in enumerate(rows)]

        def start(copies):
            for cp in copies:
                cp.start()

        def wait(copies):
            for cp in copies:
                cp.wait()

        def prep_tiles(sch, load, put, nrows, ncols):
            def tile(_, pos):
                s, k = pos
                words = {}
                for r, (_, v, _) in enumerate(sch.prods):
                    for key in v:
                        if key not in words or sch.n > 4:
                            words[key] = pltpu.bitcast(
                                load(*key, pl.multiple_of(s * 16, 16), k), U32)
                    if len(v) == 1:
                        put(r, s * 8, k, words[next(iter(v))])
                    else:
                        halves = {key: _halves(words[key]) for key in v}
                        put(r, s * 8, k, _pair(*(
                            _combine(v, {key: hv[p] for key, hv in halves.items()})
                            for p in range(2))))
                wrap = k + 1 == ncols
                return jnp.where(wrap, s + 1, s), jnp.where(wrap, 0, k + 1)
            lax.fori_loop(0, nrows // 16 * ncols, tile, (0, 0))

        def lanes_at(k):
            return pl.ds(pl.multiple_of(k * LANES, LANES), LANES)

        def words_at(row):
            return pl.ds(pl.multiple_of(row, 8), 8)

        def prep_qkv(w, c, slot):
            def heads(i, carry):
                st = qst_v.at[slot, i].bitcast(U32)
                for jp in range(H // 2):
                    for k, x in enumerate(_halves(st[pl.ds(jp, QR, stride=H // 2), :])):
                        qtr_v[i, 2 * jp + k] = x.astype(BF16)
                return carry
            lax.fori_loop(0, NA, heads, 0)

            def put(r, row, k, val):
                wqkv_v[w, k, r, words_at(c * (QR // 2) + row), :] = val
            prep_tiles(SA, lambda i, j, row, k: qtr_v[i, j * HB + k, pl.ds(row, 16), :], put, QR, HB)

        def prep_from_big(sch, dst, base, blk, c, nrows):
            ncols = D // sch.n // LANES

            def load(i, j, row, k):
                return big_v[rows_at(base + i * blk + row, 16), lanes_at(j * ncols + k)]

            def put(r, row, k, val):
                dst[k, r, words_at(c * (nrows // 2) + row), :] = val
            prep_tiles(sch, load, put, nrows, ncols)

        def prep_gu(w, c):
            def put8(r, row, k, val):
                wgu8_v[w, k, r, words_at(c * (GR // 2) + row), :] = val
            prep_tiles(SA, lambda i, j, row, k: gst_v[c, i, pl.ds(row, 16), lanes_at(j * NG + k)],
                       put8, GR, NG)

            def put4(r, row, k, val):
                rows = words_at(k * (DA // 2) + c * (GR // 2) + row)
                wgu4_v[r, rows, w * LANES:(w + 1) * LANES] = val
            prep_tiles(SB, lambda i, j, row, k: gst_v[c, 2 * i + k, pl.ds(row, 16),
                                                      F8 + j * LANES:F8 + (j + 1) * LANES],
                       put4, GR, 2)

        x_head = pltpu.make_async_copy(x_hbm.at[0:XH, :], x_v.at[0:XH, :], sem_x.at[0])
        x_tail = pltpu.make_async_copy(x_hbm.at[XH:, :], x_v.at[XH:, :], sem_x.at[1])
        NQ, NO = DA // QR, EB // WR
        ONEXT = min(QST, OST)
        for n in range(QST):
            start(q_copies(0, n, n))
        x_head.start()

        ri = lax.broadcasted_iota(jnp.int32, (2 * L, LANES), 0)
        ci = lax.broadcasted_iota(jnp.int32, (2 * L, LANES), 1)
        first = jnp.where(ri < L, 0, L)
        same = (ci >= first) & (ci < first + L)
        visible = (ri < first + M) | (ri >= ci)
        keep_v[...] = (same & visible).astype(jnp.int32)
        fill_v[...] = jnp.where(same, -1e9 / scale, -jnp.inf).astype(F32)
        kv_v[...] = jnp.zeros(kv_v.shape, BF16)
        mem_v[0:M, :] = mem0_ref[...].astype(F32)
        mem_v[M:, :] = mem0_ref[...].astype(F32)

        for w in range(3):
            def q_body(c, carry, w=w):
                slot = (w * NQ + c) % QST
                wait(q_copies(w, c, slot))
                prep_qkv(w, c, slot)
                pl.when(c + QST < NQ)(lambda: start(q_copies(w, c + QST, slot)))
                if w < 2:
                    pl.when(c + QST >= NQ)(lambda: start(q_copies(w + 1, c + QST - NQ, slot)))
                else:
                    pl.when((c + QST >= NQ) & (c + QST - NQ < ONEXT))(
                        lambda: start(o_copies(c + QST - NQ)))
                return carry
            lax.fori_loop(0, NQ, q_body, 0)

        def o_body(c, carry):
            wait(o_copies(c))
            prep_from_big(SA, wo_v, (c % OST) * NA * WR, WR, c, WR)
            pl.when(c + ONEXT < NO)(lambda: start(o_copies(c + ONEXT)))
            pl.when(c >= NO - GST)(lambda: start(g_copies(wg_hbm, c - (NO - GST))))
            return carry
        lax.fori_loop(0, NO, o_body, 0)
        for c in range(GST):
            start(d_copies(c))
        x_head.wait()
        xa_v[...] = x_v[0:XH, :].astype(F32)

        def load_glu_weights():
            def gate(c, carry):
                wait(g_copies(wg_hbm, c))
                prep_gu(0, c)
                start(g_copies(wu_hbm, c))
                return carry

            def down(c, carry):
                wait(d_copies(c))
                prep_from_big(SA, wd8_v, c * DR, FA, c, DR)
                prep_from_big(SB, wd4_v, F8 + c * ER, LANES, c, ER)
                return carry

            def up(c, carry):
                wait(g_copies(wu_hbm, c))
                prep_gu(1, c)
                return carry
            lax.fori_loop(0, GST, gate, 0)
            lax.fori_loop(0, GST, down, 0)
            lax.fori_loop(0, GST, up, 0)
            x_tail.start()

        def attention(c, paired):
            n = 2 * L if paired else L
            probs = {}

            def scores(j):
                s = _dot_nt(q_v[j, 0:n, :], kv_v[0, j])
                s = jnp.where(keep_v[0:n, :] != 0, s, fill_v[0:n, :])
                mx = jnp.max(s, axis=-1, keepdims=True)
                e = jnp.exp2((s - mx) * c_exp)
                den = jnp.sum(e, axis=-1, keepdims=True)
                inv = pl.reciprocal(den, approx=True)
                inv = inv * (2.0 - den * inv)
                probs[j] = e * inv

            def values(j):
                o = _dot(probs[j], kv_v[1, j])
                o_v[0:n, tile_of(j, EB, c)] = o
                if paired:
                    o_v[n:, tile_of(j, EB, c)] = o[:L] + o[L:]

            return ([functools.partial(scores, j) for j in range(NA)],
                    [functools.partial(values, j) for j in range(NA)])

        def project_qkv(w, c, paired, hooks):
            def block(hf, i):
                cols = slice(i * DA, (i + 1) * DA)
                return jnp.concatenate([ma_v[hf * M:(hf + 1) * M, cols],
                                        na_v[hf * SEG:(hf + 1) * SEG, cols]], axis=0)

            p = fast_dot(SA, paired, lambda r: wqkv_v[w, c, r], block, la_v, w + c == 0, hooks)
            for j in range(NA):
                x = jnp.concatenate([p[0, j], p[1, j]], axis=0) if paired else p[j]
                if w == 0:
                    q_v[j, 0:x.shape[0], :] = x
                else:
                    kv_v[w - 1, j, 0:x.shape[0], :] = x.astype(BF16)

        def project_out(c, paired, hooks=None):
            return fast_dot(SA, paired, lambda r: wo_v[c, r], blocks_of(o_v, L, EB),
                            hooks=hooks, sums=True)

        def glu_input():
            nb = _layernorm(ya_v[0:2 * SEG, :], 0.5)
            nb_v[...] = jnp.concatenate([nb, nb[:SEG] + nb[SEG:]], axis=0)

        def gate_up_pieces():
            gate = {}

            def activate(cols, g, u):
                act = [jnp.tanh(g[hf]) * u[hf] + u[hf] for hf in range(2)]
                act_v[:, cols] = jnp.concatenate(act + [act[0] + act[1]], axis=0)

            def large(k, w):
                p = fast_dot(SA, True, lambda r: wgu8_v[w, k, r], blocks_of(nb_v, SEG, DA), lb_v,
                             k + w == 0, sums=True)
                if w == 0:
                    gate.update(p)
                else:
                    for j in range(NA):
                        activate(tile_of(j, FA, k), (gate[0, j], gate[1, j]), (p[0, j], p[1, j]))

            def small():
                p = fast_dot(SB, True, lambda r: wgu4_v[r], blocks_of(nb_v, SEG, DB), sums=True)
                for j in range(NB):
                    activate(slice(F8 + j * LANES, F8 + (j + 1) * LANES),
                             [p[hf, j][:, :LANES] for hf in range(2)],
                             [p[hf, j][:, LANES:] for hf in range(2)])

            return [small] + [functools.partial(large, k, w) for k in range(NG) for w in range(2)]

        def down(hooks4=None, hooks8=None):
            acc = {}
            for k in range(DB // LANES):
                p = fast_dot(SB, True, lambda r: wd4_v[k, r], blocks_of(act_v, SEG, LANES, F8),
                             hooks=None if k else hooks4, sums=True)
                acc.update({(hf, j * (DB // LANES) + k): v for (hf, j), v in p.items()})
            acc = fast_dot(SA, True, lambda r: wd8_v[0, r], blocks_of(act_v, SEG, FA),
                           hooks=hooks8, sums=True, acc=acc)
            for (hf, j), v in acc.items():
                rows = slice(hf * SEG, (hf + 1) * SEG)
                z_v[rows, tile_of(j, DA, 0)] = ya_v[rows, tile_of(j, DA, 0)] + v

        def out_copy(row, n):
            return pltpu.make_async_copy(big_v.at[pl.ds(row, n), :],
                                         out_hbm.at[pl.ds(row, n), :], sem_out)

        def attention_single(mrow, xrow, yrow):
            ma_v[0:M, :] = mem_v[pl.ds(mrow, M), :]
            na_v[0:SEG, :] = _layernorm(xa_v[pl.ds(xrow, SEG), :])
            hooks = None
            for c in range(HB):
                scores, values = attention(c, False)
                project_qkv(0, c, False, hooks)
                project_qkv(1, c, False, None)
                project_qkv(2, c, False, spread(scores, cfg.get("a0", 20), cfg.get("a1", 7)))
                hooks = spread(values, cfg.get("a2", 24), cfg.get("a3", 9))
            for piece in values:
                piece()
            for c in range(DA // LANES):
                for j, v in project_out(c, False).items():
                    mem_v[pl.ds(mrow, M), tile_of(j, DA, c)] = v[:M]
                    ya_v[pl.ds(yrow, SEG), tile_of(j, DA, c)] = (
                        xa_v[pl.ds(xrow, SEG), tile_of(j, DA, c)] + v[M:])

        def step(t, carry):
            cur = pl.multiple_of(t * SEG, SEG)
            nxt = pl.multiple_of(jnp.minimum(t + 1, NSEG - 1) * SEG, SEG)
            row = pl.multiple_of(jnp.maximum(t - 3, 0) * SEG, SEG)
            hooks = {cfg.get("g0", 2): glu_input}
            gpos = cfg.get("gpos", [1, 3, 4, 6, 7, 9, 10])
            glu = gate_up_pieces()
            for c in range(HB):
                scores, values = attention(c, True)
                for w in range(3):
                    project_qkv(w, c, True, (hooks, None, spread(
                        scores, cfg.get("h0", 20), cfg.get("s0", 10)))[w])
                    if 3 * c + w in gpos:
                        glu[gpos.index(3 * c + w)]()
                hooks = spread(values, cfg.get("h1", 20), cfg.get("s1", 10))
            down(None, spread(values, cfg.get("d0", 4), cfg.get("s2", 6)))
            big_v[pl.ds(row, SEG), :] = z_v[SEG:, :].astype(BF16)

            def next_input():
                na_v[SEG:, :] = _layernorm(z_v[:SEG, :])

            def next_tokens():
                na_v[:SEG, :] = _layernorm(x_v[pl.ds(nxt, SEG), :].astype(F32))

            next_tokens()
            for c in range(DA // LANES):
                o = project_out(c, True, {cfg.get("h2", 2): next_input} if c == 0 else None)
                for (hf, j), v in o.items():
                    cols = tile_of(j, DA, c)
                    res = x_v[pl.ds(cur, SEG), cols].astype(F32) if hf == 0 else xa_v[SEG:, cols]
                    ma_v[hf * M:(hf + 1) * M, cols] = v[:M]
                    ya_v[hf * SEG:(hf + 1) * SEG, cols] = res + v[M:]
            xa_v[SEG:, :] = z_v[:SEG, :]
            pl.when(t >= 3)(lambda: out_copy(row, SEG).start())
            return carry

        def phase(ph, carry):
            attention_single(pl.multiple_of(jnp.where(ph < 2, 0, M), M),
                             pl.multiple_of(jnp.where(ph == 0, 0, SEG), SEG),
                             pl.multiple_of(jnp.where(ph == 3, 1, ph) * SEG, SEG))
            pl.when(ph == 1)(load_glu_weights)

            @pl.when(ph >= 1)
            def _():
                glu_input()
                for piece in gate_up_pieces():
                    piece()
                down()

            @pl.when(ph == 1)
            def _():
                x_tail.wait()
                ya_v[0:SEG, :] = ya_v[SEG:2 * SEG, :]
                xa_v[SEG:, :] = z_v[:SEG, :]
                ma_v[...] = mem_v[...]
                na_v[:SEG, :] = _layernorm(x_v[2 * SEG:3 * SEG, :].astype(F32))
                na_v[SEG:, :] = _layernorm(z_v[:SEG, :])
                lax.fori_loop(2, cfg.get("nsteps", NSEG), step, 0)
                mem_v[...] = ma_v[...]

            @pl.when(ph == 2)
            def _():
                xa_v[SEG:, :] = z_v[:SEG, :]
                ya_v[0:SEG, :] = ya_v[2 * SEG:, :]
                big_v[S - 3 * SEG:S - 2 * SEG, :] = z_v[SEG:, :].astype(BF16)
                out_copy(S - 3 * SEG, SEG).start()

            @pl.when(ph == 3)
            def _():
                big_v[S - 2 * SEG:S, :] = z_v[...].astype(BF16)
                out_copy(S - 2 * SEG, 2 * SEG).start()
            return carry

        lax.fori_loop(0, cfg.get('nph', 4), phase, 0)
        out_copy(0, cfg.get("nsteps", NSEG) * SEG).wait()

    scratch = [
        pltpu.VMEM((S, D), BF16),
        pltpu.VMEM((FF, D), BF16),
        pltpu.VMEM((GST, NA, GR, FF), BF16),
        pltpu.VMEM((QST, NA, (QR + 1) * H, DH), BF16),
        pltpu.VMEM((NA, H, QR, DH), BF16),
        pltpu.VMEM((3, HB, PA, DA // 2, DH), U32),
        pltpu.VMEM((DA // LANES, PA, EB // 2, LANES), U32),
        pltpu.VMEM((2, NG, PA, DA // 2, LANES), U32),
        pltpu.VMEM((PB, DB // 2, 2 * LANES), U32),
        pltpu.VMEM((1, PA, FA // 2, LANES), U32),
        pltpu.VMEM((DB // LANES, PB, LANES // 2, LANES), U32),
        pltpu.VMEM((PA, L, DA), F32),
        pltpu.VMEM((PA, SEG, DA), F32),
        pltpu.VMEM((3 * L, H * DH), F32),
        pltpu.VMEM((3 * SEG, FF), F32),
        pltpu.VMEM((2 * M, D), F32),
        pltpu.VMEM((2 * M, D), F32),
        pltpu.VMEM((2 * SEG, D), F32),
        pltpu.VMEM((2 * SEG, D), F32),
        pltpu.VMEM((3 * SEG, D), F32),
        pltpu.VMEM((3 * SEG, D), F32),
        pltpu.VMEM((2 * SEG, D), F32),
        pltpu.VMEM((NA, 2 * L, DH), F32),
        pltpu.VMEM((2, NA, LANES, DH), BF16),
        pltpu.VMEM((2 * L, LANES), F32),
        pltpu.VMEM((2 * L, LANES), jnp.int32),
        pltpu.SemaphoreType.DMA((2,)),
        pltpu.SemaphoreType.DMA((QST, NA)),
        pltpu.SemaphoreType.DMA((OST, NA)),
        pltpu.SemaphoreType.DMA((GST, NA)),
        pltpu.SemaphoreType.DMA((GST, NA + NB)),
        pltpu.SemaphoreType.DMA(()),
    ]
    return kernel, scratch


def _build(cfg):
    @functools.partial(jax.jit, static_argnames=("A_seg_len",))
    def fn(A_x, A_mem0, A_Wq, A_Wk, A_Wv, A_Wo, A_seg_len, B_x, B_w_gate, B_w_up, B_w_down):
        B, S, D = A_x.shape
        _, H, DH = A_Wq.shape
        M = A_mem0.shape[1]
        FF = B_w_gate.shape[1]
        kernel, scratch = _make_kernel(S, D, H, DH, M, A_seg_len, FF, cfg)
        any_spec = pl.BlockSpec(memory_space=pl.ANY)
        out = pl.pallas_call(
            kernel,
            out_shape=jax.ShapeDtypeStruct((S, D), A_x.dtype),
            in_specs=[any_spec, pl.BlockSpec(memory_space=pltpu.VMEM)] + [any_spec] * 7,
            out_specs=any_spec,
            scratch_shapes=scratch,
            compiler_params=pltpu.CompilerParams(vmem_limit_bytes=cfg.get("vmem", 126) * 1024 * 1024,
                                                 flags=cfg.get("flags")),
        )(A_x.reshape(S, D), A_mem0.reshape(M, D),
          A_Wq.reshape(D * H, DH), A_Wk.reshape(D * H, DH), A_Wv.reshape(D * H, DH),
          A_Wo.reshape(H * DH, D), B_w_gate, B_w_up, B_w_down)
        return out.reshape(B, S, D)
    return fn


pallas_interleave_layers__memory_aug_recurrent_mem_tr__glu_gated_glu__prompt_kernel = _build({})
```

```python
import functools
import math

import jax
import jax.numpy as jnp
import numpy as np
from jax import lax
import jax.experimental.pallas as pl
import jax.experimental.pallas.tpu as pltpu

F32 = jnp.float32
BF16 = jnp.bfloat16
U32 = jnp.uint32
EPS = 1e-05
LANES = 128

_SCHEME_4 = """
+00 | +00 +02 -10 +30 | +00 -10
+00 +10 | +00 -01 +20 -30 | +10

+00 -11 | +01 -10 +30 | +01 +10
+10 +11 | +01 | +10 +11
+00 +01 | +03 +10 -30 | +00 +01

+00 +10 +11 +13 | +30 | -00 -01 +03 +10
+00 +01 +03 +10 +11 +13 | -03 +30 | +00 +01 -03
+03 +10 +11 +13 | +03 | +00 +01 -03 +13

+00 +10 -12 | +02 -20 | -00 +02 +10
+10 -12 | +02 | +00 -02 -10 +12
+00 -02 +10 -12 | +20 | -00 +02

+11 | +01 -11 -12 +31 | +01 -11
+01 +11 | -03 -10 +11 +13 -21 +30 | +01

-03 +11 | -03 +13 +31 | -01 +13
+01 +03 | -03 +13 +30 | -01 +03
+11 +13 | +31 | +11 -13

+01 +02 +11 | +12 +21 | +01 -11 +12
+01 +02 | +12 | -01 +02 +11 -12
+01 +02 +11 +12 | +21 | +11 -12

+03 +12 +13 | -23 -32 | -02 +03 -13
+02 +03 +12 +13 | +23 | -02 +03
+12 +13 | +32 | -02 +03 +12 -13

+02 | -12 +20 +22 +23 | +02
+12 | +02 +21 +22 -32 | +12

+03 | +03 -13 +32 +33 | +03 -13
+03 +13 | -03 -23 +31 +33 | +13
"""
_SCHEME_8 = """
+01 +10 | +01 +10 | +00 +11
+00 -01 | +01 | +00 +01
+10 -11 | +10 | -10 -11

+00 +02 +10 | +02 +20 | +00 -10 +12
+00 +02 | +02 | -00 +02 +10 -12
+00 +02 +10 +12 | +20 | +10 -12

+00 +03 -04 +10 | +30 | +00 -10 -13 -14
+00 +03 -04 +10 +13 -14 | +03 +30 | +10 +13 +14
+00 +03 -04 +13 | +03 | +03 -10 -13 -14

+04 +10 | +04 +30 +40 -74 | +00 +14
+00 -04 | +04 -47 -74 | +00 +04
+10 -14 | -03 -30 -40 | +10 +14

+00 -05 +10 | +05 +50 | -00 +10 +15
+00 -05 | +05 | +00 +05 -10 -15
+00 -05 +10 -15 | +50 | -10 -15

+00 +06 +07 +10 | +60 | +00 -10 -16 +17
+00 +06 +07 +10 +16 +17 | +06 +60 | +10 +16 -17
+00 +06 +07 +16 | +06 | +06 -10 -16 +17

-07 +10 | +07 +47 -60 +70 | -00 +17
+00 +07 | +07 +47 +74 | -00 +07
+10 +17 | +06 +60 -70 | -10 +17

+10 | -00 -02 +05 -10 -30 -40 -60 +70 | +00 -10
+00 +10 | +00 -01 -04 +07 -20 -30 +47 +50 -60 +74 | +00

+01 +11 -12 | +12 +21 | +01 +02 -11
+11 -12 | +12 | -01 -02 +11 +12
+01 -02 +11 -12 | +21 | -01 -02

+01 +13 | +13 +31 +63 -71 | +03 +11
+11 -13 | +13 -36 +63 | +11 +13
+01 -03 | -17 -31 +71 | +01 +03

+01 +11 +14 -16 | +41 | -01 +04 +06 +11
+01 +04 -06 +11 +14 -16 | -14 +41 | +01 -04 -06
+04 +11 +14 -16 | +14 | +01 -04 -06 +14

+01 +11 +15 | +15 -51 | +01 +05 -11
+11 +15 | +15 | -01 -05 +11 +15
+01 +05 +11 +15 | +51 | +01 +05

+01 +16 | +16 +36 -41 -61 | +06 -11
+11 -16 | +16 +36 -63 | -11 +16
+01 -06 | -14 +41 +61 | -01 +06

+01 +11 -13 -17 | +71 | +01 +03 +07 -11
+01 -03 -07 +11 -13 -17 | +17 -71 | +01 +03 +07
-07 +11 -13 -17 | +17 | -01 -03 -07 +17

+01 | +01 +11 -12 -15 +31 +41 +61 -71 | +01 -11
+01 +11 | -10 +11 -13 +16 +21 +36 -41 -51 -63 +71 | +11

+02 +03 +13 | +23 -32 -52 | +03 -12 -13
+02 +03 +12 +13 | +23 | +12 +13
+02 +03 | +25 +32 +52 | +02 +03 -12 -13

-04 +12 -14 | -24 -42 | +02 +04 -14
+02 -04 +12 -14 | +24 | +02 +04
+12 -14 | +42 | +02 +04 -12 -14

+03 -05 +12 +13 -15 | +52 | -02 -03 +05 +13 -15
+12 +13 -15 | +25 +52 | +02 +03 -05 -12 -13 +15
+02 +03 +12 +13 -15 | +25 | -02 -03 +05 +12 +13

+02 +06 +16 | +26 -62 | +06 -12 -16
+02 +06 +12 +16 | +26 | +12 +16
+02 +06 | +62 | +02 +06 -12 -16

+07 +12 +17 | -27 -72 | -02 +07 -17
+02 +07 +12 +17 | +27 | -02 +07
+12 +17 | +72 | -02 +07 +12 -17

+02 | -02 -21 +22 -24 +27 -32 -52 -62 | +02
+12 | +12 +20 +22 -23 -26 +42 +52 -72 | +12

+04 +13 | +03 +34 +43 | +03 +14
+03 -04 | +34 | +03 +04
+13 -14 | -03 -30 -43 | +13 +14

+03 -05 +13 | -25 +35 -53 | +03 -13 +15
+03 -05 | -25 +35 -52 | -03 +05 +13 -15
+03 -05 +13 -15 | +53 | -13 +15

-01 +03 +06 +13 | +63 | +03 -11 -13 +16
-01 +03 +06 -11 +13 +16 | -36 +63 | +11 +13 -16
-01 +03 +06 +16 | +36 | +06 +11 +13 -16

-07 +13 | +17 +37 -73 | +03 +17
+03 +07 | +17 +37 -71 | +03 +07
+13 +17 | +73 | +13 +17

+13 | -03 -13 +25 +32 -33 -35 -43 +52 -63 +73 | +03 -13
+03 +13 | -03 -17 -23 -31 +33 -34 -37 +53 -63 +71 | +03

+04 +14 +15 | +45 -54 | +04 +05 -14
+14 +15 | +45 | -04 -05 +14 +15
+04 +05 +14 +15 | +54 | +04 +05

+04 +16 | +14 +46 +64 | +06 +14
+14 -16 | +46 | +14 +16
+04 -06 | -14 +41 -64 | +04 +06

+04 -10 +14 -17 | +74 | +00 +04 -07 -14
-00 +04 -07 -10 +14 -17 | -47 -74 | +00 +04 -07
-07 -10 +14 -17 | +47 | +00 +04 -07 +17

+04 | +04 +14 +34 -42 +44 -45 +64 -74 | +04 -14
+04 +14 | -03 -14 +24 -30 -40 -43 +44 -46 -54 +74 | +14

+05 +06 +16 | +56 -65 | +06 -15 -16
+05 +06 +15 +16 | +56 | +15 +16
+05 +06 | +65 | +05 +06 -15 -16

+07 +15 +17 | -57 -75 | -05 +07 -17
+05 +07 +15 +17 | +57 | -05 +07
+15 +17 | +75 | -05 +07 +15 -17

+05 | +05 -25 +35 -51 -54 +55 +57 -65 | +05
+15 | -15 +25 -45 -50 +53 +55 -56 -75 | +15

-07 +16 | -06 +67 +76 | -06 +17
+06 +07 | +67 | -06 +07
+16 +17 | +06 +60 -76 | -16 +17

+16 | -06 -16 -36 -46 +62 +65 -66 +76 | +06 -16
+06 +16 | -06 -14 -26 -36 +41 -56 +61 -64 +66 +67 | +06

+07 | -07 -17 -37 -47 -67 +72 +75 +77 | +07 -17
+07 +17 | -06 +17 -27 +47 -57 -60 +70 -73 +76 +77 | +17
"""


class _Scheme:
    def __init__(self, n, text):
        def terms(field):
            return {(int(t[1]), int(t[2])): 1 if t[0] == "+" else -1 for t in field.split()}

        def fold(coefs, weights):
            out = {}
            for (h, i), c in coefs.items():
                out[i] = out.get(i, 0) + weights[h] * c
            return {i: c for i, c in out.items() if c}

        self.n = n
        self.prods, self.ends = [], []
        for group in text.strip().split("\n\n"):
            self.prods += [tuple(terms(f) for f in line.split("|")) for line in group.split("\n")]
            self.ends.append(len(self.prods) - 1)
        folded = [(fold(u, (-1, 1)), fold(w, (0, 1))) for u, _, w in self.prods]
        self.single = [(u, w) if u and w else None for u, w in folded]


def _combine(coefs, vals):
    acc = None
    for key, c in sorted(coefs.items(), key=lambda kv: -kv[1]):
        v = vals[key]
        if abs(c) != 1:
            v = v * abs(c)
        if acc is None:
            acc = v if c > 0 else -v
        else:
            acc = acc + v if c > 0 else acc - v
    return acc


def _accumulate(accs, group):
    terms = {}
    for n, (coefs, _) in enumerate(group):
        for key, c in coefs.items():
            terms.setdefault(key, []).append((n, c))
    sums = {((n, 1),): v for n, (_, v) in enumerate(group)}
    for key, tm in sorted(terms.items(), key=lambda kv: len(kv[1])):
        sign = tm[0][1]
        tm = tuple((n, c * sign) for n, c in tm)
        if tm not in sums:
            base = max((s for s in sums if all(t in tm for t in s)), key=len)
            val = sums[base]
            for n, c in tm:
                if (n, c) not in base:
                    val = val + group[n][1] if c > 0 else val - group[n][1]
            sums[tm] = val
        if key not in accs:
            accs[key] = sums[tm] if sign > 0 else -sums[tm]
        else:
            accs[key] = accs[key] + sums[tm] if sign > 0 else accs[key] - sums[tm]


def _layernorm(x, gain=1.0):
    m = jnp.mean(x, axis=-1, keepdims=True)
    c = x - m
    v = jnp.mean(c * c, axis=-1, keepdims=True)
    inv = lax.rsqrt(v + EPS)
    return c * (inv if gain == 1.0 else inv * gain)


def _dot(a, b):
    return lax.dot_general(a, b, (((1,), (0,)), ((), ())), preferred_element_type=F32)


def _dot_nt(a, b):
    return lax.dot_general(a, b, (((1,), (1,)), ((), ())), preferred_element_type=F32)


def _halves(x):
    return [pltpu.unpack_elementwise(x, index=k, packed_dtype=BF16, unpacked_dtype=F32)
            for k in range(2)]


def _pair(lo, hi):
    return pltpu.pack_elementwise([lo, hi], packed_dtype=BF16)


def _make_kernel(S, D, H, DH, M, SEG, FF, cfg):
    SA = _Scheme(8, _SCHEME_8)
    SB = _Scheme(4, _SCHEME_4)
    NA, NB = SA.n, SB.n
    PA, PB = len(SA.prods), len(SB.prods)
    NSEG = S // SEG
    L = M + SEG
    DA, HB = D // NA, H // NA
    EB = HB * DH
    NG = FF // (NA * LANES)
    FA = NG * LANES
    F8 = NA * FA
    DB = D // NB
    assert DA == LANES and DH == LANES and FF - F8 == NB * LANES
    QR = cfg.get("QR", 128) // NA
    QST = cfg.get("QST", 4)
    WR = 512 // NA
    OST = FF // (WR * NA)
    GST = 4
    GR, DR, ER = DA // GST, FA // GST, LANES // GST
    XH = 4 * SEG
    scale = DH ** (-0.5)
    c_exp = scale * math.log2(math.e)

    def fast_dot(sch, paired, w_of, block, kept_ref=None, fresh=True, hooks=None, sums=False,
                 acc=None):
        acc, group = dict(acc or {}), []
        for r, (u, _, w) in enumerate(sch.prods):
            if hooks and r in hooks:
                hooks[r]()
            if paired or sch.single[r]:
                if not paired:
                    u, w = sch.single[r]
                if fresh:
                    if not paired:
                        u = {(0, i): c for i, c in u.items()}
                    elif sums:
                        u = {(2 if u.get((1 - hf, i)) == c else hf, i): c
                             for (hf, i), c in u.items()}
                    lhs = _combine(u, {key: block(*key) for key in u})
                    if kept_ref is not None:
                        kept_ref[r] = lhs
                else:
                    lhs = kept_ref[r]
                group.append((w, _dot(lhs, pltpu.bitcast(w_of(r), BF16))))
            if r in sch.ends:
                _accumulate(acc, group)
                group = []
        return acc

    def blocks_of(ref, rows, cols, c0=0):
        return lambda hf, i: ref[hf * rows:(hf + 1) * rows, c0 + i * cols:c0 + (i + 1) * cols]

    def spread(pieces, first, stride):
        return {first + n * stride: piece for n, piece in enumerate(pieces)}

    def tile_of(j, blk, c):
        return slice(j * blk + c * LANES, j * blk + (c + 1) * LANES)

    def kernel(x_hbm, mem0_hbm, wq_hbm, wk_hbm, wv_hbm, wo_hbm, wg_hbm, wu_hbm, wd_hbm,
               out_hbm,
               x_v, mem0_v, big_v, gst_v, qst_v, qtr_v, wqkv_v, wo_v, wgu8_v, wgu4_v, wd8_v, wd4_v,
               la_v, lb_v, o_v, act_v, mem_v, ma_v, xa_v, na_v, nb_v, ya_v, z_v, q_v, kv_v, fill_v, keep_v,
               sem_x, sem_q, sem_o, sem_g, sem_d, sem_out):

        def rows_at(start, size):
            return pl.ds(start if isinstance(start, int) else pl.multiple_of(start, 16), size)

        def q_copies(w, c, slot):
            src = (wq_hbm, wk_hbm, wv_hbm)[w]
            return [pltpu.make_async_copy(src.at[rows_at((i * DA + c * QR) * H, QR * H), :],
                                          qst_v.at[slot, i, 0:QR * H, :], sem_q.at[slot])
                    for i in range(NA)]

        def o_copies(c):
            slot = c % OST
            return [pltpu.make_async_copy(wo_hbm.at[rows_at(i * EB + c * WR, WR), :],
                                          big_v.at[rows_at((slot * NA + i) * WR, WR), :],
                                          sem_o.at[slot]) for i in range(NA)]

        def g_copies(w, c):
            return [pltpu.make_async_copy((wg_hbm, wu_hbm)[w].at[rows_at(i * DA + c * GR, GR), :],
                                          gst_v.at[w, c, i], sem_g.at[w, c]) for i in range(NA)]

        def d_copies(c):
            rows = ([rows_at(i * FA + c * DR, DR) for i in range(NA)]
                    + [rows_at(F8 + i * LANES + c * ER, ER) for i in range(NB)])
            return [pltpu.make_async_copy(wd_hbm.at[r, :], big_v.at[r, :], sem_d.at[c])
                    for r in rows]

        def start(copies):
            for cp in copies:
                cp.start()

        def wait(copies):
            for cp in copies:
                cp.wait()

        def prep_tiles(sch, load, put, nrows, ncols):
            def tile(_, pos):
                s, k = pos
                words = {}
                for r, (_, v, _) in enumerate(sch.prods):
                    for key in v:
                        if key not in words or sch.n > 4:
                            words[key] = pltpu.bitcast(
                                load(*key, pl.multiple_of(s * 16, 16), k), U32)
                    if len(v) == 1:
                        put(r, s * 8, k, words[next(iter(v))])
                    else:
                        halves = {key: _halves(words[key]) for key in v}
                        put(r, s * 8, k, _pair(*(
                            _combine(v, {key: hv[p] for key, hv in halves.items()})
                            for p in range(2))))
                wrap = k + 1 == ncols
                return jnp.where(wrap, s + 1, s), jnp.where(wrap, 0, k + 1)
            lax.fori_loop(0, nrows // 16 * ncols, tile, (0, 0))

        def lanes_at(k):
            return pl.ds(pl.multiple_of(k * LANES, LANES), LANES)

        def words_at(row):
            return pl.ds(pl.multiple_of(row, 8), 8)

        def prep_qkv(w, c, slot):
            def heads(i, carry):
                st = qst_v.at[slot, i].bitcast(U32)
                for jp in range(H // 2):
                    for k, x in enumerate(_halves(st[pl.ds(jp, QR, stride=H // 2), :])):
                        qtr_v[i, 2 * jp + k] = x.astype(BF16)
                return carry
            lax.fori_loop(0, NA, heads, 0)

            def put(r, row, k, val):
                wqkv_v[w, k, r, words_at(c * (QR // 2) + row), :] = val
            prep_tiles(SA, lambda i, j, row, k: qtr_v[i, j * HB + k, pl.ds(row, 16), :], put, QR, HB)

        def prep_from_big(sch, dst, base, blk, c, nrows):
            ncols = D // sch.n // LANES

            def load(i, j, row, k):
                return big_v[rows_at(base + i * blk + row, 16), lanes_at(j * ncols + k)]

            def put(r, row, k, val):
                dst[k, r, words_at(c * (nrows // 2) + row), :] = val
            prep_tiles(sch, load, put, nrows, ncols)

        def prep_gu(w, c):
            def put8(r, row, k, val):
                wgu8_v[w, k, r, words_at(c * (GR // 2) + row), :] = val
            prep_tiles(SA, lambda i, j, row, k: gst_v[w, c, i, pl.ds(row, 16),
                                                      lanes_at(j * NG + k)], put8, GR, NG)

            def put4(r, row, k, val):
                rows = words_at(k * (DA // 2) + c * (GR // 2) + row)
                wgu4_v[r, rows, w * LANES:(w + 1) * LANES] = val
            prep_tiles(SB, lambda i, j, row, k: gst_v[w, c, 2 * i + k, pl.ds(row, 16),
                                                      F8 + j * LANES:F8 + (j + 1) * LANES],
                       put4, GR, 2)

        x_head = pltpu.make_async_copy(x_hbm.at[0:XH, :], x_v.at[0:XH, :], sem_x.at[0])
        x_tail = pltpu.make_async_copy(x_hbm.at[XH:, :], x_v.at[XH:, :], sem_x.at[1])
        NQ, NO = DA // QR, EB // WR
        AHEAD = cfg.get('oa', 5)
        assert QST <= min(NQ, AHEAD) and AHEAD <= OST <= NO
        for n in range(QST):
            start(q_copies(0, n, n))
        mem0_copy = pltpu.make_async_copy(mem0_hbm, mem0_v, sem_x.at[2])
        x_head.start()
        mem0_copy.start()

        ri = lax.broadcasted_iota(jnp.int32, (2 * L, LANES), 0)
        ci = lax.broadcasted_iota(jnp.int32, (2 * L, LANES), 1)
        first = jnp.where(ri < L, 0, L)
        same = (ci >= first) & (ci < first + L)
        visible = (ri < first + M) | (ri >= ci)
        keep_v[...] = (same & visible).astype(jnp.int32)
        fill_v[...] = jnp.where(same, -1e9 / scale, -jnp.inf).astype(F32)
        kv_v[...] = jnp.zeros(kv_v.shape, BF16)

        for w in range(3):
            def q_body(c, carry, w=w):
                slot = (w * NQ + c) % QST
                wait(q_copies(w, c, slot))
                prep_qkv(w, c, slot)
                pl.when(c + QST < NQ)(lambda: start(q_copies(w, c + QST, slot)))
                if w < 2:
                    pl.when(c + QST >= NQ)(lambda: start(q_copies(w + 1, c + QST - NQ, slot)))
                else:
                    pl.when(c + QST >= NQ)(lambda: start(o_copies(c + QST - NQ)))
                return carry
            lax.fori_loop(0, NQ, q_body, 0)

        for c in range(QST, AHEAD):
            start(o_copies(c))
        x_head.wait()
        mem0_copy.wait()
        xa_v[...] = x_v[0:2 * SEG, :].astype(F32)
        mem_v[0:M, :] = mem0_v[...].astype(F32)
        mem_v[M:, :] = mem0_v[...].astype(F32)

        def load_out_weights():
            def chunk(c, carry):
                wait(o_copies(c))
                prep_from_big(SA, wo_v, (c % OST) * NA * WR, WR, c, WR)
                pl.when(c + AHEAD < NO)(lambda: start(o_copies(c + AHEAD)))
                pl.when(c >= NO - 2)(lambda: start(g_copies(0, c - (NO - 2))))
                return carry
            lax.fori_loop(0, NO, chunk, 0)
            for c in range(2, GST):
                start(g_copies(0, c))
            start(g_copies(1, 0))

        def load_gate_up_weights():
            def gate(c, carry):
                pl.when(c + 1 < GST)(lambda: start(g_copies(1, c + 1)))
                wait(g_copies(0, c))
                prep_gu(0, c)
                return carry

            def up(c, carry):
                wait(g_copies(1, c))
                prep_gu(1, c)
                start(d_copies(c))
                return carry
            lax.fori_loop(0, GST, gate, 0)
            lax.fori_loop(0, GST, up, 0)

        def load_down_weights():
            def chunk(c, carry):
                wait(d_copies(c))
                pl.when(c == cfg.get("xt", GST - 1))(lambda: x_tail.start())
                prep_from_big(SA, wd8_v, c * DR, FA, c, DR)
                prep_from_big(SB, wd4_v, F8 + c * ER, LANES, c, ER)
                return carry
            lax.fori_loop(0, GST, chunk, 0)

        def attention(c, paired):
            n = 2 * L if paired else L
            probs = {}

            def scores(j):
                s = _dot_nt(q_v[j, 0:n, :], kv_v[0, j])
                s = jnp.where(keep_v[0:n, :] != 0, s, fill_v[0:n, :])
                mx = jnp.max(s, axis=-1, keepdims=True)
                e = jnp.exp2((s - mx) * c_exp)
                den = jnp.sum(e, axis=-1, keepdims=True)
                inv = pl.reciprocal(den, approx=True)
                inv = inv * (2.0 - den * inv)
                probs[j] = e * inv

            def values(j):
                o = _dot(probs[j], kv_v[1, j])
                o_v[0:n, tile_of(j, EB, c)] = o
                if paired:
                    o_v[n:, tile_of(j, EB, c)] = o[:L] + o[L:]

            return ([functools.partial(scores, j) for j in range(NA)],
                    [functools.partial(values, j) for j in range(NA)])

        def project_qkv(w, c, paired, hooks):
            def block(hf, i):
                cols = slice(i * DA, (i + 1) * DA)
                return jnp.concatenate([ma_v[hf * M:(hf + 1) * M, cols],
                                        na_v[hf * SEG:(hf + 1) * SEG, cols]], axis=0)

            p = fast_dot(SA, paired, lambda r: wqkv_v[w, c, r], block, la_v, w + c == 0, hooks)
            for j in range(NA):
                x = jnp.concatenate([p[0, j], p[1, j]], axis=0) if paired else p[j]
                if w == 0:
                    q_v[j, 0:x.shape[0], :] = x
                else:
                    kv_v[w - 1, j, 0:x.shape[0], :] = x.astype(BF16)

        def project_out(c, paired, hooks=None):
            return fast_dot(SA, paired, lambda r: wo_v[c, r], blocks_of(o_v, L, EB),
                            hooks=hooks, sums=True)

        def glu_input():
            nb = _layernorm(ya_v[0:2 * SEG, :], 0.5)
            nb_v[...] = jnp.concatenate([nb, nb[:SEG] + nb[SEG:]], axis=0)

        def gate_up_pieces():
            gate = {}

            def activate(cols, g, u):
                act = [jnp.tanh(g[hf]) * u[hf] + u[hf] for hf in range(2)]
                act_v[:, cols] = jnp.concatenate(act + [act[0] + act[1]], axis=0)

            def large(k, w):
                p = fast_dot(SA, True, lambda r: wgu8_v[w, k, r], blocks_of(nb_v, SEG, DA), lb_v,
                             k + w == 0, sums=True)
                if w == 0:
                    gate.update(p)
                else:
                    for j in range(NA):
                        activate(tile_of(j, FA, k), (gate[0, j], gate[1, j]), (p[0, j], p[1, j]))

            def small():
                p = fast_dot(SB, True, lambda r: wgu4_v[r], blocks_of(nb_v, SEG, DB), sums=True)
                for j in range(NB):
                    activate(slice(F8 + j * LANES, F8 + (j + 1) * LANES),
                             [p[hf, j][:, :LANES] for hf in range(2)],
                             [p[hf, j][:, LANES:] for hf in range(2)])

            return [small] + [functools.partial(large, k, w) for k in range(NG) for w in range(2)]

        def down(hooks4=None, hooks8=None):
            acc = {}
            for k in range(DB // LANES):
                p = fast_dot(SB, True, lambda r: wd4_v[k, r], blocks_of(act_v, SEG, LANES, F8),
                             hooks=None if k else hooks4, sums=True)
                acc.update({(hf, j * (DB // LANES) + k): v for (hf, j), v in p.items()})
            acc = fast_dot(SA, True, lambda r: wd8_v[0, r], blocks_of(act_v, SEG, FA),
                           hooks=hooks8, sums=True, acc=acc)
            for (hf, j), v in acc.items():
                rows = slice(hf * SEG, (hf + 1) * SEG)
                z_v[rows, tile_of(j, DA, 0)] = ya_v[rows, tile_of(j, DA, 0)] + v

        def out_copy(row, n):
            return pltpu.make_async_copy(big_v.at[pl.ds(row, n), :],
                                         out_hbm.at[pl.ds(row, n), :], sem_out)

        def attention_single(mrow, xrow, yrow, before_out):
            ma_v[0:M, :] = mem_v[pl.ds(mrow, M), :]
            na_v[0:SEG, :] = _layernorm(xa_v[pl.ds(xrow, SEG), :])
            hooks = None
            for c in range(HB):
                scores, values = attention(c, False)
                project_qkv(0, c, False, hooks)
                project_qkv(1, c, False, None)
                project_qkv(2, c, False, spread(scores, cfg.get("a0", 20), cfg.get("a1", 7)))
                hooks = spread(values, cfg.get("a2", 24), cfg.get("a3", 9))
            for piece in values:
                piece()
            before_out()
            for c in range(DA // LANES):
                for j, v in project_out(c, False).items():
                    mem_v[pl.ds(mrow, M), tile_of(j, DA, c)] = v[:M]
                    ya_v[pl.ds(yrow, SEG), tile_of(j, DA, c)] = (
                        xa_v[pl.ds(xrow, SEG), tile_of(j, DA, c)] + v[M:])

        def step(t, carry):
            cur = pl.multiple_of(t * SEG, SEG)
            nxt = pl.multiple_of(jnp.minimum(t + 1, NSEG - 1) * SEG, SEG)
            pl.when(t + 1 == XH // SEG)(lambda: x_tail.wait())
            row = pl.multiple_of(jnp.maximum(t - 3, 0) * SEG, SEG)
            hooks = {cfg.get("g0", 2): glu_input}
            gpos = cfg.get("gpos", [1, 3, 4, 6, 7, 9, 10])
            glu = gate_up_pieces()
            for c in range(HB):
                scores, values = attention(c, True)
                for w in range(3):
                    project_qkv(w, c, True, (hooks, None, spread(
                        scores, cfg.get("h0", 20), cfg.get("s0", 10)))[w])
                    if 3 * c + w in gpos:
                        glu[gpos.index(3 * c + w)]()
                hooks = spread(values, cfg.get("h1", 20), cfg.get("s1", 10))
            down(None, spread(values, cfg.get("d0", 4), cfg.get("s2", 6)))
            big_v[pl.ds(row, SEG), :] = z_v[SEG:, :].astype(BF16)

            def next_input():
                na_v[SEG:, :] = _layernorm(z_v[:SEG, :])

            def next_tokens():
                na_v[:SEG, :] = _layernorm(x_v[pl.ds(nxt, SEG), :].astype(F32))

            next_tokens()
            for c in range(DA // LANES):
                o = project_out(c, True, {cfg.get("h2", 2): next_input} if c == 0 else None)
                for (hf, j), v in o.items():
                    cols = tile_of(j, DA, c)
                    res = x_v[pl.ds(cur, SEG), cols].astype(F32) if hf == 0 else xa_v[SEG:, cols]
                    ma_v[hf * M:(hf + 1) * M, cols] = v[:M]
                    ya_v[hf * SEG:(hf + 1) * SEG, cols] = res + v[M:]
            xa_v[SEG:, :] = z_v[:SEG, :]
            pl.when(t >= 3)(lambda: out_copy(row, SEG).start())
            return carry

        def phase(ph, carry):
            attention_single(pl.multiple_of(jnp.where(ph < 2, 0, M), M),
                             pl.multiple_of(jnp.where(ph == 0, 0, SEG), SEG),
                             pl.multiple_of(jnp.where(ph == 3, 1, ph) * SEG, SEG),
                             lambda: pl.when(ph == 0)(load_out_weights))
            pl.when(ph == 1)(load_gate_up_weights)

            @pl.when(ph >= 1)
            def _():
                glu_input()
                for piece in gate_up_pieces():
                    piece()
                pl.when(ph == 1)(load_down_weights)
                down()

            @pl.when(ph == 1)
            def _():
                ya_v[0:SEG, :] = ya_v[SEG:2 * SEG, :]
                xa_v[SEG:, :] = z_v[:SEG, :]
                ma_v[...] = mem_v[...]
                na_v[:SEG, :] = _layernorm(x_v[2 * SEG:3 * SEG, :].astype(F32))
                na_v[SEG:, :] = _layernorm(z_v[:SEG, :])
                lax.fori_loop(2, cfg.get("nsteps", NSEG), step, 0)
                mem_v[...] = ma_v[...]

            @pl.when(ph == 2)
            def _():
                xa_v[SEG:, :] = z_v[:SEG, :]
                ya_v[0:SEG, :] = ya_v[2 * SEG:, :]
                big_v[S - 3 * SEG:S - 2 * SEG, :] = z_v[SEG:, :].astype(BF16)
                out_copy(S - 3 * SEG, SEG).start()

            @pl.when(ph == 3)
            def _():
                big_v[S - 2 * SEG:S, :] = z_v[...].astype(BF16)
                out_copy(S - 2 * SEG, 2 * SEG).start()
            return carry

        lax.fori_loop(0, cfg.get('nph', 4), phase, 0)
        out_copy(0, cfg.get("nsteps", NSEG) * SEG).wait()

    scratch = [
        pltpu.VMEM((S, D), BF16),
        pltpu.VMEM((M, D), BF16),
        pltpu.VMEM((FF, D), BF16),
        pltpu.VMEM((2, GST, NA, GR, FF), BF16),
        pltpu.VMEM((QST, NA, (QR + 1) * H, DH), BF16),
        pltpu.VMEM((NA, H, QR, DH), BF16),
        pltpu.VMEM((3, HB, PA, DA // 2, DH), U32),
        pltpu.VMEM((DA // LANES, PA, EB // 2, LANES), U32),
        pltpu.VMEM((2, NG, PA, DA // 2, LANES), U32),
        pltpu.VMEM((PB, DB // 2, 2 * LANES), U32),
        pltpu.VMEM((1, PA, FA // 2, LANES), U32),
        pltpu.VMEM((DB // LANES, PB, LANES // 2, LANES), U32),
        pltpu.VMEM((PA, L, DA), F32),
        pltpu.VMEM((PA, SEG, DA), F32),
        pltpu.VMEM((3 * L, H * DH), F32),
        pltpu.VMEM((3 * SEG, FF), F32),
        pltpu.VMEM((2 * M, D), F32),
        pltpu.VMEM((2 * M, D), F32),
        pltpu.VMEM((2 * SEG, D), F32),
        pltpu.VMEM((2 * SEG, D), F32),
        pltpu.VMEM((3 * SEG, D), F32),
        pltpu.VMEM((3 * SEG, D), F32),
        pltpu.VMEM((2 * SEG, D), F32),
        pltpu.VMEM((NA, 2 * L, DH), F32),
        pltpu.VMEM((2, NA, LANES, DH), BF16),
        pltpu.VMEM((2 * L, LANES), F32),
        pltpu.VMEM((2 * L, LANES), jnp.int32),
        pltpu.SemaphoreType.DMA((3,)),
        pltpu.SemaphoreType.DMA((QST,)),
        pltpu.SemaphoreType.DMA((OST,)),
        pltpu.SemaphoreType.DMA((2, GST)),
        pltpu.SemaphoreType.DMA((GST,)),
        pltpu.SemaphoreType.DMA(()),
    ]
    return kernel, scratch


def _build(cfg):
    @functools.partial(jax.jit, static_argnames=("A_seg_len",))
    def fn(A_x, A_mem0, A_Wq, A_Wk, A_Wv, A_Wo, A_seg_len, B_x, B_w_gate, B_w_up, B_w_down):
        B, S, D = A_x.shape
        _, H, DH = A_Wq.shape
        M = A_mem0.shape[1]
        FF = B_w_gate.shape[1]
        kernel, scratch = _make_kernel(S, D, H, DH, M, A_seg_len, FF, cfg)
        any_spec = pl.BlockSpec(memory_space=pl.ANY)
        out = pl.pallas_call(
            kernel,
            out_shape=jax.ShapeDtypeStruct((S, D), A_x.dtype),
            in_specs=[any_spec] * 9,
            out_specs=any_spec,
            scratch_shapes=scratch,
            compiler_params=pltpu.CompilerParams(vmem_limit_bytes=cfg.get("vmem", 126) * 1024 * 1024,
                                                 flags=cfg.get("flags")),
        )(A_x.reshape(S, D), A_mem0.reshape(M, D),
          A_Wq.reshape(D * H, DH), A_Wk.reshape(D * H, DH), A_Wv.reshape(D * H, DH),
          A_Wo.reshape(H * DH, D), B_w_gate, B_w_up, B_w_down)
        return out.reshape(B, S, D)
    return fn


pallas_interleave_layers__memory_aug_recurrent_mem_tr__glu_gated_glu__prompt_kernel = _build({})
```

```python
import functools
import math

import jax
import jax.numpy as jnp
import numpy as np
from jax import lax
import jax.experimental.pallas as pl
import jax.experimental.pallas.tpu as pltpu

F32 = jnp.float32
BF16 = jnp.bfloat16
U32 = jnp.uint32
EPS = 1e-05
LANES = 128

_SCHEME_4 = """
+00 | +00 +02 -10 +30 | +00 -10
+00 +10 | +00 -01 +20 -30 | +10

+00 -11 | +01 -10 +30 | +01 +10
+10 +11 | +01 | +10 +11
+00 +01 | +03 +10 -30 | +00 +01

+00 +10 +11 +13 | +30 | -00 -01 +03 +10
+00 +01 +03 +10 +11 +13 | -03 +30 | +00 +01 -03
+03 +10 +11 +13 | +03 | +00 +01 -03 +13

+00 +10 -12 | +02 -20 | -00 +02 +10
+10 -12 | +02 | +00 -02 -10 +12
+00 -02 +10 -12 | +20 | -00 +02

+11 | +01 -11 -12 +31 | +01 -11
+01 +11 | -03 -10 +11 +13 -21 +30 | +01

-03 +11 | -03 +13 +31 | -01 +13
+01 +03 | -03 +13 +30 | -01 +03
+11 +13 | +31 | +11 -13

+01 +02 +11 | +12 +21 | +01 -11 +12
+01 +02 | +12 | -01 +02 +11 -12
+01 +02 +11 +12 | +21 | +11 -12

+03 +12 +13 | -23 -32 | -02 +03 -13
+02 +03 +12 +13 | +23 | -02 +03
+12 +13 | +32 | -02 +03 +12 -13

+02 | -12 +20 +22 +23 | +02
+12 | +02 +21 +22 -32 | +12

+03 | +03 -13 +32 +33 | +03 -13
+03 +13 | -03 -23 +31 +33 | +13
"""
_SCHEME_8 = """
+01 +10 | +01 +10 | +00 +11
+00 -01 | +01 | +00 +01
+10 -11 | +10 | -10 -11

+00 +02 +10 | +02 +20 | +00 -10 +12
+00 +02 | +02 | -00 +02 +10 -12
+00 +02 +10 +12 | +20 | +10 -12

+00 +03 -04 +10 | +30 | +00 -10 -13 -14
+00 +03 -04 +10 +13 -14 | +03 +30 | +10 +13 +14
+00 +03 -04 +13 | +03 | +03 -10 -13 -14

+04 +10 | +04 +30 +40 -74 | +00 +14
+00 -04 | +04 -47 -74 | +00 +04
+10 -14 | -03 -30 -40 | +10 +14

+00 -05 +10 | +05 +50 | -00 +10 +15
+00 -05 | +05 | +00 +05 -10 -15
+00 -05 +10 -15 | +50 | -10 -15

+00 +06 +07 +10 | +60 | +00 -10 -16 +17
+00 +06 +07 +10 +16 +17 | +06 +60 | +10 +16 -17
+00 +06 +07 +16 | +06 | +06 -10 -16 +17

-07 +10 | +07 +47 -60 +70 | -00 +17
+00 +07 | +07 +47 +74 | -00 +07
+10 +17 | +06 +60 -70 | -10 +17

+10 | -00 -02 +05 -10 -30 -40 -60 +70 | +00 -10
+00 +10 | +00 -01 -04 +07 -20 -30 +47 +50 -60 +74 | +00

+01 +11 -12 | +12 +21 | +01 +02 -11
+11 -12 | +12 | -01 -02 +11 +12
+01 -02 +11 -12 | +21 | -01 -02

+01 +13 | +13 +31 +63 -71 | +03 +11
+11 -13 | +13 -36 +63 | +11 +13
+01 -03 | -17 -31 +71 | +01 +03

+01 +11 +14 -16 | +41 | -01 +04 +06 +11
+01 +04 -06 +11 +14 -16 | -14 +41 | +01 -04 -06
+04 +11 +14 -16 | +14 | +01 -04 -06 +14

+01 +11 +15 | +15 -51 | +01 +05 -11
+11 +15 | +15 | -01 -05 +11 +15
+01 +05 +11 +15 | +51 | +01 +05

+01 +16 | +16 +36 -41 -61 | +06 -11
+11 -16 | +16 +36 -63 | -11 +16
+01 -06 | -14 +41 +61 | -01 +06

+01 +11 -13 -17 | +71 | +01 +03 +07 -11
+01 -03 -07 +11 -13 -17 | +17 -71 | +01 +03 +07
-07 +11 -13 -17 | +17 | -01 -03 -07 +17

+01 | +01 +11 -12 -15 +31 +41 +61 -71 | +01 -11
+01 +11 | -10 +11 -13 +16 +21 +36 -41 -51 -63 +71 | +11

+02 +03 +13 | +23 -32 -52 | +03 -12 -13
+02 +03 +12 +13 | +23 | +12 +13
+02 +03 | +25 +32 +52 | +02 +03 -12 -13

-04 +12 -14 | -24 -42 | +02 +04 -14
+02 -04 +12 -14 | +24 | +02 +04
+12 -14 | +42 | +02 +04 -12 -14

+03 -05 +12 +13 -15 | +52 | -02 -03 +05 +13 -15
+12 +13 -15 | +25 +52 | +02 +03 -05 -12 -13 +15
+02 +03 +12 +13 -15 | +25 | -02 -03 +05 +12 +13

+02 +06 +16 | +26 -62 | +06 -12 -16
+02 +06 +12 +16 | +26 | +12 +16
+02 +06 | +62 | +02 +06 -12 -16

+07 +12 +17 | -27 -72 | -02 +07 -17
+02 +07 +12 +17 | +27 | -02 +07
+12 +17 | +72 | -02 +07 +12 -17

+02 | -02 -21 +22 -24 +27 -32 -52 -62 | +02
+12 | +12 +20 +22 -23 -26 +42 +52 -72 | +12

+04 +13 | +03 +34 +43 | +03 +14
+03 -04 | +34 | +03 +04
+13 -14 | -03 -30 -43 | +13 +14

+03 -05 +13 | -25 +35 -53 | +03 -13 +15
+03 -05 | -25 +35 -52 | -03 +05 +13 -15
+03 -05 +13 -15 | +53 | -13 +15

-01 +03 +06 +13 | +63 | +03 -11 -13 +16
-01 +03 +06 -11 +13 +16 | -36 +63 | +11 +13 -16
-01 +03 +06 +16 | +36 | +06 +11 +13 -16

-07 +13 | +17 +37 -73 | +03 +17
+03 +07 | +17 +37 -71 | +03 +07
+13 +17 | +73 | +13 +17

+13 | -03 -13 +25 +32 -33 -35 -43 +52 -63 +73 | +03 -13
+03 +13 | -03 -17 -23 -31 +33 -34 -37 +53 -63 +71 | +03

+04 +14 +15 | +45 -54 | +04 +05 -14
+14 +15 | +45 | -04 -05 +14 +15
+04 +05 +14 +15 | +54 | +04 +05

+04 +16 | +14 +46 +64 | +06 +14
+14 -16 | +46 | +14 +16
+04 -06 | -14 +41 -64 | +04 +06

+04 -10 +14 -17 | +74 | +00 +04 -07 -14
-00 +04 -07 -10 +14 -17 | -47 -74 | +00 +04 -07
-07 -10 +14 -17 | +47 | +00 +04 -07 +17

+04 | +04 +14 +34 -42 +44 -45 +64 -74 | +04 -14
+04 +14 | -03 -14 +24 -30 -40 -43 +44 -46 -54 +74 | +14

+05 +06 +16 | +56 -65 | +06 -15 -16
+05 +06 +15 +16 | +56 | +15 +16
+05 +06 | +65 | +05 +06 -15 -16

+07 +15 +17 | -57 -75 | -05 +07 -17
+05 +07 +15 +17 | +57 | -05 +07
+15 +17 | +75 | -05 +07 +15 -17

+05 | +05 -25 +35 -51 -54 +55 +57 -65 | +05
+15 | -15 +25 -45 -50 +53 +55 -56 -75 | +15

-07 +16 | -06 +67 +76 | -06 +17
+06 +07 | +67 | -06 +07
+16 +17 | +06 +60 -76 | -16 +17

+16 | -06 -16 -36 -46 +62 +65 -66 +76 | +06 -16
+06 +16 | -06 -14 -26 -36 +41 -56 +61 -64 +66 +67 | +06

+07 | -07 -17 -37 -47 -67 +72 +75 +77 | +07 -17
+07 +17 | -06 +17 -27 +47 -57 -60 +70 -73 +76 +77 | +17
"""


class _Scheme:
    def __init__(self, n, text):
        def terms(field):
            return {(int(t[1]), int(t[2])): 1 if t[0] == "+" else -1 for t in field.split()}

        def fold(coefs, weights):
            out = {}
            for (h, i), c in coefs.items():
                out[i] = out.get(i, 0) + weights[h] * c
            return {i: c for i, c in out.items() if c}

        self.n = n
        self.prods, self.ends = [], []
        for group in text.strip().split("\n\n"):
            self.prods += [tuple(terms(f) for f in line.split("|")) for line in group.split("\n")]
            self.ends.append(len(self.prods) - 1)
        folded = [(fold(u, (-1, 1)), fold(w, (0, 1))) for u, _, w in self.prods]
        self.single = [(u, w) if u and w else None for u, w in folded]


def _combine(coefs, vals):
    acc = None
    for key, c in sorted(coefs.items(), key=lambda kv: -kv[1]):
        v = vals[key]
        if abs(c) != 1:
            v = v * abs(c)
        if acc is None:
            acc = v if c > 0 else -v
        else:
            acc = acc + v if c > 0 else acc - v
    return acc


def _accumulate(accs, group):
    terms = {}
    for n, (coefs, _) in enumerate(group):
        for key, c in coefs.items():
            terms.setdefault(key, []).append((n, c))
    sums = {((n, 1),): v for n, (_, v) in enumerate(group)}
    for key, tm in sorted(terms.items(), key=lambda kv: len(kv[1])):
        sign = tm[0][1]
        tm = tuple((n, c * sign) for n, c in tm)
        if tm not in sums:
            base = max((s for s in sums if all(t in tm for t in s)), key=len)
            val = sums[base]
            for n, c in tm:
                if (n, c) not in base:
                    val = val + group[n][1] if c > 0 else val - group[n][1]
            sums[tm] = val
        if key not in accs:
            accs[key] = sums[tm] if sign > 0 else -sums[tm]
        else:
            accs[key] = accs[key] + sums[tm] if sign > 0 else accs[key] - sums[tm]


def _layernorm(x, gain=1.0):
    m = jnp.mean(x, axis=-1, keepdims=True)
    c = x - m
    v = jnp.mean(c * c, axis=-1, keepdims=True)
    inv = lax.rsqrt(v + EPS)
    return c * (inv if gain == 1.0 else inv * gain)


def _dot(a, b):
    return lax.dot_general(a, b, (((1,), (0,)), ((), ())), preferred_element_type=F32)


def _dot_nt(a, b):
    return lax.dot_general(a, b, (((1,), (1,)), ((), ())), preferred_element_type=F32)


def _halves(x):
    return [pltpu.unpack_elementwise(x, index=k, packed_dtype=BF16, unpacked_dtype=F32)
            for k in range(2)]


def _pair(lo, hi):
    return pltpu.pack_elementwise([lo, hi], packed_dtype=BF16)


def _make_kernel(S, D, H, DH, M, SEG, FF, cfg):
    SA = _Scheme(8, _SCHEME_8)
    SB = _Scheme(4, _SCHEME_4)
    NA, NB = SA.n, SB.n
    PA, PB = len(SA.prods), len(SB.prods)
    NSEG = S // SEG
    L = M + SEG
    DA, HB = D // NA, H // NA
    EB = HB * DH
    NG = FF // (NA * LANES)
    FA = NG * LANES
    F8 = NA * FA
    DB = D // NB
    assert DA == LANES and DH == LANES and FF - F8 == NB * LANES
    QR = cfg.get("QR", 128) // NA
    QST = cfg.get("QST", 4)
    WR = 512 // NA
    OST = FF // (WR * NA)
    GST = 4
    GR, DR, ER = DA // GST, FA // GST, LANES // GST
    XH = 4 * SEG
    scale = DH ** (-0.5)
    c_exp = scale * math.log2(math.e)

    def fast_dot(sch, paired, w_of, block, kept_ref=None, fresh=True, hooks=None, sums=False,
                 acc=None):
        acc, group = dict(acc or {}), []
        for r, (u, _, w) in enumerate(sch.prods):
            if hooks and r in hooks:
                hooks[r]()
            if paired or sch.single[r]:
                if not paired:
                    u, w = sch.single[r]
                if fresh:
                    if not paired:
                        u = {(0, i): c for i, c in u.items()}
                    elif sums:
                        u = {(2 if u.get((1 - hf, i)) == c else hf, i): c
                             for (hf, i), c in u.items()}
                    lhs = _combine(u, {key: block(*key) for key in u})
                    if kept_ref is not None:
                        kept_ref[r] = lhs
                else:
                    lhs = kept_ref[r]
                group.append((w, _dot(lhs, pltpu.bitcast(w_of(r), BF16))))
            if r in sch.ends:
                _accumulate(acc, group)
                group = []
        return acc

    def blocks_of(ref, rows, cols, c0=0):
        return lambda hf, i: ref[hf * rows:(hf + 1) * rows, c0 + i * cols:c0 + (i + 1) * cols]

    def spread(pieces, first, stride):
        return {first + n * stride: piece for n, piece in enumerate(pieces)}

    def tile_of(j, blk, c):
        return slice(j * blk + c * LANES, j * blk + (c + 1) * LANES)

    def kernel(x_hbm, mem0_hbm, wq_hbm, wk_hbm, wv_hbm, wo_hbm, wg_hbm, wu_hbm, wd_hbm,
               out_hbm,
               x_v, mem0_v, big_v, gst_v, qst_v, qtr_v, wqkv_v, wo_v, wgu8_v, wgu4_v, wd8_v, wd4_v,
               la_v, lb_v, o_v, act_v, mem_v, ma_v, xa_v, na_v, nb_v, ya_v, z_v, q_v, kv_v, fill_v, keep_v,
               sem_x, sem_q, sem_o, sem_g, sem_d, sem_out):

        def rows_at(start, size):
            return pl.ds(start if isinstance(start, int) else pl.multiple_of(start, 16), size)

        def q_copies(w, c, slot):
            src = (wq_hbm, wk_hbm, wv_hbm)[w]
            return [pltpu.make_async_copy(src.at[rows_at((i * DA + c * QR) * H, QR * H), :],
                                          qst_v.at[slot, i, 0:QR * H, :], sem_q.at[slot])
                    for i in range(NA)]

        def o_copies(c):
            slot = c % OST
            return [pltpu.make_async_copy(wo_hbm.at[rows_at(i * EB + c * WR, WR), :],
                                          big_v.at[rows_at((slot * NA + i) * WR, WR), :],
                                          sem_o.at[slot]) for i in range(NA)]

        def g_copies(w, c):
            return [pltpu.make_async_copy((wg_hbm, wu_hbm)[w].at[rows_at(i * DA + c * GR, GR), :],
                                          gst_v.at[w, c, i], sem_g.at[w, c]) for i in range(NA)]

        def d_copies(c):
            rows = ([rows_at(i * FA + c * DR, DR) for i in range(NA)]
                    + [rows_at(F8 + i * LANES + c * ER, ER) for i in range(NB)])
            return [pltpu.make_async_copy(wd_hbm.at[r, :], big_v.at[r, :], sem_d.at[c])
                    for r in rows]

        def start(copies):
            for cp in copies:
                cp.start()

        def wait(copies):
            for cp in copies:
                cp.wait()

        def prep_tiles(sch, load, put, nrows, ncols):
            def tile(_, pos):
                s, k = pos
                words = {}
                for r, (_, v, _) in enumerate(sch.prods):
                    for key in v:
                        if key not in words or sch.n > 4:
                            words[key] = pltpu.bitcast(
                                load(*key, pl.multiple_of(s * 16, 16), k), U32)
                    if len(v) == 1:
                        put(r, s * 8, k, words[next(iter(v))])
                    else:
                        halves = {key: _halves(words[key]) for key in v}
                        put(r, s * 8, k, _pair(*(
                            _combine(v, {key: hv[p] for key, hv in halves.items()})
                            for p in range(2))))
                wrap = k + 1 == ncols
                return jnp.where(wrap, s + 1, s), jnp.where(wrap, 0, k + 1)
            lax.fori_loop(0, nrows // 16 * ncols, tile, (0, 0))

        def lanes_at(k):
            return pl.ds(pl.multiple_of(k * LANES, LANES), LANES)

        def words_at(row):
            return pl.ds(pl.multiple_of(row, 8), 8)

        def prep_qkv(w, c, slot):
            def heads(i, carry):
                st = qst_v.at[slot, i].bitcast(U32)
                for jp in range(H // 2):
                    for k, x in enumerate(_halves(st[pl.ds(jp, QR, stride=H // 2), :])):
                        qtr_v[i, 2 * jp + k] = x.astype(BF16)
                return carry
            lax.fori_loop(0, NA, heads, 0)

            def put(r, row, k, val):
                wqkv_v[w, k, r, words_at(c * (QR // 2) + row), :] = val
            prep_tiles(SA, lambda i, j, row, k: qtr_v[i, j * HB + k, pl.ds(row, 16), :], put, QR, HB)

        def prep_from_big(sch, dst, base, blk, c, nrows):
            ncols = D // sch.n // LANES

            def load(i, j, row, k):
                return big_v[rows_at(base + i * blk + row, 16), lanes_at(j * ncols + k)]

            def put(r, row, k, val):
                dst[k, r, words_at(c * (nrows // 2) + row), :] = val
            prep_tiles(sch, load, put, nrows, ncols)

        def prep_gu(w, c):
            def put8(r, row, k, val):
                wgu8_v[w, k, r, words_at(c * (GR // 2) + row), :] = val
            prep_tiles(SA, lambda i, j, row, k: gst_v[w, c, i, pl.ds(row, 16),
                                                      lanes_at(j * NG + k)], put8, GR, NG)

            def put4(r, row, k, val):
                rows = words_at(k * (DA // 2) + c * (GR // 2) + row)
                wgu4_v[r, rows, w * LANES:(w + 1) * LANES] = val
            prep_tiles(SB, lambda i, j, row, k: gst_v[w, c, 2 * i + k, pl.ds(row, 16),
                                                      F8 + j * LANES:F8 + (j + 1) * LANES],
                       put4, GR, 2)

        x_head = pltpu.make_async_copy(x_hbm.at[0:XH, :], x_v.at[0:XH, :], sem_x.at[0])
        x_tail = pltpu.make_async_copy(x_hbm.at[XH:, :], x_v.at[XH:, :], sem_x.at[1])
        NQ, NO = DA // QR, EB // WR
        AHEAD = cfg.get('oa', 5)
        assert QST <= min(NQ, AHEAD) and AHEAD <= OST <= NO
        for n in range(QST):
            start(q_copies(0, n, n))
        mem0_copy = pltpu.make_async_copy(mem0_hbm, mem0_v, sem_x.at[2])
        x_head.start()
        mem0_copy.start()

        ri = lax.broadcasted_iota(jnp.int32, (2 * L, LANES), 0)
        ci = lax.broadcasted_iota(jnp.int32, (2 * L, LANES), 1)
        first = jnp.where(ri < L, 0, L)
        same = (ci >= first) & (ci < first + L)
        visible = (ri < first + M) | (ri >= ci)
        keep_v[...] = (same & visible).astype(jnp.int32)
        fill_v[...] = jnp.where(same, -1e9 / scale, -jnp.inf).astype(F32)
        kv_v[...] = jnp.zeros(kv_v.shape, BF16)

        for w in range(3):
            def q_body(c, carry, w=w):
                slot = (w * NQ + c) % QST
                wait(q_copies(w, c, slot))
                prep_qkv(w, c, slot)
                pl.when(c + QST < NQ)(lambda: start(q_copies(w, c + QST, slot)))
                if w < 2:
                    pl.when(c + QST >= NQ)(lambda: start(q_copies(w + 1, c + QST - NQ, slot)))
                else:
                    pl.when(c + QST >= NQ)(lambda: start(o_copies(c + QST - NQ)))
                return carry
            lax.fori_loop(0, NQ, q_body, 0)

        for c in range(QST, AHEAD):
            start(o_copies(c))
        x_head.wait()
        mem0_copy.wait()
        xa_v[...] = x_v[0:2 * SEG, :].astype(F32)
        mem_v[0:M, :] = mem0_v[...].astype(F32)
        mem_v[M:, :] = mem0_v[...].astype(F32)

        def load_out_weights():
            def chunk(c, carry):
                wait(o_copies(c))
                prep_from_big(SA, wo_v, (c % OST) * NA * WR, WR, c, WR)
                pl.when(c + AHEAD < NO)(lambda: start(o_copies(c + AHEAD)))
                pl.when(c >= NO - 2)(lambda: start(g_copies(0, c - (NO - 2))))
                return carry
            lax.fori_loop(0, NO, chunk, 0)
            for c in range(2, GST):
                start(g_copies(0, c))
            start(g_copies(1, 0))

        def load_gate_up_weights():
            def gate(c, carry):
                pl.when(c + 1 < GST)(lambda: start(g_copies(1, c + 1)))
                wait(g_copies(0, c))
                prep_gu(0, c)
                return carry

            def up(c, carry):
                wait(g_copies(1, c))
                prep_gu(1, c)
                start(d_copies(c))
                return carry
            lax.fori_loop(0, GST, gate, 0)
            lax.fori_loop(0, GST, up, 0)

        def load_down_weights():
            def chunk(c, carry):
                wait(d_copies(c))
                pl.when(c == cfg.get("xt", GST - 1))(lambda: x_tail.start())
                prep_from_big(SA, wd8_v, c * DR, FA, c, DR)
                prep_from_big(SB, wd4_v, F8 + c * ER, LANES, c, ER)
                return carry
            lax.fori_loop(0, GST, chunk, 0)

        def attention(c, paired):
            n = 2 * L if paired else L
            probs = {}

            def scores(j):
                s = _dot_nt(q_v[j, 0:n, :], kv_v[0, j])
                s = jnp.where(keep_v[0:n, :] != 0, s, fill_v[0:n, :])
                mx = jnp.max(s, axis=-1, keepdims=True)
                e = jnp.exp2((s - mx) * c_exp)
                den = jnp.sum(e, axis=-1, keepdims=True)
                inv = pl.reciprocal(den, approx=True)
                inv = inv * (2.0 - den * inv)
                probs[j] = e * inv

            def values(j):
                o = _dot(probs[j], kv_v[1, j])
                o_v[0:n, tile_of(j, EB, c)] = o
                if paired:
                    o_v[n:, tile_of(j, EB, c)] = o[:L] + o[L:]

            return ([functools.partial(scores, j) for j in range(NA)],
                    [functools.partial(values, j) for j in range(NA)])

        def project_qkv(w, c, paired, hooks):
            def block(hf, i):
                cols = slice(i * DA, (i + 1) * DA)
                if hf == 2:
                    return jnp.concatenate([ma_v[0:M, cols] + ma_v[M:, cols],
                                            na_v[2 * SEG:, cols]], axis=0)
                return jnp.concatenate([ma_v[hf * M:(hf + 1) * M, cols],
                                        na_v[hf * SEG:(hf + 1) * SEG, cols]], axis=0)

            p = fast_dot(SA, paired, lambda r: wqkv_v[w, c, r], block, la_v, w + c == 0, hooks,
                         sums=True)
            for j in range(NA):
                x = jnp.concatenate([p[0, j], p[1, j]], axis=0) if paired else p[j]
                if w == 0:
                    q_v[j, 0:x.shape[0], :] = x
                else:
                    kv_v[w - 1, j, 0:x.shape[0], :] = x.astype(BF16)

        def project_out(c, paired, hooks=None):
            return fast_dot(SA, paired, lambda r: wo_v[c, r], blocks_of(o_v, L, EB),
                            hooks=hooks, sums=True)

        def glu_input():
            nb = _layernorm(ya_v[0:2 * SEG, :], 0.5)
            nb_v[...] = jnp.concatenate([nb, nb[:SEG] + nb[SEG:]], axis=0)

        def gate_up_pieces():
            gate = {}

            def activate(cols, g, u):
                act = [jnp.tanh(g[hf]) * u[hf] + u[hf] for hf in range(2)]
                act_v[:, cols] = jnp.concatenate(act + [act[0] + act[1]], axis=0)

            def large(k, w):
                p = fast_dot(SA, True, lambda r: wgu8_v[w, k, r], blocks_of(nb_v, SEG, DA), lb_v,
                             k + w == 0, sums=True)
                if w == 0:
                    gate.update(p)
                else:
                    for j in range(NA):
                        activate(tile_of(j, FA, k), (gate[0, j], gate[1, j]), (p[0, j], p[1, j]))

            def small():
                p = fast_dot(SB, True, lambda r: wgu4_v[r], blocks_of(nb_v, SEG, DB), sums=True)
                for j in range(NB):
                    activate(slice(F8 + j * LANES, F8 + (j + 1) * LANES),
                             [p[hf, j][:, :LANES] for hf in range(2)],
                             [p[hf, j][:, LANES:] for hf in range(2)])

            return [small] + [functools.partial(large, k, w) for k in range(NG) for w in range(2)]

        def down_small():
            acc = {}
            for k in range(DB // LANES):
                p = fast_dot(SB, True, lambda r: wd4_v[k, r], blocks_of(act_v, SEG, LANES, F8),
                             sums=True)
                acc.update({(hf, j * (DB // LANES) + k): v for (hf, j), v in p.items()})
            for (hf, j), v in acc.items():
                rows = slice(hf * SEG, (hf + 1) * SEG)
                z_v[rows, tile_of(j, DA, 0)] = ya_v[rows, tile_of(j, DA, 0)] + v

        def down_large(hooks=None):
            acc = fast_dot(SA, True, lambda r: wd8_v[0, r], blocks_of(act_v, SEG, FA),
                           hooks=hooks, sums=True)
            for (hf, j), v in acc.items():
                z_v[hf * SEG:(hf + 1) * SEG, tile_of(j, DA, 0)] += v

        def out_copy(row, n):
            return pltpu.make_async_copy(big_v.at[pl.ds(row, n), :],
                                         out_hbm.at[pl.ds(row, n), :], sem_out)

        def attention_single(mrow, xrow, yrow, before_out):
            ma_v[0:M, :] = mem_v[pl.ds(mrow, M), :]
            na_v[0:SEG, :] = _layernorm(xa_v[pl.ds(xrow, SEG), :])
            hooks = None
            for c in range(HB):
                scores, values = attention(c, False)
                project_qkv(0, c, False, hooks)
                project_qkv(1, c, False, None)
                project_qkv(2, c, False, spread(scores, cfg.get("a0", 20), cfg.get("a1", 7)))
                hooks = spread(values, cfg.get("a2", 24), cfg.get("a3", 9))
            for piece in values:
                piece()
            before_out()
            for c in range(DA // LANES):
                for j, v in project_out(c, False).items():
                    mem_v[pl.ds(mrow, M), tile_of(j, DA, c)] = v[:M]
                    ya_v[pl.ds(yrow, SEG), tile_of(j, DA, c)] = (
                        xa_v[pl.ds(xrow, SEG), tile_of(j, DA, c)] + v[M:])

        def step(t, carry):
            cur = pl.multiple_of(t * SEG, SEG)
            nxt = pl.multiple_of(jnp.minimum(t + 1, NSEG - 1) * SEG, SEG)
            pl.when(t + 1 == XH // SEG)(lambda: x_tail.wait())
            row = pl.multiple_of(jnp.maximum(t - 3, 0) * SEG, SEG)
            hooks = {cfg.get("g0", 50): glu_input}
            gpos = cfg.get("gpos", [1, 3, 4, 6, 7, 9, 10])
            def next_tokens():
                na_v[:SEG, :] = _layernorm(x_v[pl.ds(nxt, SEG), :].astype(F32))

            glu = gate_up_pieces()
            for c in range(HB):
                scores, values = attention(c, True)
                for w in range(3):
                    project_qkv(w, c, True, (hooks, None, spread(
                        scores, cfg.get("h0", 20), cfg.get("s0", 10)))[w])
                    if 3 * c + w in gpos:
                        glu[gpos.index(3 * c + w)]()
                    if 3 * c + w == cfg.get('dp', 5):
                        down_small()
                hooks = spread(values, cfg.get("h1", 26), cfg.get("s1", 10))
                if c == cfg.get('nt', 2):
                    hooks[5] = next_tokens
            down_large(spread(values, cfg.get("d0", 12), cfg.get("s2", 8)))
            big_v[pl.ds(row, SEG), :] = z_v[SEG:, :].astype(BF16)

            def next_input():
                na = _layernorm(z_v[:SEG, :])
                na_v[SEG:, :] = jnp.concatenate([na, na + na_v[:SEG, :]], axis=0)

            for c in range(DA // LANES):
                o = project_out(c, True, {cfg.get("h2", 2): next_input} if c == 0 else None)
                for (hf, j), v in o.items():
                    cols = tile_of(j, DA, c)
                    res = x_v[pl.ds(cur, SEG), cols].astype(F32) if hf == 0 else xa_v[SEG:, cols]
                    ma_v[hf * M:(hf + 1) * M, cols] = v[:M]
                    ya_v[hf * SEG:(hf + 1) * SEG, cols] = res + v[M:]
            xa_v[SEG:, :] = z_v[:SEG, :]
            pl.when(t >= 3)(lambda: out_copy(row, SEG).start())
            return carry

        def phase(ph, carry):
            attention_single(pl.multiple_of(jnp.where(ph < 2, 0, M), M),
                             pl.multiple_of(jnp.where(ph == 0, 0, SEG), SEG),
                             pl.multiple_of(jnp.where(ph == 3, 1, ph) * SEG, SEG),
                             lambda: pl.when(ph == 0)(load_out_weights))
            pl.when(ph == 1)(load_gate_up_weights)

            @pl.when(ph >= 1)
            def _():
                glu_input()
                for piece in gate_up_pieces():
                    piece()
                pl.when(ph == 1)(load_down_weights)
                down_small()
                down_large()

            @pl.when(ph == 1)
            def _():
                ya_v[0:SEG, :] = ya_v[SEG:2 * SEG, :]
                xa_v[SEG:, :] = z_v[:SEG, :]
                ma_v[...] = mem_v[...]
                na_v[:SEG, :] = _layernorm(x_v[2 * SEG:3 * SEG, :].astype(F32))
                na = _layernorm(z_v[:SEG, :])
                na_v[SEG:, :] = jnp.concatenate([na, na + na_v[:SEG, :]], axis=0)
                lax.fori_loop(2, cfg.get("nsteps", NSEG), step, 0)
                mem_v[...] = ma_v[...]

            @pl.when(ph == 2)
            def _():
                xa_v[SEG:, :] = z_v[:SEG, :]
                ya_v[0:SEG, :] = ya_v[2 * SEG:, :]
                big_v[S - 3 * SEG:S - 2 * SEG, :] = z_v[SEG:, :].astype(BF16)
                out_copy(S - 3 * SEG, SEG).start()

            @pl.when(ph == 3)
            def _():
                big_v[S - 2 * SEG:S, :] = z_v[...].astype(BF16)
                out_copy(S - 2 * SEG, 2 * SEG).start()
            return carry

        lax.fori_loop(0, cfg.get('nph', 4), phase, 0)
        out_copy(0, cfg.get("nsteps", NSEG) * SEG).wait()

    scratch = [
        pltpu.VMEM((S, D), BF16),
        pltpu.VMEM((M, D), BF16),
        pltpu.VMEM((FF, D), BF16),
        pltpu.VMEM((2, GST, NA, GR, FF), BF16),
        pltpu.VMEM((QST, NA, (QR + 1) * H, DH), BF16),
        pltpu.VMEM((NA, H, QR, DH), BF16),
        pltpu.VMEM((3, HB, PA, DA // 2, DH), U32),
        pltpu.VMEM((DA // LANES, PA, EB // 2, LANES), U32),
        pltpu.VMEM((2, NG, PA, DA // 2, LANES), U32),
        pltpu.VMEM((PB, DB // 2, 2 * LANES), U32),
        pltpu.VMEM((1, PA, FA // 2, LANES), U32),
        pltpu.VMEM((DB // LANES, PB, LANES // 2, LANES), U32),
        pltpu.VMEM((PA, L, DA), F32),
        pltpu.VMEM((PA, SEG, DA), F32),
        pltpu.VMEM((3 * L, H * DH), F32),
        pltpu.VMEM((3 * SEG, FF), F32),
        pltpu.VMEM((2 * M, D), F32),
        pltpu.VMEM((2 * M, D), F32),
        pltpu.VMEM((2 * SEG, D), F32),
        pltpu.VMEM((3 * SEG, D), F32),
        pltpu.VMEM((3 * SEG, D), F32),
        pltpu.VMEM((3 * SEG, D), F32),
        pltpu.VMEM((2 * SEG, D), F32),
        pltpu.VMEM((NA, 2 * L, DH), F32),
        pltpu.VMEM((2, NA, LANES, DH), BF16),
        pltpu.VMEM((2 * L, LANES), F32),
        pltpu.VMEM((2 * L, LANES), jnp.int32),
        pltpu.SemaphoreType.DMA((3,)),
        pltpu.SemaphoreType.DMA((QST,)),
        pltpu.SemaphoreType.DMA((OST,)),
        pltpu.SemaphoreType.DMA((2, GST)),
        pltpu.SemaphoreType.DMA((GST,)),
        pltpu.SemaphoreType.DMA(()),
    ]
    return kernel, scratch


def _build(cfg):
    @functools.partial(jax.jit, static_argnames=("A_seg_len",))
    def fn(A_x, A_mem0, A_Wq, A_Wk, A_Wv, A_Wo, A_seg_len, B_x, B_w_gate, B_w_up, B_w_down):
        B, S, D = A_x.shape
        _, H, DH = A_Wq.shape
        M = A_mem0.shape[1]
        FF = B_w_gate.shape[1]
        kernel, scratch = _make_kernel(S, D, H, DH, M, A_seg_len, FF, cfg)
        any_spec = pl.BlockSpec(memory_space=pl.ANY)
        out = pl.pallas_call(
            kernel,
            out_shape=jax.ShapeDtypeStruct((S, D), A_x.dtype),
            in_specs=[any_spec] * 9,
            out_specs=any_spec,
            scratch_shapes=scratch,
            compiler_params=pltpu.CompilerParams(vmem_limit_bytes=cfg.get("vmem", 126) * 1024 * 1024,
                                                 flags=cfg.get("flags")),
        )(A_x.reshape(S, D), A_mem0.reshape(M, D),
          A_Wq.reshape(D * H, DH), A_Wk.reshape(D * H, DH), A_Wv.reshape(D * H, DH),
          A_Wo.reshape(H * DH, D), B_w_gate, B_w_up, B_w_down)
        return out.reshape(B, S, D)
    return fn


pallas_interleave_layers__memory_aug_recurrent_mem_tr__glu_gated_glu__prompt_kernel = _build({})
```

```python
import functools
import itertools
import math

import jax
import jax.numpy as jnp
import numpy as np
from jax import lax
import jax.experimental.pallas as pl
import jax.experimental.pallas.tpu as pltpu

F32 = jnp.float32
BF16 = jnp.bfloat16
U32 = jnp.uint32
EPS = 1e-05
LANES = 128

_SCHEME_4 = """
+00 | +00 +02 -10 +30 | +00 -10
+00 +10 | +00 -01 +20 -30 | +10

+00 -11 | +01 -10 +30 | +01 +10
+10 +11 | +01 | +10 +11
+00 +01 | +03 +10 -30 | +00 +01

+00 +10 +11 +13 | +30 | -00 -01 +03 +10
+00 +01 +03 +10 +11 +13 | -03 +30 | +00 +01 -03
+03 +10 +11 +13 | +03 | +00 +01 -03 +13

+00 +10 -12 | +02 -20 | -00 +02 +10
+10 -12 | +02 | +00 -02 -10 +12
+00 -02 +10 -12 | +20 | -00 +02

+11 | +01 -11 -12 +31 | +01 -11
+01 +11 | -03 -10 +11 +13 -21 +30 | +01

-03 +11 | -03 +13 +31 | -01 +13
+01 +03 | -03 +13 +30 | -01 +03
+11 +13 | +31 | +11 -13

+01 +02 +11 | +12 +21 | +01 -11 +12
+01 +02 | +12 | -01 +02 +11 -12
+01 +02 +11 +12 | +21 | +11 -12

+03 +12 +13 | -23 -32 | -02 +03 -13
+02 +03 +12 +13 | +23 | -02 +03
+12 +13 | +32 | -02 +03 +12 -13

+02 | -12 +20 +22 +23 | +02
+12 | +02 +21 +22 -32 | +12

+03 | +03 -13 +32 +33 | +03 -13
+03 +13 | -03 -23 +31 +33 | +13
"""
_SCHEME_8 = """
+01 +10 | +01 +10 | +00 +11
+00 -01 | +01 | +00 +01
+10 -11 | +10 | -10 -11

+00 +02 +10 | +02 +20 | +00 -10 +12
+00 +02 | +02 | -00 +02 +10 -12
+00 +02 +10 +12 | +20 | +10 -12

+00 +03 -04 +10 | +30 | +00 -10 -13 -14
+00 +03 -04 +10 +13 -14 | +03 +30 | +10 +13 +14
+00 +03 -04 +13 | +03 | +03 -10 -13 -14

+04 +10 | +04 +30 +40 -74 | +00 +14
+00 -04 | +04 -47 -74 | +00 +04
+10 -14 | -03 -30 -40 | +10 +14

+00 -05 +10 | +05 +50 | -00 +10 +15
+00 -05 | +05 | +00 +05 -10 -15
+00 -05 +10 -15 | +50 | -10 -15

+00 +06 +07 +10 | +60 | +00 -10 -16 +17
+00 +06 +07 +10 +16 +17 | +06 +60 | +10 +16 -17
+00 +06 +07 +16 | +06 | +06 -10 -16 +17

-07 +10 | +07 +47 -60 +70 | -00 +17
+00 +07 | +07 +47 +74 | -00 +07
+10 +17 | +06 +60 -70 | -10 +17

+10 | -00 -02 +05 -10 -30 -40 -60 +70 | +00 -10
+00 +10 | +00 -01 -04 +07 -20 -30 +47 +50 -60 +74 | +00

+01 +11 -12 | +12 +21 | +01 +02 -11
+11 -12 | +12 | -01 -02 +11 +12
+01 -02 +11 -12 | +21 | -01 -02

+01 +13 | +13 +31 +63 -71 | +03 +11
+11 -13 | +13 -36 +63 | +11 +13
+01 -03 | -17 -31 +71 | +01 +03

+01 +11 +14 -16 | +41 | -01 +04 +06 +11
+01 +04 -06 +11 +14 -16 | -14 +41 | +01 -04 -06
+04 +11 +14 -16 | +14 | +01 -04 -06 +14

+01 +11 +15 | +15 -51 | +01 +05 -11
+11 +15 | +15 | -01 -05 +11 +15
+01 +05 +11 +15 | +51 | +01 +05

+01 +16 | +16 +36 -41 -61 | +06 -11
+11 -16 | +16 +36 -63 | -11 +16
+01 -06 | -14 +41 +61 | -01 +06

+01 +11 -13 -17 | +71 | +01 +03 +07 -11
+01 -03 -07 +11 -13 -17 | +17 -71 | +01 +03 +07
-07 +11 -13 -17 | +17 | -01 -03 -07 +17

+01 | +01 +11 -12 -15 +31 +41 +61 -71 | +01 -11
+01 +11 | -10 +11 -13 +16 +21 +36 -41 -51 -63 +71 | +11

+02 +03 +13 | +23 -32 -52 | +03 -12 -13
+02 +03 +12 +13 | +23 | +12 +13
+02 +03 | +25 +32 +52 | +02 +03 -12 -13

-04 +12 -14 | -24 -42 | +02 +04 -14
+02 -04 +12 -14 | +24 | +02 +04
+12 -14 | +42 | +02 +04 -12 -14

+03 -05 +12 +13 -15 | +52 | -02 -03 +05 +13 -15
+12 +13 -15 | +25 +52 | +02 +03 -05 -12 -13 +15
+02 +03 +12 +13 -15 | +25 | -02 -03 +05 +12 +13

+02 +06 +16 | +26 -62 | +06 -12 -16
+02 +06 +12 +16 | +26 | +12 +16
+02 +06 | +62 | +02 +06 -12 -16

+07 +12 +17 | -27 -72 | -02 +07 -17
+02 +07 +12 +17 | +27 | -02 +07
+12 +17 | +72 | -02 +07 +12 -17

+02 | -02 -21 +22 -24 +27 -32 -52 -62 | +02
+12 | +12 +20 +22 -23 -26 +42 +52 -72 | +12

+04 +13 | +03 +34 +43 | +03 +14
+03 -04 | +34 | +03 +04
+13 -14 | -03 -30 -43 | +13 +14

+03 -05 +13 | -25 +35 -53 | +03 -13 +15
+03 -05 | -25 +35 -52 | -03 +05 +13 -15
+03 -05 +13 -15 | +53 | -13 +15

-01 +03 +06 +13 | +63 | +03 -11 -13 +16
-01 +03 +06 -11 +13 +16 | -36 +63 | +11 +13 -16
-01 +03 +06 +16 | +36 | +06 +11 +13 -16

-07 +13 | +17 +37 -73 | +03 +17
+03 +07 | +17 +37 -71 | +03 +07
+13 +17 | +73 | +13 +17

+13 | -03 -13 +25 +32 -33 -35 -43 +52 -63 +73 | +03 -13
+03 +13 | -03 -17 -23 -31 +33 -34 -37 +53 -63 +71 | +03

+04 +14 +15 | +45 -54 | +04 +05 -14
+14 +15 | +45 | -04 -05 +14 +15
+04 +05 +14 +15 | +54 | +04 +05

+04 +16 | +14 +46 +64 | +06 +14
+14 -16 | +46 | +14 +16
+04 -06 | -14 +41 -64 | +04 +06

+04 -10 +14 -17 | +74 | +00 +04 -07 -14
-00 +04 -07 -10 +14 -17 | -47 -74 | +00 +04 -07
-07 -10 +14 -17 | +47 | +00 +04 -07 +17

+04 | +04 +14 +34 -42 +44 -45 +64 -74 | +04 -14
+04 +14 | -03 -14 +24 -30 -40 -43 +44 -46 -54 +74 | +14

+05 +06 +16 | +56 -65 | +06 -15 -16
+05 +06 +15 +16 | +56 | +15 +16
+05 +06 | +65 | +05 +06 -15 -16

+07 +15 +17 | -57 -75 | -05 +07 -17
+05 +07 +15 +17 | +57 | -05 +07
+15 +17 | +75 | -05 +07 +15 -17

+05 | +05 -25 +35 -51 -54 +55 +57 -65 | +05
+15 | -15 +25 -45 -50 +53 +55 -56 -75 | +15

-07 +16 | -06 +67 +76 | -06 +17
+06 +07 | +67 | -06 +07
+16 +17 | +06 +60 -76 | -16 +17

+16 | -06 -16 -36 -46 +62 +65 -66 +76 | +06 -16
+06 +16 | -06 -14 -26 -36 +41 -56 +61 -64 +66 +67 | +06

+07 | -07 -17 -37 -47 -67 +72 +75 +77 | +07 -17
+07 +17 | -06 +17 -27 +47 -57 -60 +70 -73 +76 +77 | +17
"""


class _Scheme:
    def __init__(self, n, text):
        def terms(field):
            return {(int(t[1]), int(t[2])): 1 if t[0] == "+" else -1 for t in field.split()}

        def fold(coefs, weights):
            out = {}
            for (h, i), c in coefs.items():
                out[i] = out.get(i, 0) + weights[h] * c
            return {i: c for i, c in out.items() if c}

        self.n = n
        self.prods, self.ends = [], []
        for group in text.strip().split("\n\n"):
            self.prods += [tuple(terms(f) for f in line.split("|")) for line in group.split("\n")]
            self.ends.append(len(self.prods) - 1)
        dense = np.zeros((3, len(self.prods), n, n), np.int64)
        for r, prod in enumerate(self.prods):
            for m, coefs in enumerate(prod):
                for (i, j), c in coefs.items():
                    dense[m, r, i, j] = c
        eye = np.eye(n, dtype=np.int64)
        assert np.array_equal(
            np.einsum("rai,rjk,rbl->aijkbl", dense[0, :, :2], dense[1], dense[2, :, :2]),
            np.einsum("ab,ij,kl->aijkbl", eye[:2, :2], eye, eye)), "not the matrix product"
        assert all(len(v) > 1 or sum(v.values()) == 1 for _, v, _ in self.prods)
        folded = [(fold(u, (-1, 1)), fold(w, (0, 1))) for u, _, w in self.prods]
        self.single = [(u, w) if u and w else None for u, w in folded]
        self.sums, self.shared = [dict(v) for _, v, _ in self.prods], {}
        while True:
            count = {}
            for v in self.sums:
                for a, b in itertools.combinations(sorted(v), 2):
                    count[a, b, v[a] * v[b]] = count.get((a, b, v[a] * v[b]), 0) + 1
            (a, b, sign), times = max(count.items(), key=lambda kv: kv[1])
            if times < 2:
                break
            key = (n, len(self.shared))
            self.shared[key] = {a: 1, b: sign}
            for v in self.sums:
                if a in v and b in v and v[a] * v[b] == sign:
                    v[key] = v.pop(a)
                    del v[b]


def _combine(coefs, vals):
    acc = None
    for key, c in sorted(coefs.items(), key=lambda kv: -kv[1]):
        v = vals[key]
        if abs(c) != 1:
            v = v * abs(c)
        if acc is None:
            acc = v if c > 0 else -v
        else:
            acc = acc + v if c > 0 else acc - v
    return acc


def _accumulate(accs, group):
    terms = {}
    for n, (coefs, _) in enumerate(group):
        for key, c in coefs.items():
            terms.setdefault(key, []).append((n, c))
    sums = {((n, 1),): v for n, (_, v) in enumerate(group)}
    for key, tm in sorted(terms.items(), key=lambda kv: len(kv[1])):
        sign = tm[0][1]
        tm = tuple((n, c * sign) for n, c in tm)
        if tm not in sums:
            base = max((s for s in sums if all(t in tm for t in s)), key=len)
            val = sums[base]
            for n, c in tm:
                if (n, c) not in base:
                    val = val + group[n][1] if c > 0 else val - group[n][1]
            sums[tm] = val
        if key not in accs:
            accs[key] = sums[tm] if sign > 0 else -sums[tm]
        else:
            accs[key] = accs[key] + sums[tm] if sign > 0 else accs[key] - sums[tm]


def _layernorm(x, gain=1.0):
    m = jnp.mean(x, axis=-1, keepdims=True)
    c = x - m
    v = jnp.mean(c * c, axis=-1, keepdims=True)
    inv = lax.rsqrt(v + EPS)
    return c * (inv if gain == 1.0 else inv * gain)


def _dot(a, b):
    return lax.dot_general(a, b, (((1,), (0,)), ((), ())), preferred_element_type=F32)


def _dot_nt(a, b):
    return lax.dot_general(a, b, (((1,), (1,)), ((), ())), preferred_element_type=F32)


def _halves(x):
    return pltpu.bitcast(x << 16, F32), pltpu.bitcast(x & np.uint32(0xFFFF0000), F32)


def _make_kernel(S, D, H, DH, M, SEG, FF):
    SA = _Scheme(8, _SCHEME_8)
    SB = _Scheme(4, _SCHEME_4)
    NA, NB = SA.n, SB.n
    PA, PB = len(SA.prods), len(SB.prods)
    NSEG = S // SEG
    L = M + SEG
    DA, HB = D // NA, H // NA
    EB = HB * DH
    NG = FF // (NA * LANES)
    FA = NG * LANES
    F8 = NA * FA
    DB = D // NB
    assert DA == LANES and DH == LANES and FF - F8 == NB * LANES
    QR = 128 // NA
    QST = 4
    WR = 512 // NA
    OST = FF // (WR * NA)
    GST = 4
    GR, DR, ER = DA // GST, FA // GST, LANES // GST
    XH = 4 * SEG
    scale = DH ** (-0.5)
    c_exp = scale * math.log2(math.e)

    def fast_dot(sch, paired, w_of, block, kept_ref=None, fresh=True, hooks=None):
        acc, group = {}, []
        for r, (u, _, w) in enumerate(sch.prods):
            if hooks and r in hooks:
                hooks[r]()
            if paired or sch.single[r]:
                if not paired:
                    u, w = sch.single[r]
                if fresh:
                    if not paired:
                        u = {(0, i): c for i, c in u.items()}
                    else:
                        u = {(2 if u.get((1 - hf, i)) == c else hf, i): c
                             for (hf, i), c in u.items()}
                    lhs = _combine(u, {key: block(*key) for key in u})
                    if kept_ref is not None:
                        kept_ref[r] = lhs
                else:
                    lhs = kept_ref[r]
                group.append((w, _dot(lhs, pltpu.bitcast(w_of(r), BF16))))
            if r in sch.ends:
                _accumulate(acc, group)
                group = []
        return acc

    def blocks_of(ref, rows, cols, c0=0):
        return lambda hf, i: ref[hf * rows:(hf + 1) * rows, c0 + i * cols:c0 + (i + 1) * cols]

    def spread(pieces, first, stride):
        return {first + n * stride: piece for n, piece in enumerate(pieces)}

    def tile_of(j, blk, c):
        return slice(j * blk + c * LANES, j * blk + (c + 1) * LANES)

    def kernel(x_hbm, mem0_hbm, wq_hbm, wk_hbm, wv_hbm, wo_hbm, wg_hbm, wu_hbm, wd_hbm,
               out_hbm,
               x_v, mem0_v, big_v, gst_v, qst_v, qtr_v, wqkv_v, wo_v, wgu8_v, wgu4_v, wd8_v, wd4_v,
               la_v, lb_v, o_v, act_v, mem_v, ma_v, xa_v, na_v, nb_v, ya_v, z_v,
               q_v, kv_v, fill_v, keep_v,
               sem_x, sem_q, sem_o, sem_g, sem_d, sem_out):

        def rows_at(start, size):
            return pl.ds(start if isinstance(start, int) else pl.multiple_of(start, 16), size)

        def q_copies(w, c, slot):
            src = (wq_hbm, wk_hbm, wv_hbm)[w]
            return [pltpu.make_async_copy(src.at[rows_at((i * DA + c * QR) * H, QR * H), :],
                                          qst_v.at[slot, i, 0:QR * H, :], sem_q.at[slot])
                    for i in range(NA)]

        def o_copies(c):
            slot = c % OST
            return [pltpu.make_async_copy(wo_hbm.at[rows_at(i * EB + c * WR, WR), :],
                                          big_v.at[rows_at((slot * NA + i) * WR, WR), :],
                                          sem_o.at[slot]) for i in range(NA)]

        def g_copies(w, c):
            return [pltpu.make_async_copy((wg_hbm, wu_hbm)[w].at[rows_at(i * DA + c * GR, GR), :],
                                          gst_v.at[w, c, i], sem_g.at[w, c]) for i in range(NA)]

        def d_copies(c):
            rows = ([rows_at(i * FA + c * DR, DR) for i in range(NA)]
                    + [rows_at(F8 + i * LANES + c * ER, ER) for i in range(NB)])
            return [pltpu.make_async_copy(wd_hbm.at[r, :], big_v.at[r, :], sem_d.at[c])
                    for r in rows]

        def start(copies):
            for cp in copies:
                cp.start()

        def wait(copies):
            for cp in copies:
                cp.wait()

        def prep_tiles(sch, load, put, nrows, ncols):
            def tile(_, pos):
                s, k = pos
                row = pl.multiple_of(s * 16, 16)
                known = {}

                def value(key):
                    if key not in sch.shared:
                        return load(*key, row, k).astype(F32)
                    if key not in known:
                        known[key] = _combine(sch.shared[key],
                                              {a: value(a) for a in sch.shared[key]})
                    return known[key]

                for r, v in enumerate(sch.sums):
                    if len(sch.prods[r][1]) == 1:
                        val = load(*next(iter(v)), row, k)
                    else:
                        val = _combine(v, {key: value(key) for key in v}).astype(BF16)
                    put(r, row, k, pltpu.bitcast(val, U32))
                wrap = k + 1 == ncols
                return jnp.where(wrap, s + 1, s), jnp.where(wrap, 0, k + 1)
            lax.fori_loop(0, nrows // 16 * ncols, tile, (0, 0))

        def lanes_at(k):
            return pl.ds(pl.multiple_of(k * LANES, LANES), LANES)

        def words_at(row):
            return pl.ds(pl.multiple_of(row >> 1, 8), 8)

        def prep_qkv(w, c, slot):
            def heads(i, carry):
                st = qst_v.at[slot, i].bitcast(U32)
                for jp in range(H // 2):
                    for k, x in enumerate(_halves(st[pl.ds(jp, QR, stride=H // 2), :])):
                        qtr_v[i, 2 * jp + k] = x.astype(BF16)
                return carry
            lax.fori_loop(0, NA, heads, 0)

            def put(r, row, k, val):
                wqkv_v[w, k, r, words_at(c * QR + row), :] = val
            prep_tiles(SA, lambda i, j, row, k: qtr_v[i, j * HB + k, pl.ds(row, 16), :], put, QR, HB)

        def prep_from_big(sch, dst, base, blk, c, nrows):
            ncols = D // sch.n // LANES

            def load(i, j, row, k):
                return big_v[rows_at(base + i * blk + row, 16), lanes_at(j * ncols + k)]

            def put(r, row, k, val):
                dst[k, r, words_at(c * nrows + row), :] = val
            prep_tiles(sch, load, put, nrows, ncols)

        def prep_gu(w, c):
            def put8(r, row, k, val):
                wgu8_v[w, k, r, words_at(c * GR + row), :] = val
            prep_tiles(SA, lambda i, j, row, k: gst_v[w, c, i, pl.ds(row, 16),
                                                      lanes_at(j * NG + k)], put8, GR, NG)

            def put4(r, row, k, val):
                rows = words_at(k * DA + c * GR + row)
                wgu4_v[r, rows, w * LANES:(w + 1) * LANES] = val
            prep_tiles(SB, lambda i, j, row, k: gst_v[w, c, 2 * i + k, pl.ds(row, 16),
                                                      F8 + j * LANES:F8 + (j + 1) * LANES],
                       put4, GR, 2)

        x_head = pltpu.make_async_copy(x_hbm.at[0:XH, :], x_v.at[0:XH, :], sem_x.at[0])
        x_tail = pltpu.make_async_copy(x_hbm.at[XH:, :], x_v.at[XH:, :], sem_x.at[1])
        NQ, NO = DA // QR, EB // WR
        AHEAD = 5
        assert QST <= min(NQ, AHEAD) and AHEAD <= OST <= NO
        QA = QST - 1
        for n in range(QA):
            start(q_copies(0, n, n))
        mem0_copy = pltpu.make_async_copy(mem0_hbm, mem0_v, sem_x.at[2])
        x_head.start()
        mem0_copy.start()

        ri = lax.broadcasted_iota(jnp.int32, (2 * L, LANES), 0)
        ci = lax.broadcasted_iota(jnp.int32, (2 * L, LANES), 1)
        first = jnp.where(ri < L, 0, L)
        same = (ci >= first) & (ci < first + L)
        visible = (ri < first + M) | (ri >= ci)
        keep_v[...] = (same & visible).astype(jnp.int32)
        fill_v[...] = jnp.where(same, -1e9 / scale, -jnp.inf).astype(F32)
        kv_v[...] = jnp.zeros(kv_v.shape, BF16)

        for w in range(3):
            def q_body(c, carry, w=w):
                slot, free = (w * NQ + c) % QST, (w * NQ + c + QA) % QST
                wait(q_copies(w, c, slot))
                pl.when(c + QA < NQ)(lambda: start(q_copies(w, c + QA, free)))
                if w < 2:
                    pl.when(c + QA >= NQ)(lambda: start(q_copies(w + 1, c + QA - NQ, free)))
                else:
                    pl.when(c + QA >= NQ)(lambda: start(o_copies(c + QA - NQ)))
                prep_qkv(w, c, slot)
                return carry
            lax.fori_loop(0, NQ, q_body, 0)

        for c in range(QA, AHEAD):
            start(o_copies(c))
        x_head.wait()
        mem0_copy.wait()
        xa_v[...] = x_v[0:2 * SEG, :].astype(F32)
        mem_v[0:M, :] = mem0_v[...].astype(F32)
        mem_v[M:, :] = mem0_v[...].astype(F32)

        def load_out_weights():
            def chunk(c, carry):
                wait(o_copies(c))
                prep_from_big(SA, wo_v, (c % OST) * NA * WR, WR, c, WR)
                pl.when(c + AHEAD < NO)(lambda: start(o_copies(c + AHEAD)))
                pl.when(c >= NO - 2)(lambda: start(g_copies(0, c - (NO - 2))))
                return carry
            lax.fori_loop(0, NO, chunk, 0)
            for c in range(2, GST):
                start(g_copies(0, c))
            start(g_copies(1, 0))

        def load_gate_up_weights():
            def gate(c, carry):
                pl.when(c + 1 < GST)(lambda: start(g_copies(1, c + 1)))
                wait(g_copies(0, c))
                prep_gu(0, c)
                return carry

            def up(c, carry):
                wait(g_copies(1, c))
                prep_gu(1, c)
                start(d_copies(c))
                return carry
            lax.fori_loop(0, GST, gate, 0)
            lax.fori_loop(0, GST, up, 0)

        def load_down_weights():
            def chunk(c, carry):
                wait(d_copies(c))
                pl.when(c == 0)(lambda: x_tail.start())
                prep_from_big(SA, wd8_v, c * DR, FA, c, DR)
                prep_from_big(SB, wd4_v, F8 + c * ER, LANES, c, ER)
                return carry
            lax.fori_loop(0, GST, chunk, 0)

        def attention(c, paired):
            n = 2 * L if paired else L
            probs = {}

            def scores(j):
                s = _dot_nt(q_v[j, 0:n, :], kv_v[0, j])
                s = jnp.where(keep_v[0:n, :] != 0, s, fill_v[0:n, :])
                mx = jnp.max(s, axis=-1, keepdims=True)
                e = jnp.exp2((s - mx) * c_exp)
                den = jnp.sum(e, axis=-1, keepdims=True)
                inv = pl.reciprocal(den, approx=True)
                inv = inv * (2.0 - den * inv)
                probs[j] = e * inv

            def values(j):
                o = _dot(probs[j], kv_v[1, j])
                o_v[0:n, tile_of(j, EB, c)] = o
                if paired:
                    o_v[n:, tile_of(j, EB, c)] = o[:L] + o[L:]

            return ([functools.partial(scores, j) for j in range(NA)],
                    [functools.partial(values, j) for j in range(NA)])

        def project_qkv(w, c, paired, hooks):
            def block(hf, i):
                cols = slice(i * DA, (i + 1) * DA)
                if hf == 2:
                    return jnp.concatenate([ma_v[0:M, cols] + ma_v[M:, cols],
                                            na_v[2 * SEG:, cols]], axis=0)
                return jnp.concatenate([ma_v[hf * M:(hf + 1) * M, cols],
                                        na_v[hf * SEG:(hf + 1) * SEG, cols]], axis=0)

            p = fast_dot(SA, paired, lambda r: wqkv_v[w, c, r], block, la_v, w + c == 0, hooks)
            for j in range(NA):
                x = jnp.concatenate([p[0, j], p[1, j]], axis=0) if paired else p[j]
                if w == 0:
                    q_v[j, 0:x.shape[0], :] = x
                else:
                    kv_v[w - 1, j, 0:x.shape[0], :] = x.astype(BF16)

        def project_out(c, paired, hooks=None):
            return fast_dot(SA, paired, lambda r: wo_v[c, r], blocks_of(o_v, L, EB), hooks=hooks)

        def glu_input():
            nb = _layernorm(ya_v[0:2 * SEG, :], 0.5)
            nb_v[...] = jnp.concatenate([nb, nb[:SEG] + nb[SEG:]], axis=0)

        def gate_up_pieces():
            gate = {}

            def activate(cols, g, u):
                act = [jnp.tanh(g[hf]) * u[hf] + u[hf] for hf in range(2)]
                act_v[:, cols] = jnp.concatenate(act + [act[0] + act[1]], axis=0)

            def large(k, w):
                p = fast_dot(SA, True, lambda r: wgu8_v[w, k, r], blocks_of(nb_v, SEG, DA), lb_v,
                             k + w == 0)
                if w == 0:
                    gate.update(p)
                else:
                    for j in range(NA):
                        activate(tile_of(j, FA, k), (gate[0, j], gate[1, j]), (p[0, j], p[1, j]))

            def small():
                p = fast_dot(SB, True, lambda r: wgu4_v[r], blocks_of(nb_v, SEG, DB))
                for j in range(NB):
                    activate(slice(F8 + j * LANES, F8 + (j + 1) * LANES),
                             [p[hf, j][:, :LANES] for hf in range(2)],
                             [p[hf, j][:, LANES:] for hf in range(2)])

            return [small] + [functools.partial(large, k, w) for k in range(NG) for w in range(2)]

        def down_small():
            acc = {}
            for k in range(DB // LANES):
                p = fast_dot(SB, True, lambda r: wd4_v[k, r], blocks_of(act_v, SEG, LANES, F8))
                acc.update({(hf, j * (DB // LANES) + k): v for (hf, j), v in p.items()})
            for (hf, j), v in acc.items():
                rows = slice(hf * SEG, (hf + 1) * SEG)
                z_v[rows, tile_of(j, DA, 0)] = ya_v[rows, tile_of(j, DA, 0)] + v

        def down_large(hooks=None):
            acc = fast_dot(SA, True, lambda r: wd8_v[0, r], blocks_of(act_v, SEG, FA),
                           hooks=hooks)
            for (hf, j), v in acc.items():
                z_v[hf * SEG:(hf + 1) * SEG, tile_of(j, DA, 0)] += v

        def out_copy(row, n):
            return pltpu.make_async_copy(big_v.at[pl.ds(row, n), :],
                                         out_hbm.at[pl.ds(row, n), :], sem_out)

        def attention_single(mrow, xrow, yrow, before_out):
            ma_v[0:M, :] = mem_v[pl.ds(mrow, M), :]
            na_v[0:SEG, :] = _layernorm(xa_v[pl.ds(xrow, SEG), :])
            hooks = None
            for c in range(HB):
                scores, values = attention(c, False)
                project_qkv(0, c, False, hooks)
                project_qkv(1, c, False, None)
                project_qkv(2, c, False, spread(scores, 20, 7))
                hooks = spread(values, 24, 9)
            for piece in values:
                piece()
            before_out()
            for c in range(DA // LANES):
                for j, v in project_out(c, False).items():
                    mem_v[pl.ds(mrow, M), tile_of(j, DA, c)] = v[:M]
                    ya_v[pl.ds(yrow, SEG), tile_of(j, DA, c)] = (
                        xa_v[pl.ds(xrow, SEG), tile_of(j, DA, c)] + v[M:])

        def step(t, carry):
            cur = pl.multiple_of(t * SEG, SEG)
            nxt = pl.multiple_of(jnp.minimum(t + 1, NSEG - 1) * SEG, SEG)
            pl.when(t + 1 == XH // SEG)(lambda: x_tail.wait())
            row = pl.multiple_of(jnp.maximum(t - 3, 0) * SEG, SEG)
            hooks = {50: glu_input}
            gpos = [1, 3, 4, 6, 7, 9, 10]
            def next_tokens():
                na_v[:SEG, :] = _layernorm(x_v[pl.ds(nxt, SEG), :].astype(F32))

            glu = gate_up_pieces()
            for c in range(HB):
                scores, values = attention(c, True)
                for w in range(3):
                    project_qkv(w, c, True, (hooks, None, spread(
                        scores, 20, 10))[w])
                    if 3 * c + w in gpos:
                        glu[gpos.index(3 * c + w)]()
                    if 3 * c + w == 5:
                        down_small()
                hooks = spread(values, 26, 10)
                if c == 2:
                    hooks[5] = next_tokens
            down_large(spread(values, 12, 8))
            big_v[pl.ds(row, SEG), :] = z_v[SEG:, :].astype(BF16)

            def next_input():
                na = _layernorm(z_v[:SEG, :])
                na_v[SEG:, :] = jnp.concatenate([na, na + na_v[:SEG, :]], axis=0)

            for c in range(DA // LANES):
                o = project_out(c, True, {2: next_input} if c == 0 else None)
                for (hf, j), v in o.items():
                    cols = tile_of(j, DA, c)
                    res = x_v[pl.ds(cur, SEG), cols].astype(F32) if hf == 0 else xa_v[SEG:, cols]
                    ma_v[hf * M:(hf + 1) * M, cols] = v[:M]
                    ya_v[hf * SEG:(hf + 1) * SEG, cols] = res + v[M:]
            xa_v[SEG:, :] = z_v[:SEG, :]
            pl.when(t >= 3)(lambda: out_copy(row, SEG).start())
            return carry

        def phase(ph, carry):
            attention_single(pl.multiple_of(jnp.where(ph < 2, 0, M), M),
                             pl.multiple_of(jnp.where(ph == 0, 0, SEG), SEG),
                             pl.multiple_of(jnp.where(ph == 3, 1, ph) * SEG, SEG),
                             lambda: pl.when(ph == 0)(load_out_weights))
            pl.when(ph == 1)(load_gate_up_weights)

            @pl.when(ph >= 1)
            def _():
                glu_input()
                for piece in gate_up_pieces():
                    piece()
                pl.when(ph == 1)(load_down_weights)
                down_small()
                down_large()

            @pl.when(ph == 1)
            def _():
                ya_v[0:SEG, :] = ya_v[SEG:2 * SEG, :]
                xa_v[SEG:, :] = z_v[:SEG, :]
                ma_v[...] = mem_v[...]
                na_v[:SEG, :] = _layernorm(x_v[2 * SEG:3 * SEG, :].astype(F32))
                na = _layernorm(z_v[:SEG, :])
                na_v[SEG:, :] = jnp.concatenate([na, na + na_v[:SEG, :]], axis=0)
                lax.fori_loop(2, NSEG, step, 0)
                mem_v[...] = ma_v[...]

            @pl.when(ph == 2)
            def _():
                xa_v[SEG:, :] = z_v[:SEG, :]
                ya_v[0:SEG, :] = ya_v[2 * SEG:, :]
                big_v[S - 3 * SEG:S - 2 * SEG, :] = z_v[SEG:, :].astype(BF16)
                out_copy(S - 3 * SEG, SEG).start()

            @pl.when(ph == 3)
            def _():
                big_v[S - 2 * SEG:S, :] = z_v[...].astype(BF16)
                out_copy(S - 2 * SEG, 2 * SEG).start()
            return carry

        lax.fori_loop(0, 4, phase, 0)
        out_copy(0, NSEG * SEG).wait()

    scratch = [
        pltpu.VMEM((S, D), BF16),
        pltpu.VMEM((M, D), BF16),
        pltpu.VMEM((FF, D), BF16),
        pltpu.VMEM((2, GST, NA, GR, FF), BF16),
        pltpu.VMEM((QST, NA, (QR + 1) * H, DH), BF16),
        pltpu.VMEM((NA, H, QR, DH), BF16),
        pltpu.VMEM((3, HB, PA, DA // 2, DH), U32),
        pltpu.VMEM((DA // LANES, PA, EB // 2, LANES), U32),
        pltpu.VMEM((2, NG, PA, DA // 2, LANES), U32),
        pltpu.VMEM((PB, DB // 2, 2 * LANES), U32),
        pltpu.VMEM((1, PA, FA // 2, LANES), U32),
        pltpu.VMEM((DB // LANES, PB, LANES // 2, LANES), U32),
        pltpu.VMEM((PA, L, DA), F32),
        pltpu.VMEM((PA, SEG, DA), F32),
        pltpu.VMEM((3 * L, H * DH), F32),
        pltpu.VMEM((3 * SEG, FF), F32),
        pltpu.VMEM((2 * M, D), F32),
        pltpu.VMEM((2 * M, D), F32),
        pltpu.VMEM((2 * SEG, D), F32),
        pltpu.VMEM((3 * SEG, D), F32),
        pltpu.VMEM((3 * SEG, D), F32),
        pltpu.VMEM((3 * SEG, D), F32),
        pltpu.VMEM((2 * SEG, D), F32),
        pltpu.VMEM((NA, 2 * L, DH), F32),
        pltpu.VMEM((2, NA, LANES, DH), BF16),
        pltpu.VMEM((2 * L, LANES), F32),
        pltpu.VMEM((2 * L, LANES), jnp.int32),
        pltpu.SemaphoreType.DMA((3,)),
        pltpu.SemaphoreType.DMA((QST,)),
        pltpu.SemaphoreType.DMA((OST,)),
        pltpu.SemaphoreType.DMA((2, GST)),
        pltpu.SemaphoreType.DMA((GST,)),
        pltpu.SemaphoreType.DMA(()),
    ]
    return kernel, scratch


@functools.partial(jax.jit, static_argnames=("A_seg_len",))
def pallas_interleave_layers__memory_aug_recurrent_mem_tr__glu_gated_glu__prompt_kernel(
    A_x, A_mem0, A_Wq, A_Wk, A_Wv, A_Wo, A_seg_len, B_x, B_w_gate, B_w_up, B_w_down,
):
    del B_x
    B, S, D = A_x.shape
    _, H, DH = A_Wq.shape
    M = A_mem0.shape[1]
    assert B == 1
    kernel, scratch = _make_kernel(S, D, H, DH, M, A_seg_len, B_w_gate.shape[1])
    any_spec = pl.BlockSpec(memory_space=pl.ANY)
    out = pl.pallas_call(
        kernel,
        out_shape=jax.ShapeDtypeStruct((S, D), A_x.dtype),
        in_specs=[any_spec] * 9,
        out_specs=any_spec,
        scratch_shapes=scratch,
        compiler_params=pltpu.CompilerParams(vmem_limit_bytes=126 * 1024 * 1024),
    )(A_x.reshape(S, D), A_mem0.reshape(M, D),
      A_Wq.reshape(D * H, DH), A_Wk.reshape(D * H, DH), A_Wv.reshape(D * H, DH),
      A_Wo.reshape(H * DH, D), B_w_gate, B_w_up, B_w_down)
    return out.reshape(B, S, D)
```

```python
import functools
import itertools
import math

import jax
import jax.numpy as jnp
import numpy as np
from jax import lax
import jax.experimental.pallas as pl
import jax.experimental.pallas.tpu as pltpu

F32 = jnp.float32
BF16 = jnp.bfloat16
U32 = jnp.uint32
EPS = 1e-05
LANES = 128

_SCHEME_4 = """
+00 | +00 +02 -10 +30 | +00 -10
+00 +10 | +00 -01 +20 -30 | +10

+00 -11 | +01 -10 +30 | +01 +10
+10 +11 | +01 | +10 +11
+00 +01 | +03 +10 -30 | +00 +01

+00 +10 +11 +13 | +30 | -00 -01 +03 +10
+00 +01 +03 +10 +11 +13 | -03 +30 | +00 +01 -03
+03 +10 +11 +13 | +03 | +00 +01 -03 +13

+00 +10 -12 | +02 -20 | -00 +02 +10
+10 -12 | +02 | +00 -02 -10 +12
+00 -02 +10 -12 | +20 | -00 +02

+11 | +01 -11 -12 +31 | +01 -11
+01 +11 | -03 -10 +11 +13 -21 +30 | +01

-03 +11 | -03 +13 +31 | -01 +13
+01 +03 | -03 +13 +30 | -01 +03
+11 +13 | +31 | +11 -13

+01 +02 +11 | +12 +21 | +01 -11 +12
+01 +02 | +12 | -01 +02 +11 -12
+01 +02 +11 +12 | +21 | +11 -12

+03 +12 +13 | -23 -32 | -02 +03 -13
+02 +03 +12 +13 | +23 | -02 +03
+12 +13 | +32 | -02 +03 +12 -13

+02 | -12 +20 +22 +23 | +02
+12 | +02 +21 +22 -32 | +12

+03 | +03 -13 +32 +33 | +03 -13
+03 +13 | -03 -23 +31 +33 | +13
"""
_SCHEME_8 = """
+01 +10 | +01 +10 | +00 +11
+00 -01 | +01 | +00 +01
+10 -11 | +10 | -10 -11

+00 +02 +10 | +02 +20 | +00 -10 +12
+00 +02 | +02 | -00 +02 +10 -12
+00 +02 +10 +12 | +20 | +10 -12

+00 +03 -04 +10 | +30 | +00 -10 -13 -14
+00 +03 -04 +10 +13 -14 | +03 +30 | +10 +13 +14
+00 +03 -04 +13 | +03 | +03 -10 -13 -14

+04 +10 | +04 +30 +40 -74 | +00 +14
+00 -04 | +04 -47 -74 | +00 +04
+10 -14 | -03 -30 -40 | +10 +14

+00 -05 +10 | +05 +50 | -00 +10 +15
+00 -05 | +05 | +00 +05 -10 -15
+00 -05 +10 -15 | +50 | -10 -15

+00 +06 +07 +10 | +60 | +00 -10 -16 +17
+00 +06 +07 +10 +16 +17 | +06 +60 | +10 +16 -17
+00 +06 +07 +16 | +06 | +06 -10 -16 +17

-07 +10 | +07 +47 -60 +70 | -00 +17
+00 +07 | +07 +47 +74 | -00 +07
+10 +17 | +06 +60 -70 | -10 +17

+10 | -00 -02 +05 -10 -30 -40 -60 +70 | +00 -10
+00 +10 | +00 -01 -04 +07 -20 -30 +47 +50 -60 +74 | +00

+01 +11 -12 | +12 +21 | +01 +02 -11
+11 -12 | +12 | -01 -02 +11 +12
+01 -02 +11 -12 | +21 | -01 -02

+01 +13 | +13 +31 +63 -71 | +03 +11
+11 -13 | +13 -36 +63 | +11 +13
+01 -03 | -17 -31 +71 | +01 +03

+01 +11 +14 -16 | +41 | -01 +04 +06 +11
+01 +04 -06 +11 +14 -16 | -14 +41 | +01 -04 -06
+04 +11 +14 -16 | +14 | +01 -04 -06 +14

+01 +11 +15 | +15 -51 | +01 +05 -11
+11 +15 | +15 | -01 -05 +11 +15
+01 +05 +11 +15 | +51 | +01 +05

+01 +16 | +16 +36 -41 -61 | +06 -11
+11 -16 | +16 +36 -63 | -11 +16
+01 -06 | -14 +41 +61 | -01 +06

+01 +11 -13 -17 | +71 | +01 +03 +07 -11
+01 -03 -07 +11 -13 -17 | +17 -71 | +01 +03 +07
-07 +11 -13 -17 | +17 | -01 -03 -07 +17

+01 | +01 +11 -12 -15 +31 +41 +61 -71 | +01 -11
+01 +11 | -10 +11 -13 +16 +21 +36 -41 -51 -63 +71 | +11

+02 +03 +13 | +23 -32 -52 | +03 -12 -13
+02 +03 +12 +13 | +23 | +12 +13
+02 +03 | +25 +32 +52 | +02 +03 -12 -13

-04 +12 -14 | -24 -42 | +02 +04 -14
+02 -04 +12 -14 | +24 | +02 +04
+12 -14 | +42 | +02 +04 -12 -14

+03 -05 +12 +13 -15 | +52 | -02 -03 +05 +13 -15
+12 +13 -15 | +25 +52 | +02 +03 -05 -12 -13 +15
+02 +03 +12 +13 -15 | +25 | -02 -03 +05 +12 +13

+02 +06 +16 | +26 -62 | +06 -12 -16
+02 +06 +12 +16 | +26 | +12 +16
+02 +06 | +62 | +02 +06 -12 -16

+07 +12 +17 | -27 -72 | -02 +07 -17
+02 +07 +12 +17 | +27 | -02 +07
+12 +17 | +72 | -02 +07 +12 -17

+02 | -02 -21 +22 -24 +27 -32 -52 -62 | +02
+12 | +12 +20 +22 -23 -26 +42 +52 -72 | +12

+04 +13 | +03 +34 +43 | +03 +14
+03 -04 | +34 | +03 +04
+13 -14 | -03 -30 -43 | +13 +14

+03 -05 +13 | -25 +35 -53 | +03 -13 +15
+03 -05 | -25 +35 -52 | -03 +05 +13 -15
+03 -05 +13 -15 | +53 | -13 +15

-01 +03 +06 +13 | +63 | +03 -11 -13 +16
-01 +03 +06 -11 +13 +16 | -36 +63 | +11 +13 -16
-01 +03 +06 +16 | +36 | +06 +11 +13 -16

-07 +13 | +17 +37 -73 | +03 +17
+03 +07 | +17 +37 -71 | +03 +07
+13 +17 | +73 | +13 +17

+13 | -03 -13 +25 +32 -33 -35 -43 +52 -63 +73 | +03 -13
+03 +13 | -03 -17 -23 -31 +33 -34 -37 +53 -63 +71 | +03

+04 +14 +15 | +45 -54 | +04 +05 -14
+14 +15 | +45 | -04 -05 +14 +15
+04 +05 +14 +15 | +54 | +04 +05

+04 +16 | +14 +46 +64 | +06 +14
+14 -16 | +46 | +14 +16
+04 -06 | -14 +41 -64 | +04 +06

+04 -10 +14 -17 | +74 | +00 +04 -07 -14
-00 +04 -07 -10 +14 -17 | -47 -74 | +00 +04 -07
-07 -10 +14 -17 | +47 | +00 +04 -07 +17

+04 | +04 +14 +34 -42 +44 -45 +64 -74 | +04 -14
+04 +14 | -03 -14 +24 -30 -40 -43 +44 -46 -54 +74 | +14

+05 +06 +16 | +56 -65 | +06 -15 -16
+05 +06 +15 +16 | +56 | +15 +16
+05 +06 | +65 | +05 +06 -15 -16

+07 +15 +17 | -57 -75 | -05 +07 -17
+05 +07 +15 +17 | +57 | -05 +07
+15 +17 | +75 | -05 +07 +15 -17

+05 | +05 -25 +35 -51 -54 +55 +57 -65 | +05
+15 | -15 +25 -45 -50 +53 +55 -56 -75 | +15

-07 +16 | -06 +67 +76 | -06 +17
+06 +07 | +67 | -06 +07
+16 +17 | +06 +60 -76 | -16 +17

+16 | -06 -16 -36 -46 +62 +65 -66 +76 | +06 -16
+06 +16 | -06 -14 -26 -36 +41 -56 +61 -64 +66 +67 | +06

+07 | -07 -17 -37 -47 -67 +72 +75 +77 | +07 -17
+07 +17 | -06 +17 -27 +47 -57 -60 +70 -73 +76 +77 | +17
"""


class _Scheme:
    def __init__(self, n, text):
        def terms(field):
            return {(int(t[1]), int(t[2])): 1 if t[0] == "+" else -1 for t in field.split()}

        def fold(coefs, weights):
            out = {}
            for (h, i), c in coefs.items():
                out[i] = out.get(i, 0) + weights[h] * c
            return {i: c for i, c in out.items() if c}

        self.n = n
        self.prods, self.ends = [], []
        for group in text.strip().split("\n\n"):
            self.prods += [tuple(terms(f) for f in line.split("|")) for line in group.split("\n")]
            self.ends.append(len(self.prods) - 1)
        dense = np.zeros((3, len(self.prods), n, n), np.int64)
        for r, prod in enumerate(self.prods):
            for m, coefs in enumerate(prod):
                for (i, j), c in coefs.items():
                    dense[m, r, i, j] = c
        eye = np.eye(n, dtype=np.int64)
        assert np.array_equal(
            np.einsum("rai,rjk,rbl->aijkbl", dense[0, :, :2], dense[1], dense[2, :, :2]),
            np.einsum("ab,ij,kl->aijkbl", eye[:2, :2], eye, eye)), "not the matrix product"
        assert all(len(v) > 1 or sum(v.values()) == 1 for _, v, _ in self.prods)
        folded = [(fold(u, (-1, 1)), fold(w, (0, 1))) for u, _, w in self.prods]
        self.single = [(u, w) if u and w else None for u, w in folded]
        self.sums, self.shared = [dict(v) for _, v, _ in self.prods], {}
        while True:
            count = {}
            for v in self.sums:
                for a, b in itertools.combinations(sorted(v), 2):
                    count[a, b, v[a] * v[b]] = count.get((a, b, v[a] * v[b]), 0) + 1
            (a, b, sign), times = max(count.items(), key=lambda kv: kv[1])
            if times < 2:
                break
            key = (n, len(self.shared))
            self.shared[key] = {a: 1, b: sign}
            for v in self.sums:
                if a in v and b in v and v[a] * v[b] == sign:
                    v[key] = v.pop(a)
                    del v[b]


def _combine(coefs, vals):
    acc = None
    for key, c in sorted(coefs.items(), key=lambda kv: -kv[1]):
        v = vals[key]
        if abs(c) != 1:
            v = v * abs(c)
        if acc is None:
            acc = v if c > 0 else -v
        else:
            acc = acc + v if c > 0 else acc - v
    return acc


def _accumulate(accs, group):
    terms = {}
    for n, (coefs, _) in enumerate(group):
        for key, c in coefs.items():
            terms.setdefault(key, []).append((n, c))
    sums = {((n, 1),): v for n, (_, v) in enumerate(group)}
    for key, tm in sorted(terms.items(), key=lambda kv: len(kv[1])):
        sign = tm[0][1]
        tm = tuple((n, c * sign) for n, c in tm)
        if tm not in sums:
            base = max((s for s in sums if all(t in tm for t in s)), key=len)
            val = sums[base]
            for n, c in tm:
                if (n, c) not in base:
                    val = val + group[n][1] if c > 0 else val - group[n][1]
            sums[tm] = val
        if key not in accs:
            accs[key] = sums[tm] if sign > 0 else -sums[tm]
        else:
            accs[key] = accs[key] + sums[tm] if sign > 0 else accs[key] - sums[tm]


def _layernorm(x, gain=1.0):
    m = jnp.mean(x, axis=-1, keepdims=True)
    c = x - m
    v = jnp.mean(c * c, axis=-1, keepdims=True)
    inv = lax.rsqrt(v + EPS)
    return c * (inv if gain == 1.0 else inv * gain)


def _dot(a, b):
    return lax.dot_general(a, b, (((1,), (0,)), ((), ())), preferred_element_type=F32)


def _dot_nt(a, b):
    return lax.dot_general(a, b, (((1,), (1,)), ((), ())), preferred_element_type=F32)


def _halves(x):
    return pltpu.bitcast(x << 16, F32), pltpu.bitcast(x & np.uint32(0xFFFF0000), F32)


def _make_kernel(S, D, H, DH, M, SEG, FF):
    SA = _Scheme(8, _SCHEME_8)
    SB = _Scheme(4, _SCHEME_4)
    NA, NB = SA.n, SB.n
    PA, PB = len(SA.prods), len(SB.prods)
    NSEG = S // SEG
    L = M + SEG
    DA, HB = D // NA, H // NA
    EB = HB * DH
    NG = FF // (NA * LANES)
    FA = NG * LANES
    F8 = NA * FA
    DB = D // NB
    assert DA == LANES and DH == LANES and FF - F8 == NB * LANES
    QR = 128 // NA
    QST = 4
    WR = 512 // NA
    OST = FF // (WR * NA)
    GST = 4
    GR, DR, ER = DA // GST, FA // GST, LANES // GST
    XH = 4 * SEG
    scale = DH ** (-0.5)
    c_exp = scale * math.log2(math.e)

    def fast_dot(sch, paired, w_of, block, kept_ref=None, fresh=True, hooks=None):
        acc, group = {}, []
        for r, (u, _, w) in enumerate(sch.prods):
            if hooks and r in hooks:
                hooks[r]()
            if paired or sch.single[r]:
                if not paired:
                    u, w = sch.single[r]
                if fresh:
                    if not paired:
                        u = {(0, i): c for i, c in u.items()}
                    else:
                        u = {(2 if u.get((1 - hf, i)) == c else hf, i): c
                             for (hf, i), c in u.items()}
                    lhs = _combine(u, {key: block(*key) for key in u})
                    if kept_ref is not None:
                        kept_ref[r] = lhs
                else:
                    lhs = kept_ref[r]
                group.append((w, _dot(lhs, w_of(r))))
            if r in sch.ends:
                _accumulate(acc, group)
                group = []
        return acc

    def tiles_of(ref, *index):
        return lambda r: pltpu.bitcast(ref.bitcast(U32)[(*index, r)], BF16)

    def blocks_of(ref, rows, cols, c0=0):
        return lambda hf, i: ref[hf * rows:(hf + 1) * rows, c0 + i * cols:c0 + (i + 1) * cols]

    def spread(pieces, first, stride):
        return {first + n * stride: piece for n, piece in enumerate(pieces)}

    def tile_of(j, blk, c):
        return slice(j * blk + c * LANES, j * blk + (c + 1) * LANES)

    def kernel(x_hbm, mem0_hbm, wq_hbm, wk_hbm, wv_hbm, wo_hbm, wg_hbm, wu_hbm, wd_hbm,
               out_hbm,
               x_v, mem0_v, big_v, gst_v, qst_v, qtr_v, wqkv_v, wo_v, wgu8_v, wgu4_v, wd8_v, wd4_v,
               la_v, lb_v, o_v, act_v, mem_v, ma_v, xa_v, na_v, nb_v, ya_v, z_v,
               q_v, kv_v, fill_v, keep_v,
               sem_x, sem_q, sem_o, sem_g, sem_d, sem_out):

        def rows_at(start, size):
            return pl.ds(start if isinstance(start, int) else pl.multiple_of(start, 16), size)

        def q_copies(w, c, slot):
            src = (wq_hbm, wk_hbm, wv_hbm)[w]
            return [pltpu.make_async_copy(src.at[rows_at((i * DA + c * QR) * H, QR * H), :],
                                          qst_v.at[slot, i, 0:QR * H, :], sem_q.at[slot])
                    for i in range(NA)]

        def o_copies(c):
            slot = c % OST
            return [pltpu.make_async_copy(wo_hbm.at[rows_at(i * EB + c * WR, WR), :],
                                          big_v.at[rows_at((slot * NA + i) * WR, WR), :],
                                          sem_o.at[slot]) for i in range(NA)]

        def g_copies(w, c):
            return [pltpu.make_async_copy((wg_hbm, wu_hbm)[w].at[rows_at(i * DA + c * GR, GR), :],
                                          gst_v.at[w, c, i], sem_g.at[w, c]) for i in range(NA)]

        def d_copies(c):
            rows = ([rows_at(i * FA + c * DR, DR) for i in range(NA)]
                    + [rows_at(F8 + i * LANES + c * ER, ER) for i in range(NB)])
            return [pltpu.make_async_copy(wd_hbm.at[r, :], big_v.at[r, :], sem_d.at[c])
                    for r in rows]

        def start(copies):
            for cp in copies:
                cp.start()

        def wait(copies):
            for cp in copies:
                cp.wait()

        def prep_tiles(sch, load, put, nrows, ncols):
            def tile(_, pos):
                s, k = pos
                row = pl.multiple_of(s * 16, 16)
                known = {}

                def value(key):
                    if key not in sch.shared:
                        return load(*key, row, k).astype(F32)
                    if key not in known:
                        known[key] = _combine(sch.shared[key],
                                              {a: value(a) for a in sch.shared[key]})
                    return known[key]

                for r, v in enumerate(sch.sums):
                    if len(sch.prods[r][1]) == 1:
                        val = load(*next(iter(v)), row, k)
                    else:
                        val = _combine(v, {key: value(key) for key in v}).astype(BF16)
                    put(r, row, k, val)
                wrap = k + 1 == ncols
                return jnp.where(wrap, s + 1, s), jnp.where(wrap, 0, k + 1)
            lax.fori_loop(0, nrows // 16 * ncols, tile, (0, 0))

        def lanes_at(k):
            return pl.ds(pl.multiple_of(k * LANES, LANES), LANES)

        def prep_qkv(w, c, slot):
            def heads(i, carry):
                st = qst_v.at[slot, i].bitcast(U32)
                for jp in range(H // 2):
                    for k, x in enumerate(_halves(st[pl.ds(jp, QR, stride=H // 2), :])):
                        qtr_v[i, 2 * jp + k] = x.astype(BF16)
                return carry
            lax.fori_loop(0, NA, heads, 0)

            def put(r, row, k, val):
                wqkv_v[w, k, r, rows_at(c * QR + row, 16), :] = val
            prep_tiles(SA, lambda i, j, row, k: qtr_v[i, j * HB + k, pl.ds(row, 16), :], put, QR, HB)

        def prep_from_big(sch, dst, base, blk, c, nrows):
            ncols = D // sch.n // LANES

            def load(i, j, row, k):
                return big_v[rows_at(base + i * blk + row, 16), lanes_at(j * ncols + k)]

            def put(r, row, k, val):
                dst[k, r, rows_at(c * nrows + row, 16), :] = val
            prep_tiles(sch, load, put, nrows, ncols)

        def prep_gu(w, c):
            def put8(r, row, k, val):
                wgu8_v[w, k, r, rows_at(c * GR + row, 16), :] = val
            prep_tiles(SA, lambda i, j, row, k: gst_v[w, c, i, pl.ds(row, 16),
                                                      lanes_at(j * NG + k)], put8, GR, NG)

            def put4(r, row, k, val):
                wgu4_v[w, r, rows_at(k * DA + c * GR + row, 16), :] = val
            prep_tiles(SB, lambda i, j, row, k: gst_v[w, c, 2 * i + k, pl.ds(row, 16),
                                                      F8 + j * LANES:F8 + (j + 1) * LANES],
                       put4, GR, 2)

        x_head = pltpu.make_async_copy(x_hbm.at[0:XH, :], x_v.at[0:XH, :], sem_x.at[0])
        x_tail = pltpu.make_async_copy(x_hbm.at[XH:, :], x_v.at[XH:, :], sem_x.at[1])
        NQ, NO = DA // QR, EB // WR
        AHEAD = 5
        assert QST <= min(NQ, AHEAD) and AHEAD <= OST <= NO
        QA = QST - 1
        for n in range(QA):
            start(q_copies(0, n, n))
        mem0_copy = pltpu.make_async_copy(mem0_hbm, mem0_v, sem_x.at[2])
        x_head.start()
        mem0_copy.start()

        ri = lax.broadcasted_iota(jnp.int32, (2 * L, LANES), 0)
        ci = lax.broadcasted_iota(jnp.int32, (2 * L, LANES), 1)
        first = jnp.where(ri < L, 0, L)
        same = (ci >= first) & (ci < first + L)
        visible = (ri < first + M) | (ri >= ci)
        keep_v[...] = (same & visible).astype(jnp.int32)
        fill_v[...] = jnp.where(same, -1e9 / scale, -jnp.inf).astype(F32)
        kv_v[...] = jnp.zeros(kv_v.shape, BF16)

        for w in range(3):
            def q_body(c, carry, w=w):
                slot, free = (w * NQ + c) % QST, (w * NQ + c + QA) % QST
                wait(q_copies(w, c, slot))
                pl.when(c + QA < NQ)(lambda: start(q_copies(w, c + QA, free)))
                if w < 2:
                    pl.when(c + QA >= NQ)(lambda: start(q_copies(w + 1, c + QA - NQ, free)))
                else:
                    pl.when(c + QA >= NQ)(lambda: start(o_copies(c + QA - NQ)))
                prep_qkv(w, c, slot)
                return carry
            lax.fori_loop(0, NQ, q_body, 0)

        for c in range(QA, AHEAD):
            start(o_copies(c))
        x_head.wait()
        mem0_copy.wait()
        xa_v[...] = x_v[0:2 * SEG, :].astype(F32)
        mem_v[0:M, :] = mem0_v[...].astype(F32)
        mem_v[M:, :] = mem0_v[...].astype(F32)

        def load_out_weights():
            def chunk(c, carry):
                wait(o_copies(c))
                prep_from_big(SA, wo_v, (c % OST) * NA * WR, WR, c, WR)
                pl.when(c + AHEAD < NO)(lambda: start(o_copies(c + AHEAD)))
                pl.when(c >= NO - 2)(lambda: start(g_copies(0, c - (NO - 2))))
                return carry
            lax.fori_loop(0, NO, chunk, 0)
            for c in range(2, GST):
                start(g_copies(0, c))
            start(g_copies(1, 0))

        def load_gate_up_weights():
            def gate(c, carry):
                pl.when(c + 1 < GST)(lambda: start(g_copies(1, c + 1)))
                wait(g_copies(0, c))
                prep_gu(0, c)
                return carry

            def up(c, carry):
                wait(g_copies(1, c))
                prep_gu(1, c)
                start(d_copies(c))
                return carry
            lax.fori_loop(0, GST, gate, 0)
            lax.fori_loop(0, GST, up, 0)

        def load_down_weights():
            def chunk(c, carry):
                wait(d_copies(c))
                pl.when(c == 0)(lambda: x_tail.start())
                prep_from_big(SA, wd8_v, c * DR, FA, c, DR)
                prep_from_big(SB, wd4_v, F8 + c * ER, LANES, c, ER)
                return carry
            lax.fori_loop(0, GST, chunk, 0)

        def attention(c, paired):
            n = 2 * L if paired else L
            probs = {}

            def scores(j):
                s = _dot_nt(q_v[j, 0:n, :], kv_v[0, j])
                s = jnp.where(keep_v[0:n, :] != 0, s, fill_v[0:n, :])
                mx = jnp.max(s, axis=-1, keepdims=True)
                e = jnp.exp2((s - mx) * c_exp)
                den = jnp.sum(e, axis=-1, keepdims=True)
                inv = pl.reciprocal(den, approx=True)
                inv = inv * (2.0 - den * inv)
                probs[j] = e * inv

            def values(j):
                o = _dot(probs[j], kv_v[1, j])
                o_v[0:n, tile_of(j, EB, c)] = o
                if paired:
                    o_v[n:, tile_of(j, EB, c)] = o[:L] + o[L:]

            return ([functools.partial(scores, j) for j in range(NA)],
                    [functools.partial(values, j) for j in range(NA)])

        def project_qkv(w, c, paired, hooks):
            def block(hf, i):
                cols = slice(i * DA, (i + 1) * DA)
                if hf == 2:
                    return jnp.concatenate([ma_v[0:M, cols] + ma_v[M:, cols],
                                            na_v[2 * SEG:, cols]], axis=0)
                return jnp.concatenate([ma_v[hf * M:(hf + 1) * M, cols],
                                        na_v[hf * SEG:(hf + 1) * SEG, cols]], axis=0)

            p = fast_dot(SA, paired, tiles_of(wqkv_v, w, c), block, la_v, w + c == 0, hooks)
            for j in range(NA):
                x = jnp.concatenate([p[0, j], p[1, j]], axis=0) if paired else p[j]
                if w == 0:
                    q_v[j, 0:x.shape[0], :] = x
                else:
                    kv_v[w - 1, j, 0:x.shape[0], :] = x.astype(BF16)

        def project_out(c, paired, hooks=None):
            return fast_dot(SA, paired, tiles_of(wo_v, c), blocks_of(o_v, L, EB), hooks=hooks)

        def glu_input():
            nb = _layernorm(ya_v[0:2 * SEG, :], 0.5)
            nb_v[...] = jnp.concatenate([nb, nb[:SEG] + nb[SEG:]], axis=0)

        def gate_up_pieces():
            gate = {}

            def activate(cols, g, u):
                act = [jnp.tanh(g[hf]) * u[hf] + u[hf] for hf in range(2)]
                act_v[:, cols] = jnp.concatenate(act + [act[0] + act[1]], axis=0)

            def large(k, w):
                p = fast_dot(SA, True, tiles_of(wgu8_v, w, k), blocks_of(nb_v, SEG, DA), lb_v,
                             k + w == 0)
                if w == 0:
                    gate.update(p)
                else:
                    for j in range(NA):
                        activate(tile_of(j, FA, k), (gate[0, j], gate[1, j]), (p[0, j], p[1, j]))

            def small():
                p = fast_dot(SB, True, lambda r: jnp.concatenate(
                    [tiles_of(wgu4_v, w)(r) for w in range(2)], axis=1), blocks_of(nb_v, SEG, DB))
                for j in range(NB):
                    activate(slice(F8 + j * LANES, F8 + (j + 1) * LANES),
                             [p[hf, j][:, :LANES] for hf in range(2)],
                             [p[hf, j][:, LANES:] for hf in range(2)])

            return [small] + [functools.partial(large, k, w) for k in range(NG) for w in range(2)]

        def down_small():
            acc = {}
            for k in range(DB // LANES):
                p = fast_dot(SB, True, tiles_of(wd4_v, k), blocks_of(act_v, SEG, LANES, F8))
                acc.update({(hf, j * (DB // LANES) + k): v for (hf, j), v in p.items()})
            for (hf, j), v in acc.items():
                rows = slice(hf * SEG, (hf + 1) * SEG)
                z_v[rows, tile_of(j, DA, 0)] = ya_v[rows, tile_of(j, DA, 0)] + v

        def down_large(hooks=None):
            acc = fast_dot(SA, True, tiles_of(wd8_v, 0), blocks_of(act_v, SEG, FA),
                           hooks=hooks)
            for (hf, j), v in acc.items():
                z_v[hf * SEG:(hf + 1) * SEG, tile_of(j, DA, 0)] += v

        def out_copy(row, n):
            return pltpu.make_async_copy(big_v.at[pl.ds(row, n), :],
                                         out_hbm.at[pl.ds(row, n), :], sem_out)

        def attention_single(mrow, xrow, yrow, before_out):
            ma_v[0:M, :] = mem_v[pl.ds(mrow, M), :]
            na_v[0:SEG, :] = _layernorm(xa_v[pl.ds(xrow, SEG), :])
            hooks = None
            for c in range(HB):
                scores, values = attention(c, False)
                project_qkv(0, c, False, hooks)
                project_qkv(1, c, False, None)
                project_qkv(2, c, False, spread(scores, 20, 7))
                hooks = spread(values, 24, 9)
            for piece in values:
                piece()
            before_out()
            for c in range(DA // LANES):
                for j, v in project_out(c, False).items():
                    mem_v[pl.ds(mrow, M), tile_of(j, DA, c)] = v[:M]
                    ya_v[pl.ds(yrow, SEG), tile_of(j, DA, c)] = (
                        xa_v[pl.ds(xrow, SEG), tile_of(j, DA, c)] + v[M:])

        def step(t, carry):
            cur = pl.multiple_of(t * SEG, SEG)
            nxt = pl.multiple_of(jnp.minimum(t + 1, NSEG - 1) * SEG, SEG)
            pl.when(t + 1 == XH // SEG)(lambda: x_tail.wait())
            row = pl.multiple_of(jnp.maximum(t - 3, 0) * SEG, SEG)
            hooks = {50: glu_input}
            gpos = [1, 3, 4, 6, 7, 9, 10]
            def next_tokens():
                na_v[:SEG, :] = _layernorm(x_v[pl.ds(nxt, SEG), :].astype(F32))

            glu = gate_up_pieces()
            for c in range(HB):
                scores, values = attention(c, True)
                for w in range(3):
                    project_qkv(w, c, True, (hooks, None, spread(
                        scores, 20, 10))[w])
                    if 3 * c + w in gpos:
                        glu[gpos.index(3 * c + w)]()
                    if 3 * c + w == 5:
                        down_small()
                hooks = spread(values, 26, 10)
                if c == 2:
                    hooks[5] = next_tokens
            down_large(spread(values, 12, 8))
            big_v[pl.ds(row, SEG), :] = z_v[SEG:, :].astype(BF16)

            def next_input():
                na = _layernorm(z_v[:SEG, :])
                na_v[SEG:, :] = jnp.concatenate([na, na + na_v[:SEG, :]], axis=0)

            for c in range(DA // LANES):
                o = project_out(c, True, {2: next_input} if c == 0 else None)
                for (hf, j), v in o.items():
                    cols = tile_of(j, DA, c)
                    res = x_v[pl.ds(cur, SEG), cols].astype(F32) if hf == 0 else xa_v[SEG:, cols]
                    ma_v[hf * M:(hf + 1) * M, cols] = v[:M]
                    ya_v[hf * SEG:(hf + 1) * SEG, cols] = res + v[M:]
            xa_v[SEG:, :] = z_v[:SEG, :]
            pl.when(t >= 3)(lambda: out_copy(row, SEG).start())
            return carry

        def phase(ph, carry):
            attention_single(pl.multiple_of(jnp.where(ph < 2, 0, M), M),
                             pl.multiple_of(jnp.where(ph == 0, 0, SEG), SEG),
                             pl.multiple_of(jnp.where(ph == 3, 1, ph) * SEG, SEG),
                             lambda: pl.when(ph == 0)(load_out_weights))
            pl.when(ph == 1)(load_gate_up_weights)

            @pl.when(ph >= 1)
            def _():
                glu_input()
                for piece in gate_up_pieces():
                    piece()
                pl.when(ph == 1)(load_down_weights)
                down_small()
                down_large()

            @pl.when(ph == 1)
            def _():
                ya_v[0:SEG, :] = ya_v[SEG:2 * SEG, :]
                xa_v[SEG:, :] = z_v[:SEG, :]
                ma_v[...] = mem_v[...]
                na_v[:SEG, :] = _layernorm(x_v[2 * SEG:3 * SEG, :].astype(F32))
                na = _layernorm(z_v[:SEG, :])
                na_v[SEG:, :] = jnp.concatenate([na, na + na_v[:SEG, :]], axis=0)
                lax.fori_loop(2, NSEG, step, 0)
                mem_v[...] = ma_v[...]

            @pl.when(ph == 2)
            def _():
                xa_v[SEG:, :] = z_v[:SEG, :]
                ya_v[0:SEG, :] = ya_v[2 * SEG:, :]
                big_v[S - 3 * SEG:S - 2 * SEG, :] = z_v[SEG:, :].astype(BF16)
                out_copy(S - 3 * SEG, SEG).start()

            @pl.when(ph == 3)
            def _():
                big_v[S - 2 * SEG:S, :] = z_v[...].astype(BF16)
                out_copy(S - 2 * SEG, 2 * SEG).start()
            return carry

        lax.fori_loop(0, 4, phase, 0)
        out_copy(0, NSEG * SEG).wait()

    scratch = [
        pltpu.VMEM((S, D), BF16),
        pltpu.VMEM((M, D), BF16),
        pltpu.VMEM((FF, D), BF16),
        pltpu.VMEM((2, GST, NA, GR, FF), BF16),
        pltpu.VMEM((QST, NA, (QR + 1) * H, DH), BF16),
        pltpu.VMEM((NA, H, QR, DH), BF16),
        pltpu.VMEM((3, HB, PA, DA, DH), BF16),
        pltpu.VMEM((DA // LANES, PA, EB, LANES), BF16),
        pltpu.VMEM((2, NG, PA, DA, LANES), BF16),
        pltpu.VMEM((2, PB, DB, LANES), BF16),
        pltpu.VMEM((1, PA, FA, LANES), BF16),
        pltpu.VMEM((DB // LANES, PB, LANES, LANES), BF16),
        pltpu.VMEM((PA, L, DA), F32),
        pltpu.VMEM((PA, SEG, DA), F32),
        pltpu.VMEM((3 * L, H * DH), F32),
        pltpu.VMEM((3 * SEG, FF), F32),
        pltpu.VMEM((2 * M, D), F32),
        pltpu.VMEM((2 * M, D), F32),
        pltpu.VMEM((2 * SEG, D), F32),
        pltpu.VMEM((3 * SEG, D), F32),
        pltpu.VMEM((3 * SEG, D), F32),
        pltpu.VMEM((3 * SEG, D), F32),
        pltpu.VMEM((2 * SEG, D), F32),
        pltpu.VMEM((NA, 2 * L, DH), F32),
        pltpu.VMEM((2, NA, LANES, DH), BF16),
        pltpu.VMEM((2 * L, LANES), F32),
        pltpu.VMEM((2 * L, LANES), jnp.int32),
        pltpu.SemaphoreType.DMA((3,)),
        pltpu.SemaphoreType.DMA((QST,)),
        pltpu.SemaphoreType.DMA((OST,)),
        pltpu.SemaphoreType.DMA((2, GST)),
        pltpu.SemaphoreType.DMA((GST,)),
        pltpu.SemaphoreType.DMA(()),
    ]
    return kernel, scratch


@functools.partial(jax.jit, static_argnames=("A_seg_len",))
def pallas_interleave_layers__memory_aug_recurrent_mem_tr__glu_gated_glu__prompt_kernel(
    A_x, A_mem0, A_Wq, A_Wk, A_Wv, A_Wo, A_seg_len, B_x, B_w_gate, B_w_up, B_w_down,
):
    del B_x
    B, S, D = A_x.shape
    _, H, DH = A_Wq.shape
    M = A_mem0.shape[1]
    assert B == 1
    kernel, scratch = _make_kernel(S, D, H, DH, M, A_seg_len, B_w_gate.shape[1])
    any_spec = pl.BlockSpec(memory_space=pl.ANY)
    out = pl.pallas_call(
        kernel,
        out_shape=jax.ShapeDtypeStruct((S, D), A_x.dtype),
        in_specs=[any_spec] * 9,
        out_specs=any_spec,
        scratch_shapes=scratch,
        compiler_params=pltpu.CompilerParams(vmem_limit_bytes=126 * 1024 * 1024),
    )(A_x.reshape(S, D), A_mem0.reshape(M, D),
      A_Wq.reshape(D * H, DH), A_Wk.reshape(D * H, DH), A_Wv.reshape(D * H, DH),
      A_Wo.reshape(H * DH, D), B_w_gate, B_w_up, B_w_down)
    return out.reshape(B, S, D)
```

```python
import functools
import itertools
import math

import jax
import jax.numpy as jnp
import numpy as np
from jax import lax
import jax.experimental.pallas as pl
import jax.experimental.pallas.tpu as pltpu

F32 = jnp.float32
BF16 = jnp.bfloat16
U32 = jnp.uint32
EPS = 1e-05
LANES = 128

_SCHEME_4 = """
+00 | +00 +02 -10 +30 | +00 -10
+00 +10 | +00 -01 +20 -30 | +10

+00 -11 | +01 -10 +30 | +01 +10
+10 +11 | +01 | +10 +11
+00 +01 | +03 +10 -30 | +00 +01

+00 +10 +11 +13 | +30 | -00 -01 +03 +10
+00 +01 +03 +10 +11 +13 | -03 +30 | +00 +01 -03
+03 +10 +11 +13 | +03 | +00 +01 -03 +13

+00 +10 -12 | +02 -20 | -00 +02 +10
+10 -12 | +02 | +00 -02 -10 +12
+00 -02 +10 -12 | +20 | -00 +02

+11 | +01 -11 -12 +31 | +01 -11
+01 +11 | -03 -10 +11 +13 -21 +30 | +01

-03 +11 | -03 +13 +31 | -01 +13
+01 +03 | -03 +13 +30 | -01 +03
+11 +13 | +31 | +11 -13

+01 +02 +11 | +12 +21 | +01 -11 +12
+01 +02 | +12 | -01 +02 +11 -12
+01 +02 +11 +12 | +21 | +11 -12

+03 +12 +13 | -23 -32 | -02 +03 -13
+02 +03 +12 +13 | +23 | -02 +03
+12 +13 | +32 | -02 +03 +12 -13

+02 | -12 +20 +22 +23 | +02
+12 | +02 +21 +22 -32 | +12

+03 | +03 -13 +32 +33 | +03 -13
+03 +13 | -03 -23 +31 +33 | +13
"""
_SCHEME_8 = """
+01 +10 | +01 +10 | +00 +11
+00 -01 | +01 | +00 +01
+10 -11 | +10 | -10 -11

+00 +02 +10 | +02 +20 | +00 -10 +12
+00 +02 | +02 | -00 +02 +10 -12
+00 +02 +10 +12 | +20 | +10 -12

+00 +03 -04 +10 | +30 | +00 -10 -13 -14
+00 +03 -04 +10 +13 -14 | +03 +30 | +10 +13 +14
+00 +03 -04 +13 | +03 | +03 -10 -13 -14

+04 +10 | +04 +30 +40 -74 | +00 +14
+00 -04 | +04 -47 -74 | +00 +04
+10 -14 | -03 -30 -40 | +10 +14

+00 -05 +10 | +05 +50 | -00 +10 +15
+00 -05 | +05 | +00 +05 -10 -15
+00 -05 +10 -15 | +50 | -10 -15

+00 +06 +07 +10 | +60 | +00 -10 -16 +17
+00 +06 +07 +10 +16 +17 | +06 +60 | +10 +16 -17
+00 +06 +07 +16 | +06 | +06 -10 -16 +17

-07 +10 | +07 +47 -60 +70 | -00 +17
+00 +07 | +07 +47 +74 | -00 +07
+10 +17 | +06 +60 -70 | -10 +17

+10 | -00 -02 +05 -10 -30 -40 -60 +70 | +00 -10
+00 +10 | +00 -01 -04 +07 -20 -30 +47 +50 -60 +74 | +00

+01 +11 -12 | +12 +21 | +01 +02 -11
+11 -12 | +12 | -01 -02 +11 +12
+01 -02 +11 -12 | +21 | -01 -02

+01 +13 | +13 +31 +63 -71 | +03 +11
+11 -13 | +13 -36 +63 | +11 +13
+01 -03 | -17 -31 +71 | +01 +03

+01 +11 +14 -16 | +41 | -01 +04 +06 +11
+01 +04 -06 +11 +14 -16 | -14 +41 | +01 -04 -06
+04 +11 +14 -16 | +14 | +01 -04 -06 +14

+01 +11 +15 | +15 -51 | +01 +05 -11
+11 +15 | +15 | -01 -05 +11 +15
+01 +05 +11 +15 | +51 | +01 +05

+01 +16 | +16 +36 -41 -61 | +06 -11
+11 -16 | +16 +36 -63 | -11 +16
+01 -06 | -14 +41 +61 | -01 +06

+01 +11 -13 -17 | +71 | +01 +03 +07 -11
+01 -03 -07 +11 -13 -17 | +17 -71 | +01 +03 +07
-07 +11 -13 -17 | +17 | -01 -03 -07 +17

+01 | +01 +11 -12 -15 +31 +41 +61 -71 | +01 -11
+01 +11 | -10 +11 -13 +16 +21 +36 -41 -51 -63 +71 | +11

+02 +03 +13 | +23 -32 -52 | +03 -12 -13
+02 +03 +12 +13 | +23 | +12 +13
+02 +03 | +25 +32 +52 | +02 +03 -12 -13

-04 +12 -14 | -24 -42 | +02 +04 -14
+02 -04 +12 -14 | +24 | +02 +04
+12 -14 | +42 | +02 +04 -12 -14

+03 -05 +12 +13 -15 | +52 | -02 -03 +05 +13 -15
+12 +13 -15 | +25 +52 | +02 +03 -05 -12 -13 +15
+02 +03 +12 +13 -15 | +25 | -02 -03 +05 +12 +13

+02 +06 +16 | +26 -62 | +06 -12 -16
+02 +06 +12 +16 | +26 | +12 +16
+02 +06 | +62 | +02 +06 -12 -16

+07 +12 +17 | -27 -72 | -02 +07 -17
+02 +07 +12 +17 | +27 | -02 +07
+12 +17 | +72 | -02 +07 +12 -17

+02 | -02 -21 +22 -24 +27 -32 -52 -62 | +02
+12 | +12 +20 +22 -23 -26 +42 +52 -72 | +12

+04 +13 | +03 +34 +43 | +03 +14
+03 -04 | +34 | +03 +04
+13 -14 | -03 -30 -43 | +13 +14

+03 -05 +13 | -25 +35 -53 | +03 -13 +15
+03 -05 | -25 +35 -52 | -03 +05 +13 -15
+03 -05 +13 -15 | +53 | -13 +15

-01 +03 +06 +13 | +63 | +03 -11 -13 +16
-01 +03 +06 -11 +13 +16 | -36 +63 | +11 +13 -16
-01 +03 +06 +16 | +36 | +06 +11 +13 -16

-07 +13 | +17 +37 -73 | +03 +17
+03 +07 | +17 +37 -71 | +03 +07
+13 +17 | +73 | +13 +17

+13 | -03 -13 +25 +32 -33 -35 -43 +52 -63 +73 | +03 -13
+03 +13 | -03 -17 -23 -31 +33 -34 -37 +53 -63 +71 | +03

+04 +14 +15 | +45 -54 | +04 +05 -14
+14 +15 | +45 | -04 -05 +14 +15
+04 +05 +14 +15 | +54 | +04 +05

+04 +16 | +14 +46 +64 | +06 +14
+14 -16 | +46 | +14 +16
+04 -06 | -14 +41 -64 | +04 +06

+04 -10 +14 -17 | +74 | +00 +04 -07 -14
-00 +04 -07 -10 +14 -17 | -47 -74 | +00 +04 -07
-07 -10 +14 -17 | +47 | +00 +04 -07 +17

+04 | +04 +14 +34 -42 +44 -45 +64 -74 | +04 -14
+04 +14 | -03 -14 +24 -30 -40 -43 +44 -46 -54 +74 | +14

+05 +06 +16 | +56 -65 | +06 -15 -16
+05 +06 +15 +16 | +56 | +15 +16
+05 +06 | +65 | +05 +06 -15 -16

+07 +15 +17 | -57 -75 | -05 +07 -17
+05 +07 +15 +17 | +57 | -05 +07
+15 +17 | +75 | -05 +07 +15 -17

+05 | +05 -25 +35 -51 -54 +55 +57 -65 | +05
+15 | -15 +25 -45 -50 +53 +55 -56 -75 | +15

-07 +16 | -06 +67 +76 | -06 +17
+06 +07 | +67 | -06 +07
+16 +17 | +06 +60 -76 | -16 +17

+16 | -06 -16 -36 -46 +62 +65 -66 +76 | +06 -16
+06 +16 | -06 -14 -26 -36 +41 -56 +61 -64 +66 +67 | +06

+07 | -07 -17 -37 -47 -67 +72 +75 +77 | +07 -17
+07 +17 | -06 +17 -27 +47 -57 -60 +70 -73 +76 +77 | +17
"""


class _Scheme:
    def __init__(self, n, text):
        def terms(field):
            return {(int(t[1]), int(t[2])): 1 if t[0] == "+" else -1 for t in field.split()}

        def fold(coefs, weights):
            out = {}
            for (h, i), c in coefs.items():
                out[i] = out.get(i, 0) + weights[h] * c
            return {i: c for i, c in out.items() if c}

        self.n = n
        self.prods, self.ends = [], []
        for group in text.strip().split("\n\n"):
            self.prods += [tuple(terms(f) for f in line.split("|")) for line in group.split("\n")]
            self.ends.append(len(self.prods) - 1)
        dense = np.zeros((3, len(self.prods), n, n), np.int64)
        for r, prod in enumerate(self.prods):
            for m, coefs in enumerate(prod):
                for (i, j), c in coefs.items():
                    dense[m, r, i, j] = c
        eye = np.eye(n, dtype=np.int64)
        assert np.array_equal(
            np.einsum("rai,rjk,rbl->aijkbl", dense[0, :, :2], dense[1], dense[2, :, :2]),
            np.einsum("ab,ij,kl->aijkbl", eye[:2, :2], eye, eye)), "not the matrix product"
        assert all(len(v) > 1 or sum(v.values()) == 1 for _, v, _ in self.prods)
        folded = [(fold(u, (-1, 1)), fold(w, (0, 1))) for u, _, w in self.prods]
        self.single = [(u, w) if u and w else None for u, w in folded]
        self.sums, self.shared = [dict(v) for _, v, _ in self.prods], {}
        while True:
            count = {}
            for v in self.sums:
                for a, b in itertools.combinations(sorted(v), 2):
                    count[a, b, v[a] * v[b]] = count.get((a, b, v[a] * v[b]), 0) + 1
            (a, b, sign), times = max(count.items(), key=lambda kv: kv[1])
            if times < 2:
                break
            key = (n, len(self.shared))
            self.shared[key] = {a: 1, b: sign}
            for v in self.sums:
                if a in v and b in v and v[a] * v[b] == sign:
                    v[key] = v.pop(a)
                    del v[b]


def _combine(coefs, vals):
    acc = None
    for key, c in sorted(coefs.items(), key=lambda kv: -kv[1]):
        v = vals[key]
        if abs(c) != 1:
            v = v * abs(c)
        if acc is None:
            acc = v if c > 0 else -v
        else:
            acc = acc + v if c > 0 else acc - v
    return acc


def _accumulate(accs, group):
    terms = {}
    for n, (coefs, _) in enumerate(group):
        for key, c in coefs.items():
            terms.setdefault(key, []).append((n, c))
    sums = {((n, 1),): v for n, (_, v) in enumerate(group)}
    for key, tm in sorted(terms.items(), key=lambda kv: len(kv[1])):
        sign = tm[0][1]
        tm = tuple((n, c * sign) for n, c in tm)
        if tm not in sums:
            base = max((s for s in sums if all(t in tm for t in s)), key=len)
            val = sums[base]
            for n, c in tm:
                if (n, c) not in base:
                    val = val + group[n][1] if c > 0 else val - group[n][1]
            sums[tm] = val
        if key not in accs:
            accs[key] = sums[tm] if sign > 0 else -sums[tm]
        else:
            accs[key] = accs[key] + sums[tm] if sign > 0 else accs[key] - sums[tm]


def _layernorm(x, gain=1.0):
    m = jnp.mean(x, axis=-1, keepdims=True)
    c = x - m
    v = jnp.mean(c * c, axis=-1, keepdims=True)
    inv = lax.rsqrt(v + EPS)
    return c * (inv if gain == 1.0 else inv * gain)


def _dot(a, b):
    return lax.dot_general(a, b, (((1,), (0,)), ((), ())), preferred_element_type=F32)


def _dot_nt(a, b):
    return lax.dot_general(a, b, (((1,), (1,)), ((), ())), preferred_element_type=F32)


def _halves(x):
    return pltpu.bitcast(x << 16, F32), pltpu.bitcast(x & np.uint32(0xFFFF0000), F32)


def _make_kernel(S, D, H, DH, M, SEG, FF):
    SA = _Scheme(8, _SCHEME_8)
    SB = _Scheme(4, _SCHEME_4)
    NA, NB = SA.n, SB.n
    PA, PB = len(SA.prods), len(SB.prods)
    NSEG = S // SEG
    L = M + SEG
    DA, HB = D // NA, H // NA
    EB = HB * DH
    NG = FF // (NA * LANES)
    FA = NG * LANES
    F8 = NA * FA
    DB = D // NB
    assert DA == LANES and DH == LANES and FF - F8 == NB * LANES
    QR = 128 // NA
    QST = 4
    WR = 512 // NA
    OST = FF // (WR * NA)
    GST = 4
    GR, DR, ER = DA // GST, FA // GST, LANES // GST
    XH = 4 * SEG
    scale = DH ** (-0.5)
    c_exp = scale * math.log2(math.e)

    def fast_dot(sch, paired, w_of, block, kept_ref=None, fresh=True, hooks=None):
        acc, group = {}, []
        for r, (u, _, w) in enumerate(sch.prods):
            if hooks and r in hooks:
                hooks[r]()
            if paired or sch.single[r]:
                if not paired:
                    u, w = sch.single[r]
                if fresh:
                    if not paired:
                        u = {(0, i): c for i, c in u.items()}
                    else:
                        u = {(2 if u.get((1 - hf, i)) == c else hf, i): c
                             for (hf, i), c in u.items()}
                    lhs = _combine(u, {key: block(*key) for key in u})
                    if kept_ref is not None:
                        kept_ref[r] = lhs
                else:
                    lhs = kept_ref[r]
                group.append((w, _dot(lhs, w_of(r))))
            if r in sch.ends:
                _accumulate(acc, group)
                group = []
        return acc

    def tiles_of(ref, *index):
        return lambda r: pltpu.bitcast(ref.bitcast(U32)[(*index, r)], BF16)

    def blocks_of(ref, rows, cols, c0=0):
        return lambda hf, i: ref[hf * rows:(hf + 1) * rows, c0 + i * cols:c0 + (i + 1) * cols]

    def spread(pieces, first, stride):
        return {first + n * stride: piece for n, piece in enumerate(pieces)}

    def tile_of(j, blk, c):
        return slice(j * blk + c * LANES, j * blk + (c + 1) * LANES)

    def kernel(x_hbm, mem0_hbm, wq_hbm, wk_hbm, wv_hbm, wo_hbm, wg_hbm, wu_hbm, wd_hbm,
               out_hbm,
               x_v, mem0_v, big_v, gst_v, qst_v, qtr_v, wqkv_v, wo_v, wgu8_v, wgu4_v, wd8_v, wd4_v,
               la_v, lb_v, o_v, act_v, mem_v, ma_v, xa_v, na_v, nb_v, ya_v, z_v,
               q_v, kv_v, fill_v, keep_v,
               sem_x, sem_q, sem_o, sem_g, sem_d, sem_out):

        def rows_at(start, size):
            return pl.ds(start if isinstance(start, int) else pl.multiple_of(start, 16), size)

        def q_copies(w, c, slot):
            src = (wq_hbm, wk_hbm, wv_hbm)[w]
            return [pltpu.make_async_copy(src.at[rows_at((i * DA + c * QR) * H, QR * H), :],
                                          qst_v.at[slot, i, 0:QR * H, :], sem_q.at[slot])
                    for i in range(NA)]

        def o_copies(c):
            slot = c % OST
            return [pltpu.make_async_copy(wo_hbm.at[rows_at(i * EB + c * WR, WR), :],
                                          big_v.at[rows_at((slot * NA + i) * WR, WR), :],
                                          sem_o.at[slot]) for i in range(NA)]

        def g_copies(w, c):
            return [pltpu.make_async_copy((wg_hbm, wu_hbm)[w].at[rows_at(i * DA + c * GR, GR), :],
                                          gst_v.at[w, c, i], sem_g.at[w, c]) for i in range(NA)]

        def d_copies(c):
            rows = ([rows_at(i * FA + c * DR, DR) for i in range(NA)]
                    + [rows_at(F8 + i * LANES + c * ER, ER) for i in range(NB)])
            return [pltpu.make_async_copy(wd_hbm.at[r, :], big_v.at[r, :], sem_d.at[c])
                    for r in rows]

        def start(copies):
            for cp in copies:
                cp.start()

        def wait(copies):
            for cp in copies:
                cp.wait()

        def prep_tiles(sch, load, put, nrows, ncols):
            def tile(_, pos):
                s, k = pos
                row = pl.multiple_of(s * 16, 16)
                known = {}

                def value(key):
                    if key not in sch.shared:
                        return load(*key, row, k).astype(F32)
                    if key not in known:
                        known[key] = _combine(sch.shared[key],
                                              {a: value(a) for a in sch.shared[key]})
                    return known[key]

                for r, v in enumerate(sch.sums):
                    if len(sch.prods[r][1]) == 1:
                        val = load(*next(iter(v)), row, k)
                    else:
                        val = _combine(v, {key: value(key) for key in v}).astype(BF16)
                    put(r, row, k, val)
                wrap = k + 1 == ncols
                return jnp.where(wrap, s + 1, s), jnp.where(wrap, 0, k + 1)
            lax.fori_loop(0, nrows // 16 * ncols, tile, (0, 0))

        def lanes_at(k):
            return pl.ds(pl.multiple_of(k * LANES, LANES), LANES)

        def prep_qkv(w, c, slot):
            def heads(i, carry):
                st = qst_v.at[slot, i].bitcast(U32)
                for jp in range(H // 2):
                    for k, x in enumerate(_halves(st[pl.ds(jp, QR, stride=H // 2), :])):
                        qtr_v[i, 2 * jp + k] = x.astype(BF16)
                return carry
            lax.fori_loop(0, NA, heads, 0)

            def put(r, row, k, val):
                wqkv_v[w, k, r, rows_at(c * QR + row, 16), :] = val
            prep_tiles(SA, lambda i, j, row, k: qtr_v[i, j * HB + k, pl.ds(row, 16), :],
                       put, QR, HB)

        def prep_from_big(sch, dst, base, blk, c, nrows):
            ncols = D // sch.n // LANES

            def load(i, j, row, k):
                return big_v[rows_at(base + i * blk + row, 16), lanes_at(j * ncols + k)]

            def put(r, row, k, val):
                dst[k, r, rows_at(c * nrows + row, 16), :] = val
            prep_tiles(sch, load, put, nrows, ncols)

        def prep_gu(w, c):
            def put8(r, row, k, val):
                wgu8_v[w, k, r, rows_at(c * GR + row, 16), :] = val
            prep_tiles(SA, lambda i, j, row, k: gst_v[w, c, i, pl.ds(row, 16),
                                                      lanes_at(j * NG + k)], put8, GR, NG)

            def put4(r, row, k, val):
                wgu4_v[w, r, rows_at(k * DA + c * GR + row, 16), :] = val
            prep_tiles(SB, lambda i, j, row, k: gst_v[w, c, 2 * i + k, pl.ds(row, 16),
                                                      F8 + j * LANES:F8 + (j + 1) * LANES],
                       put4, GR, 2)

        x_head = pltpu.make_async_copy(x_hbm.at[0:XH, :], x_v.at[0:XH, :], sem_x.at[0])
        x_tail = pltpu.make_async_copy(x_hbm.at[XH:, :], x_v.at[XH:, :], sem_x.at[1])
        NQ, NO = DA // QR, EB // WR
        AHEAD = OST - 1
        assert QST <= min(NQ, AHEAD) and OST <= NO
        QA = QST - 1
        for n in range(QA):
            start(q_copies(0, n, n))
        mem0_copy = pltpu.make_async_copy(mem0_hbm, mem0_v, sem_x.at[2])
        x_head.start()
        mem0_copy.start()

        ri = lax.broadcasted_iota(jnp.int32, (2 * L, LANES), 0)
        ci = lax.broadcasted_iota(jnp.int32, (2 * L, LANES), 1)
        first = jnp.where(ri < L, 0, L)
        same = (ci >= first) & (ci < first + L)
        visible = (ri < first + M) | (ri >= ci)
        keep_v[...] = (same & visible).astype(jnp.int32)
        fill_v[...] = jnp.where(same, -1e9 / scale, -jnp.inf).astype(F32)
        kv_v[...] = jnp.zeros(kv_v.shape, BF16)

        for w in range(3):
            def q_body(c, carry, w=w):
                slot, free = (w * NQ + c) % QST, (w * NQ + c + QA) % QST
                wait(q_copies(w, c, slot))
                pl.when(c + QA < NQ)(lambda: start(q_copies(w, c + QA, free)))
                if w < 2:
                    pl.when(c + QA >= NQ)(lambda: start(q_copies(w + 1, c + QA - NQ, free)))
                else:
                    pl.when(c + QA >= NQ)(lambda: start(o_copies(c + QA - NQ)))
                prep_qkv(w, c, slot)
                return carry
            lax.fori_loop(0, NQ, q_body, 0)

        for c in range(QA, AHEAD):
            start(o_copies(c))
        x_head.wait()
        mem0_copy.wait()
        xa_v[...] = x_v[0:2 * SEG, :].astype(F32)
        mem_v[0:M, :] = mem0_v[...].astype(F32)
        mem_v[M:, :] = mem0_v[...].astype(F32)

        def load_out_weights():
            def chunk(c, carry):
                pl.when(c + AHEAD < NO)(lambda: start(o_copies(c + AHEAD)))
                pl.when(c == NO // 2 - 1)(lambda: start(g_copies(0, 0)))
                pl.when(c == NO - 2)(lambda: start(g_copies(0, 1)))
                wait(o_copies(c))
                prep_from_big(SA, wo_v, (c % OST) * NA * WR, WR, c, WR)
                return carry
            lax.fori_loop(0, NO, chunk, 0)
            for c in range(2, GST):
                start(g_copies(0, c))
            start(g_copies(1, 0))
            start(g_copies(1, 1))

        def load_gate_up_weights():
            def gate(c, carry):
                pl.when(c + 2 < GST)(lambda: start(g_copies(1, c + 2)))
                wait(g_copies(0, c))
                prep_gu(0, c)
                return carry

            def up(c, carry):
                wait(g_copies(1, c))
                prep_gu(1, c)
                pl.when(c == 0)(lambda: start(d_copies(0)))
                return carry
            lax.fori_loop(0, GST, gate, 0)
            lax.fori_loop(0, GST, up, 0)
            for c in range(1, 3):
                start(d_copies(c))

        def load_down_weights():
            def chunk(c, carry):
                pl.when(c + 3 < GST)(lambda: start(d_copies(c + 3)))
                wait(d_copies(c))
                pl.when(c == GST - 1)(lambda: x_tail.start())
                prep_from_big(SA, wd8_v, c * DR, FA, c, DR)
                prep_from_big(SB, wd4_v, F8 + c * ER, LANES, c, ER)
                return carry
            lax.fori_loop(0, GST, chunk, 0)

        def attention(c, paired):
            n = 2 * L if paired else L
            probs = {}

            def scores(j):
                s = _dot_nt(q_v[j, 0:n, :], kv_v[0, j])
                s = jnp.where(keep_v[0:n, :] != 0, s, fill_v[0:n, :])
                mx = jnp.max(s, axis=-1, keepdims=True)
                e = jnp.exp2((s - mx) * c_exp)
                den = jnp.sum(e, axis=-1, keepdims=True)
                inv = pl.reciprocal(den, approx=True)
                inv = inv * (2.0 - den * inv)
                probs[j] = e * inv

            def values(j):
                o = _dot(probs[j], kv_v[1, j])
                o_v[0:n, tile_of(j, EB, c)] = o
                if paired:
                    o_v[n:, tile_of(j, EB, c)] = o[:L] + o[L:]

            return ([functools.partial(scores, j) for j in range(NA)],
                    [functools.partial(values, j) for j in range(NA)])

        def project_qkv(w, c, paired, hooks):
            def block(hf, i):
                cols = slice(i * DA, (i + 1) * DA)
                if hf == 2:
                    return jnp.concatenate([ma_v[0:M, cols] + ma_v[M:, cols],
                                            na_v[2 * SEG:, cols]], axis=0)
                return jnp.concatenate([ma_v[hf * M:(hf + 1) * M, cols],
                                        na_v[hf * SEG:(hf + 1) * SEG, cols]], axis=0)

            p = fast_dot(SA, paired, tiles_of(wqkv_v, w, c), block, la_v, w + c == 0, hooks)
            for j in range(NA):
                x = jnp.concatenate([p[0, j], p[1, j]], axis=0) if paired else p[j]
                if w == 0:
                    q_v[j, 0:x.shape[0], :] = x
                else:
                    kv_v[w - 1, j, 0:x.shape[0], :] = x.astype(BF16)

        def project_out(c, paired, hooks=None):
            return fast_dot(SA, paired, tiles_of(wo_v, c), blocks_of(o_v, L, EB), hooks=hooks)

        def glu_input():
            nb = _layernorm(ya_v[0:2 * SEG, :], 0.5)
            nb_v[...] = jnp.concatenate([nb, nb[:SEG] + nb[SEG:]], axis=0)

        def gate_up_pieces():
            gate = {}

            def activate(cols, g, u):
                act = [jnp.tanh(g[hf]) * u[hf] + u[hf] for hf in range(2)]
                act_v[:, cols] = jnp.concatenate(act + [act[0] + act[1]], axis=0)

            def large(k, w):
                p = fast_dot(SA, True, tiles_of(wgu8_v, w, k), blocks_of(nb_v, SEG, DA), lb_v,
                             k + w == 0)
                if w == 0:
                    gate.update(p)
                else:
                    for j in range(NA):
                        activate(tile_of(j, FA, k), (gate[0, j], gate[1, j]), (p[0, j], p[1, j]))

            def small():
                p = fast_dot(SB, True, lambda r: jnp.concatenate(
                    [tiles_of(wgu4_v, w)(r) for w in range(2)], axis=1), blocks_of(nb_v, SEG, DB))
                for j in range(NB):
                    activate(slice(F8 + j * LANES, F8 + (j + 1) * LANES),
                             [p[hf, j][:, :LANES] for hf in range(2)],
                             [p[hf, j][:, LANES:] for hf in range(2)])

            return [small] + [functools.partial(large, k, w) for k in range(NG) for w in range(2)]

        def down_small():
            acc = {}
            for k in range(DB // LANES):
                p = fast_dot(SB, True, tiles_of(wd4_v, k), blocks_of(act_v, SEG, LANES, F8))
                acc.update({(hf, j * (DB // LANES) + k): v for (hf, j), v in p.items()})
            for (hf, j), v in acc.items():
                rows = slice(hf * SEG, (hf + 1) * SEG)
                z_v[rows, tile_of(j, DA, 0)] = ya_v[rows, tile_of(j, DA, 0)] + v

        def down_large(hooks=None):
            acc = fast_dot(SA, True, tiles_of(wd8_v, 0), blocks_of(act_v, SEG, FA),
                           hooks=hooks)
            for (hf, j), v in acc.items():
                z_v[hf * SEG:(hf + 1) * SEG, tile_of(j, DA, 0)] += v

        def out_copy(row, n):
            return pltpu.make_async_copy(big_v.at[pl.ds(row, n), :],
                                         out_hbm.at[pl.ds(row, n), :], sem_out)

        def attention_single(mrow, xrow, yrow, before_out):
            ma_v[0:M, :] = mem_v[pl.ds(mrow, M), :]
            na_v[0:SEG, :] = _layernorm(xa_v[pl.ds(xrow, SEG), :])
            hooks = None
            for c in range(HB):
                scores, values = attention(c, False)
                project_qkv(0, c, False, hooks)
                project_qkv(1, c, False, None)
                project_qkv(2, c, False, spread(scores, 20, 7))
                hooks = spread(values, 24, 9)
            for piece in values:
                piece()
            before_out()
            for c in range(DA // LANES):
                for j, v in project_out(c, False).items():
                    mem_v[pl.ds(mrow, M), tile_of(j, DA, c)] = v[:M]
                    ya_v[pl.ds(yrow, SEG), tile_of(j, DA, c)] = (
                        xa_v[pl.ds(xrow, SEG), tile_of(j, DA, c)] + v[M:])

        def step(t, carry):
            cur = pl.multiple_of(t * SEG, SEG)
            nxt = pl.multiple_of(jnp.minimum(t + 1, NSEG - 1) * SEG, SEG)
            pl.when(t + 1 == XH // SEG)(lambda: x_tail.wait())
            row = pl.multiple_of(jnp.maximum(t - 3, 0) * SEG, SEG)
            hooks = {50: glu_input}
            gpos = [1, 3, 4, 6, 7, 9, 10]

            def next_tokens():
                na_v[:SEG, :] = _layernorm(x_v[pl.ds(nxt, SEG), :].astype(F32))

            glu = gate_up_pieces()
            for c in range(HB):
                scores, values = attention(c, True)
                for w in range(3):
                    project_qkv(w, c, True, (hooks, None, spread(scores, 20, 10))[w])
                    if 3 * c + w in gpos:
                        glu[gpos.index(3 * c + w)]()
                    if 3 * c + w == 5:
                        down_small()
                hooks = spread(values, 26, 10)
                if c == 2:
                    hooks[5] = next_tokens
            down_large(spread(values, 12, 8))
            big_v[pl.ds(row, SEG), :] = z_v[SEG:, :].astype(BF16)

            def next_input():
                na = _layernorm(z_v[:SEG, :])
                na_v[SEG:, :] = jnp.concatenate([na, na + na_v[:SEG, :]], axis=0)

            for c in range(DA // LANES):
                o = project_out(c, True, {2: next_input} if c == 0 else None)
                for (hf, j), v in o.items():
                    cols = tile_of(j, DA, c)
                    res = x_v[pl.ds(cur, SEG), cols].astype(F32) if hf == 0 else xa_v[SEG:, cols]
                    ma_v[hf * M:(hf + 1) * M, cols] = v[:M]
                    ya_v[hf * SEG:(hf + 1) * SEG, cols] = res + v[M:]
            xa_v[SEG:, :] = z_v[:SEG, :]
            pl.when(t >= 3)(lambda: out_copy(row, SEG).start())
            return carry

        def phase(ph, carry):
            attention_single(pl.multiple_of(jnp.where(ph < 2, 0, M), M),
                             pl.multiple_of(jnp.where(ph == 0, 0, SEG), SEG),
                             pl.multiple_of(jnp.where(ph == 3, 1, ph) * SEG, SEG),
                             lambda: pl.when(ph == 0)(load_out_weights))
            pl.when(ph == 1)(load_gate_up_weights)

            @pl.when(ph >= 1)
            def _():
                glu_input()
                for piece in gate_up_pieces():
                    piece()
                pl.when(ph == 1)(load_down_weights)
                down_small()
                down_large()

            @pl.when(ph == 1)
            def _():
                ya_v[0:SEG, :] = ya_v[SEG:2 * SEG, :]
                xa_v[SEG:, :] = z_v[:SEG, :]
                ma_v[...] = mem_v[...]
                na_v[:SEG, :] = _layernorm(x_v[2 * SEG:3 * SEG, :].astype(F32))
                na = _layernorm(z_v[:SEG, :])
                na_v[SEG:, :] = jnp.concatenate([na, na + na_v[:SEG, :]], axis=0)
                lax.fori_loop(2, NSEG, step, 0)
                mem_v[...] = ma_v[...]

            @pl.when(ph == 2)
            def _():
                xa_v[SEG:, :] = z_v[:SEG, :]
                ya_v[0:SEG, :] = ya_v[2 * SEG:, :]
                big_v[S - 3 * SEG:S - 2 * SEG, :] = z_v[SEG:, :].astype(BF16)
                out_copy(S - 3 * SEG, SEG).start()

            @pl.when(ph == 3)
            def _():
                big_v[S - 2 * SEG:S, :] = z_v[...].astype(BF16)
                out_copy(S - 2 * SEG, 2 * SEG).start()
            return carry

        lax.fori_loop(0, 4, phase, 0)
        out_copy(0, NSEG * SEG).wait()

    scratch = [
        pltpu.VMEM((S, D), BF16),
        pltpu.VMEM((M, D), BF16),
        pltpu.VMEM((FF, D), BF16),
        pltpu.VMEM((2, GST, NA, GR, FF), BF16),
        pltpu.VMEM((QST, NA, (QR + 1) * H, DH), BF16),
        pltpu.VMEM((NA, H, QR, DH), BF16),
        pltpu.VMEM((3, HB, PA, DA, DH), BF16),
        pltpu.VMEM((DA // LANES, PA, EB, LANES), BF16),
        pltpu.VMEM((2, NG, PA, DA, LANES), BF16),
        pltpu.VMEM((2, PB, DB, LANES), BF16),
        pltpu.VMEM((1, PA, FA, LANES), BF16),
        pltpu.VMEM((DB // LANES, PB, LANES, LANES), BF16),
        pltpu.VMEM((PA, L, DA), F32),
        pltpu.VMEM((PA, SEG, DA), F32),
        pltpu.VMEM((3 * L, H * DH), F32),
        pltpu.VMEM((3 * SEG, FF), F32),
        pltpu.VMEM((2 * M, D), F32),
        pltpu.VMEM((2 * M, D), F32),
        pltpu.VMEM((2 * SEG, D), F32),
        pltpu.VMEM((3 * SEG, D), F32),
        pltpu.VMEM((3 * SEG, D), F32),
        pltpu.VMEM((3 * SEG, D), F32),
        pltpu.VMEM((2 * SEG, D), F32),
        pltpu.VMEM((NA, 2 * L, DH), F32),
        pltpu.VMEM((2, NA, LANES, DH), BF16),
        pltpu.VMEM((2 * L, LANES), F32),
        pltpu.VMEM((2 * L, LANES), jnp.int32),
        pltpu.SemaphoreType.DMA((3,)),
        pltpu.SemaphoreType.DMA((QST,)),
        pltpu.SemaphoreType.DMA((OST,)),
        pltpu.SemaphoreType.DMA((2, GST)),
        pltpu.SemaphoreType.DMA((GST,)),
        pltpu.SemaphoreType.DMA(()),
    ]
    return kernel, scratch


@functools.partial(jax.jit, static_argnames=("A_seg_len",))
def pallas_interleave_layers__memory_aug_recurrent_mem_tr__glu_gated_glu__prompt_kernel(
    A_x, A_mem0, A_Wq, A_Wk, A_Wv, A_Wo, A_seg_len, B_x, B_w_gate, B_w_up, B_w_down,
):
    del B_x
    B, S, D = A_x.shape
    _, H, DH = A_Wq.shape
    M = A_mem0.shape[1]
    assert B == 1
    kernel, scratch = _make_kernel(S, D, H, DH, M, A_seg_len, B_w_gate.shape[1])
    any_spec = pl.BlockSpec(memory_space=pl.ANY)
    out = pl.pallas_call(
        kernel,
        out_shape=jax.ShapeDtypeStruct((S, D), A_x.dtype),
        in_specs=[any_spec] * 9,
        out_specs=any_spec,
        scratch_shapes=scratch,
        compiler_params=pltpu.CompilerParams(vmem_limit_bytes=126 * 1024 * 1024),
    )(A_x.reshape(S, D), A_mem0.reshape(M, D),
      A_Wq.reshape(D * H, DH), A_Wk.reshape(D * H, DH), A_Wv.reshape(D * H, DH),
      A_Wo.reshape(H * DH, D), B_w_gate, B_w_up, B_w_down)
    return out.reshape(B, S, D)
```

```python
import functools
import itertools
import math

import jax
import jax.numpy as jnp
import numpy as np
from jax import lax
import jax.experimental.pallas as pl
import jax.experimental.pallas.tpu as pltpu

F32 = jnp.float32
BF16 = jnp.bfloat16
U32 = jnp.uint32
EPS = 1e-05
LANES = 128

_SCHEME_4 = """
+00 | +00 +02 -10 +30 | +00 -10
+00 +10 | +00 -01 +20 -30 | +10

+00 -11 | +01 -10 +30 | +01 +10
+10 +11 | +01 | +10 +11
+00 +01 | +03 +10 -30 | +00 +01

+00 +10 +11 +13 | +30 | -00 -01 +03 +10
+00 +01 +03 +10 +11 +13 | -03 +30 | +00 +01 -03
+03 +10 +11 +13 | +03 | +00 +01 -03 +13

+00 +10 -12 | +02 -20 | -00 +02 +10
+10 -12 | +02 | +00 -02 -10 +12
+00 -02 +10 -12 | +20 | -00 +02

+11 | +01 -11 -12 +31 | +01 -11
+01 +11 | -03 -10 +11 +13 -21 +30 | +01

-03 +11 | -03 +13 +31 | -01 +13
+01 +03 | -03 +13 +30 | -01 +03
+11 +13 | +31 | +11 -13

+01 +02 +11 | +12 +21 | +01 -11 +12
+01 +02 | +12 | -01 +02 +11 -12
+01 +02 +11 +12 | +21 | +11 -12

+03 +12 +13 | -23 -32 | -02 +03 -13
+02 +03 +12 +13 | +23 | -02 +03
+12 +13 | +32 | -02 +03 +12 -13

+02 | -12 +20 +22 +23 | +02
+12 | +02 +21 +22 -32 | +12

+03 | +03 -13 +32 +33 | +03 -13
+03 +13 | -03 -23 +31 +33 | +13
"""
_SCHEME_8 = """
+01 +10 | +01 +10 | +00 +11
+00 -01 | +01 | +00 +01
+10 -11 | +10 | -10 -11

+00 +02 +10 | +02 +20 | +00 -10 +12
+00 +02 | +02 | -00 +02 +10 -12
+00 +02 +10 +12 | +20 | +10 -12

+00 +03 -04 +10 | +30 | +00 -10 -13 -14
+00 +03 -04 +10 +13 -14 | +03 +30 | +10 +13 +14
+00 +03 -04 +13 | +03 | +03 -10 -13 -14

+04 +10 | +04 +30 +40 -74 | +00 +14
+00 -04 | +04 -47 -74 | +00 +04
+10 -14 | -03 -30 -40 | +10 +14

+00 -05 +10 | +05 +50 | -00 +10 +15
+00 -05 | +05 | +00 +05 -10 -15
+00 -05 +10 -15 | +50 | -10 -15

+00 +06 +07 +10 | +60 | +00 -10 -16 +17
+00 +06 +07 +10 +16 +17 | +06 +60 | +10 +16 -17
+00 +06 +07 +16 | +06 | +06 -10 -16 +17

-07 +10 | +07 +47 -60 +70 | -00 +17
+00 +07 | +07 +47 +74 | -00 +07
+10 +17 | +06 +60 -70 | -10 +17

+10 | -00 -02 +05 -10 -30 -40 -60 +70 | +00 -10
+00 +10 | +00 -01 -04 +07 -20 -30 +47 +50 -60 +74 | +00

+01 +11 -12 | +12 +21 | +01 +02 -11
+11 -12 | +12 | -01 -02 +11 +12
+01 -02 +11 -12 | +21 | -01 -02

+01 +13 | +13 +31 +63 -71 | +03 +11
+11 -13 | +13 -36 +63 | +11 +13
+01 -03 | -17 -31 +71 | +01 +03

+01 +11 +14 -16 | +41 | -01 +04 +06 +11
+01 +04 -06 +11 +14 -16 | -14 +41 | +01 -04 -06
+04 +11 +14 -16 | +14 | +01 -04 -06 +14

+01 +11 +15 | +15 -51 | +01 +05 -11
+11 +15 | +15 | -01 -05 +11 +15
+01 +05 +11 +15 | +51 | +01 +05

+01 +16 | +16 +36 -41 -61 | +06 -11
+11 -16 | +16 +36 -63 | -11 +16
+01 -06 | -14 +41 +61 | -01 +06

+01 +11 -13 -17 | +71 | +01 +03 +07 -11
+01 -03 -07 +11 -13 -17 | +17 -71 | +01 +03 +07
-07 +11 -13 -17 | +17 | -01 -03 -07 +17

+01 | +01 +11 -12 -15 +31 +41 +61 -71 | +01 -11
+01 +11 | -10 +11 -13 +16 +21 +36 -41 -51 -63 +71 | +11

+02 +03 +13 | +23 -32 -52 | +03 -12 -13
+02 +03 +12 +13 | +23 | +12 +13
+02 +03 | +25 +32 +52 | +02 +03 -12 -13

-04 +12 -14 | -24 -42 | +02 +04 -14
+02 -04 +12 -14 | +24 | +02 +04
+12 -14 | +42 | +02 +04 -12 -14

+03 -05 +12 +13 -15 | +52 | -02 -03 +05 +13 -15
+12 +13 -15 | +25 +52 | +02 +03 -05 -12 -13 +15
+02 +03 +12 +13 -15 | +25 | -02 -03 +05 +12 +13

+02 +06 +16 | +26 -62 | +06 -12 -16
+02 +06 +12 +16 | +26 | +12 +16
+02 +06 | +62 | +02 +06 -12 -16

+07 +12 +17 | -27 -72 | -02 +07 -17
+02 +07 +12 +17 | +27 | -02 +07
+12 +17 | +72 | -02 +07 +12 -17

+02 | -02 -21 +22 -24 +27 -32 -52 -62 | +02
+12 | +12 +20 +22 -23 -26 +42 +52 -72 | +12

+04 +13 | +03 +34 +43 | +03 +14
+03 -04 | +34 | +03 +04
+13 -14 | -03 -30 -43 | +13 +14

+03 -05 +13 | -25 +35 -53 | +03 -13 +15
+03 -05 | -25 +35 -52 | -03 +05 +13 -15
+03 -05 +13 -15 | +53 | -13 +15

-01 +03 +06 +13 | +63 | +03 -11 -13 +16
-01 +03 +06 -11 +13 +16 | -36 +63 | +11 +13 -16
-01 +03 +06 +16 | +36 | +06 +11 +13 -16

-07 +13 | +17 +37 -73 | +03 +17
+03 +07 | +17 +37 -71 | +03 +07
+13 +17 | +73 | +13 +17

+13 | -03 -13 +25 +32 -33 -35 -43 +52 -63 +73 | +03 -13
+03 +13 | -03 -17 -23 -31 +33 -34 -37 +53 -63 +71 | +03

+04 +14 +15 | +45 -54 | +04 +05 -14
+14 +15 | +45 | -04 -05 +14 +15
+04 +05 +14 +15 | +54 | +04 +05

+04 +16 | +14 +46 +64 | +06 +14
+14 -16 | +46 | +14 +16
+04 -06 | -14 +41 -64 | +04 +06

+04 -10 +14 -17 | +74 | +00 +04 -07 -14
-00 +04 -07 -10 +14 -17 | -47 -74 | +00 +04 -07
-07 -10 +14 -17 | +47 | +00 +04 -07 +17

+04 | +04 +14 +34 -42 +44 -45 +64 -74 | +04 -14
+04 +14 | -03 -14 +24 -30 -40 -43 +44 -46 -54 +74 | +14

+05 +06 +16 | +56 -65 | +06 -15 -16
+05 +06 +15 +16 | +56 | +15 +16
+05 +06 | +65 | +05 +06 -15 -16

+07 +15 +17 | -57 -75 | -05 +07 -17
+05 +07 +15 +17 | +57 | -05 +07
+15 +17 | +75 | -05 +07 +15 -17

+05 | +05 -25 +35 -51 -54 +55 +57 -65 | +05
+15 | -15 +25 -45 -50 +53 +55 -56 -75 | +15

-07 +16 | -06 +67 +76 | -06 +17
+06 +07 | +67 | -06 +07
+16 +17 | +06 +60 -76 | -16 +17

+16 | -06 -16 -36 -46 +62 +65 -66 +76 | +06 -16
+06 +16 | -06 -14 -26 -36 +41 -56 +61 -64 +66 +67 | +06

+07 | -07 -17 -37 -47 -67 +72 +75 +77 | +07 -17
+07 +17 | -06 +17 -27 +47 -57 -60 +70 -73 +76 +77 | +17
"""


class _Scheme:
    def __init__(self, n, text):
        def terms(field):
            return {(int(t[1]), int(t[2])): 1 if t[0] == "+" else -1 for t in field.split()}

        def fold(coefs, weights):
            out = {}
            for (h, i), c in coefs.items():
                out[i] = out.get(i, 0) + weights[h] * c
            return {i: c for i, c in out.items() if c}

        self.n = n
        self.prods, self.ends = [], []
        for group in text.strip().split("\n\n"):
            self.prods += [tuple(terms(f) for f in line.split("|")) for line in group.split("\n")]
            self.ends.append(len(self.prods) - 1)
        dense = np.zeros((3, len(self.prods), n, n), np.int64)
        for r, prod in enumerate(self.prods):
            for m, coefs in enumerate(prod):
                for (i, j), c in coefs.items():
                    dense[m, r, i, j] = c
        eye = np.eye(n, dtype=np.int64)
        assert np.array_equal(
            np.einsum("rai,rjk,rbl->aijkbl", dense[0, :, :2], dense[1], dense[2, :, :2]),
            np.einsum("ab,ij,kl->aijkbl", eye[:2, :2], eye, eye)), "not the matrix product"
        assert all(len(v) > 1 or sum(v.values()) == 1 for _, v, _ in self.prods)
        folded = [(fold(u, (-1, 1)), fold(w, (0, 1))) for u, _, w in self.prods]
        self.single = [(u, w) if u and w else None for u, w in folded]
        self.sums, self.shared = [dict(v) for _, v, _ in self.prods], {}
        while True:
            count = {}
            for v in self.sums:
                for a, b in itertools.combinations(sorted(v), 2):
                    count[a, b, v[a] * v[b]] = count.get((a, b, v[a] * v[b]), 0) + 1
            (a, b, sign), times = max(count.items(), key=lambda kv: kv[1])
            if times < 2:
                break
            key = (n, len(self.shared))
            self.shared[key] = {a: 1, b: sign}
            for v in self.sums:
                if a in v and b in v and v[a] * v[b] == sign:
                    v[key] = v.pop(a)
                    del v[b]


def _combine(coefs, vals):
    acc = None
    for key, c in sorted(coefs.items(), key=lambda kv: -kv[1]):
        v = vals[key]
        if abs(c) != 1:
            v = v * abs(c)
        if acc is None:
            acc = v if c > 0 else -v
        else:
            acc = acc + v if c > 0 else acc - v
    return acc


def _accumulate(accs, group):
    terms = {}
    for n, (coefs, _) in enumerate(group):
        for key, c in coefs.items():
            terms.setdefault(key, []).append((n, c))
    sums = {((n, 1),): v for n, (_, v) in enumerate(group)}
    for key, tm in sorted(terms.items(), key=lambda kv: len(kv[1])):
        sign = tm[0][1]
        tm = tuple((n, c * sign) for n, c in tm)
        if tm not in sums:
            base = max((s for s in sums if all(t in tm for t in s)), key=len)
            val = sums[base]
            for n, c in tm:
                if (n, c) not in base:
                    val = val + group[n][1] if c > 0 else val - group[n][1]
            sums[tm] = val
        if key not in accs:
            accs[key] = sums[tm] if sign > 0 else -sums[tm]
        else:
            accs[key] = accs[key] + sums[tm] if sign > 0 else accs[key] - sums[tm]


def _layernorm(x, gain=1.0):
    m = jnp.mean(x, axis=-1, keepdims=True)
    c = x - m
    v = jnp.mean(c * c, axis=-1, keepdims=True)
    inv = lax.rsqrt(v + EPS)
    return c * (inv if gain == 1.0 else inv * gain)


def _dot(a, b):
    return lax.dot_general(a, b, (((1,), (0,)), ((), ())), preferred_element_type=F32)


def _dot_nt(a, b):
    return lax.dot_general(a, b, (((1,), (1,)), ((), ())), preferred_element_type=F32)


def _halves(x):
    return pltpu.bitcast(x << 16, F32), pltpu.bitcast(x & np.uint32(0xFFFF0000), F32)


def _make_kernel(S, D, H, DH, M, SEG, FF):
    SA = _Scheme(8, _SCHEME_8)
    SB = _Scheme(4, _SCHEME_4)
    NA, NB = SA.n, SB.n
    PA, PB = len(SA.prods), len(SB.prods)
    NSEG = S // SEG
    L = M + SEG
    DA, HB = D // NA, H // NA
    EB = HB * DH
    NG = FF // (NA * LANES)
    FA = NG * LANES
    F8 = NA * FA
    DB = D // NB
    assert DA == LANES and DH == LANES and FF - F8 == NB * LANES
    QR = 128 // NA
    QST = 4
    WR = 512 // NA
    OST = FF // (WR * NA)
    GST = 4
    GR, DR, ER = DA // GST, FA // GST, LANES // GST
    XH = 3 * SEG
    scale = DH ** (-0.5)
    c_exp = scale * math.log2(math.e)

    def fast_dot(sch, paired, w_of, block, kept_ref=None, fresh=True, hooks=None):
        acc, group = {}, []
        for r, (u, _, w) in enumerate(sch.prods):
            if hooks and r in hooks:
                hooks[r]()
            if paired or sch.single[r]:
                if not paired:
                    u, w = sch.single[r]
                if fresh:
                    if not paired:
                        u = {(0, i): c for i, c in u.items()}
                    else:
                        u = {(2 if u.get((1 - hf, i)) == c else hf, i): c
                             for (hf, i), c in u.items()}
                    lhs = _combine(u, {key: block(*key) for key in u})
                    if kept_ref is not None:
                        kept_ref[r] = lhs
                else:
                    lhs = kept_ref[r]
                group.append((w, _dot(lhs, w_of(r))))
            if r in sch.ends:
                _accumulate(acc, group)
                group = []
        return acc

    def tiles_of(ref, *index):
        return lambda r: pltpu.bitcast(ref.bitcast(U32)[(*index, r)], BF16)

    def blocks_of(ref, rows, cols, c0=0):
        return lambda hf, i: ref[hf * rows:(hf + 1) * rows, c0 + i * cols:c0 + (i + 1) * cols]

    def spread(pieces, first, stride):
        return {first + n * stride: piece for n, piece in enumerate(pieces)}

    def tile_of(j, blk, c):
        return slice(j * blk + c * LANES, j * blk + (c + 1) * LANES)

    def kernel(x_hbm, mem0_hbm, wq_hbm, wk_hbm, wv_hbm, wo_hbm, wg_hbm, wu_hbm, wd_hbm,
               out_hbm,
               x_v, mem0_v, big_v, gst_v, qst_v, qtr_v, wqkv_v, wo_v, wgu8_v, wgu4_v, wd8_v, wd4_v,
               la_v, lb_v, o_v, act_v, mem_v, ma_v, xa_v, na_v, nb_v, ya_v, z_v,
               q_v, kv_v, fill_v, keep_v,
               sem_x, sem_q, sem_o, sem_g, sem_d, sem_out):

        def rows_at(start, size):
            return pl.ds(start if isinstance(start, int) else pl.multiple_of(start, 16), size)

        def q_copies(w, c, slot):
            src = (wq_hbm, wk_hbm, wv_hbm)[w]
            return [pltpu.make_async_copy(src.at[rows_at((i * DA + c * QR) * H, QR * H), :],
                                          qst_v.at[slot, i, 0:QR * H, :], sem_q.at[slot])
                    for i in range(NA)]

        def o_copies(c):
            slot = c % OST
            return [pltpu.make_async_copy(wo_hbm.at[rows_at(i * EB + c * WR, WR), :],
                                          big_v.at[rows_at((slot * NA + i) * WR, WR), :],
                                          sem_o.at[slot]) for i in range(NA)]

        def g_copies(w, c):
            return [pltpu.make_async_copy((wg_hbm, wu_hbm)[w].at[rows_at(i * DA + c * GR, GR), :],
                                          gst_v.at[w, c, i], sem_g.at[w, c]) for i in range(NA)]

        def d_copies(c):
            rows = ([rows_at(i * FA + c * DR, DR) for i in range(NA)]
                    + [rows_at(F8 + i * LANES + c * ER, ER) for i in range(NB)])
            return [pltpu.make_async_copy(wd_hbm.at[r, :], big_v.at[r, :], sem_d.at[c])
                    for r in rows]

        def start(copies):
            for cp in copies:
                cp.start()

        def wait(copies):
            for cp in copies:
                cp.wait()

        def prep_tiles(sch, load, put, nrows, ncols):
            def tile(_, pos):
                s, k = pos
                row = pl.multiple_of(s * 16, 16)
                known = {}

                def value(key):
                    if key not in sch.shared:
                        return load(*key, row, k).astype(F32)
                    if key not in known:
                        known[key] = _combine(sch.shared[key],
                                              {a: value(a) for a in sch.shared[key]})
                    return known[key]

                for r, v in enumerate(sch.sums):
                    if len(sch.prods[r][1]) == 1:
                        val = load(*next(iter(v)), row, k)
                    else:
                        val = _combine(v, {key: value(key) for key in v}).astype(BF16)
                    put(r, row, k, val)
                wrap = k + 1 == ncols
                return jnp.where(wrap, s + 1, s), jnp.where(wrap, 0, k + 1)
            lax.fori_loop(0, nrows // 16 * ncols, tile, (0, 0))

        def lanes_at(k):
            return pl.ds(pl.multiple_of(k * LANES, LANES), LANES)

        def prep_qkv(w, c, slot):
            def heads(i, carry):
                st = qst_v.at[slot, i].bitcast(U32)
                for jp in range(H // 2):
                    for k, x in enumerate(_halves(st[pl.ds(jp, QR, stride=H // 2), :])):
                        qtr_v[i, 2 * jp + k] = x.astype(BF16)
                return carry
            lax.fori_loop(0, NA, heads, 0)

            def put(r, row, k, val):
                wqkv_v[w, k, r, rows_at(c * QR + row, 16), :] = val
            prep_tiles(SA, lambda i, j, row, k: qtr_v[i, j * HB + k, pl.ds(row, 16), :],
                       put, QR, HB)

        def prep_from_big(sch, dst, base, blk, c, nrows):
            ncols = D // sch.n // LANES

            def load(i, j, row, k):
                return big_v[rows_at(base + i * blk + row, 16), lanes_at(j * ncols + k)]

            def put(r, row, k, val):
                dst[k, r, rows_at(c * nrows + row, 16), :] = val
            prep_tiles(sch, load, put, nrows, ncols)

        def prep_gu(w, c):
            def put8(r, row, k, val):
                wgu8_v[w, k, r, rows_at(c * GR + row, 16), :] = val
            prep_tiles(SA, lambda i, j, row, k: gst_v[w, c, i, pl.ds(row, 16),
                                                      lanes_at(j * NG + k)], put8, GR, NG)

            def put4(r, row, k, val):
                wgu4_v[w, r, rows_at(k * DA + c * GR + row, 16), :] = val
            prep_tiles(SB, lambda i, j, row, k: gst_v[w, c, 2 * i + k, pl.ds(row, 16),
                                                      F8 + j * LANES:F8 + (j + 1) * LANES],
                       put4, GR, 2)

        x_head = pltpu.make_async_copy(x_hbm.at[0:XH, :], x_v.at[0:XH, :], sem_x.at[0])
        x_tail = pltpu.make_async_copy(x_hbm.at[XH:, :], x_v.at[XH:, :], sem_x.at[1])
        NQ, NO = DA // QR, EB // WR
        AHEAD = OST - 1
        assert QST <= min(NQ, AHEAD) and OST <= NO
        QA = QST - 1
        for n in range(QA):
            start(q_copies(0, n, n))
        mem0_copy = pltpu.make_async_copy(mem0_hbm, mem0_v, sem_x.at[2])
        x_head.start()
        mem0_copy.start()

        ri = lax.broadcasted_iota(jnp.int32, (2 * L, LANES), 0)
        ci = lax.broadcasted_iota(jnp.int32, (2 * L, LANES), 1)
        first = jnp.where(ri < L, 0, L)
        same = (ci >= first) & (ci < first + L)
        visible = (ri < first + M) | (ri >= ci)
        keep_v[...] = (same & visible).astype(jnp.int32)
        fill_v[...] = jnp.where(same, -1e9 / scale, -jnp.inf).astype(F32)
        kv_v[...] = jnp.zeros(kv_v.shape, BF16)

        for w in range(3):
            def q_body(c, carry, w=w):
                slot, free = (w * NQ + c) % QST, (w * NQ + c + QA) % QST
                wait(q_copies(w, c, slot))
                pl.when(c + QA < NQ)(lambda: start(q_copies(w, c + QA, free)))
                if w < 2:
                    pl.when(c + QA >= NQ)(lambda: start(q_copies(w + 1, c + QA - NQ, free)))
                else:
                    pl.when(c + QA >= NQ)(lambda: start(o_copies(c + QA - NQ)))
                prep_qkv(w, c, slot)
                return carry
            lax.fori_loop(0, NQ, q_body, 0)

        for c in range(QA, AHEAD):
            start(o_copies(c))
        x_head.wait()
        mem0_copy.wait()
        xa_v[...] = x_v[0:3 * SEG, :].astype(F32)
        mem_v[0:M, :] = mem0_v[...].astype(F32)
        mem_v[M:, :] = mem0_v[...].astype(F32)

        def load_out_weights():
            def chunk(c, carry):
                pl.when(c + AHEAD < NO)(lambda: start(o_copies(c + AHEAD)))
                pl.when(c == NO // 2 - 1)(lambda: start(g_copies(0, 0)))
                pl.when(c == NO - 2)(lambda: start(g_copies(0, 1)))
                wait(o_copies(c))
                prep_from_big(SA, wo_v, (c % OST) * NA * WR, WR, c, WR)
                return carry
            lax.fori_loop(0, NO, chunk, 0)
            for c in range(2, GST):
                start(g_copies(0, c))
            start(g_copies(1, 0))
            start(g_copies(1, 1))

        def request_glu_weights():
            for c in range(2, GST):
                start(g_copies(1, c))
            start(d_copies(0))

        def load_gate_up_weights():
            for w in range(2):
                def chunk(c, carry):
                    if w == 0:
                        pl.when(c + 1 < GST)(lambda: start(d_copies(c + 1)))
                    wait(g_copies(w, c))
                    prep_gu(w, c)
                    return carry
                lax.fori_loop(0, GST, chunk, 0)

        def load_down_weights():
            x_tail.start()

            def chunk(c, carry):
                wait(d_copies(c))
                prep_from_big(SA, wd8_v, c * DR, FA, c, DR)
                prep_from_big(SB, wd4_v, F8 + c * ER, LANES, c, ER)
                return carry
            lax.fori_loop(0, GST, chunk, 0)

        def attention(c, paired):
            n = 2 * L if paired else L
            probs = {}

            def scores(j):
                s = _dot_nt(q_v[j, 0:n, :], kv_v[0, j])
                s = jnp.where(keep_v[0:n, :] != 0, s, fill_v[0:n, :])
                mx = jnp.max(s, axis=-1, keepdims=True)
                e = jnp.exp2((s - mx) * c_exp)
                den = jnp.sum(e, axis=-1, keepdims=True)
                inv = pl.reciprocal(den, approx=True)
                inv = inv * (2.0 - den * inv)
                probs[j] = e * inv

            def values(j):
                o = _dot(probs[j], kv_v[1, j])
                o_v[0:n, tile_of(j, EB, c)] = o
                if paired:
                    o_v[n:, tile_of(j, EB, c)] = o[:L] + o[L:]

            return ([functools.partial(scores, j) for j in range(NA)],
                    [functools.partial(values, j) for j in range(NA)])

        def project_qkv(w, c, paired, hooks):
            def block(hf, i):
                cols = slice(i * DA, (i + 1) * DA)
                if hf == 2:
                    return jnp.concatenate([ma_v[0:M, cols] + ma_v[M:, cols],
                                            na_v[2 * SEG:, cols]], axis=0)
                return jnp.concatenate([ma_v[hf * M:(hf + 1) * M, cols],
                                        na_v[hf * SEG:(hf + 1) * SEG, cols]], axis=0)

            p = fast_dot(SA, paired, tiles_of(wqkv_v, w, c), block, la_v, w + c == 0, hooks)
            for j in range(NA):
                x = jnp.concatenate([p[0, j], p[1, j]], axis=0) if paired else p[j]
                if w == 0:
                    q_v[j, 0:x.shape[0], :] = x
                else:
                    kv_v[w - 1, j, 0:x.shape[0], :] = x.astype(BF16)

        def project_out(c, paired, hooks=None):
            return fast_dot(SA, paired, tiles_of(wo_v, c), blocks_of(o_v, L, EB), hooks=hooks)

        def glu_input():
            nb = _layernorm(ya_v[0:2 * SEG, :], 0.5)
            nb_v[...] = jnp.concatenate([nb, nb[:SEG] + nb[SEG:]], axis=0)

        def gate_up_pieces():
            gate = {}

            def activate(cols, g, u):
                act = [jnp.tanh(g[hf]) * u[hf] + u[hf] for hf in range(2)]
                act_v[:, cols] = jnp.concatenate(act + [act[0] + act[1]], axis=0)

            def large(k, w):
                p = fast_dot(SA, True, tiles_of(wgu8_v, w, k), blocks_of(nb_v, SEG, DA), lb_v,
                             k + w == 0)
                if w == 0:
                    gate.update(p)
                else:
                    for j in range(NA):
                        activate(tile_of(j, FA, k), (gate[0, j], gate[1, j]), (p[0, j], p[1, j]))

            def small():
                p = fast_dot(SB, True, lambda r: jnp.concatenate(
                    [tiles_of(wgu4_v, w)(r) for w in range(2)], axis=1), blocks_of(nb_v, SEG, DB))
                for j in range(NB):
                    activate(slice(F8 + j * LANES, F8 + (j + 1) * LANES),
                             [p[hf, j][:, :LANES] for hf in range(2)],
                             [p[hf, j][:, LANES:] for hf in range(2)])

            return [small] + [functools.partial(large, k, w) for k in range(NG) for w in range(2)]

        def down_small():
            acc = {}
            for k in range(DB // LANES):
                p = fast_dot(SB, True, tiles_of(wd4_v, k), blocks_of(act_v, SEG, LANES, F8))
                acc.update({(hf, j * (DB // LANES) + k): v for (hf, j), v in p.items()})
            for (hf, j), v in acc.items():
                rows = slice(hf * SEG, (hf + 1) * SEG)
                z_v[rows, tile_of(j, DA, 0)] = ya_v[rows, tile_of(j, DA, 0)] + v

        def down_large(hooks=None):
            acc = fast_dot(SA, True, tiles_of(wd8_v, 0), blocks_of(act_v, SEG, FA),
                           hooks=hooks)
            for (hf, j), v in acc.items():
                z_v[hf * SEG:(hf + 1) * SEG, tile_of(j, DA, 0)] += v

        def out_copy(row, n):
            return pltpu.make_async_copy(big_v.at[pl.ds(row, n), :],
                                         out_hbm.at[pl.ds(row, n), :], sem_out)

        def attention_single(mrow, xrow, yrow, before_out):
            ma_v[0:M, :] = mem_v[pl.ds(mrow, M), :]
            na_v[0:SEG, :] = _layernorm(xa_v[pl.ds(xrow, SEG), :])
            hooks = None
            for c in range(HB):
                scores, values = attention(c, False)
                project_qkv(0, c, False, hooks)
                project_qkv(1, c, False, None)
                project_qkv(2, c, False, spread(scores, 20, 7))
                hooks = spread(values, 24, 9)
            for piece in values:
                piece()
            before_out()
            for c in range(DA // LANES):
                for j, v in project_out(c, False).items():
                    mem_v[pl.ds(mrow, M), tile_of(j, DA, c)] = v[:M]
                    ya_v[pl.ds(yrow, SEG), tile_of(j, DA, c)] = (
                        xa_v[pl.ds(xrow, SEG), tile_of(j, DA, c)] + v[M:])

        def step(t, carry):
            cur = pl.multiple_of(t * SEG, SEG)
            nxt = pl.multiple_of(jnp.minimum(t + 1, NSEG - 1) * SEG, SEG)
            row = pl.multiple_of((t - 3) * SEG, SEG)
            hooks = {50: glu_input}
            gpos = [1, 3, 4, 6, 7, 9, 10]

            def next_tokens():
                na_v[:SEG, :] = _layernorm(x_v[pl.ds(nxt, SEG), :].astype(F32))

            glu = gate_up_pieces()
            for c in range(HB):
                scores, values = attention(c, True)
                for w in range(3):
                    project_qkv(w, c, True, (hooks, None, spread(scores, 20, 10))[w])
                    if 3 * c + w in gpos:
                        glu[gpos.index(3 * c + w)]()
                    if 3 * c + w == 5:
                        down_small()
                hooks = spread(values, 26, 10)
                if c == 2:
                    hooks[5] = next_tokens
            down_large(spread(values, 12, 8))
            big_v[pl.ds(row, SEG), :] = z_v[SEG:, :].astype(BF16)

            def next_input():
                na = _layernorm(z_v[:SEG, :])
                na_v[SEG:, :] = jnp.concatenate([na, na + na_v[:SEG, :]], axis=0)

            for c in range(DA // LANES):
                o = project_out(c, True, {2: next_input} if c == 0 else None)
                for (hf, j), v in o.items():
                    cols = tile_of(j, DA, c)
                    res = (x_v[pl.ds(cur, SEG), cols].astype(F32) if hf == 0
                           else xa_v[SEG:2 * SEG, cols])
                    ma_v[hf * M:(hf + 1) * M, cols] = v[:M]
                    ya_v[hf * SEG:(hf + 1) * SEG, cols] = res + v[M:]
            xa_v[SEG:2 * SEG, :] = z_v[:SEG, :]
            out_copy(row, SEG).start()
            return carry

        def phase(ph, carry):
            attention_single(
                pl.multiple_of(jnp.where(ph < 3, 0, M), M),
                pl.multiple_of(jnp.where(ph < 3, ph, 1) * SEG, SEG),
                pl.multiple_of(jnp.where(ph < 3, ph, jnp.where(ph == 4, 2, 1)) * SEG, SEG),
                lambda: pl.when(ph == 0)(load_out_weights))
            pl.when(ph == 1)(request_glu_weights)
            pl.when(ph == 2)(load_gate_up_weights)

            @pl.when((ph == 2) | (ph >= 4))
            def _():
                glu_input()
                for piece in gate_up_pieces():
                    piece()
                pl.when(ph == 2)(load_down_weights)
                down_small()
                down_large()

            @pl.when((ph == 2) | (ph == 4))
            def _():
                xa_v[SEG:2 * SEG, :] = z_v[:SEG, :]
                ya_v[0:SEG, :] = ya_v[2 * SEG:, :]

            @pl.when(ph == 3)
            def _():
                x_tail.wait()
                xa_v[SEG:2 * SEG, :] = z_v[SEG:, :]
                ma_v[...] = mem_v[...]
                na_v[:SEG, :] = _layernorm(x_v[3 * SEG:4 * SEG, :].astype(F32))
                na = _layernorm(z_v[SEG:, :])
                na_v[SEG:, :] = jnp.concatenate([na, na + na_v[:SEG, :]], axis=0)
                lax.fori_loop(3, NSEG, step, 0)
                mem_v[...] = ma_v[...]

            @pl.when(ph == 4)
            def _():
                big_v[S - 3 * SEG:S - 2 * SEG, :] = z_v[SEG:, :].astype(BF16)
                out_copy(S - 3 * SEG, SEG).start()

            @pl.when(ph == 5)
            def _():
                big_v[S - 2 * SEG:S, :] = z_v[...].astype(BF16)
                out_copy(S - 2 * SEG, 2 * SEG).start()
            return carry

        lax.fori_loop(0, 6, phase, 0)
        out_copy(0, NSEG * SEG).wait()

    scratch = [
        pltpu.VMEM((S, D), BF16),
        pltpu.VMEM((M, D), BF16),
        pltpu.VMEM((FF, D), BF16),
        pltpu.VMEM((2, GST, NA, GR, FF), BF16),
        pltpu.VMEM((QST, NA, (QR + 1) * H, DH), BF16),
        pltpu.VMEM((NA, H, QR, DH), BF16),
        pltpu.VMEM((3, HB, PA, DA, DH), BF16),
        pltpu.VMEM((DA // LANES, PA, EB, LANES), BF16),
        pltpu.VMEM((2, NG, PA, DA, LANES), BF16),
        pltpu.VMEM((2, PB, DB, LANES), BF16),
        pltpu.VMEM((1, PA, FA, LANES), BF16),
        pltpu.VMEM((DB // LANES, PB, LANES, LANES), BF16),
        pltpu.VMEM((PA, L, DA), F32),
        pltpu.VMEM((PA, SEG, DA), F32),
        pltpu.VMEM((3 * L, H * DH), F32),
        pltpu.VMEM((3 * SEG, FF), F32),
        pltpu.VMEM((2 * M, D), F32),
        pltpu.VMEM((2 * M, D), F32),
        pltpu.VMEM((3 * SEG, D), F32),
        pltpu.VMEM((3 * SEG, D), F32),
        pltpu.VMEM((3 * SEG, D), F32),
        pltpu.VMEM((3 * SEG, D), F32),
        pltpu.VMEM((2 * SEG, D), F32),
        pltpu.VMEM((NA, 2 * L, DH), F32),
        pltpu.VMEM((2, NA, LANES, DH), BF16),
        pltpu.VMEM((2 * L, LANES), F32),
        pltpu.VMEM((2 * L, LANES), jnp.int32),
        pltpu.SemaphoreType.DMA((3,)),
        pltpu.SemaphoreType.DMA((QST,)),
        pltpu.SemaphoreType.DMA((OST,)),
        pltpu.SemaphoreType.DMA((2, GST)),
        pltpu.SemaphoreType.DMA((GST,)),
        pltpu.SemaphoreType.DMA(()),
    ]
    return kernel, scratch


@functools.partial(jax.jit, static_argnames=("A_seg_len",))
def pallas_interleave_layers__memory_aug_recurrent_mem_tr__glu_gated_glu__prompt_kernel(
    A_x, A_mem0, A_Wq, A_Wk, A_Wv, A_Wo, A_seg_len, B_x, B_w_gate, B_w_up, B_w_down,
):
    del B_x
    B, S, D = A_x.shape
    _, H, DH = A_Wq.shape
    M = A_mem0.shape[1]
    assert B == 1
    kernel, scratch = _make_kernel(S, D, H, DH, M, A_seg_len, B_w_gate.shape[1])
    any_spec = pl.BlockSpec(memory_space=pl.ANY)
    out = pl.pallas_call(
        kernel,
        out_shape=jax.ShapeDtypeStruct((S, D), A_x.dtype),
        in_specs=[any_spec] * 9,
        out_specs=any_spec,
        scratch_shapes=scratch,
        compiler_params=pltpu.CompilerParams(vmem_limit_bytes=126 * 1024 * 1024),
    )(A_x.reshape(S, D), A_mem0.reshape(M, D),
      A_Wq.reshape(D * H, DH), A_Wk.reshape(D * H, DH), A_Wv.reshape(D * H, DH),
      A_Wo.reshape(H * DH, D), B_w_gate, B_w_up, B_w_down)
    return out.reshape(B, S, D)
```
